```python
import jax
import jax.numpy as jnp

def _softmax(x, axis=-1):
    return jax.nn.softmax(x, axis=axis)

def _gelu(x):
    return jax.nn.gelu(x, approximate=True)

def _silu(x):
    return jax.nn.silu(x)

def _sigmoid(x):
    return jax.nn.sigmoid(x)

def _layernorm(x, axis=-1, eps=1e-05):
    m = jnp.mean(x, axis=axis, keepdims=True)
    v = jnp.var(x, axis=axis, keepdims=True)
    return (x - m) / jnp.sqrt(v + eps)

def _scatter_add(tgt, idx, src, axis=0):
    return tgt.at[idx].add(src)

def _segment_sum(src, seg, n):
    return jax.ops.segment_sum(src, seg, n)

class _Rng:

    def __init__(self, key):
        self._k = key

    def _next(self):
        self._k, sub = jax.random.split(self._k)
        return sub

    def normal(self, shape):
        return jax.random.normal(self._next(), shape, dtype=jnp.bfloat16)

    def randint(self, lo, hi, shape):
        return jax.random.randint(self._next(), shape, lo, hi, dtype=jnp.int32)

    def uniform(self, shape, lo=0.0, hi=1.0):
        return jax.random.uniform(self._next(), shape, jnp.bfloat16, lo, hi)

    def permutation(self, n):
        return jax.random.permutation(self._next(), n)
kernel_name = 'parallel_sum__memory_aug_recurrent_mem_tr__mixer_s_mlp__prompt'

def setup_inputs():
    _rng = _Rng(jax.random.key(int.from_bytes(__import__("os").urandom(4), "little")))
    _w = lambda a: (lambda t: t.astype(jnp.bfloat16) if jnp.issubdtype(t.dtype, jnp.floating) else t)(jnp.asarray(a))

    def _A_setup():
        B, S, Dm = (1, 2048, 1024)
        H, Dh = (32, 128)
        M, seg = (8, 32)
        seg = min(seg, S)
        S = S // seg * seg
        return {'x': _w((lambda *s: _rng.normal(s) * 0.05)(B, S, Dm)), 'mem0': _w((lambda *s: _rng.normal(s) * 0.05)(B, M, Dm)), 'Wq': _w((lambda *s: _rng.normal(s) * 0.05)(Dm, H, Dh) * Dm ** (-0.5)), 'Wk': _w((lambda *s: _rng.normal(s) * 0.05)(Dm, H, Dh) * Dm ** (-0.5)), 'Wv': _w((lambda *s: _rng.normal(s) * 0.05)(Dm, H, Dh) * Dm ** (-0.5)), 'Wo': _w((lambda *s: _rng.normal(s) * 0.05)(H, Dh, Dm) * (H * Dh) ** (-0.5)), 'seg_len': seg}
    _A_in = _A_setup()

    def _B_setup():
        B, S, D, F = (1, 2048, 1024, 3584)
        return {'x': _w((lambda *s: _rng.normal(s) * 0.05)(B, S, D)), 'w1': _w((lambda *s: _rng.normal(s) * 0.05)(D, D) * D ** (-0.5)), 'w2': _w((lambda *s: _rng.normal(s) * 0.05)(D, D) * D ** (-0.5)), 'w3': _w((lambda *s: _rng.normal(s) * 0.05)(D, F) * D ** (-0.5)), 'w4': _w((lambda *s: _rng.normal(s) * 0.05)(F, D) * F ** (-0.5))}
    _B_in = _B_setup()
    return {'A_x': _A_in['x'], 'A_mem0': _A_in['mem0'], 'A_Wq': _A_in['Wq'], 'A_Wk': _A_in['Wk'], 'A_Wv': _A_in['Wv'], 'A_Wo': _A_in['Wo'], 'A_seg_len': _A_in['seg_len'], 'B_x': _B_in['x'], 'B_w1': _B_in['w1'], 'B_w2': _B_in['w2'], 'B_w3': _B_in['w3'], 'B_w4': _B_in['w4']}

def reference(A_x, A_mem0, A_Wq, A_Wk, A_Wv, A_Wo, A_seg_len, B_x, B_w1, B_w2, B_w3, B_w4):

    def _A_ref(x, mem0, Wq, Wk, Wv, Wo, seg_len):
        B, S, Dm = x.shape
        H, Dh = (Wq.shape[1], Wq.shape[2])
        M = mem0.shape[1]
        scale = Dh ** (-0.5)
        n_seg = S // seg_len
        L = M + seg_len
        idx = jnp.arange(L)
        mask = (idx[:, None] < M) | (idx[:, None] >= idx[None, :])
        mem = mem0
        outs = []
        for s in range(n_seg):
            xs = x[:, s * seg_len:(s + 1) * seg_len, :].copy()
            h = jnp.concatenate([mem, xs], axis=1)
            q = jnp.einsum('btd,dhe->bhte', h, Wq)
            k = jnp.einsum('btd,dhe->bhte', h, Wk)
            v = jnp.einsum('btd,dhe->bhte', h, Wv)
            scores = jnp.einsum('bhqe,bhke->bhqk', q, k) * scale
            scores = jnp.where(mask[None, None], scores, -1000000000.0)
            p = _softmax(scores, axis=-1)
            o = jnp.einsum('bhqk,bhke->bhqe', p, v)
            o = jnp.einsum('bhte,hed->btd', o, Wo)
            mem = o[:, :M, :].copy()
            outs.append(o[:, M:, :])
        return jnp.concatenate(outs, axis=1)

    def _B_ref(x, w1, w2, w3, w4):
        B, S, D = x.shape
        h = _gelu(_layernorm(x, axis=-1) @ w1)
        c = D // 4
        g0 = jnp.pad(h[:, :, 0 * c:1 * c], ((0, 0), (1, 0), (0, 0)))[:, :S, :]
        g1 = jnp.pad(h[:, :, 1 * c:2 * c], ((0, 0), (0, 1), (0, 0)))[:, 1:, :]
        g2 = jnp.pad(h[:, :, 2 * c:3 * c], ((0, 0), (2, 0), (0, 0)))[:, :S, :]
        g3 = jnp.pad(h[:, :, 3 * c:], ((0, 0), (0, 2), (0, 0)))[:, 2:, :]
        hs = jnp.concatenate([g0, g1, g2, g3], axis=-1) @ w2
        x1 = x + hs
        h2 = _gelu(_layernorm(x1, axis=-1) @ w3) @ w4
        return x1 + h2
    x = A_x
    xn = _layernorm(x, axis=-1)
    return x + _A_ref(xn, A_mem0, A_Wq, A_Wk, A_Wv, A_Wo, A_seg_len) + _B_ref(xn, B_w1, B_w2, B_w3, B_w4)
```

```python
import functools
import math

import jax
import jax.numpy as jnp
from jax import lax
import jax.experimental.pallas as pl
import jax.experimental.pallas.tpu as pltpu

F32 = jnp.float32
BF16 = jnp.bfloat16
U32 = jnp.uint32
LANES = 128
PAD = 8


def _dot(a, b):
    return lax.dot_general(a, b, (((1,), (0,)), ((), ())), preferred_element_type=F32)


def _dot_nt(a, b):
    return lax.dot_general(a, b, (((1,), (1,)), ((), ())), preferred_element_type=F32)


def _layernorm(x):
    m = jnp.mean(x, axis=-1, keepdims=True)
    d = x - m
    v = jnp.mean(d * d, axis=-1, keepdims=True)
    return d * lax.rsqrt(v + 1e-5)


def _gelu(x):
    c = math.sqrt(2.0 / math.pi)
    inner = x * (c + (c * 0.044715) * (x * x))
    hx = 0.5 * x
    return hx + hx * jnp.tanh(inner)


def _kernel(x_hbm, mem0_ref, wq_hbm, wk_hbm, wv_hbm, wo_hbm, w1_hbm, w2_hbm, w3_hbm, w4_hbm,
            out_hbm,
            xbuf, hbuf, res, hs, w1, w2, w3, w4, stg, wqkv, wo, obuf,
            sem_x, sem_w, sem_qkv, sem_wo, sem_out,
            *, S, D, H, Dh, M, seg, F, TM1, TM2, FC):
    L = M + seg
    n_seg = S // seg
    nd = D // LANES
    slab = D // 2 + 2
    nb1 = S // TM1
    nb2 = S // TM2

    x_cp = [pltpu.make_async_copy(x_hbm.at[pl.ds(i * TM1, TM1)], xbuf.at[pl.ds(i * TM1, TM1)], sem_x.at[i])
            for i in range(nb1)]
    w_cp = [pltpu.make_async_copy(src, dst, sem_w.at[i])
            for i, (src, dst) in enumerate(((w1_hbm, w1), (w2_hbm, w2), (w3_hbm, w3), (w4_hbm, w4)))]
    qkv_cp = [pltpu.make_async_copy(src, stg.at[i], sem_qkv.at[i])
              for i, src in enumerate((wq_hbm, wk_hbm, wv_hbm))]
    wo_cp = [pltpu.make_async_copy(wo_hbm.at[:, pl.ds(n * LANES, LANES)], wo.at[n], sem_wo.at[n])
             for n in range(nd)]
    x_cp[0].start()
    w_cp[0].start()
    for c in x_cp[1:]:
        c.start()
    for c in w_cp[1:]:
        c.start()
    for c in qkv_cp + wo_cp:
        c.start()

    zpad = jnp.zeros((PAD, LANES), F32)
    for n in range(nd):
        hs[n, 0:PAD, :] = zpad
        hs[n, PAD + S:PAD + S + PAD, :] = zpad
    hbuf[0, 0:M, :] = mem0_ref[...].astype(F32)

    w_cp[0].wait()

    def b1(i, carry):
        r0 = pl.multiple_of(i * TM1, TM1)
        pltpu.make_async_copy(x_hbm.at[pl.ds(r0, TM1)], xbuf.at[pl.ds(r0, TM1)], sem_x.at[i]).wait()
        xn = _layernorm(xbuf[pl.ds(r0, TM1), :].astype(F32))
        for j in range(TM1 // seg):
            hbuf[i * (TM1 // seg) + j, M:L, :] = xn[j * seg:(j + 1) * seg]
        h = _gelu(_dot(_layernorm(xn), w1[...]))
        for n in range(nd):
            hs[n, pl.ds(r0 + PAD, TM1), :] = h[:, n * LANES:(n + 1) * LANES]
        return carry

    lax.fori_loop(0, nb1, b1, 0)

    for c in w_cp[1:]:
        c.wait()
    shifts = (-1, 1, -2, 2)

    def b2(i, carry):
        r0 = pl.multiple_of(i * TM2, TM2)
        sh = jnp.concatenate(
            [hs[n, pl.ds(r0 + PAD + shifts[n * 4 // nd], TM2), :] for n in range(nd)], axis=1)
        xn = jnp.concatenate([hbuf[i * (TM2 // seg) + j, M:L, :] for j in range(TM2 // seg)], axis=0)
        x1 = xn + _dot(sh, w2[...])
        l2 = _layernorm(x1)
        acc = x1 + xbuf[pl.ds(r0, TM2), :].astype(F32)
        for c in range(F // FC):
            g = _gelu(_dot(l2, w3[:, c * FC:(c + 1) * FC]))
            acc = acc + _dot(g, w4[c * FC:(c + 1) * FC, :])
        res[pl.ds(r0, TM2), :] = acc
        return carry

    lax.fori_loop(0, nb2, b2, 0)

    for c in qkv_cp + wo_cp:
        c.wait()
    hp = H // 2
    for t in range(3):
        su = stg.at[t].bitcast(U32)

        def repack(i, carry, su=su, t=t):
            for u in range(8):
                p = i * 8 + u
                for j in range(hp // 8):
                    a = su[pl.ds(pl.multiple_of(p * 2 * hp + 8 * j, 8), 8), :]
                    b = su[pl.ds(pl.multiple_of(p * 2 * hp + hp + 8 * j, 8), 8), :]
                    lo = (a & 0xFFFF) | (b << 16)
                    hi = (a >> 16) | (b & jnp.uint32(0xFFFF0000))
                    base = (t * H + 16 * j) * slab + p
                    wqkv[pl.ds(base, 8, stride=2 * slab), :] = lo
                    wqkv[pl.ds(base + slab, 8, stride=2 * slab), :] = hi
            return carry

        lax.fori_loop(0, D // 16, repack, 0)

    scale = Dh ** -0.5
    row = lax.broadcasted_iota(jnp.int32, (L, L), 0)
    col = lax.broadcasted_iota(jnp.int32, (L, L), 1)
    mask = (row < M) | (row >= col)
    G = 2
    out_rows = 8 * seg

    def out_copy(j):
        r0 = pl.multiple_of(j * out_rows, out_rows)
        return pltpu.make_async_copy(xbuf.at[pl.ds(r0, out_rows)], out_hbm.at[pl.ds(r0, out_rows)], sem_out.at[j])

    def step(s, carry):
        def proj(t, h):
            w = pltpu.bitcast(wqkv[pl.ds((t * H + h) * slab, D // 2), :], BF16)
            return _dot(hbuf[s], w)

        def wo_part(n, lo, hi):
            return _dot(obuf[:, lo * Dh:hi * Dh], wo[n, lo * Dh:hi * Dh, :])

        ng = H // G
        qkv, soft, part = {}, {}, {}
        for g in range(ng + 2):
            if g < ng:
                for h in range(g * G, (g + 1) * G):
                    qkv[h] = (proj(0, h), proj(1, h).astype(BF16), proj(2, h).astype(BF16))
            else:
                for n in range((g - ng) * nd // 2, (g - ng + 1) * nd // 2):
                    part[n] = wo_part(n, 0, H // 2)
            if 1 <= g <= ng:
                for h in range((g - 1) * G, g * G):
                    q, k, _ = qkv[h]
                    sc = jnp.where(mask, _dot_nt(q, k), -1e9 / scale)
                    e = jnp.exp2((sc - jnp.max(sc, axis=-1, keepdims=True)) * (scale * math.log2(math.e)))
                    soft[h] = (e, 1.0 / jnp.sum(e, axis=-1, keepdims=True))
            if g >= 2:
                for h in range((g - 2) * G, (g - 1) * G):
                    e, r = soft[h]
                    obuf[:, h * Dh:(h + 1) * Dh] = _dot(e, qkv[h][2]) * r
        r0 = pl.multiple_of(s * seg, seg)
        nxt = jnp.minimum(s + 1, n_seg)
        for n in range(nd):
            o = part[n] + wo_part(n, H // 2, H)
            cols = slice(n * LANES, (n + 1) * LANES)
            hbuf[nxt, 0:M, cols] = o[0:M]
            xbuf[pl.ds(r0, seg), cols] = (res[pl.ds(r0, seg), cols] + o[M:L]).astype(BF16)

        @pl.when(s % 8 == 7)
        def _():
            out_copy(s // 8).start()

        return carry

    lax.fori_loop(0, n_seg, step, 0)
    for j in range(S // out_rows):
        out_copy(j).wait()


@functools.partial(jax.jit, static_argnames=("A_seg_len",))
def pallas_parallel_sum__memory_aug_recurrent_mem_tr__mixer_s_mlp__prompt_kernel(
    A_x: jax.Array,
    A_mem0: jax.Array,
    A_Wq: jax.Array,
    A_Wk: jax.Array,
    A_Wv: jax.Array,
    A_Wo: jax.Array,
    A_seg_len: int,
    B_x: jax.Array,
    B_w1: jax.Array,
    B_w2: jax.Array,
    B_w3: jax.Array,
    B_w4: jax.Array,
):
    del B_x
    _, S, D = A_x.shape
    _, H, Dh = A_Wq.shape
    M = A_mem0.shape[1]
    seg = int(A_seg_len)
    F = B_w3.shape[1]
    TM1, TM2, FC = 256, 128, 512
    L = M + seg
    nd = D // LANES

    kern = functools.partial(_kernel, S=S, D=D, H=H, Dh=Dh, M=M, seg=seg, F=F, TM1=TM1, TM2=TM2, FC=FC)
    hbm = pl.BlockSpec(memory_space=pl.ANY)
    dma = pltpu.SemaphoreType.DMA
    out = pl.pallas_call(
        kern,
        out_shape=jax.ShapeDtypeStruct((S, D), BF16),
        in_specs=[hbm, pl.BlockSpec(memory_space=pltpu.VMEM)] + [hbm] * 8,
        out_specs=hbm,
        scratch_shapes=[
            pltpu.VMEM((S, D), BF16),
            pltpu.VMEM((S // seg + 1, L, D), F32),
            pltpu.VMEM((S, D), F32),
            pltpu.VMEM((nd, S + 2 * PAD, LANES), F32),
            pltpu.VMEM((D, D), BF16),
            pltpu.VMEM((D, D), BF16),
            pltpu.VMEM((D, F), BF16),
            pltpu.VMEM((F, D), BF16),
            pltpu.VMEM((3, D * H, Dh), BF16),
            pltpu.VMEM((3 * H * (D // 2 + 2), Dh), U32),
            pltpu.VMEM((nd, H * Dh, LANES), BF16),
            pltpu.VMEM((L, H * Dh), F32),
            dma((S // TM1,)), dma((4,)), dma((3,)), dma((nd,)), dma((S // (8 * seg),)),
        ],
        compiler_params=pltpu.CompilerParams(vmem_limit_bytes=120 * 1024 * 1024),
        name="rmt_s2mlp",
    )(A_x.reshape(S, D), A_mem0.reshape(M, D),
      A_Wq.reshape(D * H, Dh), A_Wk.reshape(D * H, Dh), A_Wv.reshape(D * H, Dh),
      A_Wo.reshape(H * Dh, D), B_w1, B_w2, B_w3, B_w4)
    return out.reshape(1, S, D)
```

```python
import functools
import math

import jax
import jax.numpy as jnp
from jax import lax
import jax.experimental.pallas as pl
import jax.experimental.pallas.tpu as pltpu

F32 = jnp.float32
BF16 = jnp.bfloat16
U32 = jnp.uint32
LANES = 128
PAD = 8


def _dot(a, b):
    return lax.dot_general(a, b, (((1,), (0,)), ((), ())), preferred_element_type=F32)


def _dot_nt(a, b):
    return lax.dot_general(a, b, (((1,), (1,)), ((), ())), preferred_element_type=F32)


def _layernorm(x):
    m = jnp.mean(x, axis=-1, keepdims=True)
    d = x - m
    v = jnp.mean(d * d, axis=-1, keepdims=True)
    return d * lax.rsqrt(v + 1e-5)


def _recip(x):
    r = pl.reciprocal(x, approx=True)
    return r * (2.0 - x * r)


def _gelu(x):
    c = math.sqrt(2.0 / math.pi)
    inner = x * (c + (c * 0.044715) * (x * x))
    hx = 0.5 * x
    return hx + hx * jnp.tanh(inner)


def _kernel(x_hbm, mem0_ref, wq_hbm, wk_hbm, wv_hbm, wo_hbm, w1_hbm, w2_hbm, w3_hbm, w4_hbm,
            out_hbm,
            xbuf, hbuf, res, hs, lcur, lnxt, w1, w2, w3, w4, stg, wqkv, wo, obuf, pbuf,
            sem_x, sem_w, sem_qkv, sem_wo, sem_out,
            *, S, D, H, Dh, M, seg, F, TM1, TM2, FC):
    L = M + seg
    n_seg = S // seg
    nd = D // LANES
    slab = D // 2 + 2
    nb1 = S // TM1
    nb2 = S // TM2
    srows = D * H // nb2

    def cols(n):
        return slice(n * LANES, (n + 1) * LANES)

    def x_copy(i):
        r0 = pl.multiple_of(i * TM1, TM1)
        return pltpu.make_async_copy(x_hbm.at[pl.ds(r0, TM1)], xbuf.at[pl.ds(r0, TM1)], sem_x.at[i])

    def qkv_copy(t, i):
        src = (wq_hbm, wk_hbm, wv_hbm)[t]
        r0 = pl.multiple_of(i * srows, srows)
        return pltpu.make_async_copy(src.at[pl.ds(r0, srows)], stg.at[i % 2, t], sem_qkv.at[i % 2, t])

    w_cp = [pltpu.make_async_copy(src, dst, sem_w.at[i])
            for i, (src, dst) in enumerate(((w1_hbm, w1), (w2_hbm, w2), (w3_hbm, w3), (w4_hbm, w4)))]
    wo_cp = [pltpu.make_async_copy(wo_hbm.at[:, cols(n)], wo.at[n], sem_wo.at[n]) for n in range(nd)]
    x_copy(0).start()
    w_cp[0].start()
    x_copy(1).start()

    zpad = jnp.zeros((PAD, LANES), F32)
    for n in range(nd):
        hs[n, 0:PAD, :] = zpad
        hs[n, PAD + S:PAD + S + PAD, :] = zpad
    hbuf[0, 0:M, :] = mem0_ref[...].astype(F32)

    def norm_in(i, dst):
        r0 = pl.multiple_of(i * TM1, TM1)
        xn = _layernorm(xbuf[pl.ds(r0, TM1), :].astype(F32))
        for j in range(TM1 // seg):
            hbuf[i * (TM1 // seg) + j, M:L, :] = xn[j * seg:(j + 1) * seg]
        dst[...] = _layernorm(xn)

    x_copy(0).wait()
    norm_in(0, lnxt)
    w_cp[0].wait()
    for i in range(2, nb1):
        x_copy(i).start()
    w_cp[1].start()

    def b1(i, carry):
        @pl.when(i + 1 < nb1)
        def _():
            x_copy(i + 1).wait()

        @pl.when(i == 2)
        def _():
            w_cp[2].start()

        @pl.when(i == 5)
        def _():
            w_cp[3].start()

        r0 = pl.multiple_of(i * TM1, TM1)
        lcur[...] = lnxt[...]
        norm_in(jnp.minimum(i + 1, nb1 - 1), lnxt)
        h = _gelu(_dot(lcur[...], w1[...]))
        for n in range(nd):
            hs[n, pl.ds(r0 + PAD, TM1), :] = h[:, cols(n)]
        return carry

    lax.fori_loop(0, nb1, b1, 0)

    w_cp[1].wait()
    shifts = (-1, 1, -2, 2)

    def mix(i):
        r0 = pl.multiple_of(i * TM1, TM1)
        sh = jnp.concatenate(
            [hs[n, pl.ds(r0 + PAD + shifts[n * 4 // nd], TM1), :] for n in range(nd)], axis=1)
        xn = jnp.concatenate([hbuf[i * (TM1 // seg) + j, M:L, :] for j in range(TM1 // seg)], axis=0)
        res[pl.ds(r0, TM1), :] = xn + _dot(sh, w2[...])

    def norm_mid(i):
        r0 = pl.multiple_of(i * TM1, TM1)
        l2 = _layernorm(res[pl.ds(r0, TM1), :])
        for n in range(nd):
            hs[n, pl.ds(r0, TM1), :] = l2[:, cols(n)]

    mix(0)

    def b2(i, carry):
        r0 = pl.multiple_of((i - 1) * TM1, TM1)
        l2 = _layernorm(res[pl.ds(r0, TM1), :])
        mix(i)
        for n in range(nd):
            hs[n, pl.ds(r0, TM1), :] = l2[:, cols(n)]
        return carry

    lax.fori_loop(1, nb1, b2, 0)
    for t in range(3):
        qkv_copy(t, 0).start()
        qkv_copy(t, 1).start()
    norm_mid(nb1 - 1)

    w_cp[2].wait()
    w_cp[3].wait()
    for c in wo_cp:
        c.start()
    hp = H // 2
    npair = srows // (2 * H)

    def b3(i, carry):
        for t in range(3):
            qkv_copy(t, i).wait()

        r0 = pl.multiple_of(i * TM2, TM2)
        l2 = jnp.concatenate([hs[n, pl.ds(r0, TM2), :] for n in range(nd)], axis=1)
        acc = res[pl.ds(r0, TM2), :] + xbuf[pl.ds(r0, TM2), :].astype(F32)
        def repack(t, u):
            su = stg.at[i % 2, t].bitcast(U32)
            for j in range(hp // 8):
                a = su[pl.ds(u * 2 * hp + 8 * j, 8), :]
                b = su[pl.ds(u * 2 * hp + hp + 8 * j, 8), :]
                lo = (a & 0xFFFF) | (b << 16)
                hi = (a >> 16) | (b & jnp.uint32(0xFFFF0000))
                base = (t * H + 16 * j) * slab + u + i * npair
                wqkv[pl.ds(base, 8, stride=2 * slab), :] = lo
                wqkv[pl.ds(base + slab, 8, stride=2 * slab), :] = hi

        todo = [(t, u) for t in range(3) for u in range(npair)]
        nc = F // FC
        for c in range(nc):
            g = _gelu(_dot(l2, w3[:, c * FC:(c + 1) * FC]))
            for t, u in todo[c * len(todo) // nc:(c + 1) * len(todo) // nc]:
                repack(t, u)
            acc = acc + _dot(g, w4[c * FC:(c + 1) * FC, :])
        res[pl.ds(r0, TM2), :] = acc

        @pl.when(i + 2 < nb2)
        def _():
            for t in range(3):
                qkv_copy(t, i + 2).start()

        return carry

    lax.fori_loop(0, nb2, b3, 0)
    for c in wo_cp:
        c.wait()

    scale = Dh ** -0.5
    row = lax.broadcasted_iota(jnp.int32, (L, L), 0)
    col = lax.broadcasted_iota(jnp.int32, (L, L), 1)
    mask = (row < M) | (row >= col)
    G = 2
    out_rows = 4 * seg

    def out_copy(j):
        r0 = pl.multiple_of(j * out_rows, out_rows)
        return pltpu.make_async_copy(xbuf.at[pl.ds(r0, out_rows)], out_hbm.at[pl.ds(r0, out_rows)], sem_out.at[j])

    def step(s, carry):
        def proj(t, h):
            w = pltpu.bitcast(wqkv[pl.ds((t * H + h) * slab, D // 2), :], BF16)
            return _dot(hbuf[s], w)

        def wo_part(n, lo, hi):
            return _dot(obuf[:, lo * Dh:hi * Dh], wo[n, lo * Dh:hi * Dh, :])

        ng = H // G
        qkv, soft = {}, {}
        for g in range(ng + 2):
            if g < ng:
                for h in range(g * G, (g + 1) * G):
                    qkv[h] = (proj(0, h), proj(1, h).astype(BF16), proj(2, h).astype(BF16))
            else:
                for n in range((g - ng) * nd // 2, (g - ng + 1) * nd // 2):
                    pbuf[:, cols(n)] = wo_part(n, 0, H // 2)
            if 1 <= g <= ng:
                for h in range((g - 1) * G, g * G):
                    q, k, _ = qkv[h]
                    sc = jnp.where(mask, _dot_nt(q, k), -1e9 / scale)
                    e = jnp.exp2((sc - jnp.max(sc, axis=-1, keepdims=True)) * (scale * math.log2(math.e)))
                    soft[h] = (e, _recip(jnp.sum(e, axis=-1, keepdims=True)))
            if g >= 2:
                for h in range((g - 2) * G, (g - 1) * G):
                    e, r = soft[h]
                    obuf[:, h * Dh:(h + 1) * Dh] = _dot(e, qkv[h][2]) * r
        r0 = pl.multiple_of(s * seg, seg)
        for n in range(nd):
            o = pbuf[:, cols(n)] + wo_part(n, H // 2, H)
            hbuf[s + 1, 0:M, cols(n)] = o[0:M]
            xbuf[pl.ds(r0, seg), cols(n)] = (res[pl.ds(r0, seg), cols(n)] + o[M:L]).astype(BF16)

        @pl.when(s % 4 == 3)
        def _():
            out_copy(s // 4).start()

        return carry

    lax.fori_loop(0, n_seg, step, 0)
    for j in range(S // out_rows):
        out_copy(j).wait()


@functools.partial(jax.jit, static_argnames=("A_seg_len",))
def pallas_parallel_sum__memory_aug_recurrent_mem_tr__mixer_s_mlp__prompt_kernel(
    A_x: jax.Array,
    A_mem0: jax.Array,
    A_Wq: jax.Array,
    A_Wk: jax.Array,
    A_Wv: jax.Array,
    A_Wo: jax.Array,
    A_seg_len: int,
    B_x: jax.Array,
    B_w1: jax.Array,
    B_w2: jax.Array,
    B_w3: jax.Array,
    B_w4: jax.Array,
):
    del B_x
    _, S, D = A_x.shape
    _, H, Dh = A_Wq.shape
    M = A_mem0.shape[1]
    seg = int(A_seg_len)
    F = B_w3.shape[1]
    TM1, TM2, FC = 256, 128, 512
    L = M + seg
    nd = D // LANES

    kern = functools.partial(_kernel, S=S, D=D, H=H, Dh=Dh, M=M, seg=seg, F=F, TM1=TM1, TM2=TM2, FC=FC)
    hbm = pl.BlockSpec(memory_space=pl.ANY)
    dma = pltpu.SemaphoreType.DMA
    out = pl.pallas_call(
        kern,
        out_shape=jax.ShapeDtypeStruct((S, D), BF16),
        in_specs=[hbm, pl.BlockSpec(memory_space=pltpu.VMEM)] + [hbm] * 8,
        out_specs=hbm,
        scratch_shapes=[
            pltpu.VMEM((S, D), BF16),
            pltpu.VMEM((S // seg + 1, L, D), F32),
            pltpu.VMEM((S, D), F32),
            pltpu.VMEM((nd, S + 2 * PAD, LANES), F32),
            pltpu.VMEM((TM1, D), F32),
            pltpu.VMEM((TM1, D), F32),
            pltpu.VMEM((D, D), BF16),
            pltpu.VMEM((D, D), BF16),
            pltpu.VMEM((D, F), BF16),
            pltpu.VMEM((F, D), BF16),
            pltpu.VMEM((2, 3, D * H * TM2 // S, Dh), BF16),
            pltpu.VMEM((3 * H * (D // 2 + 2), Dh), U32),
            pltpu.VMEM((nd, H * Dh, LANES), BF16),
            pltpu.VMEM((L, H * Dh), F32),
            pltpu.VMEM((L, D), F32),
            dma((S // TM1,)), dma((4,)), dma((2, 3)), dma((nd,)), dma((S // (4 * seg),)),
        ],
        compiler_params=pltpu.CompilerParams(vmem_limit_bytes=120 * 1024 * 1024, flags={"XLA_TPU_EVENLY_DISTRIBUTE_CRITICAL_NODES": True}),
        name="rmt_s2mlp",
    )(A_x.reshape(S, D), A_mem0.reshape(M, D),
      A_Wq.reshape(D * H, Dh), A_Wk.reshape(D * H, Dh), A_Wv.reshape(D * H, Dh),
      A_Wo.reshape(H * Dh, D), B_w1, B_w2, B_w3, B_w4)
    return out.reshape(1, S, D)
```

```python
import functools
import math

import jax
import jax.numpy as jnp
from jax import lax
import jax.experimental.pallas as pl
import jax.experimental.pallas.tpu as pltpu

F32 = jnp.float32
BF16 = jnp.bfloat16
U32 = jnp.uint32
LANES = 128
PAD = 8


def _dot(a, b):
    return lax.dot_general(a, b, (((1,), (0,)), ((), ())), preferred_element_type=F32)


def _dot_nt(a, b):
    return lax.dot_general(a, b, (((1,), (1,)), ((), ())), preferred_element_type=F32)


def _layernorm(x):
    m = jnp.mean(x, axis=-1, keepdims=True)
    d = x - m
    v = jnp.mean(d * d, axis=-1, keepdims=True)
    return d * lax.rsqrt(v + 1e-5)


def _recip(x):
    r = pl.reciprocal(x, approx=True)
    return r * (2.0 - x * r)


def _gelu(x):
    c = math.sqrt(2.0 / math.pi)
    inner = x * (c + (c * 0.044715) * (x * x))
    hx = 0.5 * x
    return hx + hx * jnp.tanh(inner)


def _words(x):
    return pltpu.bitcast(x.astype(BF16), U32)


def _halves(w):
    return pltpu.bitcast(w, BF16)


def _cat(xs, axis):
    return xs[0] if len(xs) == 1 else jnp.concatenate(xs, axis=axis)


def _right(b11, b12, b21, b22):
    return (b11 + b22, b11, b12 - b22, b21 - b11, b22, b11 + b12, b21 + b22)


def _unpack(w):
    return pltpu.bitcast(w << 16, F32), pltpu.bitcast(w & U32(0xFFFF0000), F32)


def _pack(lo, hi):
    return pltpu.bitcast(pltpu.pack_elementwise([lo, hi], packed_dtype=BF16), U32)


def _right_words(w):
    lo, hi = zip(*[_unpack(x) for x in w])
    f = [_pack(a, b) for a, b in zip(_right(*lo), _right(*hi))]
    f[1], f[4] = w[0], w[3]
    return f


def _left(a11, a12, a21, a22):
    return (a11 + a22, a21 + a22, a11, a22, a11 + a12, a21 - a11, a12 - a22)


def _combine(m):
    m4 = m(3)
    m2 = m(1)
    c21 = m2 + m4
    m1 = m(0)
    c22 = m1 - m2
    c11 = m1 + m4
    c11 = c11 + m(6)
    m5 = m(4)
    c11 = c11 - m5
    m3 = m(2)
    c12 = m3 + m5
    c22 = c22 + m3
    c22 = c22 + m(5)
    return c11, c12, c21, c22


def _kernel(x_hbm, mem0_ref, wq_hbm, wk_hbm, wv_hbm, wo_hbm, w1_hbm, w2_hbm, w3_hbm, w4_hbm,
            out_hbm,
            xbuf, xnb, res, hs, la, lb, lz, w3f, w4f, arq, aro, stq, sto, membuf, hl, ol, pbuf,
            sem_x, sem_w, sem_a, sem_out,
            *, S, D, H, Dh, M, seg, F, TM1, TM2):
    L = M + seg
    nd = D // LANES
    nh = nd // 2
    Dk = D // 2
    wk = Dk // 2
    slab = wk + 1
    nf = F // (2 * LANES)
    ng = H // 2
    nb1 = S // TM1
    nb2 = S // TM2
    h1 = TM1 // 2
    h2 = TM2 // 2

    def cols(n, w=1):
        return slice(n * LANES, (n + w) * LANES)

    raw = {1: 0, 2: nd * Dk, 3: 2 * nd * Dk, 4: 2 * nd * Dk + 2 * nf * Dk}
    raw_src = {1: w1_hbm, 2: w2_hbm, 3: w3_hbm, 4: w4_hbm}
    raw_rows = {1: Dk, 2: Dk, 3: Dk, 4: F // 2}
    raw_sem = {1: 0, 2: nd, 3: 2 * nd, 4: 2 * nd + 2 * nf}

    def w_copy(j, n):
        return pltpu.make_async_copy(raw_src[j].bitcast(U32).at[:, cols(n)],
                                     arq.at[pl.ds(raw[j] + n * raw_rows[j], raw_rows[j])],
                                     sem_w.at[raw_sem[j] + n])

    def x_copy(i):
        r0 = pl.multiple_of(i * TM1, TM1)
        return pltpu.make_async_copy(x_hbm.at[pl.ds(r0, TM1)], xbuf.at[pl.ds(r0, TM1)], sem_x.at[i])

    fpi = Dk // nb2
    gpi = ng // nb2

    def a_copies(i):
        cps = []
        for t, src in enumerate((wq_hbm, wk_hbm, wv_hbm)):
            for half in range(2):
                r0 = pl.multiple_of((half * Dk + i * fpi) * (H // 2), fpi * H // 2)
                cps.append(pltpu.make_async_copy(src.bitcast(U32).at[pl.ds(r0, fpi * H // 2)],
                                                 stq.at[i % 2, 2 * t + half], sem_a.at[i % 2, 2 * t + half]))
        r0 = pl.multiple_of(i * gpi * Dh, gpi * Dh)
        for n in range(nd):
            cps.append(pltpu.make_async_copy(wo_hbm.bitcast(U32).at[pl.ds(r0, gpi * Dh), cols(n)],
                                             sto.at[i % 2, pl.ds(n * gpi * Dh, gpi * Dh)], sem_a.at[i % 2, 6 + n]))
        return cps

    def prep(src, r11, r12, r21, r22, rows, dst, base, pitch):
        for r in range(0, rows, 8):
            for i, f in enumerate(_right_words([src[pl.ds(o + r, 8), :] for o in (r11, r12, r21, r22)])):
                dst[pl.ds(base + i * pitch + r, 8), :] = f

    def prep_sq(j, n, r, rows):
        o = raw[j] + r
        prep(arq, o + n * Dk, o + (n + nh) * Dk, o + n * Dk + wk, o + (n + nh) * Dk + wk, rows,
             aro, ((j - 1) * nh + n) * 7 * wk + r, wk)

    x_copy(0).start()
    for n in range(nd):
        w_copy(1, n).start()
    x_copy(1).start()

    zpad = jnp.zeros((PAD, LANES), F32)
    for n in range(nd):
        hs[n, 0:PAD, :] = zpad
        hs[n, PAD + S:PAD + S + PAD, :] = zpad
    membuf[...] = mem0_ref[...].astype(F32)

    RC = 16

    def put_left(dst, r, a11, a12, a21, a22):
        for k, f in enumerate(_left(a11, a12, a21, a22)):
            for n in range(nh):
                dst[k, n, r:r + RC, :] = f[:, cols(n)].astype(BF16)

    def get_left(src, k):
        w = src.bitcast(U32)
        return _halves(_cat([w[k, n] for n in range(src.shape[1])], 1))

    def norm_in(i, dst):
        for r in range(0, h1, RC):
            a = []
            for half in range(2):
                rr = pl.ds(pl.multiple_of(i * TM1 + half * h1 + r, RC), RC)
                xn = _layernorm(xbuf[rr, :].astype(F32))
                xnb[rr, :] = xn.astype(BF16)
                res[rr, :] = xn
                a.append(_layernorm(xn))
            put_left(dst, r, a[0][:, :Dk], a[0][:, Dk:], a[1][:, :Dk], a[1][:, Dk:])

    x_copy(0).wait()
    norm_in(0, la)
    for n in range(nh):
        w_copy(1, n).wait()
        w_copy(1, n + nh).wait()
        if n == 0:
            x_copy(2).start()
            x_copy(3).start()
        prep_sq(1, n, 0, wk)

    later = [[w_copy(2, n) for n in range(nd)]]
    w3c = [w_copy(3, n) for n in range(2 * nf)]
    w4c = [w_copy(4, n) for n in range(nd)]
    later += [[x_copy(4 + k)] + w3c[5 * k:5 * k + 5] for k in range(4)] + [w3c[20:]]
    later += [w4c[2 * k:2 * k + 2] for k in range(4)]

    def start_later(i, lo, hi):
        for k in range(lo, min(hi, len(later))):
            @pl.when(i == k)
            def _(k=k):
                for c in later[k]:
                    c.start()

    def b1(i, cur, nxt, second):
        r0 = pl.multiple_of(i * TM1, TM1)
        norm_in(jnp.minimum(i + 1, nb1 - 1), nxt)
        for n in range(nh):
            c = _combine(lambda k: _dot(get_left(cur, k), _halves(aro[pl.ds((n * 7 + k) * wk, wk), :])))
            hs[n, pl.ds(r0 + PAD, h1), :] = _gelu(c[0])
            hs[n + nh, pl.ds(r0 + PAD, h1), :] = _gelu(c[1])
            hs[n, pl.ds(r0 + PAD + h1, h1), :] = _gelu(c[2])
            hs[n + nh, pl.ds(r0 + PAD + h1, h1), :] = _gelu(c[3])
            if second:
                prep_sq(2, i - nb1 // 2, n * wk // nh, wk // nh)
        if second:
            start_later(i, nb1 // 2, nb1)
        else:
            start_later(i, 0, nb1 // 2)

    def b1_pair(second):
        def b1p(i, carry):
            x_copy(2 * i + 1).wait()
            b1(2 * i, la, lb, second)

            @pl.when(2 * i + 2 < nb1)
            def _():
                x_copy(2 * i + 2).wait()

            b1(2 * i + 1, lb, la, second)
            return carry
        return b1p

    lax.fori_loop(0, nb1 // 4, b1_pair(False), 0)
    for n in range(nd):
        w_copy(2, n).wait()
    lax.fori_loop(nb1 // 4, nb1 // 2, b1_pair(True), 0)

    shifts = (-1, 1, -2, 2)

    def shift_in(i, dst):
        for r in range(0, h1, RC):
            def blk(half, c):
                r0 = i * TM1 + PAD + half * h1 + r
                return _cat([hs[n, pl.ds(r0 + shifts[n * 4 // nd], RC), :] for n in range(c, c + nh)], 1)

            put_left(dst, r, blk(0, 0), blk(0, nh), blk(1, 0), blk(1, nh))

    def norm_mid(i):
        for r in range(0, TM1, 2 * RC):
            rr = pl.ds(pl.multiple_of(i * TM1 + r, 2 * RC), 2 * RC)
            l2 = _layernorm(res[rr, :])
            for n in range(nd):
                hs[n, rr, :] = l2[:, cols(n)]

    def prep3(u):
        p, r = u // 2, (u % 2) * (wk // 2)
        o = raw[3] + 2 * p * Dk + r
        prep(arq, o, o + Dk, o + wk, o + Dk + wk, wk // 2, w3f, p * 7 * wk + r, wk)

    def prep4(n, p):
        o = raw[4] + n * (F // 2) + p * LANES
        rows = LANES // 2
        prep(arq, o, o + nh * (F // 2), o + rows, o + nh * (F // 2) + rows, rows,
             w4f, n * 7 * nf * rows + p * rows, nf * rows)

    def b2(i, cur, nxt, second):
        r0 = pl.multiple_of(i * TM1, TM1)
        shift_in(jnp.minimum(i + 1, nb1 - 1), nxt)
        for n in range(nh):
            c = _combine(lambda k: _dot(get_left(cur, k), _halves(aro[pl.ds(((nh + n) * 7 + k) * wk, wk), :])))
            res[pl.ds(r0, h1), cols(n)] += c[0]
            res[pl.ds(r0, h1), cols(n + nh)] += c[1]
            res[pl.ds(r0 + h1, h1), cols(n)] += c[2]
            res[pl.ds(r0 + h1, h1), cols(n + nh)] += c[3]
        if second:
            for p in range(nf):
                prep4(i - nb1 // 2, p)
        else:
            per = 2 * nf // (nb1 // 2)
            for u in range(per):
                prep3(i * per + u)
            start_later(i + nb1, nb1, nb1 + nb1 // 2)
        norm_mid(i)

    def b2_pair(second):
        def b2p(i, carry):
            b2(2 * i, la, lb, second)
            b2(2 * i + 1, lb, la, second)
            return carry
        return b2p

    shift_in(0, la)
    for c in w3c:
        c.wait()
    lax.fori_loop(0, nb1 // 4, b2_pair(False), 0)
    for c in w4c:
        c.wait()
    for c in a_copies(0) + a_copies(1):
        c.start()
    lax.fori_loop(nb1 // 4, nb1 // 2, b2_pair(True), 0)

    hp = H // 2

    def b3(i, carry):
        for c in a_copies(i):
            c.wait()

        def prep_qkv(t, u, j):
            forms = []
            for par in range(2):
                w = [stq[i % 2, 2 * t + half, pl.ds((2 * u + par) * hp + 8 * j, 8), :] for half in range(2)]
                forms.append(_right(*_unpack(w[0]), *_unpack(w[1])))
            for k in range(7):
                base = ((t * ng + 8 * j) * 7 + k) * slab + u + i * (fpi // 2)
                arq[pl.ds(base, 8, stride=7 * slab), :] = _pack(forms[0][k], forms[1][k])

        def prep_o(g, n):
            o = 2 * g * (Dh // 2)
            prep(sto.at[i % 2], o + n * gpi * Dh, o + (n + nh) * gpi * Dh,
                 o + n * gpi * Dh + Dh // 2, o + (n + nh) * gpi * Dh + Dh // 2, Dh // 2,
                 aro, pl.multiple_of((n * 7 * ng + i * gpi + g) * (Dh // 2), Dh // 2), ng * Dh // 2)

        r0 = pl.multiple_of(i * TM2, TM2)

        def blk(r, c):
            return _cat([hs[n, pl.ds(r0 + r, h2), :] for n in range(c, c + nh)], 1)

        ly = [f.astype(BF16) for f in _left(blk(0, 0), blk(0, nh), blk(h2, 0), blk(h2, nh))]
        for p in range(nf):
            c = _combine(lambda k: _dot(ly[k], _halves(w3f[pl.ds((p * 7 + k) * wk, wk), :])))
            for k, f in enumerate(_left(*[_gelu(y) for y in c])):
                lz[k, p] = f.astype(BF16)
        for t in range(3):
            for u in range(fpi // 2):
                for j in range(hp // 8):
                    prep_qkv(t, u, j)
        for g in range(gpi):
            for n in range(nh):
                prep_o(g, n)
        rows = nf * LANES // 2
        for n in range(0, nh, 2):
            c = _combine(lambda k: _dot(get_left(lz, k), _cat(
                [_halves(w4f[pl.ds(((n + e) * 7 + k) * rows, rows), :]) for e in range(2)], 1)))
            for r, cc, y in ((0, n, c[0]), (0, n + nh, c[1]), (h2, n, c[2]), (h2, n + nh, c[3])):
                rr = pl.ds(r0 + r, h2)
                res[rr, cols(cc, 2)] += xbuf[rr, cols(cc, 2)].astype(F32) + y

        @pl.when(i + 2 < nb2)
        def _():
            for c in a_copies(i + 2):
                c.start()

        return carry

    lax.fori_loop(0, nb2, b3, 0)

    scale = Dh ** -0.5
    row = lax.broadcasted_iota(jnp.int32, (L, L), 0)
    col = lax.broadcasted_iota(jnp.int32, (L, L), 1)
    mask = (row < M) | (row >= col)
    QS = 4 * seg
    R = seg - M
    rv = R // 8

    def upper(n):
        return lax.broadcasted_iota(jnp.int32, (8, n), 0) < 4

    def split8(mem, tok):
        u = upper(mem.shape[1])
        return jnp.where(u, mem, tok), pltpu.roll(jnp.where(u, tok, mem), 4, 0)

    def join8(t, b):
        u = upper(t.shape[1])
        b = pltpu.roll(b, 4, 0)
        return jnp.where(u, t, b), jnp.where(u, b, t)

    def out_copy(j):
        r0 = pl.multiple_of(j * QS, QS)
        return pltpu.make_async_copy(xbuf.at[pl.ds(r0, QS)], out_hbm.at[pl.ds(r0, QS)], sem_out.at[j])

    def vregs(y, lo, hi):
        return [y[8 * k:8 * k + 8] for k in range(lo, hi)]

    def quad(j, carry):
        xs = xnb[pl.ds(pl.multiple_of(j * QS, QS), QS), :].astype(F32)
        qkv = {(t, h): [] for t in range(3) for h in range(H)}
        att = {h: [] for h in range(H)}
        outs = {n: [] for n in range(nd)}
        mem = membuf[...]
        for st in range(4):
            if st == 0:
                t0, u0 = split8(mem, xs[2 * R:2 * R + 8])
                at = jnp.concatenate([t0, xs[0:R]], axis=0)
                au = jnp.concatenate([u0, xs[R:2 * R]], axis=0)
                for k, f in enumerate(_left(at[:, :Dk], at[:, Dk:], au[:, :Dk], au[:, Dk:])):
                    hl[st, k] = f
            else:
                r = 2 * R + 8 + (st - 1) * R
                a = jnp.concatenate([mem, xs[r:r + R]], axis=0)
                hl[st, 1] = a[:, :Dk] + a[:, Dk:]
                hl[st, 2] = a[:, :Dk]
                hl[st, 3] = a[:, Dk:]

            def proj(t, g):
                def m(k, left=None):
                    w = _halves(arq[pl.ds(((t * ng + g) * 7 + k) * slab, wk), :])
                    return _dot(hl[st, k if left is None else left], w)

                got = []
                if st == 0:
                    c = _combine(m)
                    for e in range(2):
                        ym, yt = join8(c[e][0:8], c[2 + e][0:8])
                        qkv[t, 2 * g + e] += vregs(c[e], 1, 1 + rv) + vregs(c[2 + e], 1, 1 + rv) + [yt]
                        got.append(ym)
                else:
                    for e, y in enumerate((m(3) + m(1), m(2) + m(4, 1))):
                        qkv[t, 2 * g + e] += vregs(y, 1, 1 + rv)
                        got.append(y[0:8])
                return [jnp.concatenate([got[e]] + qkv[t, 2 * g + e][4 * st:4 * st + 4], axis=0) for e in range(2)]

            def feed(g, o):
                for e in range(2):
                    att[2 * g + e] += vregs(o[e], 1, 5)
                if st < 3:
                    a = [jnp.concatenate([o[e][0:8]] + att[2 * g + e][st * rv:(st + 1) * rv], axis=0)
                         for e in range(2)]
                    ol[st, 1, :, cols(g)] = a[0] + a[1]
                    ol[st, 2, :, cols(g)] = a[0]
                    ol[st, 3, :, cols(g)] = a[1]
                else:
                    at, au = [], []
                    for e in range(2):
                        y = att[2 * g + e][3 * rv:]
                        t0, u0 = split8(o[e][0:8], y[2 * rv])
                        at.append(jnp.concatenate([t0] + y[:rv], axis=0))
                        au.append(jnp.concatenate([u0] + y[rv:2 * rv], axis=0))
                    for k, f in enumerate(_left(at[0], at[1], au[0], au[1])):
                        ol[st, k, :, cols(g)] = f

            def wo_part(n, lo, hi):
                def m(k, left=None):
                    w = _halves(aro[pl.ds(((n * 7 + k) * ng + lo) * (Dh // 2), (hi - lo) * (Dh // 2)), :])
                    return _dot(ol[st, k if left is None else left, :, lo * Dh:hi * Dh], w)

                return _combine(m) if st == 3 else (m(3) + m(1), m(2) + m(4, 1))

            aro[pl.ds(aro.shape[0] - 16 + (j % 2) * 8, 8), :] = jnp.zeros((8, LANES), U32)
            cur, soft = {}, {}
            for g in range(ng + 2):
                if g < ng:
                    cur[g] = [proj(t, g) for t in range(3)]
                else:
                    for n in range((g - ng) * nh // 2, (g - ng + 1) * nh // 2):
                        for k, y in enumerate(wo_part(n, 0, ng // 2)):
                            pbuf[st, k, :, cols(n)] = y
                if 1 <= g <= ng:
                    soft[g - 1] = []
                    for e in range(2):
                        q, k = cur[g - 1][0][e], cur[g - 1][1][e]
                        sc = jnp.where(mask, _dot_nt(q, k.astype(BF16)), -1e9 / scale)
                        p = jnp.exp2((sc - jnp.max(sc, axis=-1, keepdims=True)) * (scale * math.log2(math.e)))
                        soft[g - 1].append((p, _recip(jnp.sum(p, axis=-1, keepdims=True))))
                if g >= 2:
                    feed(g - 2, [_dot(p, cur[g - 2][2][e].astype(BF16)) * r
                                 for e, (p, r) in enumerate(soft[g - 2])])
            arq[pl.ds(arq.shape[0] - 16 + (j % 2) * 8, 8), :] = jnp.zeros((8, LANES), U32)
            new = {}
            for n in range(nh):
                c = [pbuf[st, k, :, cols(n)] + y for k, y in enumerate(wo_part(n, ng // 2, ng))]
                for e in range(2):
                    if st < 3:
                        new[n + e * nh] = c[e][0:8]
                        outs[n + e * nh] += vregs(c[e], 1, 1 + rv)
                    else:
                        ym, yt = join8(c[e][0:8], c[2 + e][0:8])
                        new[n + e * nh] = ym
                        outs[n + e * nh] += vregs(c[e], 1, 1 + rv) + vregs(c[2 + e], 1, 1 + rv) + [yt]
            mem = jnp.concatenate([new[n] for n in range(nd)], axis=1)
            lo, hi = ((0, 2), (2, 6), (6, 8), (8, 16))[st]
            rr = pl.ds(pl.multiple_of(j * QS + 8 * lo, 16), 8 * (hi - lo))
            for n in range(nd):
                xbuf[rr, cols(n)] = (res[rr, cols(n)] + jnp.concatenate(outs[n][lo:hi], axis=0)).astype(BF16)
        membuf[...] = mem
        out_copy(j).start()
        return carry

    lax.fori_loop(0, S // QS, quad, 0)
    for j in range(S // QS):
        out_copy(j).wait()


@functools.partial(jax.jit, static_argnames=("A_seg_len",))
def pallas_parallel_sum__memory_aug_recurrent_mem_tr__mixer_s_mlp__prompt_kernel(
    A_x: jax.Array,
    A_mem0: jax.Array,
    A_Wq: jax.Array,
    A_Wk: jax.Array,
    A_Wv: jax.Array,
    A_Wo: jax.Array,
    A_seg_len: int,
    B_x: jax.Array,
    B_w1: jax.Array,
    B_w2: jax.Array,
    B_w3: jax.Array,
    B_w4: jax.Array,
):
    del B_x
    _, S, D = A_x.shape
    _, H, Dh = A_Wq.shape
    M = A_mem0.shape[1]
    seg = int(A_seg_len)
    F = B_w3.shape[1]
    assert (M, seg, Dh) == (8, 32, LANES)
    TM1, TM2 = 256, 128
    nd = D // LANES
    nb2 = S // TM2

    kern = functools.partial(_kernel, S=S, D=D, H=H, Dh=Dh, M=M, seg=seg, F=F, TM1=TM1, TM2=TM2)
    hbm = pl.BlockSpec(memory_space=pl.ANY)
    dma = pltpu.SemaphoreType.DMA
    out = pl.pallas_call(
        kern,
        out_shape=jax.ShapeDtypeStruct((S, D), BF16),
        in_specs=[hbm, pl.BlockSpec(memory_space=pltpu.VMEM)] + [hbm] * 8,
        out_specs=hbm,
        scratch_shapes=[
            pltpu.VMEM((S, D), BF16),
            pltpu.VMEM((S, D), BF16),
            pltpu.VMEM((S, D), F32),
            pltpu.VMEM((nd, S + 2 * PAD, LANES), F32),
            pltpu.VMEM((7, nd // 2, TM1 // 2, LANES), BF16),
            pltpu.VMEM((7, nd // 2, TM1 // 2, LANES), BF16),
            pltpu.VMEM((7, F // (2 * LANES), TM2 // 2, LANES), BF16),
            pltpu.VMEM((7 * D * F // (8 * LANES), LANES), U32),
            pltpu.VMEM((7 * D * F // (8 * LANES), LANES), U32),
            pltpu.VMEM((3 * (H // 2) * 7 * (D // 4 + 1) + 16, LANES), U32),
            pltpu.VMEM((7 * H * Dh * D // (8 * LANES) + 16, LANES), U32),
            pltpu.VMEM((2, 6, (D // 2 // nb2) * H // 2, LANES), U32),
            pltpu.VMEM((2, nd * H * Dh // (2 * nb2), LANES), U32),
            pltpu.VMEM((M, D), F32),
            pltpu.VMEM((4, 7, seg, D // 2), F32),
            pltpu.VMEM((4, 7, seg, H * Dh // 2), F32),
            pltpu.VMEM((4, 4, seg, D // 2), F32),
            dma((S // TM1,)), dma((3 * nd + F // LANES,)), dma((2, 6 + nd)), dma((S // (4 * seg),)),
        ],
        compiler_params=pltpu.CompilerParams(vmem_limit_bytes=126 * 1024 * 1024, flags={"XLA_TPU_EVENLY_DISTRIBUTE_CRITICAL_NODES": True}),
        name="rmt_s2mlp",
    )(A_x.reshape(S, D), A_mem0.reshape(M, D),
      A_Wq.reshape(D * H, Dh), A_Wk.reshape(D * H, Dh), A_Wv.reshape(D * H, Dh),
      A_Wo.reshape(H * Dh, D), B_w1, B_w2, B_w3, B_w4)
    return out.reshape(1, S, D)
```

```python
import functools
import math

import jax
import jax.numpy as jnp
from jax import lax
import jax.experimental.pallas as pl
import jax.experimental.pallas.tpu as pltpu

F32 = jnp.float32
BF16 = jnp.bfloat16
U32 = jnp.uint32
LANES = 128
PAD = 8


def _dot(a, b):
    return lax.dot_general(a, b, (((1,), (0,)), ((), ())), preferred_element_type=F32)


def _dot_nt(a, b):
    return lax.dot_general(a, b, (((1,), (1,)), ((), ())), preferred_element_type=F32)


def _layernorm(x):
    m = jnp.mean(x, axis=-1, keepdims=True)
    d = x - m
    v = jnp.mean(d * d, axis=-1, keepdims=True)
    return d * lax.rsqrt(v + 1e-5)


def _recip(x):
    r = pl.reciprocal(x, approx=True)
    return r * (2.0 - x * r)


def _gelu(x):
    c = math.sqrt(2.0 / math.pi)
    inner = x * (c + (c * 0.044715) * (x * x))
    hx = 0.5 * x
    return hx + hx * jnp.tanh(inner)


def _words(x):
    return pltpu.bitcast(x.astype(BF16), U32)


def _halves(w):
    return pltpu.bitcast(w, BF16)


def _cat(xs, axis):
    return xs[0] if len(xs) == 1 else jnp.concatenate(xs, axis=axis)


def _right(b11, b12, b21, b22):
    return (b11 + b22, b11, b12 - b22, b21 - b11, b22, b11 + b12, b21 + b22)


def _unpack(w):
    return pltpu.bitcast(w << 16, F32), pltpu.bitcast(w & U32(0xFFFF0000), F32)


def _pack(lo, hi):
    return pltpu.bitcast(pltpu.pack_elementwise([lo, hi], packed_dtype=BF16), U32)


def _right_words(w):
    lo, hi = zip(*[_unpack(x) for x in w])
    f = [_pack(a, b) for a, b in zip(_right(*lo), _right(*hi))]
    f[1], f[4] = w[0], w[3]
    return f


def _left(a11, a12, a21, a22):
    return (a11 + a22, a21 + a22, a11, a22, a11 + a12, a21 - a11, a12 - a22)


def _combine(m):
    m4 = m(3)
    m2 = m(1)
    c21 = m2 + m4
    m1 = m(0)
    c22 = m1 - m2
    c11 = m1 + m4
    c11 = c11 + m(6)
    m5 = m(4)
    c11 = c11 - m5
    m3 = m(2)
    c12 = m3 + m5
    c22 = c22 + m3
    c22 = c22 + m(5)
    return c11, c12, c21, c22


def _kernel(x_hbm, mem0_ref, wq_hbm, wk_hbm, wv_hbm, wo_hbm, w1_hbm, w2_hbm, w3_hbm, w4_hbm,
            out_hbm,
            xbuf, xnb, res, hs, la, lb, lz, w3f, w4f, arq, aro, stq, sto, membuf, hl, ol, pbuf, qbuf,
            sem_x, sem_w, sem_a, sem_out,
            *, S, D, H, Dh, M, seg, F, TM1, TM2):
    L = M + seg
    nd = D // LANES
    nh = nd // 2
    Dk = D // 2
    wk = Dk // 2
    slab = wk + 1
    nf = F // (2 * LANES)
    ng = H // 2
    nb1 = S // TM1
    nb2 = S // TM2
    h1 = TM1 // 2
    h2 = TM2 // 2

    def cols(n, w=1):
        return slice(n * LANES, (n + w) * LANES)

    raw = {1: 0, 2: nd * Dk, 3: 2 * nd * Dk, 4: 2 * nd * Dk + 2 * nf * Dk}
    raw_src = {1: w1_hbm, 2: w2_hbm, 3: w3_hbm, 4: w4_hbm}
    raw_rows = {1: Dk, 2: Dk, 3: Dk, 4: F // 2}
    raw_sem = {1: 0, 2: nd, 3: 2 * nd, 4: 2 * nd + 2 * nf}

    def w_copy(j, n):
        return pltpu.make_async_copy(raw_src[j].bitcast(U32).at[:, cols(n)],
                                     arq.at[pl.ds(raw[j] + n * raw_rows[j], raw_rows[j])],
                                     sem_w.at[raw_sem[j] + n])

    def x_copy(i):
        r0 = pl.multiple_of(i * TM1, TM1)
        return pltpu.make_async_copy(x_hbm.at[pl.ds(r0, TM1)], xbuf.at[pl.ds(r0, TM1)], sem_x.at[i])

    fpi = Dk // nb2
    gpi = ng // nb2

    def a_copies(i):
        cps = []
        for t, src in enumerate((wq_hbm, wk_hbm, wv_hbm)):
            for half in range(2):
                r0 = pl.multiple_of((half * Dk + i * fpi) * (H // 2), fpi * H // 2)
                cps.append(pltpu.make_async_copy(src.bitcast(U32).at[pl.ds(r0, fpi * H // 2)],
                                                 stq.at[i % 2, 2 * t + half], sem_a.at[i % 2, 2 * t + half]))
        r0 = pl.multiple_of(i * gpi * Dh, gpi * Dh)
        for n in range(nd):
            cps.append(pltpu.make_async_copy(wo_hbm.bitcast(U32).at[pl.ds(r0, gpi * Dh), cols(n)],
                                             sto.at[i % 2, pl.ds(n * gpi * Dh, gpi * Dh)], sem_a.at[i % 2, 6 + n]))
        return cps

    def prep(src, r11, r12, r21, r22, rows, dst, base, pitch):
        for r in range(0, rows, 8):
            for i, f in enumerate(_right_words([src[pl.ds(o + r, 8), :] for o in (r11, r12, r21, r22)])):
                dst[pl.ds(base + i * pitch + r, 8), :] = f

    def prep_sq(j, n, r, rows):
        o = raw[j] + r
        prep(arq, o + n * Dk, o + (n + nh) * Dk, o + n * Dk + wk, o + (n + nh) * Dk + wk, rows,
             aro, ((j - 1) * nh + n) * 7 * wk + r, wk)

    x_copy(0).start()
    for n in range(nd):
        w_copy(1, n).start()
    x_copy(1).start()

    zpad = jnp.zeros((PAD, LANES), F32)
    for n in range(nd):
        hs[n, 0:PAD, :] = zpad
        hs[n, PAD + S:PAD + S + PAD, :] = zpad
    membuf[...] = mem0_ref[...].astype(F32)

    RC = 16

    def put_left(dst, r, a11, a12, a21, a22):
        for k, f in enumerate(_left(a11, a12, a21, a22)):
            for n in range(nh):
                dst[k, n, r:r + RC, :] = f[:, cols(n)].astype(BF16)

    def get_left(src, k):
        w = src.bitcast(U32)
        return _halves(_cat([w[k, n] for n in range(src.shape[1])], 1))

    def norm_in(i, dst):
        for r in range(0, h1, RC):
            a = []
            for half in range(2):
                rr = pl.ds(pl.multiple_of(i * TM1 + half * h1 + r, RC), RC)
                xn = _layernorm(xbuf[rr, :].astype(F32))
                xnb[rr, :] = xn.astype(BF16)
                res[rr, :] = xn
                a.append(_layernorm(xn))
            put_left(dst, r, a[0][:, :Dk], a[0][:, Dk:], a[1][:, :Dk], a[1][:, Dk:])

    x_copy(0).wait()
    norm_in(0, la)
    for n in range(nh):
        w_copy(1, n).wait()
        w_copy(1, n + nh).wait()
        if n == 0:
            x_copy(2).start()
            x_copy(3).start()
        prep_sq(1, n, 0, wk)

    later = [[w_copy(2, n) for n in range(nd)]]
    w3c = [w_copy(3, n) for n in range(2 * nf)]
    w4c = [w_copy(4, n) for n in range(nd)]
    later += [[x_copy(4 + k)] + w3c[5 * k:5 * k + 5] for k in range(4)] + [w3c[20:]]
    later += [w4c[2 * k:2 * k + 2] for k in range(4)]

    def start_later(i, lo, hi):
        for k in range(lo, min(hi, len(later))):
            @pl.when(i == k)
            def _(k=k):
                for c in later[k]:
                    c.start()

    def b1(i, cur, nxt, second):
        r0 = pl.multiple_of(i * TM1, TM1)
        norm_in(jnp.minimum(i + 1, nb1 - 1), nxt)
        for n in range(nh):
            c = _combine(lambda k: _dot(get_left(cur, k), _halves(aro[pl.ds((n * 7 + k) * wk, wk), :])))
            hs[n, pl.ds(r0 + PAD, h1), :] = _gelu(c[0])
            hs[n + nh, pl.ds(r0 + PAD, h1), :] = _gelu(c[1])
            hs[n, pl.ds(r0 + PAD + h1, h1), :] = _gelu(c[2])
            hs[n + nh, pl.ds(r0 + PAD + h1, h1), :] = _gelu(c[3])
            if second:
                prep_sq(2, i - nb1 // 2, n * wk // nh, wk // nh)
        if second:
            start_later(i, nb1 // 2, nb1)
        else:
            start_later(i, 0, nb1 // 2)

    def b1_pair(second):
        def b1p(i, carry):
            x_copy(2 * i + 1).wait()
            b1(2 * i, la, lb, second)

            @pl.when(2 * i + 2 < nb1)
            def _():
                x_copy(2 * i + 2).wait()

            b1(2 * i + 1, lb, la, second)
            return carry
        return b1p

    lax.fori_loop(0, nb1 // 4, b1_pair(False), 0)
    for n in range(nd):
        w_copy(2, n).wait()
    lax.fori_loop(nb1 // 4, nb1 // 2, b1_pair(True), 0)

    shifts = (-1, 1, -2, 2)

    def shift_in(i, dst):
        for r in range(0, h1, RC):
            def blk(half, c):
                r0 = i * TM1 + PAD + half * h1 + r
                return _cat([hs[n, pl.ds(r0 + shifts[n * 4 // nd], RC), :] for n in range(c, c + nh)], 1)

            put_left(dst, r, blk(0, 0), blk(0, nh), blk(1, 0), blk(1, nh))

    def norm_mid(i):
        for r in range(0, TM1, 2 * RC):
            rr = pl.ds(pl.multiple_of(i * TM1 + r, 2 * RC), 2 * RC)
            l2 = _layernorm(res[rr, :])
            for n in range(nd):
                hs[n, rr, :] = l2[:, cols(n)]

    def prep3(u):
        p, r = u // 2, (u % 2) * (wk // 2)
        o = raw[3] + 2 * p * Dk + r
        prep(arq, o, o + Dk, o + wk, o + Dk + wk, wk // 2, w3f, p * 7 * wk + r, wk)

    def prep4(n, p):
        o = raw[4] + n * (F // 2) + p * LANES
        rows = LANES // 2
        prep(arq, o, o + nh * (F // 2), o + rows, o + nh * (F // 2) + rows, rows,
             w4f, n * 7 * nf * rows + p * rows, nf * rows)

    def b2(i, cur, nxt, second):
        r0 = pl.multiple_of(i * TM1, TM1)
        shift_in(jnp.minimum(i + 1, nb1 - 1), nxt)
        for n in range(nh):
            c = _combine(lambda k: _dot(get_left(cur, k), _halves(aro[pl.ds(((nh + n) * 7 + k) * wk, wk), :])))
            res[pl.ds(r0, h1), cols(n)] += c[0]
            res[pl.ds(r0, h1), cols(n + nh)] += c[1]
            res[pl.ds(r0 + h1, h1), cols(n)] += c[2]
            res[pl.ds(r0 + h1, h1), cols(n + nh)] += c[3]
        if second:
            for p in range(nf):
                prep4(i - nb1 // 2, p)
        else:
            per = 2 * nf // (nb1 // 2)
            for u in range(per):
                prep3(i * per + u)
            start_later(i + nb1, nb1, nb1 + nb1 // 2)
        norm_mid(i)

    def b2_pair(second):
        def b2p(i, carry):
            b2(2 * i, la, lb, second)
            b2(2 * i + 1, lb, la, second)
            return carry
        return b2p

    shift_in(0, la)
    for c in w3c:
        c.wait()
    lax.fori_loop(0, nb1 // 4, b2_pair(False), 0)
    for c in w4c:
        c.wait()
    for c in a_copies(0) + a_copies(1):
        c.start()
    lax.fori_loop(nb1 // 4, nb1 // 2, b2_pair(True), 0)

    hp = H // 2

    def b3(i, carry):
        for c in a_copies(i):
            c.wait()

        def prep_qkv(t, u, j):
            forms = []
            for par in range(2):
                w = [stq[i % 2, 2 * t + half, pl.ds((2 * u + par) * hp + 8 * j, 8), :] for half in range(2)]
                forms.append(_right(*_unpack(w[0]), *_unpack(w[1])))
            for k in range(7):
                base = ((t * ng + 8 * j) * 7 + k) * slab + u + i * (fpi // 2)
                arq[pl.ds(base, 8, stride=7 * slab), :] = _pack(forms[0][k], forms[1][k])

        def prep_o(g, n):
            o = 2 * g * (Dh // 2)
            prep(sto.at[i % 2], o + n * gpi * Dh, o + (n + nh) * gpi * Dh,
                 o + n * gpi * Dh + Dh // 2, o + (n + nh) * gpi * Dh + Dh // 2, Dh // 2,
                 aro, pl.multiple_of((n * 7 * ng + i * gpi + g) * (Dh // 2), Dh // 2), ng * Dh // 2)

        r0 = pl.multiple_of(i * TM2, TM2)

        def blk(r, c):
            return _cat([hs[n, pl.ds(r0 + r, h2), :] for n in range(c, c + nh)], 1)

        ly = [f.astype(BF16) for f in _left(blk(0, 0), blk(0, nh), blk(h2, 0), blk(h2, nh))]
        for p in range(nf):
            c = _combine(lambda k: _dot(ly[k], _halves(w3f[pl.ds((p * 7 + k) * wk, wk), :])))
            for k, f in enumerate(_left(*[_gelu(y) for y in c])):
                lz[k, p] = f.astype(BF16)
        for t in range(3):
            for u in range(fpi // 2):
                for j in range(hp // 8):
                    prep_qkv(t, u, j)
        for g in range(gpi):
            for n in range(nh):
                prep_o(g, n)
        rows = nf * LANES // 2
        for n in range(0, nh, 2):
            c = _combine(lambda k: _dot(get_left(lz, k), _cat(
                [_halves(w4f[pl.ds(((n + e) * 7 + k) * rows, rows), :]) for e in range(2)], 1)))
            for r, cc, y in ((0, n, c[0]), (0, n + nh, c[1]), (h2, n, c[2]), (h2, n + nh, c[3])):
                rr = pl.ds(r0 + r, h2)
                res[rr, cols(cc, 2)] += xbuf[rr, cols(cc, 2)].astype(F32) + y

        @pl.when(i + 2 < nb2)
        def _():
            for c in a_copies(i + 2):
                c.start()

        return carry

    lax.fori_loop(0, nb2, b3, 0)

    scale = Dh ** -0.5
    row = lax.broadcasted_iota(jnp.int32, (L, L), 0)
    col = lax.broadcasted_iota(jnp.int32, (L, L), 1)
    mask = (row < M) | (row >= col)
    QS = 4 * seg
    R = seg - M
    rv = R // 8

    def upper(n):
        return lax.broadcasted_iota(jnp.int32, (8, n), 0) < 4

    def split8(mem, tok):
        u = upper(mem.shape[1])
        return jnp.where(u, mem, tok), pltpu.roll(jnp.where(u, tok, mem), 4, 0)

    def join8(t, b):
        u = upper(t.shape[1])
        b = pltpu.roll(b, 4, 0)
        return jnp.where(u, t, b), jnp.where(u, b, t)

    def out_copy(j):
        r0 = pl.multiple_of(j * QS, QS)
        return pltpu.make_async_copy(xbuf.at[pl.ds(r0, QS)], out_hbm.at[pl.ds(r0, QS)], sem_out.at[j])

    def vregs(y, lo, hi):
        return [y[8 * k:8 * k + 8] for k in range(lo, hi)]

    def quad(j, carry):
        xs = xnb[pl.ds(pl.multiple_of(j * QS, QS), QS), :].astype(F32)
        qkv = {(t, h): [] for t in range(3) for h in range(H)}
        att = {h: [] for h in range(H)}
        outs = {n: [] for n in range(nd)}
        mem = membuf[...]
        for st in range(4):
            if st == 0:
                t0, u0 = split8(mem, xs[2 * R:2 * R + 8])
                at = jnp.concatenate([t0, xs[0:R]], axis=0)
                au = jnp.concatenate([u0, xs[R:2 * R]], axis=0)
                for k, f in enumerate(_left(at[:, :Dk], at[:, Dk:], au[:, :Dk], au[:, Dk:])):
                    hl[st, k] = f
            else:
                r = 2 * R + 8 + (st - 1) * R
                a = jnp.concatenate([mem, xs[r:r + R]], axis=0)
                hl[st, 1] = a[:, :Dk] + a[:, Dk:]
                hl[st, 2] = a[:, :Dk]
                hl[st, 3] = a[:, Dk:]

            def four(m):
                return m(3) + m(1), m(2) + m(4, 1)

            def wq_part(t, g, lo, hi):
                def m(k, left=None):
                    w = _halves(arq[pl.ds(((t * ng + g) * 7 + k) * slab + lo // 2, (hi - lo) // 2), :])
                    return _dot(hl[st, k if left is None else left, :, lo:hi], w)

                return _combine(m) if st == 0 else four(m)

            def proj(t, g, head=None):
                if head is None:
                    c = wq_part(t, g, 0, Dk)
                else:
                    c = [x + y for x, y in zip(head, wq_part(t, g, Dk // 2, Dk))]
                got = []
                if st == 0:
                    for e in range(2):
                        ym, yt = join8(c[e][0:8], c[2 + e][0:8])
                        qkv[t, 2 * g + e] += vregs(c[e], 1, 1 + rv) + vregs(c[2 + e], 1, 1 + rv) + [yt]
                        got.append(ym)
                else:
                    for e, y in enumerate(c):
                        qkv[t, 2 * g + e] += vregs(y, 1, 1 + rv)
                        got.append(y[0:8])
                return [jnp.concatenate([got[e]] + qkv[t, 2 * g + e][4 * st:4 * st + 4], axis=0) for e in range(2)]

            def feed(g, o):
                for e in range(2):
                    att[2 * g + e] += vregs(o[e], 1, 5)
                if st < 3:
                    a = [jnp.concatenate([o[e][0:8]] + att[2 * g + e][st * rv:(st + 1) * rv], axis=0)
                         for e in range(2)]
                    ol[st, 1, :, cols(g)] = a[0] + a[1]
                    ol[st, 2, :, cols(g)] = a[0]
                    ol[st, 3, :, cols(g)] = a[1]
                else:
                    at, au = [], []
                    for e in range(2):
                        y = att[2 * g + e][3 * rv:]
                        t0, u0 = split8(o[e][0:8], y[2 * rv])
                        at.append(jnp.concatenate([t0] + y[:rv], axis=0))
                        au.append(jnp.concatenate([u0] + y[rv:2 * rv], axis=0))
                    for k, f in enumerate(_left(at[0], at[1], au[0], au[1])):
                        ol[st, k, :, cols(g)] = f

            def wo_part(n, lo, hi):
                def m(k, left=None):
                    w = _halves(aro[pl.ds(((n * 7 + k) * ng + lo) * (Dh // 2), (hi - lo) * (Dh // 2)), :])
                    return _dot(ol[st, k if left is None else left, :, lo * Dh:hi * Dh], w)

                return _combine(m) if st == 3 else four(m)

            cur, soft = {}, {}
            for g in range(ng + nh):
                if g == 0 and st > 0:
                    for t in range(3):
                        for k, y in enumerate(wq_part(t, g, 0, Dk // 2)):
                            qbuf[st, t, k] = y
                    cur[g] = [proj(t, g, [qbuf[st, t, k] for k in range(2)]) for t in range(3)]
                elif g < ng:
                    cur[g] = [proj(t, g) for t in range(3)]
                else:
                    for k, y in enumerate(wo_part(g - ng, 0, ng // 2)):
                        pbuf[st, k, :, cols(g - ng)] = y
                if 1 <= g <= ng:
                    soft[g - 1] = []
                    for e in range(2):
                        q, k = cur[g - 1][0][e], cur[g - 1][1][e]
                        sc = jnp.where(mask, _dot_nt(q, k.astype(BF16)), -1e9 / scale)
                        p = jnp.exp2((sc - jnp.max(sc, axis=-1, keepdims=True)) * (scale * math.log2(math.e)))
                        soft[g - 1].append(p * _recip(jnp.sum(p, axis=-1, keepdims=True)))
                if 3 <= g < ng + 3:
                    feed(g - 3, [_dot(p, cur[g - 3][2][e].astype(BF16)) for e, p in enumerate(soft[g - 3])])
            new = {}
            for n in range(nh):
                c = [pbuf[st, k, :, cols(n)] + y for k, y in enumerate(wo_part(n, ng // 2, ng))]
                for e in range(2):
                    if st < 3:
                        new[n + e * nh] = c[e][0:8]
                        outs[n + e * nh] += vregs(c[e], 1, 1 + rv)
                    else:
                        ym, yt = join8(c[e][0:8], c[2 + e][0:8])
                        new[n + e * nh] = ym
                        outs[n + e * nh] += vregs(c[e], 1, 1 + rv) + vregs(c[2 + e], 1, 1 + rv) + [yt]
            mem = jnp.concatenate([new[n] for n in range(nd)], axis=1)
            lo, hi = ((0, 2), (2, 6), (6, 8), (8, 16))[st]
            rr = pl.ds(pl.multiple_of(j * QS + 8 * lo, 16), 8 * (hi - lo))
            for n in range(nd):
                xbuf[rr, cols(n)] = (res[rr, cols(n)] + jnp.concatenate(outs[n][lo:hi], axis=0)).astype(BF16)
        membuf[...] = mem
        out_copy(j).start()
        return carry

    lax.fori_loop(0, S // QS, quad, 0)
    for j in range(S // QS):
        out_copy(j).wait()


@functools.partial(jax.jit, static_argnames=("A_seg_len",))
def pallas_parallel_sum__memory_aug_recurrent_mem_tr__mixer_s_mlp__prompt_kernel(
    A_x: jax.Array,
    A_mem0: jax.Array,
    A_Wq: jax.Array,
    A_Wk: jax.Array,
    A_Wv: jax.Array,
    A_Wo: jax.Array,
    A_seg_len: int,
    B_x: jax.Array,
    B_w1: jax.Array,
    B_w2: jax.Array,
    B_w3: jax.Array,
    B_w4: jax.Array,
):
    del B_x
    _, S, D = A_x.shape
    _, H, Dh = A_Wq.shape
    M = A_mem0.shape[1]
    seg = int(A_seg_len)
    F = B_w3.shape[1]
    assert (M, seg, Dh) == (8, 32, LANES)
    TM1, TM2 = 256, 128
    nd = D // LANES
    nb2 = S // TM2

    kern = functools.partial(_kernel, S=S, D=D, H=H, Dh=Dh, M=M, seg=seg, F=F, TM1=TM1, TM2=TM2)
    hbm = pl.BlockSpec(memory_space=pl.ANY)
    dma = pltpu.SemaphoreType.DMA
    out = pl.pallas_call(
        kern,
        out_shape=jax.ShapeDtypeStruct((S, D), BF16),
        in_specs=[hbm, pl.BlockSpec(memory_space=pltpu.VMEM)] + [hbm] * 8,
        out_specs=hbm,
        scratch_shapes=[
            pltpu.VMEM((S, D), BF16),
            pltpu.VMEM((S, D), BF16),
            pltpu.VMEM((S, D), F32),
            pltpu.VMEM((nd, S + 2 * PAD, LANES), F32),
            pltpu.VMEM((7, nd // 2, TM1 // 2, LANES), BF16),
            pltpu.VMEM((7, nd // 2, TM1 // 2, LANES), BF16),
            pltpu.VMEM((7, F // (2 * LANES), TM2 // 2, LANES), BF16),
            pltpu.VMEM((7 * D * F // (8 * LANES), LANES), U32),
            pltpu.VMEM((7 * D * F // (8 * LANES), LANES), U32),
            pltpu.VMEM((3 * (H // 2) * 7 * (D // 4 + 1), LANES), U32),
            pltpu.VMEM((7 * H * Dh * D // (8 * LANES), LANES), U32),
            pltpu.VMEM((2, 6, (D // 2 // nb2) * H // 2, LANES), U32),
            pltpu.VMEM((2, nd * H * Dh // (2 * nb2), LANES), U32),
            pltpu.VMEM((M, D), F32),
            pltpu.VMEM((4, 7, seg, D // 2), F32),
            pltpu.VMEM((4, 7, seg, H * Dh // 2), F32),
            pltpu.VMEM((4, 4, seg, D // 2), F32),
            pltpu.VMEM((4, 3, 2, seg, LANES), F32),
            dma((S // TM1,)), dma((3 * nd + F // LANES,)), dma((2, 6 + nd)), dma((S // (4 * seg),)),
        ],
        compiler_params=pltpu.CompilerParams(vmem_limit_bytes=126 * 1024 * 1024, flags={"XLA_TPU_EVENLY_DISTRIBUTE_CRITICAL_NODES": True}),
        name="rmt_s2mlp",
    )(A_x.reshape(S, D), A_mem0.reshape(M, D),
      A_Wq.reshape(D * H, Dh), A_Wk.reshape(D * H, Dh), A_Wv.reshape(D * H, Dh),
      A_Wo.reshape(H * Dh, D), B_w1, B_w2, B_w3, B_w4)
    return out.reshape(1, S, D)
```

```python
import functools
import math

import jax
import jax.numpy as jnp
from jax import lax
import jax.experimental.pallas as pl
import jax.experimental.pallas.tpu as pltpu

F32 = jnp.float32
BF16 = jnp.bfloat16
U32 = jnp.uint32
LANES = 128
PAD = 8


def _dot(a, b):
    return lax.dot_general(a, b, (((1,), (0,)), ((), ())), preferred_element_type=F32)


def _dot_nt(a, b):
    return lax.dot_general(a, b, (((1,), (1,)), ((), ())), preferred_element_type=F32)


def _layernorm(x):
    m = jnp.mean(x, axis=-1, keepdims=True)
    d = x - m
    v = jnp.mean(d * d, axis=-1, keepdims=True)
    return d * lax.rsqrt(v + 1e-5)


def _recip(x):
    r = pl.reciprocal(x, approx=True)
    return r * (2.0 - x * r)


def _gelu(x):
    c = math.sqrt(2.0 / math.pi)
    inner = x * (c + (c * 0.044715) * (x * x))
    hx = 0.5 * x
    return hx + hx * jnp.tanh(inner)


def _words(x):
    return pltpu.bitcast(x.astype(BF16), U32)


def _halves(w):
    return pltpu.bitcast(w, BF16)


def _cat(xs, axis):
    return xs[0] if len(xs) == 1 else jnp.concatenate(xs, axis=axis)


def _right(b11, b12, b21, b22):
    return (b11 + b22, b11, b12 - b22, b21 - b11, b22, b11 + b12, b21 + b22)


def _unpack(w):
    return pltpu.bitcast(w << 16, F32), pltpu.bitcast(w & U32(0xFFFF0000), F32)


def _pack(lo, hi):
    return pltpu.bitcast(pltpu.pack_elementwise([lo, hi], packed_dtype=BF16), U32)


def _right_words(w):
    lo, hi = zip(*[_unpack(x) for x in w])
    f = [_pack(a, b) for a, b in zip(_right(*lo), _right(*hi))]
    f[1], f[4] = w[0], w[3]
    return f


def _left(a11, a12, a21, a22):
    return (a11 + a22, a21 + a22, a11, a22, a11 + a12, a21 - a11, a12 - a22)


def _combine(m):
    m4 = m(3)
    m2 = m(1)
    c21 = m2 + m4
    m1 = m(0)
    c22 = m1 - m2
    c11 = m1 + m4
    c11 = c11 + m(6)
    m5 = m(4)
    c11 = c11 - m5
    m3 = m(2)
    c12 = m3 + m5
    c22 = c22 + m3
    c22 = c22 + m(5)
    return c11, c12, c21, c22


class _Filler:
    def __init__(self, slots, *job_lists):
        self.slots, self.done, self.lists = slots, 0, job_lists

    def __call__(self):
        for jobs in self.lists:
            n = len(jobs)
            for job in jobs[self.done * n // self.slots:(self.done + 1) * n // self.slots]:
                job()
        self.done += 1


def _kernel(x_hbm, mem0_ref, wq_hbm, wk_hbm, wv_hbm, wo_hbm, w1_hbm, w2_hbm, w3_hbm, w4_hbm,
            out_hbm,
            xbuf, xnb, res, hs, lf, lz, wts, stq, sto, membuf, hl, ol, pbuf, qbuf,
            sem_x, sem_w, sem_a, sem_out,
            *, S, D, H, Dh, M, seg, F, TM1, TM2):
    L = M + seg
    nd = D // LANES
    nh = nd // 2
    Dk = D // 2
    wk = Dk // 2
    slab = wk + 1
    nf = F // (2 * LANES)
    ng = H // 2
    nb1 = S // TM1
    nb2 = S // TM2
    h1 = TM1 // 2
    h2 = TM2 // 2
    RC = 16
    part = functools.partial

    def cols(n, w=1):
        return slice(n * LANES, (n + w) * LANES)

    o_w3 = 0
    o_w4 = o_w3 + nf * 7 * wk
    o_wo = o_w4 + nf * 7 * wk
    o_qkv = o_wo + ng * 7 * wk
    raw = {1: o_qkv, 2: o_qkv + nd * Dk, 3: o_qkv + 2 * nd * Dk, 4: o_qkv + 2 * nd * Dk + 2 * nf * Dk}

    raw_src = {1: w1_hbm, 2: w2_hbm, 3: w3_hbm, 4: w4_hbm}
    raw_rows = {1: Dk, 2: Dk, 3: Dk, 4: F // 2}
    raw_sem = {1: 0, 2: nd, 3: 2 * nd, 4: 2 * nd + 2 * nf}

    def w_copy(j, n):
        return pltpu.make_async_copy(raw_src[j].bitcast(U32).at[:, cols(n)],
                                     wts.at[pl.ds(raw[j] + n * raw_rows[j], raw_rows[j])],
                                     sem_w.at[raw_sem[j] + n])

    def x_copy(i):
        r0 = pl.multiple_of(i * TM1, TM1)
        return pltpu.make_async_copy(x_hbm.at[pl.ds(r0, TM1)], xbuf.at[pl.ds(r0, TM1)], sem_x.at[i])

    fpi = Dk // nb2
    gpi = ng // nb2

    def a_copies(i):
        cps = []
        for t, src in enumerate((wq_hbm, wk_hbm, wv_hbm)):
            for half in range(2):
                r0 = pl.multiple_of((half * Dk + i * fpi) * ng, fpi * ng)
                cps.append(pltpu.make_async_copy(src.bitcast(U32).at[pl.ds(r0, fpi * ng)],
                                                 stq.at[i % 2, 2 * t + half], sem_a.at[i % 2, 2 * t + half]))
        r0 = pl.multiple_of(i * gpi * Dh, gpi * Dh)
        for n in range(nd):
            cps.append(pltpu.make_async_copy(wo_hbm.bitcast(U32).at[pl.ds(r0, gpi * Dh), cols(n)],
                                             sto.at[i % 2, pl.ds(n * gpi * Dh, gpi * Dh)], sem_a.at[i % 2, 6 + n]))
        return cps

    def prep(src, offs, rows, dst, pitch):
        def job(r):
            for i, f in enumerate(_right_words([src[pl.ds(o + r, 8), :] for o in offs])):
                wts[pl.ds(dst + i * pitch + r, 8), :] = f
        return [part(job, r) for r in range(0, rows, 8)]

    def prep_sq(j, n):
        o = raw[j] + n * Dk
        return prep(wts, (o, o + nh * Dk, o + wk, o + nh * Dk + wk), wk, o_wo + ((j - 1) * nh + n) * 7 * wk, wk)

    x_copy(0).start()
    for n in range(nd):
        w_copy(1, n).start()
    x_copy(1).start()

    zpad = jnp.zeros((PAD, LANES), F32)
    for n in range(nd):
        hs[n, 0:PAD, :] = zpad
        hs[n, PAD + S:PAD + S + PAD, :] = zpad
    membuf[...] = mem0_ref[...].astype(F32)

    def put_left(slot, r, top, bot):
        for k, f in enumerate(_left(top[:, :Dk], top[:, Dk:], bot[:, :Dk], bot[:, Dk:])):
            for n in range(nh):
                lf[slot, k, n, r:r + RC, :] = f[:, cols(n)].astype(BF16)

    def get_left(slot, k, rows):
        w = lf.bitcast(U32)
        return _halves(_cat([w[slot, k, n, 0:rows // 2, :] for n in range(nh)], 1))

    def weights(r0, rows):
        return _halves(wts[pl.ds(r0, rows), :])

    def norm_in(i, slot):
        def job(r):
            a = []
            for half in range(2):
                rr = pl.ds(pl.multiple_of(i * TM1 + half * h1 + r, RC), RC)
                xn = _layernorm(xbuf[rr, :].astype(F32))
                xnb[rr, :] = xn.astype(BF16)
                res[rr, :] = xn
                a.append(_layernorm(xn))
            put_left(slot, r, *a)
        return [part(job, r) for r in range(0, h1, RC)]

    x_copy(0).wait()
    for job in norm_in(0, 0):
        job()
    for n in range(nh):
        w_copy(1, n).wait()
        w_copy(1, n + nh).wait()
        if n == 0:
            x_copy(2).start()
            x_copy(3).start()
        for job in prep_sq(1, n):
            job()

    w3c = [w_copy(3, n) for n in range(2 * nf)]
    w4c = [w_copy(4, n) for n in range(nd)]
    later = [[w_copy(2, n) for n in range(nd)]]
    later += [[x_copy(4 + k)] + w3c[5 * k:5 * k + 5] for k in range(4)] + [w3c[20:]]
    later += [w4c[2 * k:2 * k + 2] for k in range(4)]

    def start_later(i, lo, hi):
        for k in range(lo, min(hi, len(later))):
            @pl.when(i == k)
            def _(k=k):
                for c in later[k]:
                    c.start()

    def b1(second, i, carry):
        @pl.when(i + 1 < nb1)
        def _():
            x_copy(i + 1).wait()

        r0 = pl.multiple_of(i * TM1, TM1)
        fill = _Filler(7 * nh - 2, norm_in(jnp.minimum(i + 1, nb1 - 1), (i + 1) % 2),
                       prep_sq(2, i - nb1 // 2) if second else [])

        def prod(n, k):
            y = _dot(get_left(i % 2, k, h1), weights(o_wo + (n * 7 + k) * wk, wk))
            fill()
            return y

        for n in range(nh):
            c = _combine(part(prod, n))
            hs[n, pl.ds(r0 + PAD, h1), :] = _gelu(c[0])
            hs[n + nh, pl.ds(r0 + PAD, h1), :] = _gelu(c[1])
            hs[n, pl.ds(r0 + PAD + h1, h1), :] = _gelu(c[2])
            hs[n + nh, pl.ds(r0 + PAD + h1, h1), :] = _gelu(c[3])
        start_later(i, *((nb1 // 2, nb1) if second else (0, nb1 // 2)))
        return carry

    lax.fori_loop(0, nb1 // 2, part(b1, False), 0)
    for n in range(nd):
        w_copy(2, n).wait()
    lax.fori_loop(nb1 // 2, nb1, part(b1, True), 0)

    shifts = (-1, 1, -2, 2)

    def shift_in(i, slot):
        def job(r):
            put_left(slot, r, *[_cat([hs[n, pl.ds(i * TM1 + PAD + half * h1 + r + shifts[n * 4 // nd], RC), :]
                                      for n in range(nd)], 1) for half in range(2)])
        return [part(job, r) for r in range(0, h1, RC)]

    def prep3(u):
        p, r = u // 2, (u % 2) * (wk // 2)
        o = pl.multiple_of(raw[3] + 2 * p * Dk + r, 8)
        return prep(wts, (o, o + Dk, o + wk, o + Dk + wk), wk // 2, pl.multiple_of(o_w3 + p * 7 * wk + r, 8), wk)

    def prep4(n, p):
        o = raw[4] + n * (F // 2) + p * LANES
        rows = LANES // 2
        return prep(wts, (o, o + nh * (F // 2), o + rows, o + nh * (F // 2) + rows), rows,
                    o_w4 + (n * 7 * nf + p) * rows, nf * rows)

    def b2(second, i, carry):
        r0 = pl.multiple_of(i * TM1, TM1)
        per = 2 * nf // (nb1 // 2)
        jobs = ([prep4(i - nb1 // 2, p) for p in range(nf)] if second else
                [prep3(i * per + u) for u in range(per)])
        fill = _Filler(7 * nh - 2, shift_in(jnp.minimum(i + 1, nb1 - 1), (i + 1) % 2), sum(jobs, []))

        def prod(n, k):
            y = _dot(get_left(i % 2, k, h1), weights(o_wo + ((nh + n) * 7 + k) * wk, wk))
            fill()
            return y

        for n in range(nh):
            c = _combine(part(prod, n))
            res[pl.ds(r0, h1), cols(n)] += c[0]
            res[pl.ds(r0, h1), cols(n + nh)] += c[1]
            res[pl.ds(r0 + h1, h1), cols(n)] += c[2]
            res[pl.ds(r0 + h1, h1), cols(n + nh)] += c[3]
        if not second:
            start_later(i + nb1, nb1, nb1 + nb1 // 2)
        return carry

    for job in shift_in(0, 0):
        job()
    for c in w3c:
        c.wait()
    lax.fori_loop(0, nb1 // 2, part(b2, False), 0)
    for c in w4c:
        c.wait()
    for c in a_copies(0) + a_copies(1):
        c.start()
    lax.fori_loop(nb1 // 2, nb1, part(b2, True), 0)

    def norm_mid(i, slot):
        def job(r):
            put_left(slot, r, *[_layernorm(res[pl.ds(pl.multiple_of(i * TM2 + half * h2 + r, RC), RC), :])
                                for half in range(2)])
        return [part(job, r) for r in range(0, h2, RC)]

    def b3(i, carry):
        for c in a_copies(i):
            c.wait()

        def prep_qkv(t, u, j):
            forms = []
            for par in range(2):
                w = [stq[i % 2, 2 * t + half, pl.ds((2 * u + par) * ng + 8 * j, 8), :] for half in range(2)]
                forms.append(_right(*_unpack(w[0]), *_unpack(w[1])))
            for k in range(7):
                base = o_qkv + ((t * ng + 8 * j) * 7 + k) * slab + u + i * (fpi // 2)
                wts[pl.ds(base, 8, stride=7 * slab), :] = _pack(forms[0][k], forms[1][k])

        def prep_o(g, n):
            o = g * Dh + n * gpi * Dh
            return prep(sto.at[i % 2], (o, o + nh * gpi * Dh, o + Dh // 2, o + nh * gpi * Dh + Dh // 2), Dh // 2,
                        pl.multiple_of(o_wo + (n * 7 * ng + i * gpi + g) * (Dh // 2), Dh // 2), ng * Dh // 2)

        jobs = [part(prep_qkv, t, u, j) for t in range(3) for u in range(fpi // 2) for j in range(ng // 8)]
        jobs += sum([prep_o(g, n) for g in range(gpi) for n in range(nh)], [])
        fill = _Filler(7 * nf, norm_mid(jnp.minimum(i + 1, nb2 - 1), (i + 1) % 2), jobs)
        r0 = pl.multiple_of(i * TM2, TM2)

        def up(p, k):
            y = _dot(get_left(i % 2, k, h2), weights(o_w3 + (p * 7 + k) * wk, wk))
            fill()
            return y

        for p in range(nf):
            for k, f in enumerate(_left(*[_gelu(y) for y in _combine(part(up, p))])):
                lz[k, p] = f.astype(BF16)
        rows = nf * LANES // 2

        def down(n, k):
            w = lz.bitcast(U32)
            return _dot(_halves(_cat([w[k, p] for p in range(nf)], 1)),
                        _cat([weights(o_w4 + ((n + e) * 7 + k) * rows, rows) for e in range(2)], 1))

        for n in range(0, nh, 2):
            c = _combine(part(down, n))
            for r, cc, y in ((0, n, c[0]), (0, n + nh, c[1]), (h2, n, c[2]), (h2, n + nh, c[3])):
                rr = pl.ds(r0 + r, h2)
                res[rr, cols(cc, 2)] += xbuf[rr, cols(cc, 2)].astype(F32) + y

        @pl.when(i + 2 < nb2)
        def _():
            for c in a_copies(i + 2):
                c.start()

        return carry

    for job in norm_mid(0, 0):
        job()
    lax.fori_loop(0, nb2, b3, 0)

    scale = Dh ** -0.5
    row = lax.broadcasted_iota(jnp.int32, (L, L), 0)
    col = lax.broadcasted_iota(jnp.int32, (L, L), 1)
    mask = (row < M) | (row >= col)
    QS = 4 * seg
    R = seg - M
    rv = R // 8

    def upper(n):
        return lax.broadcasted_iota(jnp.int32, (8, n), 0) < 4

    def split8(mem, tok):
        u = upper(mem.shape[1])
        return jnp.where(u, mem, tok), pltpu.roll(jnp.where(u, tok, mem), 4, 0)

    def join8(t, b):
        u = upper(t.shape[1])
        b = pltpu.roll(b, 4, 0)
        return jnp.where(u, t, b), jnp.where(u, b, t)

    def out_copy(j):
        r0 = pl.multiple_of(j * QS, QS)
        return pltpu.make_async_copy(xbuf.at[pl.ds(r0, QS)], out_hbm.at[pl.ds(r0, QS)], sem_out.at[j])

    def vregs(y, lo, hi):
        return [y[8 * k:8 * k + 8] for k in range(lo, hi)]

    def quad(j, carry):
        xs = xnb[pl.ds(pl.multiple_of(j * QS, QS), QS), :].astype(F32)
        qkv = {(t, h): [] for t in range(3) for h in range(H)}
        att = {h: [] for h in range(H)}
        outs = {n: [] for n in range(nd)}
        mem = membuf[...]
        for st in range(4):
            if st == 0:
                t0, u0 = split8(mem, xs[2 * R:2 * R + 8])
                at = jnp.concatenate([t0, xs[0:R]], axis=0)
                au = jnp.concatenate([u0, xs[R:2 * R]], axis=0)
                for k, f in enumerate(_left(at[:, :Dk], at[:, Dk:], au[:, :Dk], au[:, Dk:])):
                    hl[st, k] = f
            else:
                r = 2 * R + 8 + (st - 1) * R
                a = jnp.concatenate([mem, xs[r:r + R]], axis=0)
                hl[st, 1] = a[:, :Dk] + a[:, Dk:]
                hl[st, 2] = a[:, :Dk]
                hl[st, 3] = a[:, Dk:]

            def four(m):
                return m(3) + m(1), m(2) + m(4, 1)

            def wq_part(t, g, lo, hi):
                def m(k, left=None):
                    w = weights(o_qkv + ((t * ng + g) * 7 + k) * slab + lo // 2, (hi - lo) // 2)
                    return _dot(hl[st, k if left is None else left, :, lo:hi], w)

                return _combine(m) if st == 0 else four(m)

            def proj(t, g, head=None):
                if head is None:
                    c = wq_part(t, g, 0, Dk)
                else:
                    c = [x + y for x, y in zip(head, wq_part(t, g, Dk // 2, Dk))]
                got = []
                if st == 0:
                    for e in range(2):
                        ym, yt = join8(c[e][0:8], c[2 + e][0:8])
                        qkv[t, 2 * g + e] += vregs(c[e], 1, 1 + rv) + vregs(c[2 + e], 1, 1 + rv) + [yt]
                        got.append(ym)
                else:
                    for e, y in enumerate(c):
                        qkv[t, 2 * g + e] += vregs(y, 1, 1 + rv)
                        got.append(y[0:8])
                return [jnp.concatenate([got[e]] + qkv[t, 2 * g + e][4 * st:4 * st + 4], axis=0) for e in range(2)]

            def feed(g, o):
                for e in range(2):
                    att[2 * g + e] += vregs(o[e], 1, 5)
                if st < 3:
                    a = [jnp.concatenate([o[e][0:8]] + att[2 * g + e][st * rv:(st + 1) * rv], axis=0)
                         for e in range(2)]
                    ol[st, 1, :, cols(g)] = a[0] + a[1]
                    ol[st, 2, :, cols(g)] = a[0]
                    ol[st, 3, :, cols(g)] = a[1]
                else:
                    at, au = [], []
                    for e in range(2):
                        y = att[2 * g + e][3 * rv:]
                        t0, u0 = split8(o[e][0:8], y[2 * rv])
                        at.append(jnp.concatenate([t0] + y[:rv], axis=0))
                        au.append(jnp.concatenate([u0] + y[rv:2 * rv], axis=0))
                    for k, f in enumerate(_left(at[0], at[1], au[0], au[1])):
                        ol[st, k, :, cols(g)] = f

            def wo_part(n, lo, hi):
                def m(k, left=None):
                    w = weights(o_wo + ((n * 7 + k) * ng + lo) * (Dh // 2), (hi - lo) * (Dh // 2))
                    return _dot(ol[st, k if left is None else left, :, lo * Dh:hi * Dh], w)

                return _combine(m) if st == 3 else four(m)

            cur, soft = {}, {}
            for g in range(ng + nh):
                if g == 0 and st > 0:
                    for t in range(3):
                        for k, y in enumerate(wq_part(t, g, 0, Dk // 2)):
                            qbuf[st, t, k] = y
                    cur[g] = [proj(t, g, [qbuf[st, t, k] for k in range(2)]) for t in range(3)]
                elif g < ng:
                    cur[g] = [proj(t, g) for t in range(3)]
                else:
                    for k, y in enumerate(wo_part(g - ng, 0, ng // 2)):
                        pbuf[st, k, :, cols(g - ng)] = y
                if 1 <= g <= ng:
                    soft[g - 1] = []
                    for e in range(2):
                        q, k = cur[g - 1][0][e], cur[g - 1][1][e]
                        sc = jnp.where(mask, _dot_nt(q, k.astype(BF16)), -1e9 / scale)
                        p = jnp.exp2((sc - jnp.max(sc, axis=-1, keepdims=True)) * (scale * math.log2(math.e)))
                        soft[g - 1].append(p * _recip(jnp.sum(p, axis=-1, keepdims=True)))
                if 3 <= g < ng + 3:
                    feed(g - 3, [_dot(p, cur[g - 3][2][e].astype(BF16)) for e, p in enumerate(soft[g - 3])])
            new = {}
            for n in range(nh):
                c = [pbuf[st, k, :, cols(n)] + y for k, y in enumerate(wo_part(n, ng // 2, ng))]
                for e in range(2):
                    if st < 3:
                        new[n + e * nh] = c[e][0:8]
                        outs[n + e * nh] += vregs(c[e], 1, 1 + rv)
                    else:
                        ym, yt = join8(c[e][0:8], c[2 + e][0:8])
                        new[n + e * nh] = ym
                        outs[n + e * nh] += vregs(c[e], 1, 1 + rv) + vregs(c[2 + e], 1, 1 + rv) + [yt]
            mem = jnp.concatenate([new[n] for n in range(nd)], axis=1)
            lo, hi = ((0, 2), (2, 6), (6, 8), (8, 16))[st]
            rr = pl.ds(pl.multiple_of(j * QS + 8 * lo, 16), 8 * (hi - lo))
            for n in range(nd):
                xbuf[rr, cols(n)] = (res[rr, cols(n)] + jnp.concatenate(outs[n][lo:hi], axis=0)).astype(BF16)
        membuf[...] = mem
        out_copy(j).start()
        return carry

    lax.fori_loop(0, S // QS, quad, 0)
    for j in range(S // QS):
        out_copy(j).wait()


@functools.partial(jax.jit, static_argnames=("A_seg_len",))
def pallas_parallel_sum__memory_aug_recurrent_mem_tr__mixer_s_mlp__prompt_kernel(
    A_x: jax.Array,
    A_mem0: jax.Array,
    A_Wq: jax.Array,
    A_Wk: jax.Array,
    A_Wv: jax.Array,
    A_Wo: jax.Array,
    A_seg_len: int,
    B_x: jax.Array,
    B_w1: jax.Array,
    B_w2: jax.Array,
    B_w3: jax.Array,
    B_w4: jax.Array,
):
    del B_x
    _, S, D = A_x.shape
    _, H, Dh = A_Wq.shape
    M = A_mem0.shape[1]
    seg = int(A_seg_len)
    F = B_w3.shape[1]
    assert (M, seg, Dh) == (8, 32, LANES)
    TM1, TM2 = 256, 128
    nd = D // LANES
    nb2 = S // TM2

    kern = functools.partial(_kernel, S=S, D=D, H=H, Dh=Dh, M=M, seg=seg, F=F, TM1=TM1, TM2=TM2)
    hbm = pl.BlockSpec(memory_space=pl.ANY)
    dma = pltpu.SemaphoreType.DMA
    out = pl.pallas_call(
        kern,
        out_shape=jax.ShapeDtypeStruct((S, D), BF16),
        in_specs=[hbm, pl.BlockSpec(memory_space=pltpu.VMEM)] + [hbm] * 8,
        out_specs=hbm,
        scratch_shapes=[
            pltpu.VMEM((S, D), BF16),
            pltpu.VMEM((S, D), BF16),
            pltpu.VMEM((S, D), F32),
            pltpu.VMEM((nd, S + 2 * PAD, LANES), F32),
            pltpu.VMEM((2, 7, nd // 2, max(TM1, TM2) // 2, LANES), BF16),
            pltpu.VMEM((7, F // (2 * LANES), TM2 // 2, LANES), BF16),
            pltpu.VMEM((7 * (D // 4) * (F // LANES + H // 2) + 3 * (H // 2) * 7 * (D // 4 + 1), LANES), U32),
            pltpu.VMEM((2, 6, (D // 2 // nb2) * H // 2, LANES), U32),
            pltpu.VMEM((2, nd * H * Dh // (2 * nb2), LANES), U32),
            pltpu.VMEM((M, D), F32),
            pltpu.VMEM((4, 7, seg, D // 2), F32),
            pltpu.VMEM((4, 7, seg, H * Dh // 2), F32),
            pltpu.VMEM((4, 4, seg, D // 2), F32),
            pltpu.VMEM((4, 3, 2, seg, LANES), F32),
            dma((S // TM1,)), dma((3 * nd + F // LANES,)), dma((2, 6 + nd)), dma((S // (4 * seg),)),
        ],
        compiler_params=pltpu.CompilerParams(vmem_limit_bytes=126 * 1024 * 1024),
        name="rmt_s2mlp",
    )(A_x.reshape(S, D), A_mem0.reshape(M, D),
      A_Wq.reshape(D * H, Dh), A_Wk.reshape(D * H, Dh), A_Wv.reshape(D * H, Dh),
      A_Wo.reshape(H * Dh, D), B_w1, B_w2, B_w3, B_w4)
    return out.reshape(1, S, D)
```

```python
import functools
import math

import jax
import jax.numpy as jnp
from jax import lax
import jax.experimental.pallas as pl
import jax.experimental.pallas.tpu as pltpu

F32 = jnp.float32
BF16 = jnp.bfloat16
U32 = jnp.uint32
LANES = 128
PAD = 8


def _dot(a, b):
    return lax.dot_general(a, b, (((1,), (0,)), ((), ())), preferred_element_type=F32)


def _dot_nt(a, b):
    return lax.dot_general(a, b, (((1,), (1,)), ((), ())), preferred_element_type=F32)


def _layernorm(x):
    m = jnp.mean(x, axis=-1, keepdims=True)
    d = x - m
    v = jnp.mean(d * d, axis=-1, keepdims=True)
    return d * lax.rsqrt(v + 1e-5)


def _layernorm_twice(x):
    m = jnp.mean(x, axis=-1, keepdims=True)
    d = x - m
    v = jnp.mean(d * d, axis=-1, keepdims=True)
    r = lax.rsqrt(v + 1e-5)
    return d * r, d * (r * lax.rsqrt(v * r * r + 1e-5))


def _recip(x):
    r = pl.reciprocal(x, approx=True)
    return r * (2.0 - x * r)


def _gelu(x):
    c = math.sqrt(2.0 / math.pi)
    inner = x * (c + (c * 0.044715) * (x * x))
    hx = 0.5 * x
    return hx + hx * jnp.tanh(inner)


def _words(x):
    return pltpu.bitcast(x.astype(BF16), U32)


def _halves(w):
    return pltpu.bitcast(w, BF16)


def _cat(xs, axis):
    return xs[0] if len(xs) == 1 else jnp.concatenate(xs, axis=axis)


def _right(b11, b12, b21, b22):
    return (b11 + b22, b11, b12 - b22, b21 - b11, b22, b11 + b12, b21 + b22)


def _unpack(w):
    return pltpu.bitcast(w << 16, F32), pltpu.bitcast(w & U32(0xFFFF0000), F32)


def _pack(lo, hi):
    return pltpu.bitcast(pltpu.pack_elementwise([lo, hi], packed_dtype=BF16), U32)


def _right_words(w):
    lo, hi = zip(*[_unpack(x) for x in w])
    f = [_pack(a, b) for a, b in zip(_right(*lo), _right(*hi))]
    f[1], f[4] = w[0], w[3]
    return f


def _left(a11, a12, a21, a22):
    return (a11 + a22, a21 + a22, a11, a22, a11 + a12, a21 - a11, a12 - a22)


def _combine(m):
    m4 = m(3)
    m2 = m(1)
    c21 = m2 + m4
    m1 = m(0)
    c22 = m1 - m2
    c11 = m1 + m4
    c11 = c11 + m(6)
    m5 = m(4)
    c11 = c11 - m5
    m3 = m(2)
    c12 = m3 + m5
    c22 = c22 + m3
    c22 = c22 + m(5)
    return c11, c12, c21, c22


class _Filler:
    def __init__(self, slots, *job_lists):
        self.slots, self.done, self.lists = slots, 0, job_lists

    def __call__(self):
        for jobs in self.lists:
            n = len(jobs)
            for job in jobs[self.done * n // self.slots:(self.done + 1) * n // self.slots]:
                job()
        self.done += 1


def _kernel(x_hbm, mem0_ref, wq_hbm, wk_hbm, wv_hbm, wo_hbm, w1_hbm, w2_hbm, w3_hbm, w4_hbm,
            out_hbm,
            xbuf, xnb, res, hs, lf, lz, wts, stq, sto, membuf, hl, ol, pbuf, qbuf,
            sem_x, sem_w, sem_a, sem_out,
            *, S, D, H, Dh, M, seg, F, TM1, TM2):
    L = M + seg
    nd = D // LANES
    nh = nd // 2
    Dk = D // 2
    wk = Dk // 2
    slab = wk + 1
    nf = F // (2 * LANES)
    ng = H // 2
    nb1 = S // TM1
    nb2 = S // TM2
    h1 = TM1 // 2
    h2 = TM2 // 2
    RC = 16
    part = functools.partial

    def cols(n, w=1):
        return slice(n * LANES, (n + w) * LANES)

    o_w3 = 0
    o_w4 = o_w3 + nf * 7 * wk
    o_wo = o_w4 + nf * 7 * wk
    o_qkv = o_wo + ng * 7 * wk
    raw = {1: o_qkv, 2: o_qkv + nd * Dk, 3: o_qkv + 2 * nd * Dk, 4: o_qkv + 2 * nd * Dk + 2 * nf * Dk}

    raw_src = {1: w1_hbm, 2: w2_hbm, 3: w3_hbm, 4: w4_hbm}
    raw_rows = {1: Dk, 2: Dk, 3: Dk, 4: F // 2}
    raw_sem = {1: 0, 2: nd, 3: 2 * nd, 4: 2 * nd + 2 * nf}

    def w_copy(j, n):
        return pltpu.make_async_copy(raw_src[j].bitcast(U32).at[:, cols(n)],
                                     wts.at[pl.ds(raw[j] + n * raw_rows[j], raw_rows[j])],
                                     sem_w.at[raw_sem[j] + n])

    def x_copy(i):
        r0 = pl.multiple_of(i * TM1, TM1)
        return pltpu.make_async_copy(x_hbm.at[pl.ds(r0, TM1)], xbuf.at[pl.ds(r0, TM1)], sem_x.at[i])

    fpi = Dk // nb2
    gpi = ng // nb2

    def a_copies(i):
        cps = []
        for t, src in enumerate((wq_hbm, wk_hbm, wv_hbm)):
            for half in range(2):
                r0 = pl.multiple_of((half * Dk + i * fpi) * ng, fpi * ng)
                cps.append(pltpu.make_async_copy(src.bitcast(U32).at[pl.ds(r0, fpi * ng)],
                                                 stq.at[i % 2, 2 * t + half], sem_a.at[i % 2, 2 * t + half]))
        r0 = pl.multiple_of(i * gpi * Dh, gpi * Dh)
        for n in range(nd):
            cps.append(pltpu.make_async_copy(wo_hbm.bitcast(U32).at[pl.ds(r0, gpi * Dh), cols(n)],
                                             sto.at[i % 2, pl.ds(n * gpi * Dh, gpi * Dh)], sem_a.at[i % 2, 6 + n]))
        return cps

    def prep(src, offs, rows, dst, pitch):
        def job(r):
            for i, f in enumerate(_right_words([src[pl.ds(o + r, 8), :] for o in offs])):
                wts[pl.ds(dst + i * pitch + r, 8), :] = f
        return [part(job, r) for r in range(0, rows, 8)]

    def prep_sq(u, r, rows):
        o = pl.multiple_of(raw[1] + (u + (u // nh) * nh) * Dk + r, 8)
        return prep(wts, (o, o + nh * Dk, o + wk, o + nh * Dk + wk), rows,
                    pl.multiple_of(o_wo + u * 7 * wk + r, 8), wk)

    first = [pltpu.make_async_copy(x_hbm.at[pl.ds(r, TM1 // 8)], xbuf.at[pl.ds(r, TM1 // 8)], sem_x.at[0])
             for r in range(0, TM1, TM1 // 8)]
    for c in first:
        c.start()
    for n in range(nh // 2):
        w_copy(1, n).start()
        w_copy(1, n + nh).start()

    zpad = jnp.zeros((PAD, LANES), F32)
    for n in range(nd):
        hs[n, 0:PAD, :] = zpad
        hs[n, PAD + S:PAD + S + PAD, :] = zpad
    membuf[...] = mem0_ref[...].astype(F32)

    def put_left(slot, r, top, bot):
        for k, f in enumerate(_left(top[:, :Dk], top[:, Dk:], bot[:, :Dk], bot[:, Dk:])):
            for n in range(nh):
                lf[slot, k, n, pl.ds(r, RC), :] = f[:, cols(n)].astype(BF16)

    def get_left(slot, k, rows):
        w = lf.bitcast(U32)
        return _halves(_cat([w[slot, k, n, 0:rows // 2, :] for n in range(nh)], 1))

    def weights(r0, rows):
        return _halves(wts[pl.ds(r0, rows), :])

    def norm_pair(i, slot, r):
        a = []
        for half in range(2):
            rr = pl.ds(pl.multiple_of(i * TM1 + half * h1 + r, RC), RC)
            xn, xnn = _layernorm_twice(xbuf[rr, :].astype(F32))
            xnb[rr, :] = xn.astype(BF16)
            res[rr, :] = xn
            a.append(xnn)
        put_left(slot, r, *a)

    for c in first:
        c.wait()
    for n in range(nh // 2, nh):
        w_copy(1, n).start()
        w_copy(1, n + nh).start()
    x_copy(1).start()

    def norm_first(q, carry):
        for e in range(2):
            norm_pair(0, 0, pl.multiple_of((2 * q + e) * RC, RC))
        return carry

    lax.fori_loop(0, h1 // (2 * RC), norm_first, 0)

    def prep_first(n, carry):
        for e in range(2):
            pltpu.make_async_copy(wts.at[pl.ds(0, Dk)], wts.at[pl.ds(0, Dk)], sem_w.at[n + e * nh]).wait()
        for job in prep_sq(n, 0, wk):
            job()
        return carry

    lax.fori_loop(0, nh, prep_first, 0)
    x_copy(2).start()
    x_copy(3).start()

    def w3_copies(lo, hi):
        return [w_copy(3, n) for n in range(2 * lo, 2 * hi)]

    def w4_copies(n):
        return [w_copy(4, n), w_copy(4, n + nh)]

    later = [
        lambda: [w_copy(2, n) for n in range(nd)],
        lambda: [x_copy(4)] + w3_copies(0, 2),
        lambda: [x_copy(5)] + w4_copies(0)[:1],
        lambda: [x_copy(6)] + w4_copies(0)[1:],
        lambda: [x_copy(7)] + w3_copies(2, 4),
        lambda: w4_copies(1),
        lambda: w3_copies(4, 7),
        lambda: w4_copies(2),
        lambda: w3_copies(7, 11),
        lambda: w4_copies(3),
        lambda: w3_copies(11, 14),
        lambda: a_copies(0),
        lambda: a_copies(1),
    ]

    def start_later(i, lo, hi):
        for k in range(lo, min(hi, len(later))):
            @pl.when(i == k - lo)
            def _(k=k):
                for c in later[k]():
                    c.start()

    def b1(i, carry):
        @pl.when(i + 1 < nb1)
        def _():
            x_copy(i + 1).wait()

        @pl.when(i == nh)
        def _():
            for n in range(nd):
                w_copy(2, n).wait()

        r0 = pl.multiple_of(i * TM1, TM1)
        nxt = jnp.minimum(i + 1, nb1 - 1)
        fill = _Filler(7 * nh - 2, [part(norm_pair, nxt, (i + 1) % 2, r) for r in range(0, h1, RC)],
                       prep_sq(i, 0, wk))

        def prod(n, k):
            y = _dot(get_left(i % 2, k, h1), weights(o_wo + (n * 7 + k) * wk, wk))
            fill()
            return y

        for n in range(nh):
            c = _combine(part(prod, n))
            hs[n, pl.ds(r0 + PAD, h1), :] = _gelu(c[0])
            hs[n + nh, pl.ds(r0 + PAD, h1), :] = _gelu(c[1])
            hs[n, pl.ds(r0 + PAD + h1, h1), :] = _gelu(c[2])
            hs[n + nh, pl.ds(r0 + PAD + h1, h1), :] = _gelu(c[3])
        start_later(i, 0, nb1)
        return carry

    lax.fori_loop(0, nb1, b1, 0)

    shifts = (-1, 1, -2, 2)

    def shift_in(i, slot):
        def job(r):
            put_left(slot, r, *[_cat([hs[n, pl.ds(i * TM1 + PAD + half * h1 + r + shifts[n * 4 // nd], RC), :]
                                      for n in range(nd)], 1) for half in range(2)])
        return [part(job, r) for r in range(0, h1, RC)]

    rq = LANES // 2
    per = 4 * nf // nb1

    def prep3(u):
        p, r = u // 4, (u % 4) * rq
        o = pl.multiple_of(raw[3] + 2 * p * Dk + r, 8)
        return prep(wts, (o, o + Dk, o + wk, o + Dk + wk), rq, pl.multiple_of(o_w3 + p * 7 * wk + r, 8), wk)

    def prep4(n, p):
        o = pl.multiple_of(raw[4] + n * (F // 2) + p * LANES, 8)
        return prep(wts, (o, o + nh * (F // 2), o + rq, o + nh * (F // 2) + rq), rq,
                    pl.multiple_of(o_w4 + (n * 7 * nf + p) * rq, 8), nf * rq)

    def b2(i, carry):
        for k in range(nb1):
            @pl.when(i == k)
            def _(k=k):
                for c in w3_copies((k * per + 3) // 4, ((k + 1) * per + 3) // 4) + (
                        [] if k % 2 else w4_copies(k // 2)):
                    c.wait()

        r0 = pl.multiple_of(i * TM1, TM1)
        jobs = [prep3(i * per + u) + prep4(i // 2, (i % 2) * per + u) for u in range(per)]
        fill = _Filler(7 * nh - 2, shift_in(jnp.minimum(i + 1, nb1 - 1), (i + 1) % 2), sum(jobs, []))

        def prod(n, k):
            y = _dot(get_left(i % 2, k, h1), weights(o_wo + ((nh + n) * 7 + k) * wk, wk))
            fill()
            return y

        for n in range(nh):
            c = _combine(part(prod, n))
            res[pl.ds(r0, h1), cols(n)] += c[0]
            res[pl.ds(r0, h1), cols(n + nh)] += c[1]
            res[pl.ds(r0 + h1, h1), cols(n)] += c[2]
            res[pl.ds(r0 + h1, h1), cols(n + nh)] += c[3]
        start_later(i, nb1, 2 * nb1)
        return carry

    for job in shift_in(0, 0):
        job()
    lax.fori_loop(0, nb1, b2, 0)

    def norm_mid(i, slot):
        def job(r):
            put_left(slot, r, *[_layernorm(res[pl.ds(pl.multiple_of(i * TM2 + half * h2 + r, RC), RC), :])
                                for half in range(2)])
        return [part(job, r) for r in range(0, h2, RC)]

    def b3(i, carry):
        for c in a_copies(i):
            c.wait()

        def prep_qkv(t, u, j):
            forms = []
            for par in range(2):
                w = [stq[i % 2, 2 * t + half, pl.ds((2 * u + par) * ng + 8 * j, 8), :] for half in range(2)]
                forms.append(_right(*_unpack(w[0]), *_unpack(w[1])))
            for k in range(7):
                base = o_qkv + ((t * ng + 8 * j) * 7 + k) * slab + u + i * (fpi // 2)
                wts[pl.ds(base, 8, stride=7 * slab), :] = _pack(forms[0][k], forms[1][k])

        def prep_o(g, n):
            o = g * Dh + n * gpi * Dh
            return prep(sto.at[i % 2], (o, o + nh * gpi * Dh, o + Dh // 2, o + nh * gpi * Dh + Dh // 2), Dh // 2,
                        pl.multiple_of(o_wo + (n * 7 * ng + i * gpi + g) * (Dh // 2), Dh // 2), ng * Dh // 2)

        jobs = [part(prep_qkv, t, u, j) for t in range(3) for u in range(fpi // 2) for j in range(ng // 8)]
        jobs += sum([prep_o(g, n) for g in range(gpi) for n in range(nh)], [])
        fill = _Filler((nf // 2) * 7 * (nh // 2) - 4, norm_mid(jnp.minimum(i + 1, nb2 - 1), (i + 1) % 2), jobs)
        r0 = pl.multiple_of(i * TM2, TM2)

        def up(p, k):
            return _dot(get_left(i % 2, k, h2), weights(o_w3 + (p * 7 + k) * wk, wk))

        for p in range(nf):
            for k, f in enumerate(_left(*[_gelu(y) for y in _combine(part(up, p))])):
                lz[k, p] = f.astype(BF16)

        def down(n, k):
            w = lz.bitcast(U32)
            y = None
            for p in range(0, nf, 2):
                z = _dot(_halves(_cat([w[k, p], w[k, p + 1]], 1)),
                         _cat([weights(o_w4 + (((n + e) * 7 + k) * nf + p) * rq, 2 * rq) for e in range(2)], 1))
                y = z if y is None else z + y
                fill()
            return y

        for n in range(0, nh, 2):
            c = _combine(part(down, n))
            for r, cc, y in ((0, n, c[0]), (0, n + nh, c[1]), (h2, n, c[2]), (h2, n + nh, c[3])):
                rr = pl.ds(r0 + r, h2)
                res[rr, cols(cc, 2)] += xbuf[rr, cols(cc, 2)].astype(F32) + y

        @pl.when(i + 2 < nb2)
        def _():
            for c in a_copies(i + 2):
                c.start()

        return carry

    for job in norm_mid(0, 0):
        job()
    lax.fori_loop(0, nb2, b3, 0)

    scale = Dh ** -0.5
    row = lax.broadcasted_iota(jnp.int32, (L, L), 0)
    col = lax.broadcasted_iota(jnp.int32, (L, L), 1)
    mask = (row < M) | (row >= col)
    QS = 4 * seg
    R = seg - M
    rv = R // 8

    def upper(n):
        return lax.broadcasted_iota(jnp.int32, (8, n), 0) < 4

    def split8(mem, tok):
        u = upper(mem.shape[1])
        return jnp.where(u, mem, tok), pltpu.roll(jnp.where(u, tok, mem), 4, 0)

    def join8(t, b):
        u = upper(t.shape[1])
        b = pltpu.roll(b, 4, 0)
        return jnp.where(u, t, b), jnp.where(u, b, t)

    def out_copy(j):
        r0 = pl.multiple_of(j * QS, QS)
        return pltpu.make_async_copy(xbuf.at[pl.ds(r0, QS)], out_hbm.at[pl.ds(r0, QS)], sem_out.at[j])

    def vregs(y, lo, hi):
        return [y[8 * k:8 * k + 8] for k in range(lo, hi)]

    def quad(j, carry):
        xs = xnb[pl.ds(pl.multiple_of(j * QS, QS), QS), :].astype(F32)
        qkv = {(t, h): [] for t in range(3) for h in range(H)}
        att = {h: [] for h in range(H)}
        outs = {n: [] for n in range(nd)}
        mem = membuf[...]
        for st in range(4):
            if st == 0:
                t0, u0 = split8(mem, xs[2 * R:2 * R + 8])
                at = jnp.concatenate([t0, xs[0:R]], axis=0)
                au = jnp.concatenate([u0, xs[R:2 * R]], axis=0)
                for k, f in enumerate(_left(at[:, :Dk], at[:, Dk:], au[:, :Dk], au[:, Dk:])):
                    hl[st, k] = f
            else:
                r = 2 * R + 8 + (st - 1) * R
                a = jnp.concatenate([mem, xs[r:r + R]], axis=0)
                hl[st, 1] = a[:, :Dk] + a[:, Dk:]
                hl[st, 2] = a[:, :Dk]
                hl[st, 3] = a[:, Dk:]

            def four(m):
                return m(3) + m(1), m(2) + m(4, 1)

            def wq_part(t, g, lo, hi):
                def m(k, left=None):
                    w = weights(o_qkv + ((t * ng + g) * 7 + k) * slab + lo // 2, (hi - lo) // 2)
                    return _dot(hl[st, k if left is None else left, :, lo:hi], w)

                return _combine(m) if st == 0 else four(m)

            def proj(t, g, head=None):
                if head is None:
                    c = wq_part(t, g, 0, Dk)
                else:
                    c = [x + y for x, y in zip(head, wq_part(t, g, Dk // 2, Dk))]
                got = []
                if st == 0:
                    for e in range(2):
                        ym, yt = join8(c[e][0:8], c[2 + e][0:8])
                        qkv[t, 2 * g + e] += vregs(c[e], 1, 1 + rv) + vregs(c[2 + e], 1, 1 + rv) + [yt]
                        got.append(ym)
                else:
                    for e, y in enumerate(c):
                        qkv[t, 2 * g + e] += vregs(y, 1, 1 + rv)
                        got.append(y[0:8])
                return [jnp.concatenate([got[e]] + qkv[t, 2 * g + e][4 * st:4 * st + 4], axis=0) for e in range(2)]

            def feed(g, o):
                for e in range(2):
                    att[2 * g + e] += vregs(o[e], 1, 5)
                if st < 3:
                    a = [jnp.concatenate([o[e][0:8]] + att[2 * g + e][st * rv:(st + 1) * rv], axis=0)
                         for e in range(2)]
                    ol[st, 1, :, cols(g)] = a[0] + a[1]
                    ol[st, 2, :, cols(g)] = a[0]
                    ol[st, 3, :, cols(g)] = a[1]
                else:
                    at, au = [], []
                    for e in range(2):
                        y = att[2 * g + e][3 * rv:]
                        t0, u0 = split8(o[e][0:8], y[2 * rv])
                        at.append(jnp.concatenate([t0] + y[:rv], axis=0))
                        au.append(jnp.concatenate([u0] + y[rv:2 * rv], axis=0))
                    for k, f in enumerate(_left(at[0], at[1], au[0], au[1])):
                        ol[st, k, :, cols(g)] = f

            def wo_part(n, lo, hi):
                def m(k, left=None):
                    w = weights(o_wo + ((n * 7 + k) * ng + lo) * (Dh // 2), (hi - lo) * (Dh // 2))
                    return _dot(ol[st, k if left is None else left, :, lo * Dh:hi * Dh], w)

                return _combine(m) if st == 3 else four(m)

            cur, soft = {}, {}
            for g in range(ng + nh):
                if g == 0 and st > 0:
                    for t in range(3):
                        for k, y in enumerate(wq_part(t, g, 0, Dk // 2)):
                            qbuf[st, t, k] = y
                    cur[g] = [proj(t, g, [qbuf[st, t, k] for k in range(2)]) for t in range(3)]
                elif g < ng:
                    cur[g] = [proj(t, g) for t in range(3)]
                else:
                    for k, y in enumerate(wo_part(g - ng, 0, ng // 2)):
                        pbuf[st, k, :, cols(g - ng)] = y
                if 1 <= g <= ng:
                    soft[g - 1] = []
                    for e in range(2):
                        q, k = cur[g - 1][0][e], cur[g - 1][1][e]
                        sc = jnp.where(mask, _dot_nt(q, k.astype(BF16)), -1e9 / scale)
                        p = jnp.exp2((sc - jnp.max(sc, axis=-1, keepdims=True)) * (scale * math.log2(math.e)))
                        soft[g - 1].append(p * _recip(jnp.sum(p, axis=-1, keepdims=True)))
                if 3 <= g < ng + 3:
                    feed(g - 3, [_dot(p, cur[g - 3][2][e].astype(BF16)) for e, p in enumerate(soft[g - 3])])
            new = {}
            for n in range(nh):
                c = [pbuf[st, k, :, cols(n)] + y for k, y in enumerate(wo_part(n, ng // 2, ng))]
                for e in range(2):
                    if st < 3:
                        new[n + e * nh] = c[e][0:8]
                        outs[n + e * nh] += vregs(c[e], 1, 1 + rv)
                    else:
                        ym, yt = join8(c[e][0:8], c[2 + e][0:8])
                        new[n + e * nh] = ym
                        outs[n + e * nh] += vregs(c[e], 1, 1 + rv) + vregs(c[2 + e], 1, 1 + rv) + [yt]
            mem = jnp.concatenate([new[n] for n in range(nd)], axis=1)
            lo, hi = ((0, 2), (2, 6), (6, 8), (8, 16))[st]
            rr = pl.ds(pl.multiple_of(j * QS + 8 * lo, 16), 8 * (hi - lo))
            for n in range(nd):
                xbuf[rr, cols(n)] = (res[rr, cols(n)] + jnp.concatenate(outs[n][lo:hi], axis=0)).astype(BF16)
        membuf[...] = mem
        out_copy(j).start()
        return carry

    lax.fori_loop(0, S // QS, quad, 0)
    for j in range(S // QS):
        out_copy(j).wait()


@functools.partial(jax.jit, static_argnames=("A_seg_len",))
def pallas_parallel_sum__memory_aug_recurrent_mem_tr__mixer_s_mlp__prompt_kernel(
    A_x: jax.Array,
    A_mem0: jax.Array,
    A_Wq: jax.Array,
    A_Wk: jax.Array,
    A_Wv: jax.Array,
    A_Wo: jax.Array,
    A_seg_len: int,
    B_x: jax.Array,
    B_w1: jax.Array,
    B_w2: jax.Array,
    B_w3: jax.Array,
    B_w4: jax.Array,
):
    del B_x
    _, S, D = A_x.shape
    _, H, Dh = A_Wq.shape
    M = A_mem0.shape[1]
    seg = int(A_seg_len)
    F = B_w3.shape[1]
    assert (M, seg, Dh) == (8, 32, LANES)
    TM1, TM2 = 256, 128
    nd = D // LANES
    nb2 = S // TM2

    kern = functools.partial(_kernel, S=S, D=D, H=H, Dh=Dh, M=M, seg=seg, F=F, TM1=TM1, TM2=TM2)
    hbm = pl.BlockSpec(memory_space=pl.ANY)
    dma = pltpu.SemaphoreType.DMA
    out = pl.pallas_call(
        kern,
        out_shape=jax.ShapeDtypeStruct((S, D), BF16),
        in_specs=[hbm, pl.BlockSpec(memory_space=pltpu.VMEM)] + [hbm] * 8,
        out_specs=hbm,
        scratch_shapes=[
            pltpu.VMEM((S, D), BF16),
            pltpu.VMEM((S, D), BF16),
            pltpu.VMEM((S, D), F32),
            pltpu.VMEM((nd, S + 2 * PAD, LANES), F32),
            pltpu.VMEM((2, 7, nd // 2, max(TM1, TM2) // 2, LANES), BF16),
            pltpu.VMEM((7, F // (2 * LANES), TM2 // 2, LANES), BF16),
            pltpu.VMEM((7 * (D // 4) * (F // LANES + H // 2) + 3 * (H // 2) * 7 * (D // 4 + 1), LANES), U32),
            pltpu.VMEM((2, 6, (D // 2 // nb2) * H // 2, LANES), U32),
            pltpu.VMEM((2, nd * H * Dh // (2 * nb2), LANES), U32),
            pltpu.VMEM((M, D), F32),
            pltpu.VMEM((4, 7, seg, D // 2), F32),
            pltpu.VMEM((4, 7, seg, H * Dh // 2), F32),
            pltpu.VMEM((4, 4, seg, D // 2), F32),
            pltpu.VMEM((4, 3, 2, seg, LANES), F32),
            dma((S // TM1,)), dma((3 * nd + F // LANES,)), dma((2, 6 + nd)), dma((S // (4 * seg),)),
        ],
        compiler_params=pltpu.CompilerParams(vmem_limit_bytes=126 * 1024 * 1024, disable_bounds_checks=True, disable_semaphore_checks=True),
        name="rmt_s2mlp",
    )(A_x.reshape(S, D), A_mem0.reshape(M, D),
      A_Wq.reshape(D * H, Dh), A_Wk.reshape(D * H, Dh), A_Wv.reshape(D * H, Dh),
      A_Wo.reshape(H * Dh, D), B_w1, B_w2, B_w3, B_w4)
    return out.reshape(1, S, D)
```

```python
import functools
import math

import jax
import jax.numpy as jnp
from jax import lax
import jax.experimental.pallas as pl
import jax.experimental.pallas.tpu as pltpu

F32 = jnp.float32
BF16 = jnp.bfloat16
U32 = jnp.uint32
LANES = 128
EPS = 1e-5
PAD = 8


def _dot(a, b):
    return lax.dot_general(a, b, (((1,), (0,)), ((), ())), preferred_element_type=F32)


def _dot_nt(a, b):
    return lax.dot_general(a, b, (((1,), (1,)), ((), ())), preferred_element_type=F32)


def _moments(x, z):
    s = _cat([pltpu.bitcast(z, F32)] * (x.shape[0] // 8), 0)
    for c in range(0, x.shape[1], LANES):
        s = s + x[:, c:c + LANES]
    m = jnp.sum(s, axis=-1, keepdims=True) * (1.0 / x.shape[1])
    d = x - m
    return m, d, jnp.mean(d * d, axis=-1, keepdims=True)


def _recip(x):
    r = pl.reciprocal(x, approx=True)
    return r * (2.0 - x * r)


def _gelu(x):
    c = math.sqrt(2.0 / math.pi)
    inner = x * (c + (c * 0.044715) * (x * x))
    hx = 0.5 * x
    return hx + hx * jnp.tanh(inner)


def _words(x):
    return pltpu.bitcast(x.astype(BF16), U32)


def _halves(w):
    return pltpu.bitcast(w, BF16)


def _cat(xs, axis):
    return xs[0] if len(xs) == 1 else jnp.concatenate(xs, axis=axis)


def _right(b11, b12, b21, b22):
    return (b11 + b22, b11, b12 - b22, b21 - b11, b22, b11 + b12, b21 + b22)


def _unpack(w, z):
    return pltpu.bitcast(w << (z | 16), F32), pltpu.bitcast(w & (z | U32(0xFFFF0000)), F32)


def _pack(lo, hi):
    return pltpu.bitcast(pltpu.pack_elementwise([lo, hi], packed_dtype=BF16), U32)


def _right_words(w, z):
    lo, hi = zip(*[_unpack(x, z) for x in w])
    f = [_pack(a, b) for a, b in zip(_right(*lo), _right(*hi))]
    f[1], f[4] = w[0], w[3]
    return f


def _left(a11, a12, a21, a22):
    return (a11 + a22, a21 + a22, a11, a22, a11 + a12, a21 - a11, a12 - a22)


def _combine(m):
    m4 = m(3)
    m2 = m(1)
    c21 = m2 + m4
    m1 = m(0)
    c22 = m1 - m2
    c11 = m1 + m4
    c11 = c11 + m(6)
    m5 = m(4)
    c11 = c11 - m5
    m3 = m(2)
    c12 = m3 + m5
    c22 = c22 + m3
    c22 = c22 + m(5)
    return c11, c12, c21, c22


class _Blocks(tuple):
    def __add__(self, other):
        return _Blocks(a + b for a, b in zip(self, other))

    def __sub__(self, other):
        return _Blocks(a - b for a, b in zip(self, other))


def _nest(a):
    return [_Blocks(a[2 * i + u][2 * j + w] for u in range(2) for w in range(2)) for i in range(2) for j in range(2)]


def _combine2(m, outer):
    c = outer(lambda a: _Blocks(_combine(lambda b: m(7 * a + b))))
    return [[c[2 * (i // 2) + j // 2][2 * (i % 2) + j % 2] for j in range(4)] for i in range(4)]


def _combine_late(m):
    m3 = m(2)
    m5 = m(4)
    c12 = m3 + m5
    c22 = m3 + m(5)
    m1 = m(0)
    c11 = m1 - m5
    c22 = c22 + m1
    m2 = m(1)
    c22 = c22 - m2
    m4 = m(3)
    c21 = m2 + m4
    c11 = c11 + m4
    c11 = c11 + m(6)
    return c11, c12, c21, c22


class _Filler:
    def __init__(self, slots, *job_lists):
        self.slots, self.done, self.lists, self.live = slots, 0, job_lists, []

    def __call__(self, z):
        def step(g, v):
            try:
                g.send(v)
                return True
            except StopIteration:
                return False

        new = []
        for jobs in self.lists:
            n = len(jobs)
            new += [job(z) for job in jobs[self.done * n // self.slots:(self.done + 1) * n // self.slots]]
        self.live = [g for g in new if step(g, None)] + [g for g in self.live if step(g, z)]
        self.done += 1

    def finish(self):
        while self.live or self.done < self.slots:
            self(jnp.zeros((8, LANES), U32))


def _run(jobs, group):
    _Filler(len(jobs) // group, jobs).finish()


def _kernel(x_hbm, mem0_hbm, wq_hbm, wk_hbm, wv_hbm, wo_hbm, w1_hbm, w2_hbm, w3_hbm, w4_hbm,
            out_hbm,
            xbuf, stat, hs, lf, lt, ly, lz, wa, wb, zero, stq, sto, mem0, membuf, pbuf, qbuf,
            sem_x, sem_w, sem_a, sem_out,
            *, S, D, H, Dh, M, seg, F, TM1, TM2):
    L = M + seg
    nd = D // LANES
    nh = nd // 2
    Dk = D // 2
    wk = Dk // 2
    slab = wk + 1
    wq = wk // 2
    nf = F // (4 * LANES)
    ng = H // 2
    nb1 = S // TM1
    nb2 = S // TM2
    h1 = TM1 // 2
    q2 = TM2 // 4
    SUB = 1
    hb = h1 // SUB
    LAG = 2
    NW = 3
    HB = 128
    LAG2 = 2
    RN = 8
    RC = 16
    part = functools.partial

    def cols(n, w=1):
        return slice(n * LANES, (n + w) * LANES)

    o_w3 = 0
    o_w4 = o_w3 + nf * 49 * wq
    o_wo = 0
    o_qkv = o_wo + ng * 7 * wk
    raw = {1: o_qkv, 2: o_qkv + nd * Dk, 3: o_qkv + 2 * nd * Dk, 4: o_qkv + 2 * nd * Dk + 4 * nf * Dk}

    raw_src = {1: w1_hbm, 2: w2_hbm, 3: w3_hbm, 4: w4_hbm}
    raw_rows = {1: Dk, 2: Dk, 3: Dk, 4: F // 2}
    raw_sem = {1: 0, 2: nd, 3: 2 * nd, 4: 2 * nd + 4 * nf}

    def w_copy(j, n):
        return pltpu.make_async_copy(raw_src[j].bitcast(U32).at[:, cols(n)],
                                     wa.at[pl.ds(raw[j] + n * raw_rows[j], raw_rows[j])],
                                     sem_w.at[raw_sem[j] + n])

    def x_copy(i):
        r0 = pl.multiple_of(i * TM1, TM1)
        return pltpu.make_async_copy(x_hbm.at[pl.ds(r0, TM1)], xbuf.at[pl.ds(r0, TM1)], sem_x.at[i])

    fpi = Dk // nb2
    gpi = ng // nb2

    def a_copies(i):
        cps = []
        for t, src in enumerate((wq_hbm, wk_hbm, wv_hbm)):
            for half in range(2):
                r0 = pl.multiple_of((half * Dk + i * fpi) * ng, fpi * ng)
                cps.append(pltpu.make_async_copy(src.bitcast(U32).at[pl.ds(r0, fpi * ng)],
                                                 stq.at[i % 2, 2 * t + half], sem_a.at[i % 2, 2 * t + half]))
        r0 = pl.multiple_of(i * gpi * Dh, gpi * Dh)
        for n in range(nd):
            cps.append(pltpu.make_async_copy(wo_hbm.bitcast(U32).at[pl.ds(r0, gpi * Dh), cols(n)],
                                             sto.at[i % 2, pl.ds(n * gpi * Dh, gpi * Dh)], sem_a.at[i % 2, 6 + n]))
        return cps

    def prep(src, offs, rows, out, dst, pitch):
        def job(r, _):
            w = [src[pl.ds(o + r, 8), :] for o in offs]
            z = yield
            for i, f in enumerate(_right_words(w, z)):
                out[pl.ds(dst + i * pitch + r, 8), :] = f
        return [part(job, r) for r in range(0, rows, 8)]

    def prep_sq(u, out, base):
        o = pl.multiple_of(raw[1] + (u + (u // nh) * nh) * Dk, 8)
        return prep(wa, (o, o + nh * Dk, o + wk, o + nh * Dk + wk), wk,
                    out, pl.multiple_of(base + u * 7 * wk, 8), wk)

    first = [pltpu.make_async_copy(x_hbm.at[pl.ds(r, TM1 // 8)], xbuf.at[pl.ds(r, TM1 // 8)], sem_x.at[0])
             for r in range(0, TM1, TM1 // 8)]
    for c in first:
        c.start()
    for n in range(nh // 2):
        w_copy(1, n).start()
        w_copy(1, n + nh).start()

    zpad = jnp.zeros((PAD, LANES), F32)
    for n in range(nd):
        hs[n, 0:PAD, :] = zpad
        hs[n, PAD + S:PAD + S + PAD, :] = zpad
    wa[0:8, :] = jnp.zeros((8, LANES), U32)
    wb[0:8, :] = jnp.zeros((8, LANES), U32)

    def put_left(slot, r, top, bot):
        for k, f in enumerate(_left(top[:, :Dk], top[:, Dk:], bot[:, :Dk], bot[:, Dk:])):
            for n in range(nh):
                lf[slot, k, n, pl.ds(r, RC), :] = f[:, cols(n)].astype(BF16)
            if k in (1, 4):
                yield

    def get_left(slot, k, r):
        w = lf.bitcast(U32)
        return _cat([w[slot, k, n, r // 2:(r + hb) // 2, :] for n in range(nh)], 1)

    def weights(ref, r0, rows):
        return _halves(ref[pl.ds(r0, rows), :])

    zero[0] = 0

    class Deadline:
        def __init__(self, probe, lag):
            self.probe, self.queue = probe, [None] * lag
            self.zero = jnp.full((8, LANES), zero[0], jnp.int32).astype(U32)

        def after(self, y):
            return pltpu.bitcast(y[0:8, 0:LANES], U32) & self.zero

        def __call__(self, w):
            self.queue.append(self.probe() & self.zero)
            z = self.queue.pop(0)
            if z is not None:
                rest = [w[8:, 0:LANES]] if w.shape[0] > 8 else []
                w = _cat([_cat([w[0:8, 0:LANES] | z] + rest, 0), w[:, LANES:]], 1)
            return w

    def norm_pair(i, slot, r, z):
        a = []
        for half in range(2):
            rr = pl.ds(pl.multiple_of(i * TM1 + half * h1 + r, RC), RC)
            m, d, v = _moments(xbuf[rr, :].astype(F32), z)
            q = lax.rsqrt(v + EPS)
            stat[0, rr, :] = jnp.broadcast_to(m, (RC, LANES))
            stat[1, rr, :] = jnp.broadcast_to(q, (RC, LANES))
            a.append(d * (q * lax.rsqrt(v * q * q + EPS)))
        for _ in range(NW):
            yield
        yield from put_left(slot, r, *a)

    def normed(rr, lo=0, hi=nd):
        m, q = (_cat([stat[k, rr, :]] * (hi - lo), 1) for k in range(2))
        return (xbuf[rr, lo * LANES:hi * LANES].astype(F32) - m) * q

    for c in first:
        c.wait()
    for n in range(nh // 2, nh):
        w_copy(1, n).start()
        w_copy(1, n + nh).start()

    def norm_first(q, carry):
        _run([part(norm_pair, 0, 0, pl.multiple_of((4 * q + e) * RC, RC)) for e in range(4)], 4)
        return carry

    lax.fori_loop(0, h1 // (4 * RC), norm_first, 0)
    x_copy(1).start()

    def prep_first(n, carry):
        for e in range(2):
            pltpu.make_async_copy(wa.at[pl.ds(0, Dk)], wa.at[pl.ds(0, Dk)], sem_w.at[n + e * nh]).wait()
        _run(prep_sq(n, wb, o_w4), 2)
        return carry

    lax.fori_loop(0, nh, prep_first, 0)
    x_copy(2).start()
    x_copy(3).start()
    mem_copy = pltpu.make_async_copy(mem0_hbm, mem0, sem_x.at[nb1])
    mem_copy.start()

    def w3_copies(lo, hi):
        return [w_copy(3, n) for n in range(4 * lo, 4 * hi)]

    def w4_copies(n):
        return [w_copy(4, 2 * j + n) for j in range(4)]

    later = [
        lambda: [x_copy(4)] + [w_copy(2, n) for n in range(nh)],
        lambda: [x_copy(5)] + [w_copy(2, n) for n in range(nh, nd)],
        lambda: [x_copy(6)] + w3_copies(0, 1),
        lambda: [x_copy(7)] + [w_copy(4, 0)],
        lambda: [w_copy(4, 2), w_copy(4, 4)],
        lambda: [w_copy(4, 6)] + w3_copies(1, 2),
        lambda: w3_copies(2, 4),
        lambda: [w_copy(4, 1), w_copy(4, 3)],
        lambda: [w_copy(4, 5), w_copy(4, 7)],
        lambda: w3_copies(4, 6),
        lambda: w3_copies(6, 7),
        lambda: a_copies(0),
        lambda: a_copies(1),
    ]

    def start_later(i, lo, hi):
        for k in range(lo, min(hi, len(later))):
            @pl.when(i == k - lo)
            def _(k=k):
                for c in later[k]():
                    c.start()

    def b1(i, carry):
        @pl.when(i + 1 < nb1)
        def _():
            x_copy(i + 1).wait()

        r0 = pl.multiple_of(i * TM1, TM1)
        nxt = jnp.minimum(i + 1, nb1 - 1)
        fill = _Filler((7 * nh - 3) * SUB, [part(norm_pair, nxt, (i + 1) % 2, r) for r in range(0, h1, RC)])
        due = Deadline(None, 0)

        def prod(n, r, k):
            y = _dot(_halves(get_left(i % 2, k, r)), weights(wb, o_w4 + (n * 7 + k) * wk, wk))
            fill(due.after(y))
            return y

        for n in range(nh):
            for r in range(0, h1, hb):
                for k, y in enumerate(_combine(part(prod, n, r))):
                    hs[n + k % 2 * nh, pl.ds(r0 + PAD + k // 2 * h1 + r, hb), :] = _gelu(y)
        fill.finish()
        start_later(i, 0, nb1)
        return carry

    lax.fori_loop(0, nb1, b1, 0)

    shifts = (-1, 1, -2, 2)

    rq = LANES // 2
    per = nf * (wq // 8) // nb1

    def prep2(src, down, right, dst, pitch, _):
        w = [[wa[pl.ds(src + k * down + j * right, 8), :] for j in range(4)] for k in range(4)]
        z = yield
        w = [[_unpack(x, z) for x in row] for row in w]
        lo, hi = (_right(*_nest([[x[e] for x in row] for row in w])) for e in range(2))
        for a in range(7):
            for b, (u, v) in enumerate(zip(_right(*lo[a]), _right(*hi[a]))):
                wb[pl.ds(dst + (7 * a + b) * pitch, 8), :] = _pack(u, v)

    def prep3(u):
        p, r = u // (wq // 8), u % (wq // 8) * 8
        return part(prep2, pl.multiple_of(raw[3] + 4 * p * Dk + r, 8), wq, Dk,
                    pl.multiple_of(o_w3 + p * 49 * wq + r, 8), wq)

    def prep4(e, u):
        p, r = u // (rq // 8), u % (rq // 8) * 8
        return part(prep2, pl.multiple_of(raw[4] + e * (F // 2) + p * 4 * rq + r, 8), rq, F,
                    pl.multiple_of(o_w4 + (e * 49 * nf + p) * rq + r, 8), nf * rq)

    def b2(i, carry):
        def groups(k):
            return (k * per + wq // 8 - 1) // (wq // 8)

        for k in range(nb1):
            @pl.when(i == k)
            def _(k=k):
                for c in w3_copies(groups(k), groups(k + 1)) + (
                        [] if k % (nb1 // 2) else w4_copies(k // (nb1 // 2))):
                    c.wait()

        r0 = pl.multiple_of(i * TM1, TM1)
        ui = i.astype(U32)
        jobs = [[prep3((ui * per + u).astype(jnp.int32)),
                 prep4(i // (nb1 // 2), ((ui % (nb1 // 2)) * per + u).astype(jnp.int32))] for u in range(per)]
        fill = _Filler(2 * nd * TM1 // HB - 4, sum(jobs, []))
        due = Deadline(lambda: wb[0:8, :], LAG2)
        for r in range(0, TM1, HB):
            sh = [hs[n, pl.ds(r0 + PAD + r + shifts[n * 4 // nd], HB), :] for n in range(nd)]
            for c in range(nd):
                y = None
                for k in range(0, nd, nh):
                    a = pltpu.bitcast(due(pltpu.bitcast(_cat(sh[k:k + nh], 1), U32)), F32)
                    p = _dot(a, weights(wa, raw[2] + c * Dk + k * rq, nh * rq))
                    y = p if y is None else p + y
                    fill(due.after(y))
                hs[c, pl.ds(r0 + r, HB), :] = y
        fill.finish()
        start_later(i, nb1, 2 * nb1)
        return carry

    for n in range(nd):
        w_copy(2, n).wait()
    lax.fori_loop(0, nb1, b2, 0)

    def norm_mid(i):
        def job(r, z):
            rr = pl.ds(pl.multiple_of(i * TM2 + r, RN), RN)
            _, d, v = _moments(_cat([hs[n, rr, :] for n in range(nd)], 1) + normed(rr), z)
            lt[r:r + RN, :] = d * lax.rsqrt(v + EPS)
            yield
        return [part(job, r) for r in range(0, TM2, RN)]

    def left_mid():
        def job(r, n, z):
            a = [[lt[u * q2 + r:u * q2 + r + RC, cols(2 * j + n)] for j in range(4)] for u in range(4)]
            for k, g in enumerate(_left(*_nest(a))):
                for b, f in enumerate(_left(*g)):
                    ly[7 * k + b, n, r:r + RC, :] = f.astype(BF16)
                yield
        return [part(job, r, n) for r in range(0, q2, RC) for n in range(2)]

    def b3(i, carry):
        for c in a_copies(i):
            c.wait()

        def prep_qkv(t, u, j, _):
            w = [[stq[i % 2, 2 * t + half, pl.ds((2 * u + par) * ng + 8 * j, 8), :] for half in range(2)]
                 for par in range(2)]
            z = yield
            forms = [_right(*_unpack(x[0], z), *_unpack(x[1], z)) for x in w]
            for k in range(7):
                base = o_qkv + ((t * ng + 8 * j) * 7 + k) * slab + u + i * (fpi // 2)
                wa[pl.ds(base, 8, stride=7 * slab), :] = _pack(forms[0][k], forms[1][k])

        def prep_o(g, n):
            o = g * Dh + n * gpi * Dh
            return prep(sto.at[i % 2], (o, o + nh * gpi * Dh, o + Dh // 2, o + nh * gpi * Dh + Dh // 2), Dh // 2,
                        wa, pl.multiple_of(o_wo + (n * 7 * ng + i * gpi + g) * (Dh // 2), Dh // 2), ng * Dh // 2)

        jobs = [part(prep_qkv, t, u, j) for t in range(3) for u in range(fpi // 2) for j in range(ng // 8)]
        jobs += sum([prep_o(g, n) for g in range(gpi) for n in range(nh)], [])
        r0 = pl.multiple_of(i * TM2, TM2)
        here = pl.ds(pl.multiple_of(zero[0], 8), 8)
        SLOTS = [k for k in range(49) if k // 7 in (1, 0)]
        YS = SLOTS[::4]
        fill = _Filler(nf * len(YS) + 2 * 49 - 8, jobs)
        due = Deadline(lambda: wa[0:8, :], 5)
        fill_y = _Filler((nf - 1) * len(SLOTS), norm_mid(jnp.minimum(i + 1, nb2 - 1)))
        due_y = Deadline(lambda: pltpu.bitcast(lt[here, 0:LANES], U32), 14)
        fill_z = _Filler(2 * 49 - 24, left_mid())
        due_z = Deadline(lambda: ly.bitcast(U32)[zero[0], 0, 0:8, :], 6)

        def up(p, k):
            w = ly.bitcast(U32)
            w = _cat([w[k, n] for n in range(2)], 1)
            slot = k in SLOTS
            if k in YS:
                w = due(w)
            y = _dot(_halves(due_y(w) if slot else w), weights(wb, o_w3 + (p * 49 + k) * wq, wq))
            if slot:
                z = due.after(y)
                fill_y(z)
                if k in YS:
                    fill(z)
            return y

        for p in range(nf):
            g = [[_gelu(y) for y in row] for row in _combine2(part(up, p), _combine)]
            for a, blocks in enumerate(_left(*_nest(g))):
                for b, f in enumerate(_left(*blocks)):
                    lz[7 * a + b, p] = f.astype(BF16)
        fill_y.finish()

        def down(e, k):
            w = lz.bitcast(U32)
            y = _dot(_halves(due_z(due(_cat([w[k, p] for p in range(nf)], 1)))),
                     weights(wb, o_w4 + (e * 49 + k) * nf * rq, nf * rq))
            z = due.after(y)
            fill(z)
            fill_z(z)
            return y

        for e in range(2):
            for u, row in enumerate(_combine2(part(down, e), _combine_late)):
                for j, y in enumerate(row):
                    rr = pl.ds(r0 + u * q2, q2)
                    c = 2 * j + e
                    hs[c, rr, :] += (xbuf[rr, cols(c)].astype(F32) + normed(rr, c, c + 1)) + y

        fill_z.finish()
        fill.finish()

        @pl.when(i + 2 < nb2)
        def _():
            for c in a_copies(i + 2):
                c.start()

        return carry

    _run(norm_mid(0), 1)
    _run(left_mid(), 1)
    lax.fori_loop(0, nb2, b3, 0)

    scale = Dh ** -0.5
    row = lax.broadcasted_iota(jnp.int32, (L, L), 0)
    col = lax.broadcasted_iota(jnp.int32, (L, L), 1)
    mask = (row < M) | (row >= col)
    QS = 4 * seg
    R = seg - M
    rv = R // 8

    def upper(n):
        return lax.broadcasted_iota(jnp.int32, (8, n), 0) < 4

    def split8(mem, tok):
        u = upper(mem.shape[1])
        return jnp.where(u, mem, tok), pltpu.roll(jnp.where(u, tok, mem), 4, 0)

    def join8(t, b):
        u = upper(t.shape[1])
        b = pltpu.roll(b, 4, 0)
        return jnp.where(u, t, b), jnp.where(u, b, t)

    def out_copy(j):
        r0 = pl.multiple_of(j * QS, QS)
        return pltpu.make_async_copy(xbuf.at[pl.ds(r0, QS)], out_hbm.at[pl.ds(r0, QS)], sem_out.at[j])

    def vregs(y, lo, hi):
        return [y[8 * k:8 * k + 8] for k in range(lo, hi)]

    def quad(j, carry):
        xs = normed(pl.ds(pl.multiple_of(j * QS, QS), QS))
        qkv = {(t, h): [] for t in range(3) for h in range(H)}
        att = {h: [] for h in range(H)}
        outs = {n: [] for n in range(nd)}
        mem = membuf[...]
        for st in range(4):
            if st == 0:
                t0, u0 = split8(mem, xs[2 * R:2 * R + 8])
                at = jnp.concatenate([t0, xs[0:R]], axis=0)
                au = jnp.concatenate([u0, xs[R:2 * R]], axis=0)
                hl = _left(at[:, :Dk], at[:, Dk:], au[:, :Dk], au[:, Dk:])
            else:
                r = 2 * R + 8 + (st - 1) * R
                a = jnp.concatenate([mem, xs[r:r + R]], axis=0)
                hl = {1: a[:, :Dk] + a[:, Dk:], 2: a[:, :Dk], 3: a[:, Dk:]}
            ol = {}

            def four(m):
                return m(3) + m(1), m(2) + m(4, 1)

            def wq_part(t, g, lo, hi):
                def m(k, left=None):
                    w = weights(wa, o_qkv + ((t * ng + g) * 7 + k) * slab + lo // 2, (hi - lo) // 2)
                    return _dot(hl[k if left is None else left][:, lo:hi], w)

                return _combine(m) if st == 0 else four(m)

            def proj(t, g, head=None):
                if head is None:
                    c = wq_part(t, g, 0, Dk)
                else:
                    c = [x + y for x, y in zip(head, wq_part(t, g, Dk // 2, Dk))]
                got = []
                if st == 0:
                    for e in range(2):
                        ym, yt = join8(c[e][0:8], c[2 + e][0:8])
                        qkv[t, 2 * g + e] += vregs(c[e], 1, 1 + rv) + vregs(c[2 + e], 1, 1 + rv) + [yt]
                        got.append(ym)
                else:
                    for e, y in enumerate(c):
                        qkv[t, 2 * g + e] += vregs(y, 1, 1 + rv)
                        got.append(y[0:8])
                return [jnp.concatenate([got[e]] + qkv[t, 2 * g + e][4 * st:4 * st + 4], axis=0) for e in range(2)]

            def feed(g, o):
                for e in range(2):
                    att[2 * g + e] += vregs(o[e], 1, 5)
                if st < 3:
                    a = [jnp.concatenate([o[e][0:8]] + att[2 * g + e][st * rv:(st + 1) * rv], axis=0)
                         for e in range(2)]
                    ol[g] = {1: a[0] + a[1], 2: a[0], 3: a[1]}
                else:
                    at, au = [], []
                    for e in range(2):
                        y = att[2 * g + e][3 * rv:]
                        t0, u0 = split8(o[e][0:8], y[2 * rv])
                        at.append(jnp.concatenate([t0] + y[:rv], axis=0))
                        au.append(jnp.concatenate([u0] + y[rv:2 * rv], axis=0))
                    ol[g] = _left(at[0], at[1], au[0], au[1])

            def wo_part(n, lo, hi):
                def m(k, left=None):
                    w = weights(wa, o_wo + ((n * 7 + k) * ng + lo) * (Dh // 2), (hi - lo) * (Dh // 2))
                    return _dot(_cat([ol[g][k if left is None else left] for g in range(lo, hi)], 1), w)

                return _combine(m) if st == 3 else four(m)

            cur, soft = {}, {}
            for g in range(ng + nh):
                if g == 0 and st > 0:
                    for t in range(3):
                        for k, y in enumerate(wq_part(t, g, 0, Dk // 2)):
                            qbuf[st, t, k] = y
                    cur[g] = [proj(t, g, [qbuf[st, t, k] for k in range(2)]) for t in range(3)]
                elif g < ng:
                    cur[g] = [proj(t, g) for t in range(3)]
                else:
                    for k, y in enumerate(wo_part(g - ng, 0, ng // 2)):
                        pbuf[st, k, :, cols(g - ng)] = y
                if 1 <= g <= ng:
                    soft[g - 1] = []
                    for e in range(2):
                        q, k = cur[g - 1][0][e], cur[g - 1][1][e]
                        sc = jnp.where(mask, _dot_nt(q, k.astype(BF16)), -1e9 / scale)
                        p = jnp.exp2((sc - jnp.max(sc, axis=-1, keepdims=True)) * (scale * math.log2(math.e)))
                        soft[g - 1].append(p * _recip(jnp.sum(p, axis=-1, keepdims=True)))
                if 3 <= g < ng + 3:
                    feed(g - 3, [_dot(p, cur[g - 3][2][e].astype(BF16)) for e, p in enumerate(soft[g - 3])])
            new = {}
            for n in range(nh):
                c = [pbuf[st, k, :, cols(n)] + y for k, y in enumerate(wo_part(n, ng // 2, ng))]
                for e in range(2):
                    if st < 3:
                        new[n + e * nh] = c[e][0:8]
                        outs[n + e * nh] += vregs(c[e], 1, 1 + rv)
                    else:
                        ym, yt = join8(c[e][0:8], c[2 + e][0:8])
                        new[n + e * nh] = ym
                        outs[n + e * nh] += vregs(c[e], 1, 1 + rv) + vregs(c[2 + e], 1, 1 + rv) + [yt]
            mem = jnp.concatenate([new[n] for n in range(nd)], axis=1)
            lo, hi = ((0, 2), (2, 6), (6, 8), (8, 16))[st]
            rr = pl.ds(pl.multiple_of(j * QS + 8 * lo, 16), 8 * (hi - lo))
            for n in range(nd):
                xbuf[rr, cols(n)] = (hs[n, rr, :] + jnp.concatenate(outs[n][lo:hi], axis=0)).astype(BF16)
        membuf[...] = mem
        out_copy(j).start()
        return carry

    mem_copy.wait()
    membuf[...] = mem0[...].astype(F32)
    lax.fori_loop(0, S // QS, quad, 0)
    for j in range(S // QS):
        out_copy(j).wait()


@functools.partial(jax.jit, static_argnames=("A_seg_len",))
def pallas_parallel_sum__memory_aug_recurrent_mem_tr__mixer_s_mlp__prompt_kernel(
    A_x: jax.Array,
    A_mem0: jax.Array,
    A_Wq: jax.Array,
    A_Wk: jax.Array,
    A_Wv: jax.Array,
    A_Wo: jax.Array,
    A_seg_len: int,
    B_x: jax.Array,
    B_w1: jax.Array,
    B_w2: jax.Array,
    B_w3: jax.Array,
    B_w4: jax.Array,
):
    del B_x
    _, S, D = A_x.shape
    _, H, Dh = A_Wq.shape
    M = A_mem0.shape[1]
    seg = int(A_seg_len)
    F = B_w3.shape[1]
    assert (M, seg, Dh) == (8, 32, LANES)
    TM1, TM2 = 256, 128
    nd = D // LANES
    nb2 = S // TM2

    kern = functools.partial(_kernel, S=S, D=D, H=H, Dh=Dh, M=M, seg=seg, F=F, TM1=TM1, TM2=TM2)
    hbm = pl.BlockSpec(memory_space=pl.ANY)
    dma = pltpu.SemaphoreType.DMA
    out = pl.pallas_call(
        kern,
        out_shape=jax.ShapeDtypeStruct((S, D), BF16),
        in_specs=[hbm] * 10,
        out_specs=hbm,
        scratch_shapes=[
            pltpu.VMEM((S, D), BF16),
            pltpu.VMEM((2, S, LANES), F32),
            pltpu.VMEM((nd, S + 2 * PAD, LANES), F32),
            pltpu.VMEM((2, 7, nd // 2, TM1 // 2, LANES), BF16),
            pltpu.VMEM((TM2, D), F32),
            pltpu.VMEM((49, nd // 4, TM2 // 4, LANES), BF16),
            pltpu.VMEM((49, F // (4 * LANES), TM2 // 4, LANES), BF16),
            pltpu.VMEM(((H // 2) * 7 * (D // 4 + 3 * (D // 4 + 1)), LANES), U32),
            pltpu.VMEM((2 * 49 * (D // 8) * (F // (4 * LANES)), LANES), U32),
            pltpu.SMEM((1,), jnp.int32),
            pltpu.VMEM((2, 6, (D // 2 // nb2) * H // 2, LANES), U32),
            pltpu.VMEM((2, nd * H * Dh // (2 * nb2), LANES), U32),
            pltpu.VMEM((M, D), BF16),
            pltpu.VMEM((M, D), F32),
            pltpu.VMEM((4, 4, seg, D // 2), F32),
            pltpu.VMEM((4, 3, 2, seg, LANES), F32),
            dma((S // TM1 + 1,)), dma((3 * nd + F // LANES,)), dma((2, 6 + nd)), dma((S // (4 * seg),)),
        ],
        compiler_params=pltpu.CompilerParams(vmem_limit_bytes=128 * 1024 * 1024, disable_bounds_checks=True, disable_semaphore_checks=True),
        name="rmt_s2mlp",
    )(A_x.reshape(S, D), A_mem0.reshape(M, D),
      A_Wq.reshape(D * H, Dh), A_Wk.reshape(D * H, Dh), A_Wv.reshape(D * H, Dh),
      A_Wo.reshape(H * Dh, D), B_w1, B_w2, B_w3, B_w4)
    return out.reshape(1, S, D)
```

```python
import functools
import math

import jax
import jax.numpy as jnp
from jax import lax
import jax.experimental.pallas as pl
import jax.experimental.pallas.tpu as pltpu

F32 = jnp.float32
BF16 = jnp.bfloat16
U32 = jnp.uint32
LANES = 128
EPS = 1e-5
PAD = 8


def _dot(a, b):
    return lax.dot_general(a, b, (((1,), (0,)), ((), ())), preferred_element_type=F32)


def _dot_nt(a, b):
    return lax.dot_general(a, b, (((1,), (1,)), ((), ())), preferred_element_type=F32)


def _moments(x, z):
    s = _cat([pltpu.bitcast(z, F32)] * (x.shape[0] // 8), 0)
    for c in range(0, x.shape[1], LANES):
        s = s + x[:, c:c + LANES]
    m = jnp.sum(s, axis=-1, keepdims=True) * (1.0 / x.shape[1])
    d = x - m
    return m, d, jnp.mean(d * d, axis=-1, keepdims=True)


def _recip(x):
    r = pl.reciprocal(x, approx=True)
    return r * (2.0 - x * r)


def _gelu(x):
    c = math.sqrt(2.0 / math.pi)
    inner = x * (c + (c * 0.044715) * (x * x))
    hx = 0.5 * x
    return hx + hx * jnp.tanh(inner)


def _words(x):
    return pltpu.bitcast(x.astype(BF16), U32)


def _halves(w):
    return pltpu.bitcast(w, BF16)


def _cat(xs, axis):
    return xs[0] if len(xs) == 1 else jnp.concatenate(xs, axis=axis)


def _right(b11, b12, b21, b22):
    return (b11 + b22, b11, b12 - b22, b21 - b11, b22, b11 + b12, b21 + b22)


def _unpack(w, z):
    return pltpu.bitcast(w << (z | 16), F32), pltpu.bitcast(w & (z | U32(0xFFFF0000)), F32)


def _pack(lo, hi):
    return pltpu.bitcast(pltpu.pack_elementwise([lo, hi], packed_dtype=BF16), U32)


def _right_words(w, z):
    lo, hi = zip(*[_unpack(x, z) for x in w])
    f = [_pack(a, b) for a, b in zip(_right(*lo), _right(*hi))]
    f[1], f[4] = w[0], w[3]
    return f


def _left(a11, a12, a21, a22):
    return (a11 + a22, a21 + a22, a11, a22, a11 + a12, a21 - a11, a12 - a22)


def _combine(m):
    m4 = m(3)
    m2 = m(1)
    c21 = m2 + m4
    m1 = m(0)
    c22 = m1 - m2
    c11 = m1 + m4
    c11 = c11 + m(6)
    m5 = m(4)
    c11 = c11 - m5
    m3 = m(2)
    c12 = m3 + m5
    c22 = c22 + m3
    c22 = c22 + m(5)
    return c11, c12, c21, c22


class _Blocks(tuple):
    def __add__(self, other):
        return _Blocks(a + b for a, b in zip(self, other))

    def __sub__(self, other):
        return _Blocks(a - b for a, b in zip(self, other))


def _nest(a):
    return [_Blocks(a[2 * i + u][2 * j + w] for u in range(2) for w in range(2)) for i in range(2) for j in range(2)]


def _combine2(m, outer):
    c = outer(lambda a: _Blocks(_combine(lambda b: m(7 * a + b))))
    return [[c[2 * (i // 2) + j // 2][2 * (i % 2) + j % 2] for j in range(4)] for i in range(4)]


def _combine_late(m):
    m3 = m(2)
    m5 = m(4)
    c12 = m3 + m5
    c22 = m3 + m(5)
    m1 = m(0)
    c11 = m1 - m5
    c22 = c22 + m1
    m2 = m(1)
    c22 = c22 - m2
    m4 = m(3)
    c21 = m2 + m4
    c11 = c11 + m4
    c11 = c11 + m(6)
    return c11, c12, c21, c22


def _hopcroft_kerr(types):
    n = len(types)
    prods = []

    def add(left, out):
        prods.append((left, {}, out))
        return len(prods) - 1

    def use(weight, terms):
        for f, s in terms:
            for k, c in weight.items():
                prods[f][1][k] = prods[f][1].get(k, 0) + s * c

    class Node:
        def __init__(self, t, xs, ys, plus, minus):
            self.t, self.xs, self.ys, self.plus, self.minus = t, xs, ys, plus, minus

    def mix(*parts):
        return {(i, t % 3): s * c for d, t, s in parts for i, c in d.items()}

    def pair(u, w):
        if (u.t - w.t) % 3 != 1:
            zwu, zuw, free = pair(w, u)
            return zuw, zwu, free
        t = u.t
        s = add(mix((u.xs, t + 2, 1), (w.xs, t, 1)), mix((u.ys, t + 2, 1), (w.ys, t, -1)))
        o1 = add(mix((u.xs, t, -1), (w.xs, t, 1)), mix((u.ys, t + 2, 1), (w.ys, t + 2, 1)))
        o2 = add(mix((u.xs, t + 2, -1), (w.xs, t + 2, 1)), mix((u.ys, t, 1), (w.ys, t, 1)))
        free = Node((t + 1) % 3, {**{i: -c for i, c in u.xs.items()}, **w.xs}, {**u.ys, **w.ys}, o1, o2)
        return ([(s, 1), (o1, -1), (u.minus, 1), (w.minus, -1)],
                [(s, 1), (o2, -1), (u.plus, 1), (w.plus, -1)], free)

    nodes = []
    for i, t in enumerate(types):
        e = {i: 1}
        nodes.append(Node(t, e, e, add(mix((e, t + 2, 1)), mix((e, t + 1, 1))),
                          add(mix((e, t + 1, 1)), mix((e, t + 2, 1)))))
        use({(i, i): 1}, [(nodes[i].plus, 1), (nodes[i].minus, -1)])
    z, free = {}, {}
    for i in range(n):
        for j in range(i + 1, n):
            if types[i] != types[j]:
                z[i, j], z[j, i], free[i, j] = pair(nodes[i], nodes[j])
                free[j, i] = free[i, j]
    for i in range(n):
        for j in range(i + 1, n):
            if types[i] == types[j]:
                k = next(k for k in range(n) if types[k] != types[i])
                w = free[i, k]
                zwj, zjw, _ = pair(w, nodes[j])
                s = w.xs[i]
                z[i, j] = [(f, s * c) for f, c in zwj] + z[k, j]
                z[j, i] = zjw + [(f, -c) for f, c in z[j, k]]
    for key, terms in z.items():
        use({key: 1}, terms)
    return [(l, {k: c for k, c in r.items() if c}, o) for l, r, o in prods]


_HK = _hopcroft_kerr((0, 1, 2, 0))
_HK_ROW = [f for f, (l, _, o) in enumerate(_HK) if any(t != 2 for _, t in l) and any(t != 0 for _, t in o)]


def _signed_sum(terms):
    terms = sorted(terms, key=lambda t: -t[0])
    sign, y = terms[0]
    for s, x in terms[1:]:
        y = y + x if s == sign else y - x
    return sign, y


def _signed_value(terms):
    sign, y = _signed_sum(terms)
    return y if sign > 0 else -y


_HK_RIGHT_SIGN = [_signed_sum([(c, 0) for c in r.values()])[0] for _, r, _ in _HK]


def _hk_left(upper, lower=None):
    if lower is None:
        base = [((1, u), (-1, u), None) for u in upper]
    else:
        base = [((1, u), (1, w), (-1, u + w)) for u, w in zip(upper, lower)]
    return {f: _signed_sum([(c * base[i][t][0], base[i][t][1]) for (i, t), c in _HK[f][0].items() if base[i][t]])
            for f in (_HK_ROW if lower is None else range(len(_HK)))}


def _hk_combine(signs, m):
    both = len(signs) == len(_HK)
    acc = {}
    for f, sign in signs.items():
        y = m(f)
        for (j, t), c in _HK[f][2].items():
            c *= sign * _HK_RIGHT_SIGN[f]
            if both:
                acc[j, t] = _signed_sum([acc[j, t], (c, y)]) if (j, t) in acc else (c, y)
            elif t:
                c *= (0, -1, 1)[t]
                acc[j] = _signed_sum([acc[j], (c, y)]) if j in acc else (c, y)
    if not both:
        return [[_signed_value([acc[j]]) for j in range(4)]]
    return [[_signed_value([acc[j, p], (-acc[j, q][0], acc[j, q][1])]) for j in range(4)]
            for p, q in ((2, 1), (0, 2))]


class _Filler:
    def __init__(self, slots, *job_lists):
        self.slots, self.done, self.lists, self.live = slots, 0, job_lists, []

    def __call__(self, z):
        def step(g, v):
            try:
                g.send(v)
                return True
            except StopIteration:
                return False

        new = []
        for jobs in self.lists:
            n = len(jobs)
            new += [job(z) for job in jobs[self.done * n // self.slots:(self.done + 1) * n // self.slots]]
        self.live = [g for g in new if step(g, None)] + [g for g in self.live if step(g, z)]
        self.done += 1

    def finish(self):
        while self.live or self.done < self.slots:
            self(jnp.zeros((8, LANES), U32))


def _run(jobs, group):
    _Filler(len(jobs) // group, jobs).finish()


def _kernel(x_hbm, mem0_hbm, wq_hbm, wk_hbm, wv_hbm, wo_hbm, w1_hbm, w2_hbm, w3_hbm, w4_hbm,
            out_hbm,
            xbuf, stat, hs, lf, lt, ly, lz, wa, wb, zero, stq, sto, mem0, membuf, pbuf,
            sem_x, sem_w, sem_a, sem_out,
            *, S, D, H, Dh, M, seg, F, TM1, TM2):
    L = M + seg
    nd = D // LANES
    nh = nd // 2
    Dk = D // 2
    wk = Dk // 2
    slab = wk // 2 + 2
    wq = wk // 2
    nf = F // (4 * LANES)
    hp = H // 2
    ng = H // 4
    nk = len(_HK)
    nb1 = S // TM1
    nb2 = S // TM2
    h1 = TM1 // 2
    q2 = TM2 // 4
    SUB = 1
    hb = h1 // SUB
    LAG = 2
    NW = 3
    HB = 128
    LAG2 = 2
    RN = 8
    RC = 16
    part = functools.partial

    def cols(n, w=1):
        return slice(n * LANES, (n + w) * LANES)

    o_w3 = 0
    o_w4 = o_w3 + nf * 49 * wq
    o_wo = 0
    o_qkv = o_wo + 2 * nk * ng * (Dh // 2)
    raw = {1: o_qkv, 2: o_qkv + nd * Dk, 3: o_qkv + 2 * nd * Dk, 4: o_qkv + 2 * nd * Dk + 4 * nf * Dk}

    raw_src = {1: w1_hbm, 2: w2_hbm, 3: w3_hbm, 4: w4_hbm}
    raw_rows = {1: Dk, 2: Dk, 3: Dk, 4: F // 2}
    raw_sem = {1: 0, 2: nd, 3: 2 * nd, 4: 2 * nd + 4 * nf}

    def w_copy(j, n):
        return pltpu.make_async_copy(raw_src[j].bitcast(U32).at[:, cols(n)],
                                     wa.at[pl.ds(raw[j] + n * raw_rows[j], raw_rows[j])],
                                     sem_w.at[raw_sem[j] + n])

    def x_copy(i):
        r0 = pl.multiple_of(i * TM1, TM1)
        return pltpu.make_async_copy(x_hbm.at[pl.ds(r0, TM1)], xbuf.at[pl.ds(r0, TM1)], sem_x.at[i])

    fpi = D // 4 // nb2
    opi = ng * (Dh // 2) // nb2

    def heads(g):
        return [2 * g, 2 * g + 1, hp + 2 * g, hp + 2 * g + 1]

    def a_copies(i):
        cps = []
        for t, src in enumerate((wq_hbm, wk_hbm, wv_hbm)):
            for k in range(4):
                r0 = pl.multiple_of((k * (D // 4) + i * fpi) * hp, fpi * hp)
                cps.append(pltpu.make_async_copy(src.bitcast(U32).at[pl.ds(r0, fpi * hp)],
                                                 stq.at[i % 2, 4 * t + k], sem_a.at[i % 2]))
        per_group = Dh // 2 // opi
        for k, h in enumerate(heads(i // per_group)):
            r0 = pl.multiple_of(h * (Dh // 2) + i % per_group * opi, opi)
            for n in range(nd):
                cps.append(pltpu.make_async_copy(wo_hbm.bitcast(U32).at[pl.ds(r0, opi), cols(n)],
                                                 sto.at[i % 2, k, n], sem_a.at[i % 2]))
        return cps

    def prep(src, offs, rows, out, dst, pitch):
        def job(r, _):
            w = [src[pl.ds(o + r, 8), :] for o in offs]
            z = yield
            for i, f in enumerate(_right_words(w, z)):
                out[pl.ds(dst + i * pitch + r, 8), :] = f
        return [part(job, r) for r in range(0, rows, 8)]

    def prep_sq(u, out, base):
        o = pl.multiple_of(raw[1] + (u + (u // nh) * nh) * Dk, 8)
        return prep(wa, (o, o + nh * Dk, o + wk, o + nh * Dk + wk), wk,
                    out, pl.multiple_of(base + u * 7 * wk, 8), wk)

    first = [pltpu.make_async_copy(x_hbm.at[pl.ds(r, TM1 // 8)], xbuf.at[pl.ds(r, TM1 // 8)], sem_x.at[0])
             for r in range(0, TM1, TM1 // 8)]
    for c in first:
        c.start()
    for n in range(nh // 2):
        w_copy(1, n).start()
        w_copy(1, n + nh).start()

    zpad = jnp.zeros((PAD, LANES), F32)
    for n in range(nd):
        hs[n, 0:PAD, :] = zpad
        hs[n, PAD + S:PAD + S + PAD, :] = zpad
    wa[0:8, :] = jnp.zeros((8, LANES), U32)
    wb[0:8, :] = jnp.zeros((8, LANES), U32)

    def put_left(slot, r, top, bot):
        for k, f in enumerate(_left(top[:, :Dk], top[:, Dk:], bot[:, :Dk], bot[:, Dk:])):
            for n in range(nh):
                lf[slot, k, n, pl.ds(r, RC), :] = f[:, cols(n)].astype(BF16)
            if k in (1, 4):
                yield

    def get_left(slot, k, r):
        w = lf.bitcast(U32)
        return _cat([w[slot, k, n, r // 2:(r + hb) // 2, :] for n in range(nh)], 1)

    def weights(ref, r0, rows):
        return _halves(ref[pl.ds(r0, rows), :])

    zero[0] = 0

    class Deadline:
        def __init__(self, probe, lag):
            self.probe, self.queue = probe, [None] * lag
            self.zero = jnp.full((8, LANES), zero[0], jnp.int32).astype(U32)

        def after(self, y):
            return pltpu.bitcast(y[0:8, 0:LANES], U32) & self.zero

        def __call__(self, w):
            self.queue.append(self.probe() & self.zero)
            z = self.queue.pop(0)
            if z is not None:
                rest = [w[8:, 0:LANES]] if w.shape[0] > 8 else []
                w = _cat([_cat([w[0:8, 0:LANES] | z] + rest, 0), w[:, LANES:]], 1)
            return w

    def norm_pair(i, slot, r, z):
        a = []
        for half in range(2):
            rr = pl.ds(pl.multiple_of(i * TM1 + half * h1 + r, RC), RC)
            m, d, v = _moments(xbuf[rr, :].astype(F32), z)
            q = lax.rsqrt(v + EPS)
            stat[0, rr, :] = jnp.broadcast_to(m, (RC, LANES))
            stat[1, rr, :] = jnp.broadcast_to(q, (RC, LANES))
            a.append(d * (q * lax.rsqrt(v * q * q + EPS)))
        for _ in range(NW):
            yield
        yield from put_left(slot, r, *a)

    def normed(rr, lo=0, hi=nd):
        m, q = (_cat([stat[k, rr, :]] * (hi - lo), 1) for k in range(2))
        return (xbuf[rr, lo * LANES:hi * LANES].astype(F32) - m) * q

    for c in first:
        c.wait()
    for n in range(nh // 2, nh):
        w_copy(1, n).start()
        w_copy(1, n + nh).start()

    def norm_first(q, carry):
        _run([part(norm_pair, 0, 0, pl.multiple_of((4 * q + e) * RC, RC)) for e in range(4)], 4)
        return carry

    lax.fori_loop(0, h1 // (4 * RC), norm_first, 0)
    x_copy(1).start()

    def prep_first(n, carry):
        for e in range(2):
            pltpu.make_async_copy(wa.at[pl.ds(0, Dk)], wa.at[pl.ds(0, Dk)], sem_w.at[n + e * nh]).wait()
        _run(prep_sq(n, wb, o_w4), 2)
        return carry

    lax.fori_loop(0, nh, prep_first, 0)
    x_copy(2).start()
    x_copy(3).start()
    mem_copy = pltpu.make_async_copy(mem0_hbm, mem0, sem_x.at[nb1])
    mem_copy.start()

    def w3_copies(lo, hi):
        return [w_copy(3, n) for n in range(4 * lo, 4 * hi)]

    def w4_copies(n):
        return [w_copy(4, 2 * j + n) for j in range(4)]

    later = [
        lambda: [x_copy(4)] + [w_copy(2, n) for n in range(nh)],
        lambda: [x_copy(5)] + [w_copy(2, n) for n in range(nh, nd)],
        lambda: [x_copy(6)] + w3_copies(0, 1),
        lambda: [x_copy(7)] + w3_copies(1, 2),
        lambda: w3_copies(2, 3),
        lambda: w3_copies(3, 4),
        lambda: w3_copies(4, 6),
        lambda: w3_copies(6, 7),
        lambda: [w_copy(4, 0), w_copy(4, 2)],
        lambda: [w_copy(4, 4), w_copy(4, 6)],
        lambda: [w_copy(4, 1), w_copy(4, 3)],
        lambda: [w_copy(4, 5), w_copy(4, 7)],
        lambda: a_copies(0),
        lambda: a_copies(1),
    ]

    def start_later(i, lo, hi):
        for k in range(lo, min(hi, len(later))):
            @pl.when(i == k - lo)
            def _(k=k):
                for c in later[k]():
                    c.start()

    def b1(i, carry):
        @pl.when(i + 1 < nb1)
        def _():
            x_copy(i + 1).wait()

        r0 = pl.multiple_of(i * TM1, TM1)
        nxt = jnp.minimum(i + 1, nb1 - 1)
        fill = _Filler((7 * nh - 3) * SUB, [part(norm_pair, nxt, (i + 1) % 2, r) for r in range(0, h1, RC)])
        due = Deadline(None, 0)

        def prod(n, r, k):
            y = _dot(_halves(get_left(i % 2, k, r)), weights(wb, o_w4 + (n * 7 + k) * wk, wk))
            fill(due.after(y))
            return y

        for n in range(nh):
            for r in range(0, h1, hb):
                for k, y in enumerate(_combine(part(prod, n, r))):
                    hs[n + k % 2 * nh, pl.ds(r0 + PAD + k // 2 * h1 + r, hb), :] = _gelu(y)
        fill.finish()
        start_later(i, 0, nb1)
        return carry

    lax.fori_loop(0, nb1, b1, 0)

    shifts = (-1, 1, -2, 2)

    rq = LANES // 2
    BK = 32
    per = nf * (wq // BK) // (nb1 // 2)

    def prep2(second, u):
        u4 = u % (nf * rq // BK)
        e, p4, r4 = u // (nf * rq // BK), u4 // (rq // BK), u4 % (rq // BK) * BK
        p3, r3 = u // (wq // BK), u % (wq // BK) * BK
        src, down, right, dst, pitch = (jnp.where(second, b, a).astype(jnp.int32) for a, b in zip(
            (raw[3] + 4 * p3 * Dk + r3, wq, Dk, o_w3 + p3 * 49 * wq + r3, wq),
            (raw[4] + e * (F // 2) + p4 * 4 * rq + r4, rq, F, o_w4 + (e * 49 * nf + p4) * rq + r4, nf * rq)))

        def job(r, _):
            w = [[wa[pl.ds(pl.multiple_of(src + k * down + j * right, BK) + r, 8), :] for j in range(4)]
                 for k in range(4)]
            z = yield
            w = [[_unpack(x, z) for x in row] for row in w]
            lo, hi = (_right(*_nest([[x[h] for x in row] for row in w])) for h in range(2))
            for a in range(7):
                for b, (x, y) in enumerate(zip(_right(*lo[a]), _right(*hi[a]))):
                    wb[pl.ds(pl.multiple_of(dst + (7 * a + b) * pitch, BK) + r, 8), :] = _pack(x, y)
        return [part(job, r) for r in range(0, BK, 8)]

    def b2(i, carry):
        def groups(k):
            return (k * per + wq // BK - 1) // (wq // BK)

        for k in range(nb1):
            cps = w3_copies(groups(k), groups(k + 1)) if k < nb1 // 2 else [] if k % 2 else w4_copies(k // 2 - 2)
            if cps:
                @pl.when(i == k)
                def _(cps=cps):
                    for c in cps:
                        c.wait()

        r0 = pl.multiple_of(i * TM1, TM1)
        jobs = [prep2(i >= nb1 // 2, (i.astype(U32) % (nb1 // 2)) * per + u) for u in range(per)]
        fill = _Filler(2 * nd * TM1 // HB - 4, sum(jobs, []))
        due = Deadline(lambda: wb[0:8, :], LAG2)
        for r in range(0, TM1, HB):
            sh = [hs[n, pl.ds(r0 + PAD + r + shifts[n * 4 // nd], HB), :] for n in range(nd)]
            for c in range(nd):
                y = None
                for k in range(0, nd, nh):
                    a = pltpu.bitcast(due(pltpu.bitcast(_cat(sh[k:k + nh], 1), U32)), F32)
                    p = _dot(a, weights(wa, raw[2] + c * Dk + k * rq, nh * rq))
                    y = p if y is None else p + y
                    fill(due.after(y))
                hs[c, pl.ds(r0 + r, HB), :] = y
        fill.finish()
        start_later(i, nb1, 2 * nb1)
        return carry

    for n in range(nd):
        w_copy(2, n).wait()
    lax.fori_loop(0, nb1, b2, 0)

    def norm_mid(i):
        def job(r, z):
            rr = pl.ds(pl.multiple_of(i * TM2 + r, RN), RN)
            _, d, v = _moments(_cat([hs[n, rr, :] for n in range(nd)], 1) + normed(rr), z)
            lt[r:r + RN, :] = d * lax.rsqrt(v + EPS)
            yield
        return [part(job, r) for r in range(0, TM2, RN)]

    def left_mid():
        def job(r, n, z):
            a = [[lt[u * q2 + r:u * q2 + r + RC, cols(2 * j + n)] for j in range(4)] for u in range(4)]
            for k, g in enumerate(_left(*_nest(a))):
                for b, f in enumerate(_left(*g)):
                    ly[7 * k + b, n, r:r + RC, :] = f.astype(BF16)
                yield
        return [part(job, r, n) for r in range(0, q2, RC) for n in range(2)]

    def b3(i, carry):
        for c in a_copies(i):
            c.wait()

        stages = [range(8, 17), range(17, 26), range(0, 4), range(4, 8)]

        def prep_qkv(t, u, z):
            for fs in stages:
                def block(par, k, j):
                    w = stq[i % 2, 4 * t + k, pl.ds((2 * u + par) * hp + 8 * (j // 2), 8), :]
                    return _unpack(w, z)[j % 2]

                for f in fs:
                    y = [_signed_sum([(c, block(par, *key)) for key, c in _HK[f][1].items()])[1] for par in range(2)]
                    base = o_qkv + (t * ng * nk + f) * slab + u + i * (fpi // 2)
                    wa[pl.ds(base, 8, stride=nk * slab), :] = _pack(*y)
                z = yield

        def prep_o(e, r, z):
            for fs in stages:
                for f in fs:
                    w = [(c, sto[i % 2, k, 2 * j + e, r:r + 8, :]) for (k, j), c in _HK[f][1].items()]
                    rr = pl.ds(pl.multiple_of(o_wo + (e * nk + f) * ng * (Dh // 2) + i * opi, opi) + r, 8)
                    wa[rr, :] = w[0][1] if len(w) == 1 else _pack(
                        *[_signed_sum([(c, _unpack(x, z)[h]) for c, x in w])[1] for h in range(2)])
                z = yield

        jobs = [part(prep_qkv, t, u) for t in range(3) for u in range(fpi // 2)]
        jobs += [part(prep_o, e, r) for e in range(2) for r in range(0, opi, 8)]
        r0 = pl.multiple_of(i * TM2, TM2)
        here = pl.ds(pl.multiple_of(zero[0], 8), 8)
        SLOTS = [k for k in range(49) if k // 7 in (1, 0)]
        YS = SLOTS[::4]
        fill = _Filler(nf * len(YS) + 2 * 49 - 8, jobs)
        due = Deadline(lambda: wa[0:8, :], 5)
        fill_y = _Filler((nf - 1) * len(SLOTS), norm_mid(jnp.minimum(i + 1, nb2 - 1)))
        due_y = Deadline(lambda: pltpu.bitcast(lt[here, 0:LANES], U32), 14)
        fill_z = _Filler(2 * 49 - 24, left_mid())
        due_z = Deadline(lambda: ly.bitcast(U32)[zero[0], 0, 0:8, :], 6)

        def up(p, k):
            w = ly.bitcast(U32)
            w = _cat([w[k, n] for n in range(2)], 1)
            slot = k in SLOTS
            if k in YS:
                w = due(w)
            y = _dot(_halves(due_y(w) if slot else w), weights(wb, o_w3 + (p * 49 + k) * wq, wq))
            if slot:
                z = due.after(y)
                fill_y(z)
                if k in YS:
                    fill(z)
            return y

        for p in range(nf):
            g = [[_gelu(y) for y in row] for row in _combine2(part(up, p), _combine)]
            for a, blocks in enumerate(_left(*_nest(g))):
                for b, f in enumerate(_left(*blocks)):
                    lz[7 * a + b, p] = f.astype(BF16)
        fill_y.finish()

        def down(e, k):
            w = lz.bitcast(U32)
            y = _dot(_halves(due_z(due(_cat([w[k, p] for p in range(nf)], 1)))),
                     weights(wb, o_w4 + (e * 49 + k) * nf * rq, nf * rq))
            z = due.after(y)
            fill(z)
            fill_z(z)
            return y

        for e in range(2):
            for u, row in enumerate(_combine2(part(down, e), _combine_late)):
                for j, y in enumerate(row):
                    rr = pl.ds(r0 + u * q2, q2)
                    c = 2 * j + e
                    hs[c, rr, :] += (xbuf[rr, cols(c)].astype(F32) + normed(rr, c, c + 1)) + y

        fill_z.finish()
        fill.finish()

        @pl.when(i + 2 < nb2)
        def _():
            for c in a_copies(i + 2):
                c.start()

        return carry

    _run(norm_mid(0), 1)
    _run(left_mid(), 1)
    lax.fori_loop(0, nb2, b3, 0)

    scale = Dh ** -0.5
    row = lax.broadcasted_iota(jnp.int32, (L, L), 0)
    col = lax.broadcasted_iota(jnp.int32, (L, L), 1)
    mask = (col < M) | (col >= row)
    QS = 4 * seg
    R = seg - M
    rv = R // 8

    def upper(n):
        return lax.broadcasted_iota(jnp.int32, (8, n), 0) < 4

    def split8(mem, tok):
        u = upper(mem.shape[1])
        return jnp.where(u, mem, tok), pltpu.roll(jnp.where(u, tok, mem), 4, 0)

    def join8(t, b):
        u = upper(t.shape[1])
        b = pltpu.roll(b, 4, 0)
        return jnp.where(u, t, b), jnp.where(u, b, t)

    def out_copy(j):
        r0 = pl.multiple_of(j * QS, QS)
        return pltpu.make_async_copy(xbuf.at[pl.ds(r0, QS)], out_hbm.at[pl.ds(r0, QS)], sem_out.at[j])

    def vregs(y, lo, hi):
        return [y[8 * k:8 * k + 8] for k in range(lo, hi)]

    def quad(j, carry):
        xs = normed(pl.ds(pl.multiple_of(j * QS, QS), QS))
        qkv = {(t, h): [] for t in range(3) for h in range(H)}
        att = {h: [] for h in range(H)}
        outs = {n: [] for n in range(nd)}
        mem = membuf[...]
        for st in range(4):
            def left_operands(mem, tok, big):
                if not big:
                    return _hk_left([_cat([m] + y, 0) for m, y in zip(mem, tok)])
                pairs = [split8(m, y[2 * rv]) for m, y in zip(mem, tok)]
                return _hk_left(*[[_cat([p[c]] + y[c * rv:(c + 1) * rv], 0) for p, y in zip(pairs, tok)]
                                  for c in range(2)])

            def rows_out(c):
                if len(c) == 1:
                    return [(y[0:8], vregs(y, 1, 1 + rv)) for y in c[0]]
                got = []
                for y, w in zip(*c):
                    ym, yt = join8(y[0:8], w[0:8])
                    got.append((ym, vregs(y, 1, 1 + rv) + vregs(w, 1, 1 + rv) + [yt]))
                return got

            r, n_tok = (0, 2 * rv + 1) if st == 0 else ((st + 1) * rv + 1, rv)
            hl = left_operands([mem[:, cols(2 * k, 2)] for k in range(4)],
                               [vregs(xs[:, cols(2 * k, 2)], r, r + n_tok) for k in range(4)], st == 0)
            ol = {}

            def wq_part(t, g, lo, hi):
                return _hk_combine({f: s for f, (s, _) in hl.items()}, lambda f: _dot(
                    hl[f][1][:, lo:hi],
                    weights(wa, o_qkv + ((t * ng + g) * nk + f) * slab + lo // 2, (hi - lo) // 2)))

            def wo_part(e, lo, hi):
                return _hk_combine({f: s for f, (s, _) in ol[lo].items()}, lambda f: _dot(
                    _cat([ol[g][f][1] for g in range(lo, hi)], 1),
                    weights(wa, o_wo + ((e * nk + f) * ng + lo) * (Dh // 2), (hi - lo) * (Dh // 2))))

            def stash(q, c):
                for a, blocks in enumerate(c):
                    for b, y in enumerate(blocks):
                        pbuf[st, q, a, b] = y

            def resume(q, c):
                return [[pbuf[st, q, a, b] + y for b, y in enumerate(blocks)] for a, blocks in enumerate(c)]

            def proj(t, g):
                if g == 0 and st > 0 and t < 2:
                    c = resume(2 + t, wq_part(t, g, LANES, 2 * LANES))
                else:
                    c = wq_part(t, g, 0, 2 * LANES)
                got = []
                for h, (ym, yt) in zip(heads(g), rows_out(c)):
                    qkv[t, h] += yt
                    got.append(_cat([ym] + qkv[t, h][4 * st:4 * st + 4], 0))
                return got

            def probs(q, k):
                sc = jnp.where(mask, _dot_nt(k, q.astype(BF16)), -1e9 / scale)
                p = jnp.exp2((sc - jnp.max(sc, axis=0, keepdims=True)) * (scale * math.log2(math.e)))
                return p * _recip(jnp.sum(p, axis=0, keepdims=True))

            cur, p, o = {}, {}, {}

            def attend(g, c):
                for e in (2 * c, 2 * c + 1):
                    if 0 <= g < ng:
                        p[g, e] = probs(cur[0, g][e], cur[1, g][e])
                if g > 0:
                    for e in (2 * c, 2 * c + 1):
                        o[e] = _dot(p[g - 1, e].T, cur[2, g - 1][e].astype(BF16))
                        att[heads(g - 1)[e]] += vregs(o[e], 1, 5)
                    if c:
                        ol[g - 1] = left_operands(
                            [o[e][0:8] for e in range(4)],
                            [att[h][st * rv:None if st == 3 else (st + 1) * rv] for h in heads(g - 1)], st == 3)

            if st > 0:
                for t in range(2):
                    stash(2 + t, wq_part(t, 0, 0, LANES))
            for g in range(ng):
                cur[0, g] = proj(0, g)
                cur[1, g] = proj(1, g)
                attend(g - 1, 1)
                cur[2, g] = proj(2, g)
                attend(g, 0)
            stash(0, wo_part(0, 0, 2))
            attend(ng - 1, 1)
            stash(1, wo_part(1, 0, 2))
            attend(ng, 0)
            stash(0, resume(0, wo_part(0, 2, 4)))
            attend(ng, 1)
            stash(1, resume(1, wo_part(1, 2, 4)))
            new = {}
            for e in range(2):
                for c, (ym, yt) in enumerate(rows_out(resume(e, wo_part(e, ng // 2, ng)))):
                    new[2 * c + e] = ym
                    outs[2 * c + e] += yt
            mem = jnp.concatenate([new[n] for n in range(nd)], axis=1)
            lo, hi = ((0, 2), (2, 6), (6, 8), (8, 16))[st]
            rr = pl.ds(pl.multiple_of(j * QS + 8 * lo, 16), 8 * (hi - lo))
            for n in range(nd):
                xbuf[rr, cols(n)] = (hs[n, rr, :] + jnp.concatenate(outs[n][lo:hi], axis=0)).astype(BF16)
        membuf[...] = mem
        out_copy(j).start()
        return carry

    mem_copy.wait()
    membuf[...] = mem0[...].astype(F32)
    lax.fori_loop(0, S // QS, quad, 0)
    for j in range(S // QS):
        out_copy(j).wait()


@functools.partial(jax.jit, static_argnames=("A_seg_len",))
def pallas_parallel_sum__memory_aug_recurrent_mem_tr__mixer_s_mlp__prompt_kernel(
    A_x: jax.Array,
    A_mem0: jax.Array,
    A_Wq: jax.Array,
    A_Wk: jax.Array,
    A_Wv: jax.Array,
    A_Wo: jax.Array,
    A_seg_len: int,
    B_x: jax.Array,
    B_w1: jax.Array,
    B_w2: jax.Array,
    B_w3: jax.Array,
    B_w4: jax.Array,
):
    del B_x
    _, S, D = A_x.shape
    _, H, Dh = A_Wq.shape
    M = A_mem0.shape[1]
    seg = int(A_seg_len)
    F = B_w3.shape[1]
    assert (M, seg, Dh) == (8, 32, LANES)
    TM1, TM2 = 256, 128
    nd = D // LANES
    nb2 = S // TM2

    kern = functools.partial(_kernel, S=S, D=D, H=H, Dh=Dh, M=M, seg=seg, F=F, TM1=TM1, TM2=TM2)
    hbm = pl.BlockSpec(memory_space=pl.ANY)
    dma = pltpu.SemaphoreType.DMA
    out = pl.pallas_call(
        kern,
        out_shape=jax.ShapeDtypeStruct((S, D), BF16),
        in_specs=[hbm] * 10,
        out_specs=hbm,
        scratch_shapes=[
            pltpu.VMEM((S, D), BF16),
            pltpu.VMEM((2, S, LANES), F32),
            pltpu.VMEM((nd, S + 2 * PAD, LANES), F32),
            pltpu.VMEM((2, 7, nd // 2, TM1 // 2, LANES), BF16),
            pltpu.VMEM((TM2, D), F32),
            pltpu.VMEM((49, nd // 4, TM2 // 4, LANES), BF16),
            pltpu.VMEM((49, F // (4 * LANES), TM2 // 4, LANES), BF16),
            pltpu.VMEM(((H // 4) * len(_HK) * (Dh + 3 * (D // 8 + 2)), LANES), U32),
            pltpu.VMEM((2 * 49 * (D // 8) * (F // (4 * LANES)), LANES), U32),
            pltpu.SMEM((1,), jnp.int32),
            pltpu.VMEM((2, 12, (D // 4 // nb2) * H // 2, LANES), U32),
            pltpu.VMEM((2, 4, nd, H * Dh // (8 * nb2), LANES), U32),
            pltpu.VMEM((M, D), BF16),
            pltpu.VMEM((M, D), F32),
            pltpu.VMEM((4, 4, 2, 4, seg, LANES), F32),
            dma((S // TM1 + 1,)), dma((3 * nd + F // LANES,)), dma((2,)), dma((S // (4 * seg),)),
        ],
        compiler_params=pltpu.CompilerParams(vmem_limit_bytes=128 * 1024 * 1024, disable_bounds_checks=True, disable_semaphore_checks=True),
        name="rmt_s2mlp",
    )(A_x.reshape(S, D), A_mem0.reshape(M, D),
      A_Wq.reshape(D * H, Dh), A_Wk.reshape(D * H, Dh), A_Wv.reshape(D * H, Dh),
      A_Wo.reshape(H * Dh, D), B_w1, B_w2, B_w3, B_w4)
    return out.reshape(1, S, D)
```

```python
import functools
import math

import jax
import jax.numpy as jnp
from jax import lax
import jax.experimental.pallas as pl
import jax.experimental.pallas.tpu as pltpu

F32 = jnp.float32
BF16 = jnp.bfloat16
U32 = jnp.uint32
LANES = 128
EPS = 1e-5
PAD = 8


def _dot(a, b):
    return lax.dot_general(a, b, (((1,), (0,)), ((), ())), preferred_element_type=F32)


def _dot_nt(a, b):
    return lax.dot_general(a, b, (((1,), (1,)), ((), ())), preferred_element_type=F32)


def _moments(x, z):
    s = _cat([pltpu.bitcast(z, F32)] * (x.shape[0] // 8), 0)
    for c in range(0, x.shape[1], LANES):
        s = s + x[:, c:c + LANES]
    m = jnp.sum(s, axis=-1, keepdims=True) * (1.0 / x.shape[1])
    d = x - m
    return m, d, jnp.mean(d * d, axis=-1, keepdims=True)


def _recip(x):
    r = pl.reciprocal(x, approx=True)
    return r * (2.0 - x * r)


def _gelu_of_twice(h):
    c = math.sqrt(2.0 / math.pi)
    return h + h * jnp.tanh(h * (2.0 * c + (8.0 * c * 0.044715) * (h * h)))


def _words(x):
    return pltpu.bitcast(x.astype(BF16), U32)


def _halves(w):
    return pltpu.bitcast(w, BF16)


def _cat(xs, axis):
    return xs[0] if len(xs) == 1 else jnp.concatenate(xs, axis=axis)


def _right(b11, b12, b21, b22):
    return (b11 + b22, b11, b12 - b22, b21 - b11, b22, b11 + b12, b21 + b22)


def _unpack(w, z):
    return pltpu.bitcast(w << (z | 16), F32), pltpu.bitcast(w & (z | U32(0xFFFF0000)), F32)


def _pack(lo, hi):
    return pltpu.bitcast(pltpu.pack_elementwise([lo, hi], packed_dtype=BF16), U32)


def _right_words(w, z):
    lo, hi = zip(*[_unpack(x, z) for x in w])
    f = [_pack(a, b) for a, b in zip(_right(*lo), _right(*hi))]
    f[1], f[4] = w[0], w[3]
    return f


def _left(a11, a12, a21, a22):
    return (a11 + a22, a21 + a22, a11, a22, a11 + a12, a21 - a11, a12 - a22)


def _combine(m):
    m4 = m(3)
    m2 = m(1)
    c21 = m2 + m4
    m1 = m(0)
    c22 = m1 - m2
    c11 = m1 + m4
    c11 = c11 + m(6)
    m5 = m(4)
    c11 = c11 - m5
    m3 = m(2)
    c12 = m3 + m5
    c22 = c22 + m3
    c22 = c22 + m(5)
    return c11, c12, c21, c22


class _Blocks(tuple):
    def __add__(self, other):
        return _Blocks(a + b for a, b in zip(self, other))

    def __sub__(self, other):
        return _Blocks(a - b for a, b in zip(self, other))


def _nest(a):
    return [_Blocks(a[2 * i + u][2 * j + w] for u in range(2) for w in range(2)) for i in range(2) for j in range(2)]


def _combine2(m, outer):
    c = outer(lambda a: _Blocks(_combine(lambda b: m(7 * a + b))))
    return [[c[2 * (i // 2) + j // 2][2 * (i % 2) + j % 2] for j in range(4)] for i in range(4)]


def _combine_late(m):
    m3 = m(2)
    m5 = m(4)
    c12 = m3 + m5
    c22 = m3 + m(5)
    m1 = m(0)
    c11 = m1 - m5
    c22 = c22 + m1
    m2 = m(1)
    c22 = c22 - m2
    m4 = m(3)
    c21 = m2 + m4
    c11 = c11 + m4
    c11 = c11 + m(6)
    return c11, c12, c21, c22


def _hopcroft_kerr(types):
    n = len(types)
    prods = []

    def add(left, out):
        prods.append((left, {}, out))
        return len(prods) - 1

    def use(weight, terms):
        for f, s in terms:
            for k, c in weight.items():
                prods[f][1][k] = prods[f][1].get(k, 0) + s * c

    class Node:
        def __init__(self, t, xs, ys, plus, minus):
            self.t, self.xs, self.ys, self.plus, self.minus = t, xs, ys, plus, minus

    def mix(*parts):
        return {(i, t % 3): s * c for d, t, s in parts for i, c in d.items()}

    def pair(u, w):
        if (u.t - w.t) % 3 != 1:
            zwu, zuw, free = pair(w, u)
            return zuw, zwu, free
        t = u.t
        s = add(mix((u.xs, t + 2, 1), (w.xs, t, 1)), mix((u.ys, t + 2, 1), (w.ys, t, -1)))
        o1 = add(mix((u.xs, t, -1), (w.xs, t, 1)), mix((u.ys, t + 2, 1), (w.ys, t + 2, 1)))
        o2 = add(mix((u.xs, t + 2, -1), (w.xs, t + 2, 1)), mix((u.ys, t, 1), (w.ys, t, 1)))
        free = Node((t + 1) % 3, {**{i: -c for i, c in u.xs.items()}, **w.xs}, {**u.ys, **w.ys}, o1, o2)
        return ([(s, 1), (o1, -1), (u.minus, 1), (w.minus, -1)],
                [(s, 1), (o2, -1), (u.plus, 1), (w.plus, -1)], free)

    nodes = []
    for i, t in enumerate(types):
        e = {i: 1}
        nodes.append(Node(t, e, e, add(mix((e, t + 2, 1)), mix((e, t + 1, 1))),
                          add(mix((e, t + 1, 1)), mix((e, t + 2, 1)))))
        use({(i, i): 1}, [(nodes[i].plus, 1), (nodes[i].minus, -1)])
    z, free = {}, {}
    for i in range(n):
        for j in range(i + 1, n):
            if types[i] != types[j]:
                z[i, j], z[j, i], free[i, j] = pair(nodes[i], nodes[j])
                free[j, i] = free[i, j]
    for i in range(n):
        for j in range(i + 1, n):
            if types[i] == types[j]:
                k = next(k for k in range(n) if types[k] != types[i])
                w = free[i, k]
                zwj, zjw, _ = pair(w, nodes[j])
                s = w.xs[i]
                z[i, j] = [(f, s * c) for f, c in zwj] + z[k, j]
                z[j, i] = zjw + [(f, -c) for f, c in z[j, k]]
    for key, terms in z.items():
        use({key: 1}, terms)
    return [(l, {k: c for k, c in r.items() if c}, o) for l, r, o in prods]


_HK = _hopcroft_kerr((0, 1, 2, 0))
_HK_ROW = [f for f, (l, _, o) in enumerate(_HK) if any(t != 2 for _, t in l) and any(t != 0 for _, t in o)]


def _signed_sum(terms):
    terms = sorted(terms, key=lambda t: -t[0])
    sign, y = terms[0]
    for s, x in terms[1:]:
        y = y + x if s == sign else y - x
    return sign, y


def _signed_value(terms):
    sign, y = _signed_sum(terms)
    return y if sign > 0 else -y


_HK_RIGHT_SIGN = [_signed_sum([(c, 0) for c in r.values()])[0] for _, r, _ in _HK]


def _hk_left(upper, lower=None):
    if lower is None:
        base = [((1, u), (-1, u), None) for u in upper]
    else:
        base = [((1, u), (1, w), (-1, u + w)) for u, w in zip(upper, lower)]
    return {f: _signed_sum([(c * base[i][t][0], base[i][t][1]) for (i, t), c in _HK[f][0].items() if base[i][t]])
            for f in (_HK_ROW if lower is None else range(len(_HK)))}


def _hk_combine(signs, m):
    both = len(signs) == len(_HK)
    acc = {}
    for f, sign in signs.items():
        y = m(f)
        for (j, t), c in _HK[f][2].items():
            c *= sign * _HK_RIGHT_SIGN[f]
            if both:
                acc[j, t] = _signed_sum([acc[j, t], (c, y)]) if (j, t) in acc else (c, y)
            elif t:
                c *= (0, -1, 1)[t]
                acc[j] = _signed_sum([acc[j], (c, y)]) if j in acc else (c, y)
    if not both:
        return [[_signed_value([acc[j]]) for j in range(4)]]
    return [[_signed_value([acc[j, p], (-acc[j, q][0], acc[j, q][1])]) for j in range(4)]
            for p, q in ((2, 1), (0, 2))]


class _Filler:
    def __init__(self, slots, *job_lists):
        self.slots, self.done, self.lists, self.live = slots, 0, job_lists, []

    def __call__(self, z):
        def step(g, v):
            try:
                g.send(v)
                return True
            except StopIteration:
                return False

        new = []
        for jobs in self.lists:
            n = len(jobs)
            new += [job(z) for job in jobs[self.done * n // self.slots:(self.done + 1) * n // self.slots]]
        self.live = [g for g in new if step(g, None)] + [g for g in self.live if step(g, z)]
        self.done += 1

    def finish(self):
        while self.live or self.done < self.slots:
            self(jnp.zeros((8, LANES), U32))


def _run(jobs, group):
    _Filler(len(jobs) // group, jobs).finish()


def _kernel(x_hbm, mem0_hbm, wq_hbm, wk_hbm, wv_hbm, wo_hbm, w1_hbm, w2_hbm, w3_hbm, w4_hbm,
            out_hbm,
            xbuf, stat, hs, lf, lt, ly, lz, wa, wb, zero, stq, sto, mem0, membuf, pbuf,
            sem_x, sem_w, sem_a, sem_out,
            *, S, D, H, Dh, M, seg, F, TM1, TM2):
    L = M + seg
    nd = D // LANES
    nh = nd // 2
    Dk = D // 2
    wk = Dk // 2
    slab = wk // 2 + 2
    wq = wk // 2
    nf = F // (4 * LANES)
    hp = H // 2
    ng = H // 4
    nk = len(_HK)
    nb1 = S // TM1
    nb2 = S // TM2
    h1 = TM1 // 2
    q2 = TM2 // 4
    SUB = 1
    hb = h1 // SUB
    LAG = 2
    NW = 3
    HB = 32
    LAG2 = 6
    GROUPS = ((1, 5), (3, 0), (4, 2), (6,))
    RN = 8
    RC = 16
    part = functools.partial

    def cols(n, w=1):
        return slice(n * LANES, (n + w) * LANES)

    o_w3 = 0
    fp = nf * wq + 8
    o_w4 = o_w3 + 49 * fp
    o_wo = 0
    o_qkv = o_wo + 2 * nk * ng * (Dh // 2)
    raw = {1: o_qkv, 2: o_qkv + nd * Dk, 3: o_qkv + 2 * nd * Dk, 4: o_qkv + 2 * nd * Dk + 4 * nf * Dk}

    raw_src = {1: w1_hbm, 2: w2_hbm, 3: w3_hbm, 4: w4_hbm}
    raw_rows = {1: Dk, 2: Dk, 3: Dk, 4: F // 2}
    raw_sem = {1: lambda n: n % nh, 2: lambda n: nh, 3: lambda n: nh + 1 + n % nf // 2, 4: lambda n: nh + 5 + n % 2}

    def w_copy(j, n):
        return pltpu.make_async_copy(raw_src[j].bitcast(U32).at[:, cols(n)],
                                     wa.at[pl.ds(raw[j] + n * raw_rows[j], raw_rows[j])],
                                     sem_w.at[raw_sem[j](n)])

    def w_wait(sem, rows):
        pltpu.make_async_copy(wa.at[pl.ds(0, rows)], wa.at[pl.ds(0, rows)], sem_w.at[sem]).wait()

    def x_copy(i):
        r0 = pl.multiple_of(i * TM1, TM1)
        return pltpu.make_async_copy(x_hbm.at[pl.ds(r0, TM1)], xbuf.at[pl.ds(r0, TM1)], sem_x.at[i])

    fpi = D // 4 // nb2
    opi = ng * (Dh // 2) // nb2

    def heads(g):
        return [2 * g, 2 * g + 1, hp + 2 * g, hp + 2 * g + 1]

    def a_copies(i):
        cps = []
        for t, src in enumerate((wq_hbm, wk_hbm, wv_hbm)):
            for k in range(4):
                r0 = pl.multiple_of((k * (D // 4) + i * fpi) * hp, fpi * hp)
                cps.append(pltpu.make_async_copy(src.bitcast(U32).at[pl.ds(r0, fpi * hp)],
                                                 stq.at[i % 2, 4 * t + k], sem_a.at[i % 2]))
        per_group = Dh // 2 // opi
        for k, h in enumerate(heads(i // per_group)):
            r0 = pl.multiple_of(h * (Dh // 2) + i % per_group * opi, opi)
            for n in range(nd):
                cps.append(pltpu.make_async_copy(wo_hbm.bitcast(U32).at[pl.ds(r0, opi), cols(n)],
                                                 sto.at[i % 2, k, n], sem_a.at[i % 2]))
        return cps

    def prep(src, offs, rows, out, dst, pitch):
        def job(r, _):
            w = [src[pl.ds(o + r, 8), :] for o in offs]
            z = yield
            for i, f in enumerate(_right_words(w, z)):
                out[pl.ds(dst + i * pitch + r, 8), :] = f
        return [part(job, r) for r in range(0, rows, 8)]

    def prep_sq(u, out, base):
        o = pl.multiple_of(raw[1] + (u + (u // nh) * nh) * Dk, 8)
        return prep(wa, (o, o + nh * Dk, o + wk, o + nh * Dk + wk), wk,
                    out, pl.multiple_of(base + u * 7 * wk, 8), wk)

    first = [pltpu.make_async_copy(x_hbm.at[pl.ds(r, TM1 // 8)], xbuf.at[pl.ds(r, TM1 // 8)], sem_x.at[0])
             for r in range(0, TM1, TM1 // 8)]
    for c in first:
        c.start()
    for n in range(nh // 2):
        w_copy(1, n).start()
        w_copy(1, n + nh).start()

    zpad = jnp.zeros((PAD, LANES), F32)
    for n in range(nd):
        hs[n, 0:PAD, :] = zpad
        hs[n, PAD + S:PAD + S + PAD, :] = zpad
    wa[0:8, :] = jnp.zeros((8, LANES), U32)
    wb[0:8, :] = jnp.zeros((8, LANES), U32)

    def put_left(slot, r, top, bot):
        for k, f in enumerate(_left(top[:, :Dk], top[:, Dk:], bot[:, :Dk], bot[:, Dk:])):
            for n in range(nh):
                lf[slot, k, n, pl.ds(r, RC), :] = f[:, cols(n)].astype(BF16)
            if k in (1, 4):
                yield

    def get_left(slot, k, r):
        w = lf.bitcast(U32)
        return _cat([w[slot, k, n, r // 2:(r + hb) // 2, :] for n in range(nh)], 1)

    def weights(ref, r0, rows):
        return _halves(ref[pl.ds(r0, rows), :])

    zero[0] = 0

    class Deadline:
        def __init__(self, probe, lag):
            self.probe, self.queue = probe, [None] * lag
            self.zero = jnp.full((8, LANES), zero[0], jnp.int32).astype(U32)

        def after(self, y):
            return pltpu.bitcast(y[0:8, 0:LANES], U32) & self.zero

        def __call__(self, w):
            self.queue.append(self.probe() & self.zero)
            z = self.queue.pop(0)
            if z is not None:
                rest = [w[8:, 0:LANES]] if w.shape[0] > 8 else []
                w = _cat([_cat([w[0:8, 0:LANES] | z] + rest, 0), w[:, LANES:]], 1)
            return w

    def norm_pair(i, slot, r, z):
        a = []
        for half in range(2):
            rr = pl.ds(pl.multiple_of(i * TM1 + half * h1 + r, RC), RC)
            m, d, v = _moments(xbuf[rr, :].astype(F32), z)
            q = lax.rsqrt(v + EPS)
            stat[0, rr, :] = jnp.broadcast_to(m, (RC, LANES))
            stat[1, rr, :] = jnp.broadcast_to(q, (RC, LANES))
            a.append(d * (0.5 * q * lax.rsqrt(v * q * q + EPS)))
        for _ in range(NW):
            yield
        yield from put_left(slot, r, *a)

    def normed(rr, lo=0, hi=nd):
        m, q = (_cat([stat[k, rr, :]] * (hi - lo), 1) for k in range(2))
        return (xbuf[rr, lo * LANES:hi * LANES].astype(F32) - m) * q

    for c in first:
        c.wait()
    for n in range(nh // 2, nh):
        w_copy(1, n).start()
        w_copy(1, n + nh).start()

    def norm_first(q, carry):
        _run([part(norm_pair, 0, 0, pl.multiple_of((4 * q + e) * RC, RC)) for e in range(4)], 4)
        return carry

    lax.fori_loop(0, h1 // (4 * RC), norm_first, 0)
    x_copy(1).start()

    def prep_first(n, carry):
        w_wait(n, 2 * Dk)
        _run(prep_sq(n, wb, o_w4), 2)
        return carry

    lax.fori_loop(0, nh, prep_first, 0)
    x_copy(2).start()
    x_copy(3).start()
    mem_copy = pltpu.make_async_copy(mem0_hbm, mem0, sem_x.at[nb1])
    mem_copy.start()

    def w3_copies(lo, hi):
        return [w_copy(3, p + j * nf) for p in range(lo, hi) for j in range(4)]

    later = [
        lambda: [x_copy(4)] + [w_copy(2, n) for n in range(nh)],
        lambda: [x_copy(5)] + [w_copy(2, n) for n in range(nh, nd)],
        lambda: [x_copy(6)] + w3_copies(0, 1),
        lambda: [x_copy(7)] + w3_copies(1, 2),
        lambda: w3_copies(2, 3),
        lambda: w3_copies(3, 4),
        lambda: w3_copies(4, 6),
        lambda: w3_copies(6, 7),
        lambda: [w_copy(4, 0), w_copy(4, 2)],
        lambda: [w_copy(4, 4), w_copy(4, 6)],
        lambda: [w_copy(4, 1), w_copy(4, 3)],
        lambda: [w_copy(4, 5), w_copy(4, 7)],
        lambda: a_copies(0),
        lambda: a_copies(1),
    ]

    def start_later(i, lo, hi):
        for k in range(lo, min(hi, len(later))):
            @pl.when(i == k - lo)
            def _(k=k):
                for c in later[k]():
                    c.start()

    def b1(i, carry):
        @pl.when(i + 1 < nb1)
        def _():
            x_copy(i + 1).wait()

        r0 = pl.multiple_of(i * TM1, TM1)
        nxt = jnp.minimum(i + 1, nb1 - 1)
        fill = _Filler((7 * nh - 3) * SUB, [part(norm_pair, nxt, (i + 1) % 2, r) for r in range(0, h1, RC)])
        due = Deadline(None, 0)

        def prod(n, r, k):
            y = _dot(_halves(get_left(i % 2, k, r)), weights(wb, o_w4 + (n * 7 + k) * wk, wk))
            fill(due.after(y))
            return y

        for n in range(nh):
            for r in range(0, h1, hb):
                for k, y in enumerate(_combine(part(prod, n, r))):
                    hs[n + k % 2 * nh, pl.ds(r0 + PAD + k // 2 * h1 + r, hb), :] = _gelu_of_twice(y)
        fill.finish()
        start_later(i, 0, nb1)
        return carry

    lax.fori_loop(0, nb1, b1, 0)

    shifts = (-1, 1, -2, 2)

    rq = LANES // 2
    BK = 32
    per = nf * (wq // BK) // (nb1 // 2)

    def prep2(second, u):
        src = jnp.where(second, raw[4] + u // (nf * rq // BK) * (F // 2) + u % (nf * rq // BK) * BK,
                        raw[3] + u // (wq // BK) * Dk + u % (wq // BK) * BK).astype(jnp.int32)
        src = [pl.multiple_of(src + k * jnp.where(second, nf * rq, wq), BK) for k in range(4)]
        dst = pl.multiple_of(jnp.where(second, o_w4, o_w3) + u.astype(jnp.int32) * BK, 8)

        def job(r, z):
            def quarter(u, v):
                x = [_unpack(wa[pl.ds(src[2 * u + k] + ((2 * v + j) * F + r), 8), :], z)
                     for k in range(2) for j in range(2)]
                return [_Blocks(y[h] for y in x) for h in range(2)]

            for group in GROUPS:
                lo, hi = (_right(*y) for y in zip(*[quarter(u, v) for u in range(2) for v in range(2)]))
                for a in group:
                    for b, (x, y) in enumerate(zip(_right(*lo[a]), _right(*hi[a]))):
                        wb[pl.ds(dst + ((7 * a + b) * fp + r), 8), :] = _pack(x, y)
                z = yield
        return [part(job, r) for r in range(0, BK, 8)]

    def b2(i, carry):
        for k, sem, rows in ((0, 1, 8 * Dk), (1, 2, 8 * Dk), (2, 3, 8 * Dk), (3, 4, 4 * Dk),
                             (4, 5, 2 * F), (6, 6, 2 * F)):
            pl.when(i == k)(part(w_wait, nh + sem, rows))

        r0 = pl.multiple_of(i * TM1, TM1)
        jobs = [prep2(i >= nb1 // 2, (i.astype(U32) % (nb1 // 2)) * per + u) for u in range(per)]
        fill = _Filler(2 * nd * TM1 // HB - 6, sum(jobs, []))
        due = Deadline(lambda: wb[0:8, :], LAG2)
        def shifted(r):
            return [hs[n, pl.ds(r0 + PAD + r + shifts[n * 4 // nd], HB), :] for n in range(nd)]

        ahead = shifted(0)
        for r in range(0, TM1, HB):
            sh = ahead
            for c in range(nd):
                if c == nd - 2 and r + HB < TM1:
                    ahead = shifted(r + HB)
                y = None
                for k in range(0, nd, nh):
                    a = pltpu.bitcast(due(pltpu.bitcast(_cat(sh[k:k + nh], 1), U32)), F32)
                    p = _dot(a.astype(BF16), weights(wa, raw[2] + c * Dk + k * rq, nh * rq))
                    y = p if y is None else p + y
                    fill(due.after(y))
                hs[c, pl.ds(r0 + r, HB), :] = y
        fill.finish()
        start_later(i, nb1, 2 * nb1)
        return carry

    w_wait(nh, nd * Dk)
    lax.fori_loop(0, nb1, b2, 0)

    def norm_mid(i):
        def job(r, z):
            rr = pl.ds(pl.multiple_of(jnp.minimum(i, nb2 - 1) * TM2 + r, RN), RN)
            x1 = _cat([hs[n, rr, :] for n in range(nd)], 1) + normed(rr)
            _, d, v = _moments(x1, z)
            lt[r:r + RN, :] = d * (0.5 * lax.rsqrt(v + EPS))
            x1 = x1 + xbuf[rr, :].astype(F32)
            for n in range(nd):
                hs[n, pl.ds(pl.multiple_of(i * TM2 + r, RN), RN), :] = x1[:, cols(n)]
            yield
        return [part(job, r) for r in range(0, TM2, RN)]

    def left_mid():
        def job(r, n, z):
            a = [[lt[u * q2 + r:u * q2 + r + RC, cols(2 * j + n)] for j in range(4)] for u in range(4)]
            for k, g in enumerate(_left(*_nest(a))):
                for b, f in enumerate(_left(*g)):
                    ly[7 * k + b, n, r:r + RC, :] = f.astype(BF16)
                yield
        return [part(job, r, n) for r in range(0, q2, RC) for n in range(2)]

    def b3(i, carry):
        for buf in (stq, sto):
            pltpu.make_async_copy(buf.at[i % 2], buf.at[i % 2], sem_a.at[i % 2]).wait()

        stages = [range(8, 17), range(17, 26), range(0, 4), range(4, 8)]

        def prep_qkv(t, u, z):
            for fs in stages:
                def block(par, k, j):
                    w = stq[i % 2, 4 * t + k, pl.ds((2 * u + par) * hp + 8 * (j // 2), 8), :]
                    return _unpack(w, z)[j % 2]

                for f in fs:
                    y = [_signed_sum([(c, block(par, *key)) for key, c in _HK[f][1].items()])[1] for par in range(2)]
                    base = o_qkv + (t * ng * nk + f) * slab + u + i * (fpi // 2)
                    wa[pl.ds(base, 8, stride=nk * slab), :] = _pack(*y)
                z = yield

        def prep_o(e, r, z):
            for fs in stages:
                for f in fs:
                    w = [(c, sto[i % 2, k, 2 * j + e, r:r + 8, :]) for (k, j), c in _HK[f][1].items()]
                    rr = pl.ds(pl.multiple_of(o_wo + (e * nk + f) * ng * (Dh // 2) + i * opi, opi) + r, 8)
                    wa[rr, :] = w[0][1] if len(w) == 1 else _pack(
                        *[_signed_sum([(c, _unpack(x, z)[h]) for c, x in w])[1] for h in range(2)])
                z = yield

        jobs = [part(prep_qkv, t, u) for t in range(3) for u in range(fpi // 2)]
        jobs += [part(prep_o, e, r) for e in range(2) for r in range(0, opi, 8)]
        r0 = pl.multiple_of(i * TM2, TM2)
        here = pl.ds(pl.multiple_of(zero[0], 8), 8)
        SLOTS = [k for k in range(49) if k // 7 in (1, 0)]
        YS = SLOTS[::4]
        fill = _Filler(nf * len(YS) + 2 * 49 - 8, jobs)
        due = Deadline(lambda: wa[0:8, :], 5)
        fill_y = _Filler((nf - 1) * len(SLOTS), norm_mid(i + 1))
        due_y = Deadline(lambda: pltpu.bitcast(lt[here, 0:LANES], U32), 14)
        fill_z = _Filler(2 * 49 - 24, left_mid())
        due_z = Deadline(lambda: ly.bitcast(U32)[zero[0], 0, 0:8, :], 6)

        def up(p, k):
            w = ly.bitcast(U32)
            w = _cat([w[k, n] for n in range(2)], 1)
            slot = k in SLOTS
            if k in YS:
                w = due(w)
            y = _dot(_halves(due_y(w) if slot else w), weights(wb, o_w3 + k * fp + p * wq, wq))
            if slot:
                z = due.after(y)
                fill_y(z)
                if k in YS:
                    fill(z)
            return y

        for p in range(nf):
            g = [[_gelu_of_twice(y) for y in row] for row in _combine2(part(up, p), _combine)]
            for a, blocks in enumerate(_left(*_nest(g))):
                for b, f in enumerate(_left(*blocks)):
                    lz[7 * a + b, p] = f.astype(BF16)
        fill_y.finish()

        def down(e, k):
            w = lz.bitcast(U32)
            y = _dot(_halves(due_z(due(_cat([w[k, p] for p in range(nf)], 1)))),
                     weights(wb, o_w4 + k * fp + e * nf * rq, nf * rq))
            z = due.after(y)
            fill(z)
            fill_z(z)
            return y

        for e in range(2):
            for u, row in enumerate(_combine2(part(down, e), _combine_late)):
                for j, y in enumerate(row):
                    rr = pl.ds(r0 + u * q2, q2)
                    c = 2 * j + e
                    hs[c, rr, :] += y

        fill_z.finish()
        fill.finish()

        @pl.when(i + 2 < nb2)
        def _():
            for c in a_copies(i + 2):
                c.start()

        return carry

    _run(norm_mid(0), 1)
    _run(left_mid(), 1)
    lax.fori_loop(0, nb2, b3, 0)

    scale = Dh ** -0.5
    row = lax.broadcasted_iota(jnp.int32, (seg, L), 0) + M
    col = lax.broadcasted_iota(jnp.int32, (seg, L), 1)
    mask = (col < M) | (col >= row)
    QS = 4 * seg
    R = seg - M
    rv = R // 8

    def upper(n):
        return lax.broadcasted_iota(jnp.int32, (8, n), 0) < 4

    def split8(mem, tok):
        u = upper(mem.shape[1])
        return jnp.where(u, mem, tok), pltpu.roll(jnp.where(u, tok, mem), 4, 0)

    def join8(t, b):
        u = upper(t.shape[1])
        b = pltpu.roll(b, 4, 0)
        return jnp.where(u, t, b), jnp.where(u, b, t)

    def out_copy(j):
        r0 = pl.multiple_of(j * QS, QS)
        return pltpu.make_async_copy(xbuf.at[pl.ds(r0, QS)], out_hbm.at[pl.ds(r0, QS)], sem_out.at[j])

    def vregs(y, lo, hi):
        return [y[8 * k:8 * k + 8] for k in range(lo, hi)]

    def quad(j, carry):
        xs = normed(pl.ds(pl.multiple_of(j * QS, QS), QS))
        qkv = {(t, h): [] for t in range(3) for h in range(H)}
        att = {h: [] for h in range(H)}
        outs = {n: [] for n in range(nd)}
        mem = membuf[...]
        for st in range(4):
            def left_operands(mem, tok, big):
                if not big:
                    return _hk_left([_cat([m] + y, 0) for m, y in zip(mem, tok)])
                pairs = [split8(m, y[2 * rv]) for m, y in zip(mem, tok)]
                return _hk_left(*[[_cat([p[c]] + y[c * rv:(c + 1) * rv], 0) for p, y in zip(pairs, tok)]
                                  for c in range(2)])

            def rows_out(c):
                if len(c) == 1:
                    return [(y[0:8], vregs(y, 1, 1 + rv)) for y in c[0]]
                got = []
                for y, w in zip(*c):
                    ym, yt = join8(y[0:8], w[0:8])
                    got.append((ym, vregs(y, 1, 1 + rv) + vregs(w, 1, 1 + rv) + [yt]))
                return got

            r, n_tok = (0, 2 * rv + 1) if st == 0 else ((st + 1) * rv + 1, rv)
            hl = left_operands([mem[:, cols(2 * k, 2)] for k in range(4)],
                               [vregs(xs[:, cols(2 * k, 2)], r, r + n_tok) for k in range(4)], st == 0)
            ol = {}

            def wq_part(t, g, lo, hi):
                return _hk_combine({f: s for f, (s, _) in hl.items()}, lambda f: _dot(
                    hl[f][1][:, lo:hi].astype(BF16),
                    weights(wa, o_qkv + ((t * ng + g) * nk + f) * slab + lo // 2, (hi - lo) // 2)))

            def wo_part(e, lo, hi):
                return _hk_combine({f: s for f, (s, _) in ol[lo].items()}, lambda f: _dot(
                    _cat([ol[g][f][1] for g in range(lo, hi)], 1).astype(BF16),
                    weights(wa, o_wo + ((e * nk + f) * ng + lo) * (Dh // 2), (hi - lo) * (Dh // 2))))

            def stash(q, c):
                for a, blocks in enumerate(c):
                    for b, y in enumerate(blocks):
                        pbuf[st, q, a, b] = y

            def resume(q, c):
                return [[pbuf[st, q, a, b] + y for b, y in enumerate(blocks)] for a, blocks in enumerate(c)]

            def proj(t, g):
                if g == 0 and st > 0 and t < 2:
                    c = resume(2 + t, wq_part(t, g, LANES, 2 * LANES))
                else:
                    c = wq_part(t, g, 0, 2 * LANES)
                got = []
                for h, (ym, yt) in zip(heads(g), rows_out(c)):
                    qkv[t, h] += yt
                    got.append(_cat([ym] + qkv[t, h][4 * st:4 * st + 4], 0))
                return got

            def probs(q, k):
                sc = _dot_nt(k, q.astype(BF16))
                sc = _cat([sc[0:M], jnp.where(mask, sc[M:L], -1e9 / scale)], 0)
                p = jnp.exp2((sc - jnp.max(sc, axis=0, keepdims=True)) * (scale * math.log2(math.e)))
                return p * _recip(jnp.sum(p, axis=0, keepdims=True))

            cur, p, o = {}, {}, {}

            def attend(g, c):
                for e in (2 * c, 2 * c + 1):
                    if 0 <= g < ng:
                        p[g, e] = probs(cur[0, g][e], cur[1, g][e])
                if g > 0:
                    for e in (2 * c, 2 * c + 1):
                        o[e] = _dot(p[g - 1, e].T, cur[2, g - 1][e].astype(BF16))
                        att[heads(g - 1)[e]] += vregs(o[e], 1, 5)
                    if c:
                        ol[g - 1] = left_operands(
                            [o[e][0:8] for e in range(4)],
                            [att[h][st * rv:None if st == 3 else (st + 1) * rv] for h in heads(g - 1)], st == 3)

            if st > 0:
                for t in range(2):
                    stash(2 + t, wq_part(t, 0, 0, LANES))
            for g in range(ng):
                cur[0, g] = proj(0, g)
                cur[1, g] = proj(1, g)
                attend(g - 1, 1)
                cur[2, g] = proj(2, g)
                attend(g, 0)
            stash(0, wo_part(0, 0, 2))
            attend(ng - 1, 1)
            stash(1, wo_part(1, 0, 2))
            attend(ng, 0)
            stash(0, resume(0, wo_part(0, 2, 4)))
            attend(ng, 1)
            stash(1, resume(1, wo_part(1, 2, 4)))
            new = {}
            for e in range(2):
                for c, (ym, yt) in enumerate(rows_out(resume(e, wo_part(e, ng // 2, ng)))):
                    new[2 * c + e] = ym
                    outs[2 * c + e] += yt
            mem = jnp.concatenate([new[n] for n in range(nd)], axis=1)
            lo, hi = ((0, 2), (2, 6), (6, 8), (8, 16))[st]
            rr = pl.ds(pl.multiple_of(j * QS + 8 * lo, 16), 8 * (hi - lo))
            for n in range(nd):
                xbuf[rr, cols(n)] = (hs[n, rr, :] + jnp.concatenate(outs[n][lo:hi], axis=0)).astype(BF16)
        membuf[...] = mem
        out_copy(j).start()
        return carry

    mem_copy.wait()
    membuf[...] = mem0[...].astype(F32)
    lax.fori_loop(0, S // QS, quad, 0)
    for j in range(S // QS):
        out_copy(j).wait()


@functools.partial(jax.jit, static_argnames=("A_seg_len",))
def pallas_parallel_sum__memory_aug_recurrent_mem_tr__mixer_s_mlp__prompt_kernel(
    A_x: jax.Array,
    A_mem0: jax.Array,
    A_Wq: jax.Array,
    A_Wk: jax.Array,
    A_Wv: jax.Array,
    A_Wo: jax.Array,
    A_seg_len: int,
    B_x: jax.Array,
    B_w1: jax.Array,
    B_w2: jax.Array,
    B_w3: jax.Array,
    B_w4: jax.Array,
):
    del B_x
    _, S, D = A_x.shape
    _, H, Dh = A_Wq.shape
    M = A_mem0.shape[1]
    seg = int(A_seg_len)
    F = B_w3.shape[1]
    assert (M, seg, Dh) == (8, 32, LANES)
    TM1, TM2 = 256, 128
    nd = D // LANES
    nb2 = S // TM2

    kern = functools.partial(_kernel, S=S, D=D, H=H, Dh=Dh, M=M, seg=seg, F=F, TM1=TM1, TM2=TM2)
    hbm = pl.BlockSpec(memory_space=pl.ANY)
    dma = pltpu.SemaphoreType.DMA
    out = pl.pallas_call(
        kern,
        out_shape=jax.ShapeDtypeStruct((S, D), BF16),
        in_specs=[hbm] * 10,
        out_specs=hbm,
        scratch_shapes=[
            pltpu.VMEM((S, D), BF16),
            pltpu.VMEM((2, S, LANES), F32),
            pltpu.VMEM((nd, S + TM2, LANES), F32),
            pltpu.VMEM((2, 7, nd // 2, TM1 // 2, LANES), BF16),
            pltpu.VMEM((TM2, D), F32),
            pltpu.VMEM((49, nd // 4, TM2 // 4, LANES), BF16),
            pltpu.VMEM((49, F // (4 * LANES), TM2 // 4, LANES), BF16),
            pltpu.VMEM(((H // 4) * len(_HK) * (Dh + 3 * (D // 8 + 2)), LANES), U32),
            pltpu.VMEM((2 * 49 * ((D // 8) * (F // (4 * LANES)) + 8), LANES), U32),
            pltpu.SMEM((1,), jnp.int32),
            pltpu.VMEM((2, 12, (D // 4 // nb2) * H // 2, LANES), U32),
            pltpu.VMEM((2, 4, nd, H * Dh // (8 * nb2), LANES), U32),
            pltpu.VMEM((M, D), BF16),
            pltpu.VMEM((M, D), F32),
            pltpu.VMEM((4, 4, 2, 4, seg, LANES), F32),
            dma((S // TM1 + 1,)), dma((nd // 2 + 7,)), dma((2,)), dma((S // (4 * seg),)),
        ],
        compiler_params=pltpu.CompilerParams(vmem_limit_bytes=128 * 1024 * 1024, disable_bounds_checks=True, disable_semaphore_checks=True),
        name="rmt_s2mlp",
    )(A_x.reshape(S, D), A_mem0.reshape(M, D),
      A_Wq.reshape(D * H, Dh), A_Wk.reshape(D * H, Dh), A_Wv.reshape(D * H, Dh),
      A_Wo.reshape(H * Dh, D), B_w1, B_w2, B_w3, B_w4)
    return out.reshape(1, S, D)
```

```python
import functools
import math

import jax
import jax.numpy as jnp
from jax import lax
import jax.experimental.pallas as pl
import jax.experimental.pallas.tpu as pltpu

F32 = jnp.float32
BF16 = jnp.bfloat16
U32 = jnp.uint32
LANES = 128
EPS = 1e-5
PAD = 8


def _dot(a, b):
    return lax.dot_general(a, b, (((1,), (0,)), ((), ())), preferred_element_type=F32)


def _dot_nt(a, b):
    return lax.dot_general(a, b, (((1,), (1,)), ((), ())), preferred_element_type=F32)


def _cat(xs, axis):
    return xs[0] if len(xs) == 1 else jnp.concatenate(xs, axis=axis)


def _moments(x, z):
    s = _cat([pltpu.bitcast(z, F32)] * (x.shape[0] // 8), 0)
    for c in range(0, x.shape[1], LANES):
        s = s + x[:, c:c + LANES]
    m = jnp.sum(s, axis=-1, keepdims=True) * (1.0 / x.shape[1])
    d = x - m
    return m, d, jnp.mean(d * d, axis=-1, keepdims=True)


def _recip(x):
    r = pl.reciprocal(x, approx=True)
    return r * (2.0 - x * r)


def _gelu_of_twice(h):
    c = math.sqrt(2.0 / math.pi)
    return h + h * jnp.tanh(h * (2.0 * c + (8.0 * c * 0.044715) * (h * h)))


def _halves(w):
    return pltpu.bitcast(w, BF16)


def _unpack(w, z):
    return pltpu.bitcast(w << (z | 16), F32), pltpu.bitcast(w & (z | U32(0xFFFF0000)), F32)


def _pack(lo, hi):
    return pltpu.bitcast(pltpu.pack_elementwise([lo, hi], packed_dtype=BF16), U32)


def _left(a11, a12, a21, a22):
    return (a11 + a22, a21 + a22, a11, a22, a11 + a12, a21 - a11, a12 - a22)


def _right(b11, b12, b21, b22):
    return (b11 + b22, b11, b12 - b22, b21 - b11, b22, b11 + b12, b21 + b22)


def _combine(m):
    m4 = m(3)
    m2 = m(1)
    c21 = m2 + m4
    m1 = m(0)
    c22 = m1 - m2
    c11 = m1 + m4
    c11 = c11 + m(6)
    m5 = m(4)
    c11 = c11 - m5
    m3 = m(2)
    c12 = m3 + m5
    c22 = c22 + m3
    c22 = c22 + m(5)
    return c11, c12, c21, c22


def _combine_late(m):
    m3 = m(2)
    m5 = m(4)
    c12 = m3 + m5
    c22 = m3 + m(5)
    m1 = m(0)
    c11 = m1 - m5
    c22 = c22 + m1
    m2 = m(1)
    c22 = c22 - m2
    m4 = m(3)
    c21 = m2 + m4
    c11 = c11 + m4
    c11 = c11 + m(6)
    return c11, c12, c21, c22


class _Blocks(tuple):
    def __add__(self, other):
        return _Blocks(a + b for a, b in zip(self, other))

    def __sub__(self, other):
        return _Blocks(a - b for a, b in zip(self, other))


def _left2(a):
    nested = [_Blocks(a[2 * i + u][2 * j + w] for u in range(2) for w in range(2))
              for i in range(2) for j in range(2)]
    return (_left(*g) for g in _left(*nested))


def _combine2(m, outer):
    c = outer(lambda a: _Blocks(_combine(lambda b: m(7 * a + b))))
    return [[c[2 * (i // 2) + j // 2][2 * (i % 2) + j % 2] for j in range(4)] for i in range(4)]


def _hopcroft_kerr(types):
    n = len(types)
    prods = []

    def add(left, out):
        prods.append((left, {}, out))
        return len(prods) - 1

    def use(block, terms):
        for f, s in terms:
            prods[f][1][block] = prods[f][1].get(block, 0) + s

    class Node:
        def __init__(self, t, xs, ys, plus, minus):
            self.t, self.xs, self.ys, self.plus, self.minus = t, xs, ys, plus, minus

    def mix(*parts):
        return {(i, t % 3): s * c for d, t, s in parts for i, c in d.items()}

    def pair(u, w):
        if (u.t - w.t) % 3 != 1:
            zwu, zuw, free = pair(w, u)
            return zuw, zwu, free
        t = u.t
        s = add(mix((u.xs, t + 2, 1), (w.xs, t, 1)), mix((u.ys, t + 2, 1), (w.ys, t, -1)))
        o1 = add(mix((u.xs, t, -1), (w.xs, t, 1)), mix((u.ys, t + 2, 1), (w.ys, t + 2, 1)))
        o2 = add(mix((u.xs, t + 2, -1), (w.xs, t + 2, 1)), mix((u.ys, t, 1), (w.ys, t, 1)))
        free = Node((t + 1) % 3, {**{i: -c for i, c in u.xs.items()}, **w.xs}, {**u.ys, **w.ys}, o1, o2)
        return ([(s, 1), (o1, -1), (u.minus, 1), (w.minus, -1)],
                [(s, 1), (o2, -1), (u.plus, 1), (w.plus, -1)], free)

    nodes = []
    for i, t in enumerate(types):
        e = {i: 1}
        nodes.append(Node(t, e, e, add(mix((e, t + 2, 1)), mix((e, t + 1, 1))),
                          add(mix((e, t + 1, 1)), mix((e, t + 2, 1)))))
        use((i, i), [(nodes[i].plus, 1), (nodes[i].minus, -1)])
    z, free = {}, {}
    for i in range(n):
        for j in range(i + 1, n):
            if types[i] != types[j]:
                z[i, j], z[j, i], free[i, j] = pair(nodes[i], nodes[j])
                free[j, i] = free[i, j]
    for i in range(n):
        for j in range(i + 1, n):
            if types[i] == types[j]:
                k = next(k for k in range(n) if types[k] != types[i])
                w = free[i, k]
                zwj, zjw, _ = pair(w, nodes[j])
                z[i, j] = [(f, w.xs[i] * c) for f, c in zwj] + z[k, j]
                z[j, i] = zjw + [(f, -c) for f, c in z[j, k]]
    for block, terms in z.items():
        use(block, terms)
    return [(left, {k: c for k, c in right.items() if c}, out) for left, right, out in prods]


def _signed_sum(terms):
    terms = sorted(terms, key=lambda t: -t[0])
    sign, y = terms[0]
    for s, x in terms[1:]:
        y = y + x if s == sign else y - x
    return sign, y


def _signed_value(terms):
    sign, y = _signed_sum(terms)
    return y if sign > 0 else -y


_HK = _hopcroft_kerr((0, 1, 2, 0))
_HK_ROW = [f for f, (left, _, out) in enumerate(_HK)
           if any(t != 2 for _, t in left) and any(t != 0 for _, t in out)]
_HK_RIGHT_SIGN = [_signed_sum([(c, 0) for c in right.values()])[0] for _, right, _ in _HK]


def _hk_left(upper, lower=None):
    if lower is None:
        base = [((1, u), (-1, u), None) for u in upper]
    else:
        base = [((1, u), (1, w), (-1, u + w)) for u, w in zip(upper, lower)]
    return {f: _signed_sum([(c * base[i][t][0], base[i][t][1]) for (i, t), c in _HK[f][0].items() if base[i][t]])
            for f in (_HK_ROW if lower is None else range(len(_HK)))}


def _hk_combine(left, m):
    both = len(left) == len(_HK)
    acc = {}
    for f, (sign, _) in left.items():
        y = m(f)
        for (j, t), c in _HK[f][2].items():
            c *= sign * _HK_RIGHT_SIGN[f]
            if both:
                acc[j, t] = _signed_sum([acc[j, t], (c, y)]) if (j, t) in acc else (c, y)
            elif t:
                c *= (0, -1, 1)[t]
                acc[j] = _signed_sum([acc[j], (c, y)]) if j in acc else (c, y)
    if not both:
        return [[_signed_value([acc[j]]) for j in range(4)]]
    return [[_signed_value([acc[j, p], (-acc[j, q][0], acc[j, q][1])]) for j in range(4)]
            for p, q in ((2, 1), (0, 2))]


class _Filler:
    def __init__(self, slots, jobs):
        self.slots, self.done, self.jobs, self.live = slots, 0, jobs, []

    def __call__(self, z):
        def step(g, v):
            try:
                g.send(v)
                return True
            except StopIteration:
                return False

        n = len(self.jobs)
        new = [job(z) for job in self.jobs[self.done * n // self.slots:(self.done + 1) * n // self.slots]]
        self.live = [g for g in new if step(g, None)] + [g for g in self.live if step(g, z)]
        self.done += 1

    def finish(self):
        while self.live or self.done < self.slots:
            self(jnp.zeros((8, LANES), U32))


def _run(jobs, group):
    _Filler(len(jobs) // group, jobs).finish()


def _kernel(x_hbm, mem0_hbm, wq_hbm, wk_hbm, wv_hbm, wo_hbm, w1_hbm, w2_hbm, w3_hbm, w4_hbm,
            out_hbm,
            xbuf, stat, hs, lf, lt, ly, lz, wa, wb, zero, stq, sto, mem0, membuf, pbuf,
            sem_x, sem_w, sem_a, sem_out,
            *, S, D, H, Dh, M, seg, F, TM1, TM2):
    part = functools.partial
    L = M + seg
    nd = D // LANES
    nh = nd // 2
    Dk = D // 2
    rq = LANES // 2
    wk = Dk // 2
    wq = wk // 2
    nf = F // (4 * LANES)
    hp = H // 2
    ng = H // 4
    nk = len(_HK)
    nb1, nb2 = S // TM1, S // TM2
    h1, q2 = TM1 // 2, TM2 // 4
    RC = 16

    def cols(n, w=1):
        return slice(n * LANES, (n + w) * LANES)

    def heads(g):
        return [2 * g, 2 * g + 1, hp + 2 * g, hp + 2 * g + 1]

    fp = nf * wq + 8
    slab = wq + 2
    o_w3 = 0
    o_w4 = o_w3 + 49 * fp
    o_wo = 0
    o_qkv = o_wo + 2 * nk * ng * rq
    raw = {1: o_qkv, 2: o_qkv + nd * Dk, 3: o_qkv + 2 * nd * Dk, 4: o_qkv + 2 * nd * Dk + 4 * F}

    def weights(ref, r0, rows):
        return _halves(ref[pl.ds(r0, rows), :])

    def w_copy(j, n):
        src, rows, sem = {1: (w1_hbm, Dk, n % nh), 2: (w2_hbm, Dk, nh),
                          3: (w3_hbm, Dk, nh + 1 + n % nf // 2), 4: (w4_hbm, F // 2, nh + 5 + n % 2)}[j]
        return pltpu.make_async_copy(src.bitcast(U32).at[:, cols(n)], wa.at[pl.ds(raw[j] + n * rows, rows)],
                                     sem_w.at[sem])

    def w_wait(sem, *spans):
        for r0, rows in spans:
            pltpu.make_async_copy(wa.at[pl.ds(r0, rows)], wa.at[pl.ds(r0, rows)], sem_w.at[sem]).wait()

    def w3_copies(lo, hi):
        return [w_copy(3, p + j * nf) for p in range(lo, hi) for j in range(4)]

    def x_copy(i):
        r0 = pl.multiple_of(i * TM1, TM1)
        return pltpu.make_async_copy(x_hbm.at[pl.ds(r0, TM1)], xbuf.at[pl.ds(r0, TM1)], sem_x.at[i])

    fpi = D // 4 // nb2
    opi = ng * rq // nb2

    def a_copies(i):
        cps = []
        for t, src in enumerate((wq_hbm, wk_hbm, wv_hbm)):
            for k in range(4):
                r0 = pl.multiple_of((k * (D // 4) + i * fpi) * hp, fpi * hp)
                cps.append(pltpu.make_async_copy(src.bitcast(U32).at[pl.ds(r0, fpi * hp)],
                                                 stq.at[i % 2, 4 * t + k], sem_a.at[i % 2]))
        for k, h in enumerate(heads(i // (rq // opi))):
            r0 = pl.multiple_of(h * rq + i % (rq // opi) * opi, opi)
            for n in range(nd):
                cps.append(pltpu.make_async_copy(wo_hbm.bitcast(U32).at[pl.ds(r0, opi), cols(n)],
                                                 sto.at[i % 2, k, n], sem_a.at[i % 2]))
        return cps

    later = [
        lambda: [x_copy(4)] + [w_copy(2, n) for n in range(nh)],
        lambda: [x_copy(5)] + [w_copy(2, n) for n in range(nh, nd)],
        lambda: [x_copy(6)] + w3_copies(0, 1),
        lambda: [x_copy(7)] + w3_copies(1, 2),
        lambda: w3_copies(2, 3),
        lambda: w3_copies(3, 4),
        lambda: w3_copies(4, 6),
        lambda: w3_copies(6, 7),
        lambda: [w_copy(4, 0), w_copy(4, 2)],
        lambda: [w_copy(4, 4), w_copy(4, 6)],
        lambda: [w_copy(4, 1), w_copy(4, 3)],
        lambda: [w_copy(4, 5), w_copy(4, 7)],
        lambda: a_copies(0),
        lambda: a_copies(1),
    ]

    def start_later(i, lo, hi):
        for k in range(lo, min(hi, len(later))):
            @pl.when(i == k - lo)
            def _(k=k):
                for c in later[k]():
                    c.start()

    first = [pltpu.make_async_copy(x_hbm.at[pl.ds(r, TM1 // 8)], xbuf.at[pl.ds(r, TM1 // 8)], sem_x.at[0])
             for r in range(0, TM1, TM1 // 8)]
    for c in first:
        c.start()
    for n in range(nh // 2):
        w_copy(1, n).start()
        w_copy(1, n + nh).start()

    for n in range(nd):
        hs[n, 0:PAD, :] = jnp.zeros((PAD, LANES), F32)
        hs[n, PAD + S:PAD + S + PAD, :] = jnp.zeros((PAD, LANES), F32)
    wa[0:8, :] = jnp.zeros((8, LANES), U32)
    wb[0:8, :] = jnp.zeros((8, LANES), U32)
    zero[0] = 0

    class Deadline:
        def __init__(self, probe=None, lag=0):
            self.probe, self.queue = probe, [None] * lag
            self.zero = jnp.full((8, LANES), zero[0], jnp.int32).astype(U32)

        def after(self, y):
            return pltpu.bitcast(y[0:8, 0:LANES], U32) & self.zero

        def __call__(self, w):
            self.queue.append(self.probe() & self.zero)
            z = self.queue.pop(0)
            if z is None:
                return w
            return _cat([_cat([w[0:8, 0:LANES] | z, w[8:, 0:LANES]], 0), w[:, LANES:]], 1)

    def norm_in(i, slot, r, z):
        a = []
        for half in range(2):
            rr = pl.ds(pl.multiple_of(i * TM1 + half * h1 + r, RC), RC)
            m, d, v = _moments(xbuf[rr, :].astype(F32), z)
            q = lax.rsqrt(v + EPS)
            stat[0, rr, :] = jnp.broadcast_to(m, (RC, LANES))
            stat[1, rr, :] = jnp.broadcast_to(q, (RC, LANES))
            a.append(d * (0.5 * q * lax.rsqrt(v * q * q + EPS)))
        for _ in range(3):
            yield
        for k, f in enumerate(_left(a[0][:, :Dk], a[0][:, Dk:], a[1][:, :Dk], a[1][:, Dk:])):
            for n in range(nh):
                lf[slot, k, n, pl.ds(r, RC), :] = f[:, cols(n)].astype(BF16)
            if k in (1, 4):
                yield

    def normed(rr):
        m, q = (_cat([stat[k, rr, :]] * nd, 1) for k in range(2))
        return (xbuf[rr, :].astype(F32) - m) * q

    def norm_first(q, carry):
        _run([part(norm_in, 0, 0, pl.multiple_of((4 * q + e) * RC, RC)) for e in range(4)], 4)
        return carry

    def prep1(n, carry):
        o = pl.multiple_of(raw[1] + n * Dk, Dk)
        dst = pl.multiple_of(o_w4 + n * 7 * wk, 8)
        w_wait(n, (o, Dk), (o + nh * Dk, Dk))

        def job(r, _):
            w = [wa[pl.ds(o + (e + r), 8), :] for e in (0, nh * Dk, wk, nh * Dk + wk)]
            z = yield
            lo, hi = (_right(*y) for y in zip(*[_unpack(x, z) for x in w]))
            for k in range(7):
                wb[pl.ds(dst + (k * wk + r), 8), :] = {1: w[0], 4: w[3]}[k] if k in (1, 4) else _pack(lo[k], hi[k])

        _run([part(job, r) for r in range(0, wk, 8)], 2)
        return carry

    def b1(i, carry):
        @pl.when(i + 1 < nb1)
        def _():
            x_copy(i + 1).wait()

        r0 = pl.multiple_of(i * TM1, TM1)
        nxt = jnp.minimum(i + 1, nb1 - 1)
        fill = _Filler(7 * nh - 3, [part(norm_in, nxt, (i + 1) % 2, r) for r in range(0, h1, RC)])
        due = Deadline()

        def prod(n, k):
            w = lf.bitcast(U32)
            y = _dot(_halves(_cat([w[i % 2, k, c] for c in range(nh)], 1)), weights(wb, o_w4 + (n * 7 + k) * wk, wk))
            fill(due.after(y))
            return y

        for n in range(nh):
            for k, y in enumerate(_combine(part(prod, n))):
                hs[n + k % 2 * nh, pl.ds(r0 + PAD + k // 2 * h1, h1), :] = _gelu_of_twice(y)
        fill.finish()
        start_later(i, 0, nb1)
        return carry

    for c in first:
        c.wait()
    for n in range(nh // 2, nh):
        w_copy(1, n).start()
        w_copy(1, n + nh).start()
    lax.fori_loop(0, h1 // (4 * RC), norm_first, 0)
    x_copy(1).start()
    lax.fori_loop(0, nh, prep1, 0)
    x_copy(2).start()
    x_copy(3).start()
    mem_copy = pltpu.make_async_copy(mem0_hbm, mem0, sem_x.at[nb1])
    mem_copy.start()
    lax.fori_loop(0, nb1, b1, 0)

    shifts = (-1, 1, -2, 2)
    BK = 32
    HB = 32
    per = nf * (wq // BK) // (nb1 // 2)

    def prep34(second, u):
        src = jnp.where(second, raw[4] + u // (nf * rq // BK) * (F // 2) + u % (nf * rq // BK) * BK,
                        raw[3] + u // (wq // BK) * Dk + u % (wq // BK) * BK).astype(jnp.int32)
        src = [pl.multiple_of(src + k * jnp.where(second, nf * rq, wq), BK) for k in range(4)]
        dst = pl.multiple_of(jnp.where(second, o_w4, o_w3) + u.astype(jnp.int32) * BK, 8)

        def job(r, z):
            def quarter(a, b):
                x = [_unpack(wa[pl.ds(src[2 * a + k] + ((2 * b + j) * F + r), 8), :], z)
                     for k in range(2) for j in range(2)]
                return [_Blocks(y[h] for y in x) for h in range(2)]

            for stage in ((1, 5), (3, 0), (4, 2), (6,)):
                lo, hi = (_right(*y) for y in zip(*[quarter(a, b) for a in range(2) for b in range(2)]))
                for a in stage:
                    for b, (x, y) in enumerate(zip(_right(*lo[a]), _right(*hi[a]))):
                        wb[pl.ds(dst + ((7 * a + b) * fp + r), 8), :] = _pack(x, y)
                z = yield

        return [part(job, r) for r in range(0, BK, 8)]

    def b2(i, carry):
        for k in range(4):
            pl.when(i == k)(part(w_wait, nh + 1 + k, *[
                (raw[3] + j * F + 2 * k * Dk, min(2, nf - 2 * k) * Dk) for j in range(4)]))
        for e in range(2):
            pl.when(i == 4 + 2 * e)(part(w_wait, nh + 5 + e, *[
                (raw[4] + j * F + e * (F // 2), F // 2) for j in range(4)]))

        r0 = pl.multiple_of(i * TM1, TM1)
        jobs = [prep34(i >= nb1 // 2, (i.astype(U32) % (nb1 // 2)) * per + u) for u in range(per)]
        fill = _Filler(2 * nd * TM1 // HB - 6, sum(jobs, []))
        due = Deadline(lambda: wb[0:8, :], 6)

        def shifted(r):
            return [hs[n, pl.ds(r0 + PAD + r + shifts[n * 4 // nd], HB), :] for n in range(nd)]

        ahead = shifted(0)
        for r in range(0, TM1, HB):
            sh = ahead
            for c in range(nd):
                if c == nd - 2 and r + HB < TM1:
                    ahead = shifted(r + HB)
                y = None
                for k in range(0, nd, nh):
                    a = pltpu.bitcast(due(pltpu.bitcast(_cat(sh[k:k + nh], 1), U32)), F32)
                    p = _dot(a.astype(BF16), weights(wa, raw[2] + c * Dk + k * rq, nh * rq))
                    y = p if y is None else p + y
                    fill(due.after(y))
                hs[c, pl.ds(r0 + r, HB), :] = y
        fill.finish()
        start_later(i, nb1, 2 * nb1)
        return carry

    w_wait(nh, (raw[2], nd * Dk))
    lax.fori_loop(0, nb1, b2, 0)

    def norm_mid(i):
        def job(r, _):
            rr = pl.ds(pl.multiple_of(jnp.minimum(i, nb2 - 1) * TM2 + r, 8), 8)
            x1 = _cat([hs[n, rr, :] for n in range(nd)], 1) + normed(rr)
            y = x1 + xbuf[rr, :].astype(F32)
            z = yield
            for n in range(nd):
                hs[n, pl.ds(pl.multiple_of(i * TM2 + r, 8), 8), :] = y[:, cols(n)]
            _, d, v = _moments(x1, z)
            lt[r:r + 8, :] = d * (0.5 * lax.rsqrt(v + EPS))

        return [part(job, r) for r in range(0, TM2, 8)]

    def left_mid():
        def job(r, n, _):
            a = [[lt[u * q2 + r:u * q2 + r + RC, cols(2 * j + n)] for j in range(4)] for u in range(4)]
            for k, g in enumerate(_left2(a)):
                for b, f in enumerate(g):
                    ly[7 * k + b, n, r:r + RC, :] = f.astype(BF16)
                yield

        return [part(job, r, n) for r in range(0, q2, RC) for n in range(2)]

    def b3(i, carry):
        for buf in (stq, sto):
            pltpu.make_async_copy(buf.at[i % 2], buf.at[i % 2], sem_a.at[i % 2]).wait()

        stages = [range(8, 17), range(17, 26), range(0, 4), range(4, 8)]

        def prep_qkv(t, u, z):
            for stage in stages:
                def block(par, k, j):
                    w = stq[i % 2, 4 * t + k, pl.ds((2 * u + par) * hp + 8 * (j // 2), 8), :]
                    return _unpack(w, z)[j % 2]

                for f in stage:
                    y = [_signed_sum([(c, block(par, *key)) for key, c in _HK[f][1].items()])[1] for par in range(2)]
                    base = o_qkv + (t * ng * nk + f) * slab + u + i * (fpi // 2)
                    wa[pl.ds(base, 8, stride=nk * slab), :] = _pack(*y)
                z = yield

        def prep_o(e, r, z):
            for stage in stages:
                for f in stage:
                    w = [(c, sto[i % 2, k, 2 * j + e, r:r + 8, :]) for (k, j), c in _HK[f][1].items()]
                    rr = pl.ds(pl.multiple_of(o_wo + (e * nk + f) * ng * rq + i * opi, opi) + r, 8)
                    wa[rr, :] = w[0][1] if len(w) == 1 else _pack(
                        *[_signed_sum([(c, _unpack(x, z)[h]) for c, x in w])[1] for h in range(2)])
                z = yield

        jobs = [part(prep_qkv, t, u) for t in range(3) for u in range(fpi // 2)]
        jobs += [part(prep_o, e, r) for e in range(2) for r in range(0, opi, 8)]
        r0 = pl.multiple_of(i * TM2, TM2)
        here = pl.ds(pl.multiple_of(zero[0], 8), 8)
        norm_slots = [k for k in range(49) if k // 7 in (3, 1)]
        prep_slots = norm_slots[::4]
        fill = _Filler(nf * len(prep_slots) + 2 * 49 - 8, jobs)
        due = Deadline(lambda: wa[0:8, :], 5)
        fill_y = _Filler((nf - 1) * len(norm_slots), norm_mid(i + 1))
        due_y = Deadline(lambda: pltpu.bitcast(lt[here, 0:LANES], U32), 14)
        fill_z = _Filler(2 * 49 - 24, left_mid())
        due_z = Deadline(lambda: ly.bitcast(U32)[zero[0], 0, 0:8, :], 6)

        def up(p, k):
            w = ly.bitcast(U32)
            w = _cat([w[k, n] for n in range(2)], 1)
            if k in prep_slots:
                w = due(w)
            y = _dot(_halves(due_y(w) if k in norm_slots else w), weights(wb, o_w3 + k * fp + p * wq, wq))
            if k in norm_slots:
                z = due.after(y)
                fill_y(z)
                if k in prep_slots:
                    fill(z)
            return y

        for p in range(nf):
            g = [[_gelu_of_twice(y) for y in row] for row in _combine2(part(up, p), _combine)]
            for a, group in enumerate(_left2(g)):
                for b, f in enumerate(group):
                    lz[7 * a + b, p] = f.astype(BF16)
        fill_y.finish()

        def down(e, k):
            w = lz.bitcast(U32)
            y = _dot(_halves(due_z(due(_cat([w[k, p] for p in range(nf)], 1)))),
                     weights(wb, o_w4 + k * fp + e * nf * rq, nf * rq))
            z = due.after(y)
            fill(z)
            fill_z(z)
            return y

        for e in range(2):
            for u, row in enumerate(_combine2(part(down, e), _combine_late)):
                for j, y in enumerate(row):
                    hs[2 * j + e, pl.ds(r0 + u * q2, q2), :] += y
        fill_z.finish()
        fill.finish()

        @pl.when(i + 2 < nb2)
        def _():
            for c in a_copies(i + 2):
                c.start()

        return carry

    _run(norm_mid(0), 2)
    _run(left_mid(), 1)
    lax.fori_loop(0, nb2, b3, 0)

    scale = Dh ** -0.5
    key = lax.broadcasted_iota(jnp.int32, (seg, L), 0) + M
    query = lax.broadcasted_iota(jnp.int32, (seg, L), 1)
    mask = (query < M) | (query >= key)
    QS = 4 * seg
    rv = (seg - M) // 8

    def upper(n):
        return lax.broadcasted_iota(jnp.int32, (8, n), 0) < 4

    def split8(mem, tok):
        u = upper(mem.shape[1])
        return jnp.where(u, mem, tok), pltpu.roll(jnp.where(u, tok, mem), 4, 0)

    def join8(t, b):
        u = upper(t.shape[1])
        b = pltpu.roll(b, 4, 0)
        return jnp.where(u, t, b), jnp.where(u, b, t)

    def vregs(y, lo, hi):
        return [y[8 * k:8 * k + 8] for k in range(lo, hi)]

    def left_operands(mem, tok, big):
        if not big:
            return _hk_left([_cat([m] + y, 0) for m, y in zip(mem, tok)])
        pairs = [split8(m, y[2 * rv]) for m, y in zip(mem, tok)]
        return _hk_left(*[[_cat([p[c]] + y[c * rv:(c + 1) * rv], 0) for p, y in zip(pairs, tok)] for c in range(2)])

    def rows_out(c):
        if len(c) == 1:
            return [(y[0:8], vregs(y, 1, 1 + rv)) for y in c[0]]
        got = []
        for y, w in zip(*c):
            ym, yt = join8(y[0:8], w[0:8])
            got.append((ym, vregs(y, 1, 1 + rv) + vregs(w, 1, 1 + rv) + [yt]))
        return got

    def probs(q, k):
        sc = _dot_nt(k, q.astype(BF16))
        sc = _cat([sc[0:M], jnp.where(mask, sc[M:L], -1e9 / scale)], 0)
        p = jnp.exp2((sc - jnp.max(sc, axis=0, keepdims=True)) * (scale * math.log2(math.e)))
        return p * _recip(jnp.sum(p, axis=0, keepdims=True))

    def out_copy(j):
        r0 = pl.multiple_of(j * QS, QS)
        return pltpu.make_async_copy(xbuf.at[pl.ds(r0, QS)], out_hbm.at[pl.ds(r0, QS)], sem_out.at[j])

    def quad(j, carry):
        xs = normed(pl.ds(pl.multiple_of(j * QS, QS), QS))
        qkv = {(t, h): [] for t in range(3) for h in range(H)}
        att = {h: [] for h in range(H)}
        outs = {n: [] for n in range(nd)}
        mem = membuf[...]
        for st in range(4):
            r, n_tok = (0, 2 * rv + 1) if st == 0 else ((st + 1) * rv + 1, rv)
            hl = left_operands([mem[:, cols(2 * k, 2)] for k in range(4)],
                               [vregs(xs[:, cols(2 * k, 2)], r, r + n_tok) for k in range(4)], st == 0)
            ol, cur, p, o = {}, {}, {}, {}

            def wq_part(t, g, lo, hi):
                return _hk_combine(hl, lambda f: _dot(
                    hl[f][1][:, lo:hi].astype(BF16),
                    weights(wa, o_qkv + ((t * ng + g) * nk + f) * slab + lo // 2, (hi - lo) // 2)))

            def wo_part(e, lo, hi):
                return _hk_combine(ol[lo], lambda f: _dot(
                    _cat([ol[g][f][1] for g in range(lo, hi)], 1).astype(BF16),
                    weights(wa, o_wo + ((e * nk + f) * ng + lo) * rq, (hi - lo) * rq)))

            def stash(q, c):
                for a, blocks in enumerate(c):
                    for b, y in enumerate(blocks):
                        pbuf[st, q, a, b] = y

            def resume(q, c):
                return [[pbuf[st, q, a, b] + y for b, y in enumerate(blocks)] for a, blocks in enumerate(c)]

            def proj(t, g):
                if g == 0 and st > 0 and t < 2:
                    c = resume(2 + t, wq_part(t, g, LANES, 2 * LANES))
                else:
                    c = wq_part(t, g, 0, 2 * LANES)
                got = []
                for h, (ym, yt) in zip(heads(g), rows_out(c)):
                    qkv[t, h] += yt
                    got.append(_cat([ym] + qkv[t, h][4 * st:4 * st + 4], 0))
                return got

            def attend(g, c):
                for e in (2 * c, 2 * c + 1):
                    if 0 <= g < ng:
                        p[g, e] = probs(cur[0, g][e], cur[1, g][e])
                if g > 0:
                    for e in (2 * c, 2 * c + 1):
                        o[e] = _dot(p[g - 1, e].T, cur[2, g - 1][e].astype(BF16))
                        att[heads(g - 1)[e]] += vregs(o[e], 1, 5)
                    if c:
                        ol[g - 1] = left_operands(
                            [o[e][0:8] for e in range(4)],
                            [att[h][st * rv:None if st == 3 else (st + 1) * rv] for h in heads(g - 1)], st == 3)

            if st > 0:
                for t in range(2):
                    stash(2 + t, wq_part(t, 0, 0, LANES))
            for g in range(ng):
                cur[0, g] = proj(0, g)
                cur[1, g] = proj(1, g)
                attend(g - 1, 1)
                cur[2, g] = proj(2, g)
                attend(g, 0)
            stash(0, wo_part(0, 0, 2))
            attend(ng - 1, 1)
            stash(1, wo_part(1, 0, 2))
            attend(ng, 0)
            stash(0, resume(0, wo_part(0, 2, 4)))
            attend(ng, 1)
            stash(1, resume(1, wo_part(1, 2, 4)))
            new = {}
            for e in range(2):
                for c, (ym, yt) in enumerate(rows_out(resume(e, wo_part(e, 4, ng)))):
                    new[2 * c + e] = ym
                    outs[2 * c + e] += yt
            mem = _cat([new[n] for n in range(nd)], 1)
            lo, hi = ((0, 2), (2, 6), (6, 8), (8, 16))[st]
            rr = pl.ds(pl.multiple_of(j * QS + 8 * lo, RC), 8 * (hi - lo))
            for n in range(nd):
                xbuf[rr, cols(n)] = (hs[n, rr, :] + _cat(outs[n][lo:hi], 0)).astype(BF16)
        membuf[...] = mem
        out_copy(j).start()
        return carry

    mem_copy.wait()
    membuf[...] = mem0[...].astype(F32)
    lax.fori_loop(0, S // QS, quad, 0)
    for j in range(S // QS):
        out_copy(j).wait()


@functools.partial(jax.jit, static_argnames=("A_seg_len",))
def pallas_parallel_sum__memory_aug_recurrent_mem_tr__mixer_s_mlp__prompt_kernel(
    A_x: jax.Array,
    A_mem0: jax.Array,
    A_Wq: jax.Array,
    A_Wk: jax.Array,
    A_Wv: jax.Array,
    A_Wo: jax.Array,
    A_seg_len: int,
    B_x: jax.Array,
    B_w1: jax.Array,
    B_w2: jax.Array,
    B_w3: jax.Array,
    B_w4: jax.Array,
):
    del B_x
    B, S, D = A_x.shape
    _, H, Dh = A_Wq.shape
    M = A_mem0.shape[1]
    seg = int(A_seg_len)
    F = B_w3.shape[1]
    assert (B, S, D, H, Dh, M, seg, F) == (1, 2048, 1024, 32, LANES, 8, 32, 3584)
    TM1, TM2 = 256, 128
    nd, nf, nk, nb2 = D // LANES, F // (4 * LANES), len(_HK), S // TM2

    hbm = pl.BlockSpec(memory_space=pl.ANY)
    dma = pltpu.SemaphoreType.DMA
    out = pl.pallas_call(
        functools.partial(_kernel, S=S, D=D, H=H, Dh=Dh, M=M, seg=seg, F=F, TM1=TM1, TM2=TM2),
        out_shape=jax.ShapeDtypeStruct((S, D), BF16),
        in_specs=[hbm] * 10,
        out_specs=hbm,
        scratch_shapes=[
            pltpu.VMEM((S, D), BF16),
            pltpu.VMEM((2, S, LANES), F32),
            pltpu.VMEM((nd, S + TM2, LANES), F32),
            pltpu.VMEM((2, 7, nd // 2, TM1 // 2, LANES), BF16),
            pltpu.VMEM((TM2, D), F32),
            pltpu.VMEM((49, nd // 4, TM2 // 4, LANES), BF16),
            pltpu.VMEM((49, nf, TM2 // 4, LANES), BF16),
            pltpu.VMEM(((H // 4) * nk * (Dh + 3 * (D // 8 + 2)), LANES), U32),
            pltpu.VMEM((2 * 49 * (nf * D // 8 + 8), LANES), U32),
            pltpu.SMEM((1,), jnp.int32),
            pltpu.VMEM((2, 12, (D // 4 // nb2) * H // 2, LANES), U32),
            pltpu.VMEM((2, 4, nd, H * Dh // (8 * nb2), LANES), U32),
            pltpu.VMEM((M, D), BF16),
            pltpu.VMEM((M, D), F32),
            pltpu.VMEM((4, 4, 2, 4, seg, LANES), F32),
            dma((S // TM1 + 1,)), dma((nd // 2 + 7,)), dma((2,)), dma((S // (4 * seg),)),
        ],
        compiler_params=pltpu.CompilerParams(
            vmem_limit_bytes=128 * 1024 * 1024, disable_bounds_checks=True, disable_semaphore_checks=True),
        name="rmt_s2mlp",
    )(A_x.reshape(S, D), A_mem0.reshape(M, D),
      A_Wq.reshape(D * H, Dh), A_Wk.reshape(D * H, Dh), A_Wv.reshape(D * H, Dh),
      A_Wo.reshape(H * Dh, D), B_w1, B_w2, B_w3, B_w4)
    return out.reshape(B, S, D)
```

```python
import functools
import math

import jax
import jax.numpy as jnp
from jax import lax
import jax.experimental.pallas as pl
import jax.experimental.pallas.tpu as pltpu

F32 = jnp.float32
BF16 = jnp.bfloat16
U32 = jnp.uint32
LANES = 128
EPS = 1e-5
PAD = 8


def _dot(a, b):
    return lax.dot_general(a, b, (((1,), (0,)), ((), ())), preferred_element_type=F32)


def _dot_nt(a, b):
    return lax.dot_general(a, b, (((1,), (1,)), ((), ())), preferred_element_type=F32)


def _cat(xs, axis):
    return xs[0] if len(xs) == 1 else jnp.concatenate(xs, axis=axis)


def _moments(x, z):
    s = _cat([pltpu.bitcast(z, F32)] * (x.shape[0] // 8), 0)
    for c in range(0, x.shape[1], LANES):
        s = s + x[:, c:c + LANES]
    m = jnp.sum(s, axis=-1, keepdims=True) * (1.0 / x.shape[1])
    d = x - m
    return m, d, jnp.mean(d * d, axis=-1, keepdims=True)


def _recip(x):
    r = pl.reciprocal(x, approx=True)
    return r * (2.0 - x * r)


def _gelu_of_twice(h):
    c = math.sqrt(2.0 / math.pi)
    return h + h * jnp.tanh(h * (2.0 * c + (8.0 * c * 0.044715) * (h * h)))


def _halves(w):
    return pltpu.bitcast(w, BF16)


def _unpack(w, z):
    return pltpu.bitcast(w << (z | 16), F32), pltpu.bitcast(w & (z | U32(0xFFFF0000)), F32)


def _pack(lo, hi):
    return pltpu.bitcast(pltpu.pack_elementwise([lo, hi], packed_dtype=BF16), U32)


def _left(a11, a12, a21, a22):
    return (a11 + a22, a21 + a22, a11, a22, a11 + a12, a21 - a11, a12 - a22)


def _right(b11, b12, b21, b22):
    return (b11 + b22, b11, b12 - b22, b21 - b11, b22, b11 + b12, b21 + b22)


def _combine(m):
    m4 = m(3)
    m2 = m(1)
    c21 = m2 + m4
    m1 = m(0)
    c22 = m1 - m2
    c11 = m1 + m4
    c11 = c11 + m(6)
    m5 = m(4)
    c11 = c11 - m5
    m3 = m(2)
    c12 = m3 + m5
    c22 = c22 + m3
    c22 = c22 + m(5)
    return c11, c12, c21, c22


def _combine_late(m):
    m3 = m(2)
    m5 = m(4)
    c12 = m3 + m5
    c22 = m3 + m(5)
    m1 = m(0)
    c11 = m1 - m5
    c22 = c22 + m1
    m2 = m(1)
    c22 = c22 - m2
    m4 = m(3)
    c21 = m2 + m4
    c11 = c11 + m4
    c11 = c11 + m(6)
    return c11, c12, c21, c22


class _Blocks(tuple):
    def __add__(self, other):
        return _Blocks(a + b for a, b in zip(self, other))

    def __sub__(self, other):
        return _Blocks(a - b for a, b in zip(self, other))


def _left2(a):
    nested = [_Blocks(a[2 * i + u][2 * j + w] for u in range(2) for w in range(2))
              for i in range(2) for j in range(2)]
    return (_left(*g) for g in _left(*nested))


def _combine2(m, outer):
    c = outer(lambda a: _Blocks(_combine(lambda b: m(7 * a + b))))
    return [[c[2 * (i // 2) + j // 2][2 * (i % 2) + j % 2] for j in range(4)] for i in range(4)]


def _hopcroft_kerr(types):
    n = len(types)
    prods = []

    def add(left, out):
        prods.append((left, {}, out))
        return len(prods) - 1

    def use(block, terms):
        for f, s in terms:
            prods[f][1][block] = prods[f][1].get(block, 0) + s

    class Node:
        def __init__(self, t, xs, ys, plus, minus):
            self.t, self.xs, self.ys, self.plus, self.minus = t, xs, ys, plus, minus

    def mix(*parts):
        return {(i, t % 3): s * c for d, t, s in parts for i, c in d.items()}

    def pair(u, w):
        if (u.t - w.t) % 3 != 1:
            zwu, zuw, free = pair(w, u)
            return zuw, zwu, free
        t = u.t
        s = add(mix((u.xs, t + 2, 1), (w.xs, t, 1)), mix((u.ys, t + 2, 1), (w.ys, t, -1)))
        o1 = add(mix((u.xs, t, -1), (w.xs, t, 1)), mix((u.ys, t + 2, 1), (w.ys, t + 2, 1)))
        o2 = add(mix((u.xs, t + 2, -1), (w.xs, t + 2, 1)), mix((u.ys, t, 1), (w.ys, t, 1)))
        free = Node((t + 1) % 3, {**{i: -c for i, c in u.xs.items()}, **w.xs}, {**u.ys, **w.ys}, o1, o2)
        return ([(s, 1), (o1, -1), (u.minus, 1), (w.minus, -1)],
                [(s, 1), (o2, -1), (u.plus, 1), (w.plus, -1)], free)

    nodes = []
    for i, t in enumerate(types):
        e = {i: 1}
        nodes.append(Node(t, e, e, add(mix((e, t + 2, 1)), mix((e, t + 1, 1))),
                          add(mix((e, t + 1, 1)), mix((e, t + 2, 1)))))
        use((i, i), [(nodes[i].plus, 1), (nodes[i].minus, -1)])
    z, free = {}, {}
    for i in range(n):
        for j in range(i + 1, n):
            if types[i] != types[j]:
                z[i, j], z[j, i], free[i, j] = pair(nodes[i], nodes[j])
                free[j, i] = free[i, j]
    for i in range(n):
        for j in range(i + 1, n):
            if types[i] == types[j]:
                k = next(k for k in range(n) if types[k] != types[i])
                w = free[i, k]
                zwj, zjw, _ = pair(w, nodes[j])
                z[i, j] = [(f, w.xs[i] * c) for f, c in zwj] + z[k, j]
                z[j, i] = zjw + [(f, -c) for f, c in z[j, k]]
    for block, terms in z.items():
        use(block, terms)
    return [(left, {k: c for k, c in right.items() if c}, out) for left, right, out in prods]


def _signed_sum(terms):
    terms = sorted(terms, key=lambda t: -t[0])
    sign, y = terms[0]
    for s, x in terms[1:]:
        y = y + x if s == sign else y - x
    return sign, y


def _signed_value(terms):
    sign, y = _signed_sum(terms)
    return y if sign > 0 else -y


_HK = _hopcroft_kerr((0, 1, 2, 0))
_HK_ROW = [f for f, (left, _, out) in enumerate(_HK)
           if any(t != 2 for _, t in left) and any(t != 0 for _, t in out)]
_HK_RIGHT_SIGN = [_signed_sum([(c, 0) for c in right.values()])[0] for _, right, _ in _HK]


def _hk_left(upper, lower=None):
    if lower is None:
        base = [((1, u), (-1, u), None) for u in upper]
    else:
        base = [((1, u), (1, w), (-1, u + w)) for u, w in zip(upper, lower)]
    return {f: _signed_sum([(c * base[i][t][0], base[i][t][1]) for (i, t), c in _HK[f][0].items() if base[i][t]])
            for f in (_HK_ROW if lower is None else range(len(_HK)))}


def _hk_combine(left, m):
    both = len(left) == len(_HK)
    acc = {}
    for f, (sign, _) in left.items():
        y = m(f)
        for (j, t), c in _HK[f][2].items():
            c *= sign * _HK_RIGHT_SIGN[f]
            if both:
                acc[j, t] = _signed_sum([acc[j, t], (c, y)]) if (j, t) in acc else (c, y)
            elif t:
                c *= (0, -1, 1)[t]
                acc[j] = _signed_sum([acc[j], (c, y)]) if j in acc else (c, y)
    if not both:
        return [[_signed_value([acc[j]]) for j in range(4)]]
    return [[_signed_value([acc[j, p], (-acc[j, q][0], acc[j, q][1])]) for j in range(4)]
            for p, q in ((2, 1), (0, 2))]


class _Filler:
    def __init__(self, slots, jobs):
        self.slots, self.done, self.jobs, self.live = slots, 0, jobs, []

    def __call__(self, z):
        def step(g, v):
            try:
                g.send(v)
                return True
            except StopIteration:
                return False

        n = len(self.jobs)
        new = [job(z) for job in self.jobs[self.done * n // self.slots:(self.done + 1) * n // self.slots]]
        self.live = [g for g in new if step(g, None)] + [g for g in self.live if step(g, z)]
        self.done += 1

    def finish(self):
        while self.live or self.done < self.slots:
            self(jnp.zeros((8, LANES), U32))


def _run(jobs, group):
    _Filler(len(jobs) // group, jobs).finish()


def _kernel(x_hbm, mem0_hbm, wq_hbm, wk_hbm, wv_hbm, wo_hbm, w1_hbm, w2_hbm, w3_hbm, w4_hbm,
            out_hbm,
            xbuf, stat, hs, lf, lt, ly, lz, wa, wb, zero, stq, sto, mem0, membuf, pbuf,
            sem_x, sem_w, sem_a, sem_out,
            *, S, D, H, Dh, M, seg, F, TM1, TM2):
    part = functools.partial
    L = M + seg
    nd = D // LANES
    nh = nd // 2
    Dk = D // 2
    rq = LANES // 2
    wk = Dk // 2
    wq = wk // 2
    nf = F // (4 * LANES)
    hp = H // 2
    ng = H // 4
    nk = len(_HK)
    nb1, nb2 = S // TM1, S // TM2
    h1, q2 = TM1 // 2, TM2 // 4
    RC = 16

    def cols(n, w=1):
        return slice(n * LANES, (n + w) * LANES)

    def heads(g):
        return [2 * g, 2 * g + 1, hp + 2 * g, hp + 2 * g + 1]

    fp = nf * wq + 8
    slab = wq + 2
    o_w3 = 0
    o_w4 = o_w3 + 49 * fp
    o_qkv = 0
    o_wo = o_qkv + 3 * ng * nk * slab
    raw = {1: o_qkv, 2: o_qkv + nd * Dk, 3: o_qkv + 2 * nd * Dk, 4: o_qkv + 2 * nd * Dk + 4 * F}

    def weights(ref, r0, rows):
        return _halves(ref[pl.ds(r0, rows), :])

    def w_copy(j, n):
        src, rows, sem = {1: (w1_hbm, Dk, n % nh), 2: (w2_hbm, Dk, nh),
                          3: (w3_hbm, Dk, nh + 1 + n % nf // 2), 4: (w4_hbm, F // 2, nh + 5 + n % 2)}[j]
        return pltpu.make_async_copy(src.bitcast(U32).at[:, cols(n)], wa.at[pl.ds(raw[j] + n * rows, rows)],
                                     sem_w.at[sem])

    def w_wait(sem, *spans):
        for r0, rows in spans:
            pltpu.make_async_copy(wa.at[pl.ds(r0, rows)], wa.at[pl.ds(r0, rows)], sem_w.at[sem]).wait()

    def w3_copies(lo, hi):
        return [w_copy(3, p + j * nf) for p in range(lo, hi) for j in range(4)]

    def x_copy(i):
        r0 = pl.multiple_of(i * TM1, TM1)
        return pltpu.make_async_copy(x_hbm.at[pl.ds(r0, TM1)], xbuf.at[pl.ds(r0, TM1)], sem_x.at[i])

    fpi = D // 4 // nb2
    opi = ng * rq // nb2

    def a_copies(i):
        cps = []
        for t, src in enumerate((wq_hbm, wk_hbm, wv_hbm)):
            for k in range(4):
                r0 = pl.multiple_of((k * (D // 4) + i * fpi) * hp, fpi * hp)
                cps.append(pltpu.make_async_copy(src.bitcast(U32).at[pl.ds(r0, fpi * hp)],
                                                 stq.at[i % 2, 4 * t + k], sem_a.at[i % 2]))
        for k, h in enumerate(heads(i // (rq // opi))):
            r0 = pl.multiple_of(h * rq + i % (rq // opi) * opi, opi)
            for n in range(nd):
                cps.append(pltpu.make_async_copy(wo_hbm.bitcast(U32).at[pl.ds(r0, opi), cols(n)],
                                                 sto.at[i % 2, k, n], sem_a.at[i % 2]))
        return cps

    later = [
        lambda: [x_copy(4)] + [w_copy(2, n) for n in range(nh)],
        lambda: [x_copy(5)] + [w_copy(2, n) for n in range(nh, nd)],
        lambda: [x_copy(6)] + w3_copies(0, 1),
        lambda: [x_copy(7)] + w3_copies(1, 2),
        lambda: w3_copies(2, 3),
        lambda: w3_copies(3, 4),
        lambda: w3_copies(4, 6),
        lambda: w3_copies(6, 7),
        lambda: [w_copy(4, 0), w_copy(4, 2)],
        lambda: [w_copy(4, 4), w_copy(4, 6)],
        lambda: [w_copy(4, 1), w_copy(4, 3)],
        lambda: [w_copy(4, 5), w_copy(4, 7)],
        lambda: a_copies(0),
        lambda: a_copies(1),
    ]

    def start_later(i, lo, hi):
        for k in range(lo, min(hi, len(later))):
            @pl.when(i == k - lo)
            def _(k=k):
                for c in later[k]():
                    c.start()

    first = [pltpu.make_async_copy(x_hbm.at[pl.ds(r, TM1 // 8)], xbuf.at[pl.ds(r, TM1 // 8)], sem_x.at[0])
             for r in range(0, TM1, TM1 // 8)]
    for c in first:
        c.start()
    for n in range(nh // 2):
        w_copy(1, n).start()
        w_copy(1, n + nh).start()

    for n in range(nd):
        hs[n, 0:PAD, :] = jnp.zeros((PAD, LANES), F32)
        hs[n, PAD + S:PAD + S + PAD, :] = jnp.zeros((PAD, LANES), F32)
    wa[o_wo:o_wo + 8, :] = jnp.zeros((8, LANES), U32)
    wb[0:8, :] = jnp.zeros((8, LANES), U32)
    zero[0] = 0

    class Deadline:
        def __init__(self, probe=None, lag=0):
            self.probe, self.queue = probe, [None] * lag
            self.zero = jnp.full((8, LANES), zero[0], jnp.int32).astype(U32)

        def after(self, y):
            return pltpu.bitcast(y[0:8, 0:LANES], U32) & self.zero

        def __call__(self, w):
            self.queue.append(self.probe() & self.zero)
            z = self.queue.pop(0)
            if z is None:
                return w
            return _cat([_cat([w[0:8, 0:LANES] | z, w[8:, 0:LANES]], 0), w[:, LANES:]], 1)

    def norm_in(i, slot, r, z):
        a = []
        for half in range(2):
            rr = pl.ds(pl.multiple_of(i * TM1 + half * h1 + r, RC), RC)
            m, d, v = _moments(xbuf[rr, :].astype(F32), z)
            q = lax.rsqrt(v + EPS)
            stat[0, rr, :] = jnp.broadcast_to(m, (RC, LANES))
            stat[1, rr, :] = jnp.broadcast_to(q, (RC, LANES))
            a.append(d * (0.5 * q * lax.rsqrt(v * q * q + EPS)))
        for _ in range(3):
            yield
        for k, f in enumerate(_left(a[0][:, :Dk], a[0][:, Dk:], a[1][:, :Dk], a[1][:, Dk:])):
            for n in range(nh):
                lf[slot, k, n, pl.ds(r, RC), :] = f[:, cols(n)].astype(BF16)
            if k in (1, 4):
                yield

    def normed(rr):
        m, q = (_cat([stat[k, rr, :]] * nd, 1) for k in range(2))
        return (xbuf[rr, :].astype(F32) - m) * q

    def norm_first(q, carry):
        _run([part(norm_in, 0, 0, pl.multiple_of((4 * q + e) * RC, RC)) for e in range(4)], 4)
        return carry

    def prep1(n, carry):
        o = pl.multiple_of(raw[1] + n * Dk, Dk)
        dst = pl.multiple_of(o_w4 + n * 7 * wk, 8)
        w_wait(n, (o, Dk), (o + nh * Dk, Dk))

        def job(r, _):
            w = [wa[pl.ds(o + (e + r), 8), :] for e in (0, nh * Dk, wk, nh * Dk + wk)]
            z = yield
            lo, hi = (_right(*y) for y in zip(*[_unpack(x, z) for x in w]))
            for k in range(7):
                wb[pl.ds(dst + (k * wk + r), 8), :] = {1: w[0], 4: w[3]}[k] if k in (1, 4) else _pack(lo[k], hi[k])

        _run([part(job, r) for r in range(0, wk, 8)], 2)
        return carry

    def b1(i, carry):
        @pl.when(i + 1 < nb1)
        def _():
            x_copy(i + 1).wait()

        r0 = pl.multiple_of(i * TM1, TM1)
        nxt = jnp.minimum(i + 1, nb1 - 1)
        fill = _Filler(7 * nh - 3, [part(norm_in, nxt, (i + 1) % 2, r) for r in range(0, h1, RC)])
        due = Deadline()

        def prod(n, k):
            w = lf.bitcast(U32)
            y = _dot(_halves(_cat([w[i % 2, k, c] for c in range(nh)], 1)), weights(wb, o_w4 + (n * 7 + k) * wk, wk))
            fill(due.after(y))
            return y

        for n in range(nh):
            for k, y in enumerate(_combine(part(prod, n))):
                hs[n + k % 2 * nh, pl.ds(r0 + PAD + k // 2 * h1, h1), :] = _gelu_of_twice(y)
        fill.finish()
        start_later(i, 0, nb1)
        return carry

    for c in first:
        c.wait()
    for n in range(nh // 2, nh):
        w_copy(1, n).start()
        w_copy(1, n + nh).start()
    lax.fori_loop(0, h1 // (4 * RC), norm_first, 0)
    x_copy(1).start()
    lax.fori_loop(0, nh, prep1, 0)
    x_copy(2).start()
    x_copy(3).start()
    mem_copy = pltpu.make_async_copy(mem0_hbm, mem0, sem_x.at[nb1])
    mem_copy.start()
    lax.fori_loop(0, nb1, b1, 0)

    shifts = (-1, 1, -2, 2)
    BK = 32
    HB = 32
    per = nf * (wq // BK) // (nb1 // 2)

    def prep34(second, u):
        src = jnp.where(second, raw[4] + u // (nf * rq // BK) * (F // 2) + u % (nf * rq // BK) * BK,
                        raw[3] + u // (wq // BK) * Dk + u % (wq // BK) * BK).astype(jnp.int32)
        src = [pl.multiple_of(src + k * jnp.where(second, nf * rq, wq), BK) for k in range(4)]
        dst = pl.multiple_of(jnp.where(second, o_w4, o_w3) + u.astype(jnp.int32) * BK, 8)

        def job(r, z):
            def quarter(a, b):
                x = [_unpack(wa[pl.ds(src[2 * a + k] + ((2 * b + j) * F + r), 8), :], z)
                     for k in range(2) for j in range(2)]
                return [_Blocks(y[h] for y in x) for h in range(2)]

            for stage in ((1, 5), (3, 0), (4, 2), (6,)):
                lo, hi = (_right(*y) for y in zip(*[quarter(a, b) for a in range(2) for b in range(2)]))
                for a in stage:
                    for b, (x, y) in enumerate(zip(_right(*lo[a]), _right(*hi[a]))):
                        wb[pl.ds(dst + ((7 * a + b) * fp + r), 8), :] = _pack(x, y)
                z = yield

        return [part(job, r) for r in range(0, BK, 8)]

    def b2(i, carry):
        for k in range(4):
            pl.when(i == k)(part(w_wait, nh + 1 + k, *[
                (raw[3] + j * F + 2 * k * Dk, min(2, nf - 2 * k) * Dk) for j in range(4)]))
        for e in range(2):
            pl.when(i == 4 + 2 * e)(part(w_wait, nh + 5 + e, *[
                (raw[4] + j * F + e * (F // 2), F // 2) for j in range(4)]))

        r0 = pl.multiple_of(i * TM1, TM1)
        jobs = [prep34(i >= nb1 // 2, (i.astype(U32) % (nb1 // 2)) * per + u) for u in range(per)]
        fill = _Filler(2 * nd * TM1 // HB - 6, sum(jobs, []))
        due = Deadline(lambda: wb[0:8, :], 6)

        def shifted(r):
            return [hs[n, pl.ds(r0 + PAD + r + shifts[n * 4 // nd], HB), :] for n in range(nd)]

        ahead = shifted(0)
        for r in range(0, TM1, HB):
            sh = ahead
            for c in range(nd):
                if c == nd - 2 and r + HB < TM1:
                    ahead = shifted(r + HB)
                y = None
                for k in range(0, nd, nh):
                    a = pltpu.bitcast(due(pltpu.bitcast(_cat(sh[k:k + nh], 1), U32)), F32)
                    p = _dot(a.astype(BF16), weights(wa, raw[2] + c * Dk + k * rq, nh * rq))
                    y = p if y is None else p + y
                    fill(due.after(y))
                hs[c, pl.ds(r0 + r, HB), :] = y
        fill.finish()
        start_later(i, nb1, 2 * nb1)
        return carry

    w_wait(nh, (raw[2], nd * Dk))
    lax.fori_loop(0, nb1, b2, 0)

    def norm_mid(i):
        def job(r, _):
            rr = pl.ds(pl.multiple_of(jnp.minimum(i, nb2 - 1) * TM2 + r, 8), 8)
            x1 = _cat([hs[n, rr, :] for n in range(nd)], 1) + normed(rr)
            y = x1 + xbuf[rr, :].astype(F32)
            z = yield
            for n in range(nd):
                hs[n, pl.ds(pl.multiple_of(i * TM2 + r, 8), 8), :] = y[:, cols(n)]
            _, d, v = _moments(x1, z)
            lt[r:r + 8, :] = d * (0.5 * lax.rsqrt(v + EPS))

        return [part(job, r) for r in range(0, TM2, 8)]

    def left_mid():
        def job(r, n, _):
            a = [[lt[u * q2 + r:u * q2 + r + RC, cols(2 * j + n)] for j in range(4)] for u in range(4)]
            for k, g in enumerate(_left2(a)):
                for b, f in enumerate(g):
                    ly[7 * k + b, n, r:r + RC, :] = f.astype(BF16)
                yield

        return [part(job, r, n) for r in range(0, q2, RC) for n in range(2)]

    def b3(i, carry):
        for buf in (stq, sto):
            pltpu.make_async_copy(buf.at[i % 2], buf.at[i % 2], sem_a.at[i % 2]).wait()

        stages = [range(8, 17), range(17, 26), range(0, 4), range(4, 8)]

        def prep_qkv(t, u, z):
            for stage in stages:
                def block(par, k, j):
                    w = stq[i % 2, 4 * t + k, pl.ds((2 * u + par) * hp + 8 * (j // 2), 8), :]
                    return _unpack(w, z)[j % 2]

                for f in stage:
                    y = [_signed_sum([(c, block(par, *key)) for key, c in _HK[f][1].items()])[1] for par in range(2)]
                    base = o_qkv + (t * ng * nk + f) * slab + u + i * (fpi // 2)
                    wa[pl.ds(base, 8, stride=nk * slab), :] = _pack(*y)
                z = yield

        def prep_o(e, r, z):
            for stage in stages:
                for f in stage:
                    w = [(c, sto[i % 2, k, 2 * j + e, r:r + 8, :]) for (k, j), c in _HK[f][1].items()]
                    rr = pl.ds(pl.multiple_of(o_wo + (e * nk + f) * ng * rq + i * opi, opi) + r, 8)
                    wa[rr, :] = w[0][1] if len(w) == 1 else _pack(
                        *[_signed_sum([(c, _unpack(x, z)[h]) for c, x in w])[1] for h in range(2)])
                z = yield

        jobs = [part(prep_qkv, t, u) for t in range(3) for u in range(fpi // 2)]
        jobs += [part(prep_o, e, r) for e in range(2) for r in range(0, opi, 8)]
        r0 = pl.multiple_of(i * TM2, TM2)
        here = pl.ds(pl.multiple_of(zero[0], 8), 8)
        norm_slots = [k for k in range(49) if k // 7 in (3, 1)]
        prep_slots = norm_slots[::4]
        fill = _Filler(nf * len(prep_slots) + 2 * 49 - 8, jobs)
        due = Deadline(lambda: wa[o_wo:o_wo + 8, :], 5)
        fill_y = _Filler((nf - 1) * len(norm_slots), norm_mid(i + 1))
        due_y = Deadline(lambda: pltpu.bitcast(lt[here, 0:LANES], U32), 14)
        fill_z = _Filler(2 * 49 - 24, left_mid())
        due_z = Deadline(lambda: ly.bitcast(U32)[zero[0], 0, 0:8, :], 6)

        def up(p, k):
            w = ly.bitcast(U32)
            w = _cat([w[k, n] for n in range(2)], 1)
            if k in prep_slots:
                w = due(w)
            y = _dot(_halves(due_y(w) if k in norm_slots else w), weights(wb, o_w3 + k * fp + p * wq, wq))
            if k in norm_slots:
                z = due.after(y)
                fill_y(z)
                if k in prep_slots:
                    fill(z)
            return y

        for p in range(nf):
            g = [[_gelu_of_twice(y) for y in row] for row in _combine2(part(up, p), _combine)]
            for a, group in enumerate(_left2(g)):
                for b, f in enumerate(group):
                    lz[7 * a + b, p] = f.astype(BF16)
        fill_y.finish()

        def down(e, k):
            w = lz.bitcast(U32)
            y = _dot(_halves(due_z(due(_cat([w[k, p] for p in range(nf)], 1)))),
                     weights(wb, o_w4 + k * fp + e * nf * rq, nf * rq))
            z = due.after(y)
            fill(z)
            fill_z(z)
            return y

        for e in range(2):
            for u, row in enumerate(_combine2(part(down, e), _combine_late)):
                for j, y in enumerate(row):
                    hs[2 * j + e, pl.ds(r0 + u * q2, q2), :] += y
        fill_z.finish()
        fill.finish()

        @pl.when(i + 2 < nb2)
        def _():
            for c in a_copies(i + 2):
                c.start()

        return carry

    _run(norm_mid(0), 2)
    _run(left_mid(), 1)
    lax.fori_loop(0, nb2, b3, 0)

    scale = Dh ** -0.5
    key = lax.broadcasted_iota(jnp.int32, (seg, L), 0) + M
    query = lax.broadcasted_iota(jnp.int32, (seg, L), 1)
    mask = (query < M) | (query >= key)
    QS = 4 * seg
    rv = (seg - M) // 8

    def upper(n):
        return lax.broadcasted_iota(jnp.int32, (8, n), 0) < 4

    def split8(mem, tok):
        u = upper(mem.shape[1])
        return jnp.where(u, mem, tok), pltpu.roll(jnp.where(u, tok, mem), 4, 0)

    def join8(t, b):
        u = upper(t.shape[1])
        b = pltpu.roll(b, 4, 0)
        return jnp.where(u, t, b), jnp.where(u, b, t)

    def vregs(y, lo, hi):
        return [y[8 * k:8 * k + 8] for k in range(lo, hi)]

    def left_operands(mem, tok, big):
        if not big:
            return _hk_left([_cat([m] + y, 0) for m, y in zip(mem, tok)])
        pairs = [split8(m, y[2 * rv]) for m, y in zip(mem, tok)]
        return _hk_left(*[[_cat([p[c]] + y[c * rv:(c + 1) * rv], 0) for p, y in zip(pairs, tok)] for c in range(2)])

    def rows_out(c):
        if len(c) == 1:
            return [(y[0:8], vregs(y, 1, 1 + rv)) for y in c[0]]
        got = []
        for y, w in zip(*c):
            ym, yt = join8(y[0:8], w[0:8])
            got.append((ym, vregs(y, 1, 1 + rv) + vregs(w, 1, 1 + rv) + [yt]))
        return got

    def probs(q, k):
        sc = _dot_nt(k, q.astype(BF16))
        sc = _cat([sc[0:M], jnp.where(mask, sc[M:L], -1e9 / scale)], 0)
        p = jnp.exp2((sc - jnp.max(sc, axis=0, keepdims=True)) * (scale * math.log2(math.e)))
        return p * _recip(jnp.sum(p, axis=0, keepdims=True))

    def out_copy(j):
        r0 = pl.multiple_of(j * QS, QS)
        return pltpu.make_async_copy(xbuf.at[pl.ds(r0, QS)], out_hbm.at[pl.ds(r0, QS)], sem_out.at[j])

    def quad(j, carry):
        xs = normed(pl.ds(pl.multiple_of(j * QS, QS), QS))
        qkv = {(t, h): [] for t in range(3) for h in range(H)}
        att = {h: [] for h in range(H)}
        outs = {n: [] for n in range(nd)}
        mem = membuf[...]
        for st in range(4):
            r, n_tok = (0, 2 * rv + 1) if st == 0 else ((st + 1) * rv + 1, rv)
            hl = left_operands([mem[:, cols(2 * k, 2)] for k in range(4)],
                               [vregs(xs[:, cols(2 * k, 2)], r, r + n_tok) for k in range(4)], st == 0)
            ol, cur, p, o = {}, {}, {}, {}

            def wq_part(t, g, lo, hi):
                return _hk_combine(hl, lambda f: _dot(
                    hl[f][1][:, lo:hi].astype(BF16),
                    weights(wa, o_qkv + ((t * ng + g) * nk + f) * slab + lo // 2, (hi - lo) // 2)))

            def wo_part(e, lo, hi):
                return _hk_combine(ol[lo], lambda f: _dot(
                    _cat([ol[g][f][1] for g in range(lo, hi)], 1).astype(BF16),
                    weights(wa, o_wo + ((e * nk + f) * ng + lo) * rq, (hi - lo) * rq)))

            def stash(q, c):
                for a, blocks in enumerate(c):
                    for b, y in enumerate(blocks):
                        pbuf[st, q, a, b] = y

            def resume(q, c):
                return [[pbuf[st, q, a, b] + y for b, y in enumerate(blocks)] for a, blocks in enumerate(c)]

            def proj(t, g):
                if g == 0 and st > 0 and t < 2:
                    c = resume(2 + t, wq_part(t, g, LANES, 2 * LANES))
                else:
                    c = wq_part(t, g, 0, 2 * LANES)
                got = []
                for h, (ym, yt) in zip(heads(g), rows_out(c)):
                    qkv[t, h] += yt
                    got.append(_cat([ym] + qkv[t, h][4 * st:4 * st + 4], 0))
                return got

            def attend(g, c):
                for e in (2 * c, 2 * c + 1):
                    if 0 <= g < ng:
                        p[g, e] = probs(cur[0, g][e], cur[1, g][e])
                if g > 0:
                    for e in (2 * c, 2 * c + 1):
                        o[e] = _dot(p[g - 1, e].T, cur[2, g - 1][e].astype(BF16))
                        att[heads(g - 1)[e]] += vregs(o[e], 1, 5)
                    if c:
                        ol[g - 1] = left_operands(
                            [o[e][0:8] for e in range(4)],
                            [att[h][st * rv:None if st == 3 else (st + 1) * rv] for h in heads(g - 1)], st == 3)

            if st > 0:
                for t in range(2):
                    stash(2 + t, wq_part(t, 0, 0, LANES))
            for g in range(ng):
                cur[0, g] = proj(0, g)
                cur[1, g] = proj(1, g)
                attend(g - 1, 1)
                cur[2, g] = proj(2, g)
                attend(g, 0)
            stash(0, wo_part(0, 0, 2))
            attend(ng - 1, 1)
            stash(1, wo_part(1, 0, 2))
            attend(ng, 0)
            stash(0, resume(0, wo_part(0, 2, 4)))
            attend(ng, 1)
            stash(1, resume(1, wo_part(1, 2, 4)))
            new = {}
            for e in range(2):
                for c, (ym, yt) in enumerate(rows_out(resume(e, wo_part(e, 4, ng)))):
                    new[2 * c + e] = ym
                    outs[2 * c + e] += yt
            mem = _cat([new[n] for n in range(nd)], 1)
            lo, hi = ((0, 2), (2, 6), (6, 8), (8, 16))[st]
            rr = pl.ds(pl.multiple_of(j * QS + 8 * lo, RC), 8 * (hi - lo))
            for n in range(nd):
                xbuf[rr, cols(n)] = (hs[n, rr, :] + _cat(outs[n][lo:hi], 0)).astype(BF16)
        membuf[...] = mem
        out_copy(j).start()
        return carry

    mem_copy.wait()
    membuf[...] = mem0[...].astype(F32)
    lax.fori_loop(0, S // QS, quad, 0)
    for j in range(S // QS):
        out_copy(j).wait()


@functools.partial(jax.jit, static_argnames=("A_seg_len",))
def pallas_parallel_sum__memory_aug_recurrent_mem_tr__mixer_s_mlp__prompt_kernel(
    A_x: jax.Array,
    A_mem0: jax.Array,
    A_Wq: jax.Array,
    A_Wk: jax.Array,
    A_Wv: jax.Array,
    A_Wo: jax.Array,
    A_seg_len: int,
    B_x: jax.Array,
    B_w1: jax.Array,
    B_w2: jax.Array,
    B_w3: jax.Array,
    B_w4: jax.Array,
):
    del B_x
    B, S, D = A_x.shape
    _, H, Dh = A_Wq.shape
    M = A_mem0.shape[1]
    seg = int(A_seg_len)
    F = B_w3.shape[1]
    assert (B, S, D, H, Dh, M, seg, F) == (1, 2048, 1024, 32, LANES, 8, 32, 3584)
    TM1, TM2 = 256, 128
    nd, nf, nk, nb2 = D // LANES, F // (4 * LANES), len(_HK), S // TM2

    hbm = pl.BlockSpec(memory_space=pl.ANY)
    dma = pltpu.SemaphoreType.DMA
    out = pl.pallas_call(
        functools.partial(_kernel, S=S, D=D, H=H, Dh=Dh, M=M, seg=seg, F=F, TM1=TM1, TM2=TM2),
        out_shape=jax.ShapeDtypeStruct((S, D), BF16),
        in_specs=[hbm] * 10,
        out_specs=hbm,
        scratch_shapes=[
            pltpu.VMEM((S, D), BF16),
            pltpu.VMEM((2, S, LANES), F32),
            pltpu.VMEM((nd, S + TM2, LANES), F32),
            pltpu.VMEM((2, 7, nd // 2, TM1 // 2, LANES), BF16),
            pltpu.VMEM((TM2, D), F32),
            pltpu.VMEM((49, nd // 4, TM2 // 4, LANES), BF16),
            pltpu.VMEM((49, nf, TM2 // 4, LANES), BF16),
            pltpu.VMEM(((H // 4) * nk * (Dh + 3 * (D // 8 + 2)), LANES), U32),
            pltpu.VMEM((2 * 49 * (nf * D // 8 + 8), LANES), U32),
            pltpu.SMEM((1,), jnp.int32),
            pltpu.VMEM((2, 12, (D // 4 // nb2) * H // 2, LANES), U32),
            pltpu.VMEM((2, 4, nd, H * Dh // (8 * nb2), LANES), U32),
            pltpu.VMEM((M, D), BF16),
            pltpu.VMEM((M, D), F32),
            pltpu.VMEM((4, 4, 2, 4, seg, LANES), F32),
            dma((S // TM1 + 1,)), dma((nd // 2 + 7,)), dma((2,)), dma((S // (4 * seg),)),
        ],
        compiler_params=pltpu.CompilerParams(
            vmem_limit_bytes=128 * 1024 * 1024, disable_bounds_checks=True, disable_semaphore_checks=True),
        name="rmt_s2mlp",
    )(A_x.reshape(S, D), A_mem0.reshape(M, D),
      A_Wq.reshape(D * H, Dh), A_Wk.reshape(D * H, Dh), A_Wv.reshape(D * H, Dh),
      A_Wo.reshape(H * Dh, D), B_w1, B_w2, B_w3, B_w4)
    return out.reshape(B, S, D)
```

```python
import functools
import math

import jax
import jax.numpy as jnp
from jax import lax
import jax.experimental.pallas as pl
import jax.experimental.pallas.tpu as pltpu

F32 = jnp.float32
BF16 = jnp.bfloat16
U32 = jnp.uint32
LANES = 128
EPS = 1e-5
PAD = 8


def _dot(a, b):
    return lax.dot_general(a, b, (((1,), (0,)), ((), ())), preferred_element_type=F32)


def _dot_nt(a, b):
    return lax.dot_general(a, b, (((1,), (1,)), ((), ())), preferred_element_type=F32)


def _cat(xs, axis):
    return xs[0] if len(xs) == 1 else jnp.concatenate(xs, axis=axis)


def _moments(x, z):
    s = _cat([pltpu.bitcast(z, F32)] * (x.shape[0] // 8), 0)
    for c in range(0, x.shape[1], LANES):
        s = s + x[:, c:c + LANES]
    m = jnp.sum(s, axis=-1, keepdims=True) * (1.0 / x.shape[1])
    d = x - m
    return m, d, jnp.mean(d * d, axis=-1, keepdims=True)


def _recip(x):
    r = pl.reciprocal(x, approx=True)
    return r * (2.0 - x * r)


def _gelu_of_twice(h):
    c = math.sqrt(2.0 / math.pi)
    return h + h * jnp.tanh(h * (2.0 * c + (8.0 * c * 0.044715) * (h * h)))


def _halves(w):
    return pltpu.bitcast(w, BF16)


def _unpack(w, z):
    return pltpu.bitcast(w << (z | 16), F32), pltpu.bitcast(w & (z | U32(0xFFFF0000)), F32)


def _widen(w, z):
    return _halves(w if z is None else w | z).astype(F32)


def _left(a11, a12, a21, a22):
    return (a11 + a22, a21 + a22, a11, a22, a11 + a12, a21 - a11, a12 - a22)


def _right(b11, b12, b21, b22):
    return (b11 + b22, b11, b12 - b22, b21 - b11, b22, b11 + b12, b21 + b22)


def _combine(m):
    m4 = m(3)
    m2 = m(1)
    c21 = m2 + m4
    m1 = m(0)
    c22 = m1 - m2
    c11 = m1 + m4
    c11 = c11 + m(6)
    m5 = m(4)
    c11 = c11 - m5
    m3 = m(2)
    c12 = m3 + m5
    c22 = c22 + m3
    c22 = c22 + m(5)
    return c11, c12, c21, c22


def _combine_late(m):
    m3 = m(2)
    m5 = m(4)
    c12 = m3 + m5
    c22 = m3 + m(5)
    m1 = m(0)
    c11 = m1 - m5
    c22 = c22 + m1
    m2 = m(1)
    c22 = c22 - m2
    m4 = m(3)
    c21 = m2 + m4
    c11 = c11 + m4
    c11 = c11 + m(6)
    return c11, c12, c21, c22


class _Blocks(tuple):
    def __add__(self, other):
        return _Blocks(a + b for a, b in zip(self, other))

    def __sub__(self, other):
        return _Blocks(a - b for a, b in zip(self, other))


def _left2(a):
    nested = [_Blocks(a[2 * i + u][2 * j + w] for u in range(2) for w in range(2))
              for i in range(2) for j in range(2)]
    return (_left(*g) for g in _left(*nested))


def _combine2(m, outer):
    c = outer(lambda a: _Blocks(_combine(lambda b: m(7 * a + b))))
    return [[c[2 * (i // 2) + j // 2][2 * (i % 2) + j % 2] for j in range(4)] for i in range(4)]


def _hopcroft_kerr(types):
    n = len(types)
    prods = []

    def add(left, out):
        prods.append((left, {}, out))
        return len(prods) - 1

    def use(block, terms):
        for f, s in terms:
            prods[f][1][block] = prods[f][1].get(block, 0) + s

    class Node:
        def __init__(self, t, xs, ys, plus, minus):
            self.t, self.xs, self.ys, self.plus, self.minus = t, xs, ys, plus, minus

    def mix(*parts):
        return {(i, t % 3): s * c for d, t, s in parts for i, c in d.items()}

    def pair(u, w):
        if (u.t - w.t) % 3 != 1:
            zwu, zuw, free = pair(w, u)
            return zuw, zwu, free
        t = u.t
        s = add(mix((u.xs, t + 2, 1), (w.xs, t, 1)), mix((u.ys, t + 2, 1), (w.ys, t, -1)))
        o1 = add(mix((u.xs, t, -1), (w.xs, t, 1)), mix((u.ys, t + 2, 1), (w.ys, t + 2, 1)))
        o2 = add(mix((u.xs, t + 2, -1), (w.xs, t + 2, 1)), mix((u.ys, t, 1), (w.ys, t, 1)))
        free = Node((t + 1) % 3, {**{i: -c for i, c in u.xs.items()}, **w.xs}, {**u.ys, **w.ys}, o1, o2)
        return ([(s, 1), (o1, -1), (u.minus, 1), (w.minus, -1)],
                [(s, 1), (o2, -1), (u.plus, 1), (w.plus, -1)], free)

    nodes = []
    for i, t in enumerate(types):
        e = {i: 1}
        nodes.append(Node(t, e, e, add(mix((e, t + 2, 1)), mix((e, t + 1, 1))),
                          add(mix((e, t + 1, 1)), mix((e, t + 2, 1)))))
        use((i, i), [(nodes[i].plus, 1), (nodes[i].minus, -1)])
    z, free = {}, {}
    for i in range(n):
        for j in range(i + 1, n):
            if types[i] != types[j]:
                z[i, j], z[j, i], free[i, j] = pair(nodes[i], nodes[j])
                free[j, i] = free[i, j]
    for i in range(n):
        for j in range(i + 1, n):
            if types[i] == types[j]:
                k = next(k for k in range(n) if types[k] != types[i])
                w = free[i, k]
                zwj, zjw, _ = pair(w, nodes[j])
                z[i, j] = [(f, w.xs[i] * c) for f, c in zwj] + z[k, j]
                z[j, i] = zjw + [(f, -c) for f, c in z[j, k]]
    for block, terms in z.items():
        use(block, terms)
    return [(left, {k: c for k, c in right.items() if c}, out) for left, right, out in prods]


def _signed_sum(terms):
    terms = sorted(terms, key=lambda t: -t[0])
    sign, y = terms[0]
    for s, x in terms[1:]:
        y = y + x if s == sign else y - x
    return sign, y


def _signed_value(terms):
    sign, y = _signed_sum(terms)
    return y if sign > 0 else -y


_HK = _hopcroft_kerr((0, 1, 2, 0))
_HK_ROW = [f for f, (left, _, out) in enumerate(_HK)
           if any(t != 2 for _, t in left) and any(t != 0 for _, t in out)]
_HK_RIGHT_SIGN = [_signed_sum([(c, 0) for c in right.values()])[0] for _, right, _ in _HK]


def _hk_left(upper, lower=None):
    if lower is None:
        base = [((1, u), (-1, u), None) for u in upper]
    else:
        base = [((1, u), (1, w), (-1, u + w)) for u, w in zip(upper, lower)]
    return {f: _signed_sum([(c * base[i][t][0], base[i][t][1]) for (i, t), c in _HK[f][0].items() if base[i][t]])
            for f in (_HK_ROW if lower is None else range(len(_HK)))}


def _hk_combine(left, m):
    both = len(left) == len(_HK)
    acc = {}
    for f, (sign, _) in left.items():
        y = m(f)
        for (j, t), c in _HK[f][2].items():
            c *= sign * _HK_RIGHT_SIGN[f]
            if both:
                acc[j, t] = _signed_sum([acc[j, t], (c, y)]) if (j, t) in acc else (c, y)
            elif t:
                c *= (0, -1, 1)[t]
                acc[j] = _signed_sum([acc[j], (c, y)]) if j in acc else (c, y)
    if not both:
        return [[_signed_value([acc[j]]) for j in range(4)]]
    return [[_signed_value([acc[j, p], (-acc[j, q][0], acc[j, q][1])]) for j in range(4)]
            for p, q in ((2, 1), (0, 2))]


class _Filler:
    def __init__(self, slots, jobs):
        self.slots, self.done, self.jobs, self.live = slots, 0, jobs, []

    def __call__(self, z):
        def step(g, v):
            try:
                g.send(v)
                return True
            except StopIteration:
                return False

        n = len(self.jobs)
        new = [job(z) for job in self.jobs[self.done * n // self.slots:(self.done + 1) * n // self.slots]]
        self.live = [g for g in new if step(g, None)] + [g for g in self.live if step(g, z)]
        self.done += 1

    def finish(self):
        while self.live or self.done < self.slots:
            self(jnp.zeros((8, LANES), U32))


def _run(jobs, group):
    _Filler(len(jobs) // group, jobs).finish()


def _kernel(x_hbm, mem0_hbm, wq_hbm, wk_hbm, wv_hbm, wo_hbm, w1_hbm, w2_hbm, w3_hbm, w4_hbm,
            out_hbm,
            xbuf, stat, hs, lf, lt, ly, lz, wa, wb, zero, stq, stt, sto, mem0, membuf, pbuf,
            sem_x, sem_w, sem_a, sem_out,
            *, S, D, H, Dh, M, seg, F, TM1, TM2):
    part = functools.partial
    L = M + seg
    nd = D // LANES
    nh = nd // 2
    Dk = D // 2
    rq = LANES // 2
    wk = Dk // 2
    wq = wk // 2
    nf = F // (4 * LANES)
    hp = H // 2
    ng = H // 4
    nk = len(_HK)
    nb1, nb2 = S // TM1, S // TM2
    h1, q2 = TM1 // 2, TM2 // 4
    RC = 16

    def cols(n, w=1):
        return slice(n * LANES, (n + w) * LANES)

    def heads(g):
        return [2 * g, 2 * g + 1, hp + 2 * g, hp + 2 * g + 1]

    fp = nf * wq + 8
    o_w3 = 0
    o_w4 = o_w3 + 49 * fp
    o_wo = 0
    o_qkv = o_wo + 2 * nk * ng * rq
    raw = {1: o_qkv, 2: o_qkv + nd * Dk, 3: o_qkv + 2 * nd * Dk, 4: o_qkv + 2 * nd * Dk + 4 * F}

    def words(ref, r0, rows):
        return ref.bitcast(U32)[pl.ds(r0, rows), :]

    def weights(ref, r0, rows):
        return _halves(words(ref, r0, rows))

    def view(ref, r0, rows):
        return ref.at[pl.ds(pl.multiple_of(2 * r0, RC), 2 * rows)]

    def put(ref, r, y):
        ref[2 * r:2 * r + RC, :] = y.astype(BF16)

    def w_copy(j, n):
        src, rows, sem = {1: (w1_hbm, Dk, n % nh), 2: (w2_hbm, Dk, nh),
                          3: (w3_hbm, Dk, nh + 1 + n % nf // 2), 4: (w4_hbm, F // 2, nh + 5 + n % 2)}[j]
        return pltpu.make_async_copy(src.at[:, cols(n)], wa.at[pl.ds(2 * (raw[j] + n * rows), 2 * rows)],
                                     sem_w.at[sem])

    def w_wait(sem, *spans):
        for r0, rows in spans:
            span = wa.at[pl.ds(2 * r0, 2 * rows)]
            pltpu.make_async_copy(span, span, sem_w.at[sem]).wait()

    def w3_copies(lo, hi):
        return [w_copy(3, p + j * nf) for p in range(lo, hi) for j in range(4)]

    def x_copy(i):
        r0 = pl.multiple_of(i * TM1, TM1)
        return pltpu.make_async_copy(x_hbm.at[pl.ds(r0, TM1)], xbuf.at[pl.ds(r0, TM1)], sem_x.at[i])

    fpi = D // 4 // nb2
    tp = fpi + 4
    opi = ng * rq // nb2

    def a_copies(i):
        cps = []
        for t, src in enumerate((wq_hbm, wk_hbm, wv_hbm)):
            for k in range(4):
                r0 = pl.multiple_of((k * (D // 4) + i * fpi) * H, fpi * H)
                cps.append(pltpu.make_async_copy(src.at[pl.ds(r0, fpi * H)],
                                                 stq.at[i % 2, 4 * t + k], sem_a.at[i % 2]))
        for k, h in enumerate(heads(i // (rq // opi))):
            r0 = pl.multiple_of(2 * (h * rq + i % (rq // opi) * opi), 2 * opi)
            for n in range(nd):
                cps.append(pltpu.make_async_copy(wo_hbm.at[pl.ds(r0, 2 * opi), cols(n)],
                                                 sto.at[i % 2, k, n], sem_a.at[i % 2]))
        return cps

    later = [
        lambda: [x_copy(4)] + [w_copy(2, n) for n in range(nh)],
        lambda: [x_copy(5)] + [w_copy(2, n) for n in range(nh, nd)],
        lambda: [x_copy(6)] + w3_copies(0, 1),
        lambda: [x_copy(7)] + w3_copies(1, 2),
        lambda: w3_copies(2, 3),
        lambda: w3_copies(3, 4),
        lambda: w3_copies(4, 6),
        lambda: w3_copies(6, 7),
        lambda: [w_copy(4, 0), w_copy(4, 2)],
        lambda: [w_copy(4, 4), w_copy(4, 6)],
        lambda: [w_copy(4, 1), w_copy(4, 3)],
        lambda: [w_copy(4, 5), w_copy(4, 7)],
        lambda: a_copies(0),
        lambda: a_copies(1),
    ]

    def start_later(i, lo, hi):
        for k in range(lo, min(hi, len(later))):
            @pl.when(i == k - lo)
            def _(k=k):
                for c in later[k]():
                    c.start()

    first = [pltpu.make_async_copy(x_hbm.at[pl.ds(r, TM1 // 8)], xbuf.at[pl.ds(r, TM1 // 8)], sem_x.at[0])
             for r in range(0, TM1, TM1 // 8)]
    for c in first:
        c.start()
    for n in range(nh // 2):
        w_copy(1, n).start()
        w_copy(1, n + nh).start()

    for n in range(nd):
        hs[n, 0:PAD, :] = jnp.zeros((PAD, LANES), F32)
        hs[n, PAD + S:PAD + S + PAD, :] = jnp.zeros((PAD, LANES), F32)
    for ref in (wa, wb):
        ref[0:RC, :] = jnp.zeros((RC, LANES), BF16)
    for c in range(stt.shape[0]):
        stt[c, 0:8, :] = jnp.zeros((8, LANES), U32)
    zero[0] = 0

    class Deadline:
        def __init__(self, probe=None, lag=0):
            self.probe, self.queue = probe, [None] * lag
            self.zero = jnp.full((8, LANES), zero[0], jnp.int32).astype(U32)

        def after(self, y):
            return pltpu.bitcast(y[0:8, 0:LANES], U32) & self.zero

        def __call__(self, w):
            self.queue.append(self.probe() & self.zero)
            z = self.queue.pop(0)
            if z is None:
                return w
            return _cat([_cat([w[0:8, 0:LANES] | z, w[8:, 0:LANES]], 0), w[:, LANES:]], 1)

    def norm_in(i, slot, r, z):
        a = []
        for half in range(2):
            rr = pl.ds(pl.multiple_of(i * TM1 + half * h1 + r, RC), RC)
            m, d, v = _moments(xbuf[rr, :].astype(F32), z)
            q = lax.rsqrt(v + EPS)
            stat[0, rr, :] = jnp.broadcast_to(m, (RC, LANES))
            stat[1, rr, :] = jnp.broadcast_to(q, (RC, LANES))
            a.append(d * (0.5 * q * lax.rsqrt(v * q * q + EPS)))
        for _ in range(3):
            yield
        for k, f in enumerate(_left(a[0][:, :Dk], a[0][:, Dk:], a[1][:, :Dk], a[1][:, Dk:])):
            for n in range(nh):
                lf[slot, k, n, pl.ds(r, RC), :] = f[:, cols(n)].astype(BF16)
            if k in (1, 4):
                yield

    def normed(rr):
        m, q = (_cat([stat[k, rr, :]] * nd, 1) for k in range(2))
        return (xbuf[rr, :].astype(F32) - m) * q

    def norm_first(q, carry):
        _run([part(norm_in, 0, 0, pl.multiple_of((4 * q + e) * RC, RC)) for e in range(4)], 4)
        return carry

    def prep1(n, carry):
        o = pl.multiple_of(raw[1] + n * Dk, Dk)
        src, dst = view(wa, o, (nh + 1) * Dk), view(wb, o_w4 + n * 7 * wk, 7 * wk)
        w_wait(n, (o, Dk), (o + nh * Dk, Dk))

        def job(r, _):
            w = [words(src, e + r, 8) for e in (0, nh * Dk, wk, nh * Dk + wk)]
            z = yield
            for k, f in enumerate(_right(*[_widen(x, z) for x in w])):
                put(dst, k * wk + r, f)

        _run([part(job, r) for r in range(0, wk, 8)], 2)
        return carry

    def b1(i, carry):
        @pl.when(i + 1 < nb1)
        def _():
            x_copy(i + 1).wait()

        r0 = pl.multiple_of(i * TM1, TM1)
        nxt = jnp.minimum(i + 1, nb1 - 1)
        fill = _Filler(7 * nh - 3, [part(norm_in, nxt, (i + 1) % 2, r) for r in range(0, h1, RC)])
        due = Deadline()

        def prod(n, k):
            w = lf.bitcast(U32)
            y = _dot(_halves(_cat([w[i % 2, k, c] for c in range(nh)], 1)), weights(wb, o_w4 + (n * 7 + k) * wk, wk))
            fill(due.after(y))
            return y

        for n in range(nh):
            for k, y in enumerate(_combine(part(prod, n))):
                hs[n + k % 2 * nh, pl.ds(r0 + PAD + k // 2 * h1, h1), :] = _gelu_of_twice(y)
        fill.finish()
        start_later(i, 0, nb1)
        return carry

    for c in first:
        c.wait()
    for n in range(nh // 2, nh):
        w_copy(1, n).start()
        w_copy(1, n + nh).start()
    lax.fori_loop(0, h1 // (4 * RC), norm_first, 0)
    x_copy(1).start()
    lax.fori_loop(0, nh, prep1, 0)
    x_copy(2).start()
    x_copy(3).start()
    mem_copy = pltpu.make_async_copy(mem0_hbm, mem0, sem_x.at[nb1])
    mem_copy.start()
    lax.fori_loop(0, nb1, b1, 0)

    shifts = (-1, 1, -2, 2)
    BK = 32
    HB = 64
    per = nf * (wq // BK) // (nb1 // 2)

    def prep34(second, u):
        src = jnp.where(second, raw[4] + u // (nf * rq // BK) * (F // 2) + u % (nf * rq // BK) * BK,
                        raw[3] + u // (wq // BK) * Dk + u % (wq // BK) * BK).astype(jnp.int32)
        src = [view(wa, src + k * jnp.where(second, nf * rq, wq), 3 * F + BK) for k in range(4)]
        dst = view(wb, jnp.where(second, o_w4, o_w3) + u.astype(jnp.int32) * BK, 48 * fp + BK)

        def job(r, z):
            def quarter(a, b):
                return _Blocks(_widen(words(src[2 * a + k], (2 * b + j) * F + r, 8), z if k == j else None)
                               for k in range(2) for j in range(2))

            for stage in ((1, 5, 3), (0, 4, 2, 6)):
                outer = _right(*[quarter(a, b) for a in range(2) for b in range(2)])
                for a in stage:
                    for b, f in enumerate(_right(*outer[a])):
                        put(dst, (7 * a + b) * fp + r, f)
                z = yield

        return [part(job, r) for r in range(0, BK, 8)]

    def b2(i, carry):
        for k in range(4):
            pl.when(i == k)(part(w_wait, nh + 1 + k, *[
                (raw[3] + j * F + 2 * k * Dk, min(2, nf - 2 * k) * Dk) for j in range(4)]))
        for e in range(2):
            pl.when(i == 4 + 2 * e)(part(w_wait, nh + 5 + e, *[
                (raw[4] + j * F + e * (F // 2), F // 2) for j in range(4)]))

        r0 = pl.multiple_of(i * TM1, TM1)
        jobs = [prep34(i >= nb1 // 2, (i.astype(U32) % (nb1 // 2)) * per + u) for u in range(per)]
        fill = _Filler(2 * nd * TM1 // HB - 6, sum(jobs, []))
        due = Deadline(lambda: words(wb, 0, 8), 4)

        def shifted(r):
            return [hs[n, pl.ds(r0 + PAD + r + shifts[n * 4 // nd], HB), :] for n in range(nd)]

        ahead = shifted(0)
        for r in range(0, TM1, HB):
            sh = ahead
            for c in range(nd):
                if c == nd - 2 and r + HB < TM1:
                    ahead = shifted(r + HB)
                y = None
                for k in range(0, nd, nh):
                    a = pltpu.bitcast(due(pltpu.bitcast(_cat(sh[k:k + nh], 1), U32)), F32)
                    p = _dot(a.astype(BF16), weights(wa, raw[2] + c * Dk + k * rq, nh * rq))
                    y = p if y is None else p + y
                    fill(due.after(y))
                hs[c, pl.ds(r0 + r, HB), :] = y
        fill.finish()
        start_later(i, nb1, 2 * nb1)
        return carry

    w_wait(nh, (raw[2], nd * Dk))
    lax.fori_loop(0, nb1, b2, 0)

    def norm_mid(i):
        def job(r, _):
            rr = pl.ds(pl.multiple_of(jnp.minimum(i, nb2 - 1) * TM2 + r, 8), 8)
            x1 = _cat([hs[n, rr, :] for n in range(nd)], 1) + normed(rr)
            y = x1 + xbuf[rr, :].astype(F32)
            z = yield
            for n in range(nd):
                hs[n, pl.ds(pl.multiple_of(i * TM2 + r, 8), 8), :] = y[:, cols(n)]
            _, d, v = _moments(x1, z)
            lt[r:r + 8, :] = d * (0.5 * lax.rsqrt(v + EPS))

        return [part(job, r) for r in range(0, TM2, 8)]

    def left_mid():
        def job(r, n, _):
            a = [[lt[u * q2 + r:u * q2 + r + RC, cols(2 * j + n)] for j in range(4)] for u in range(4)]
            for k, g in enumerate(_left2(a)):
                for b, f in enumerate(g):
                    ly[7 * k + b, n, r:r + RC, :] = f.astype(BF16)
                yield

        return [part(job, r, n) for r in range(0, q2, RC) for n in range(2)]

    def b3(i, carry):
        for buf in (stq, sto):
            pltpu.make_async_copy(buf.at[i % 2], buf.at[i % 2], sem_a.at[i % 2]).wait()

        dst_qkv = view(wa, o_qkv + i * (fpi // 2), (3 * ng * nk - 1) * wq + fpi // 2)
        dst_o = view(wa, o_wo + i * opi, (2 * nk - 1) * ng * rq + opi)
        stages = [range(8, 17), range(17, 26), range(0, 4), range(4, 8)]

        def turn(c, d, _):
            w = [stq.bitcast(U32)[i % 2, c, pl.ds(e * 8, 8), :] for e in range(2 * d, 2 * d + 4)]
            w[0] = w[0] | (yield)
            for e, x in enumerate(w):
                stt[c, pl.ds(e % 2 * 8 * tp + d + e // 2, 8, stride=tp), :] = x

        def prep_qkv(t, g, z):
            for stage in stages:
                def block(k, j):
                    r = heads(g)[j] // 2 * tp
                    return _cat([_unpack(stt[4 * t + k, r + e:r + e + 8, :], z)[j % 2] for e in (0, 8)], 0)

                for f in stage:
                    y = _signed_sum([(c, block(*key)) for key, c in _HK[f][1].items()])[1]
                    put(dst_qkv, ((t * ng + g) * nk + f) * wq, y)
                z = yield

        def prep_o(e, r, z):
            for stage in stages:
                for f in stage:
                    y = [(c, _widen(sto.bitcast(U32)[i % 2, k, 2 * j + e, r:r + 8, :], None if n else z))
                         for n, ((k, j), c) in enumerate(_HK[f][1].items())]
                    put(dst_o, (e * nk + f) * ng * rq + r, _signed_sum(y)[1])
                z = yield

        jobs = [part(prep_o, e, r) for e in range(2) for r in range(0, opi, 8)]
        jobs += [part(prep_qkv, t, g) for t in range(3) for g in range(ng)]
        r0 = pl.multiple_of(i * TM2, TM2)
        here = pl.ds(pl.multiple_of(zero[0], 8), 8)
        norm_slots = [k for k in range(49) if k // 7 in (3, 1)]
        prep_slots = norm_slots[3::3]
        fill = _Filler(nf * len(prep_slots) + 2 * 49 - 8, jobs)
        due = Deadline(lambda: words(wa, 0, 8), 5)
        fill_y = _Filler((nf - 1) * len(norm_slots), norm_mid(i + 1))
        due_y = Deadline(lambda: pltpu.bitcast(lt[here, 0:LANES], U32) | stt[zero[0], 0:8, :], 14)
        fill_t = _Filler((nf - 1) * len(norm_slots),
                         [part(turn, c, d) for c in range(12) for d in range(0, fpi, 2)])
        fill_z = _Filler(7 * 7, left_mid())
        due_z = Deadline(lambda: ly.bitcast(U32)[zero[0], 0, 0:8, :], 6)

        def up(p, k):
            w = ly.bitcast(U32)
            w = _cat([w[k, n] for n in range(2)], 1)
            if k in prep_slots:
                w = due(w)
            y = _dot(_halves(due_y(w) if k in norm_slots else w), weights(wb, o_w3 + k * fp + p * wq, wq))
            if k in norm_slots:
                z = due.after(y)
                fill_y(z)
                fill_t(z)
                if k in prep_slots:
                    fill(z)
            return y

        for p in range(nf):
            g = [[_gelu_of_twice(y) for y in row] for row in _combine2(part(up, p), _combine)]
            for a, group in enumerate(_left2(g)):
                for b, f in enumerate(group):
                    lz[7 * a + b, p] = f.astype(BF16)
        fill_y.finish()
        fill_t.finish()
        assert fill.done * len(jobs) // fill.slots <= 2 * opi // 8

        def down(e, k):
            w = lz.bitcast(U32)
            y = _dot(_halves(due_z(due(_cat([w[k, p] for p in range(nf)], 1)))),
                     weights(wb, o_w4 + k * fp + e * nf * rq, nf * rq))
            z = due.after(y)
            fill(z)
            fill_z(z)
            return y

        for e in range(2):
            for u, row in enumerate(_combine2(part(down, e), _combine_late)):
                for j, y in enumerate(row):
                    hs[2 * j + e, pl.ds(r0 + u * q2, q2), :] += y
        fill_z.finish()
        fill.finish()

        @pl.when(i + 2 < nb2)
        def _():
            for c in a_copies(i + 2):
                c.start()

        return carry

    _run(norm_mid(0), 2)
    _run(left_mid(), 1)
    lax.fori_loop(0, nb2, b3, 0)

    scale = Dh ** -0.5
    key = lax.broadcasted_iota(jnp.int32, (seg, L), 0) + M
    query = lax.broadcasted_iota(jnp.int32, (seg, L), 1)
    mask = (query < M) | (query >= key)
    QS = 4 * seg
    rv = (seg - M) // 8

    def upper(n):
        return lax.broadcasted_iota(jnp.int32, (8, n), 0) < 4

    def split8(mem, tok):
        u = upper(mem.shape[1])
        return jnp.where(u, mem, tok), pltpu.roll(jnp.where(u, tok, mem), 4, 0)

    def join8(t, b):
        u = upper(t.shape[1])
        b = pltpu.roll(b, 4, 0)
        return jnp.where(u, t, b), jnp.where(u, b, t)

    def vregs(y, lo, hi):
        return [y[8 * k:8 * k + 8] for k in range(lo, hi)]

    def left_operands(mem, tok, big):
        if not big:
            return _hk_left([_cat([m] + y, 0) for m, y in zip(mem, tok)])
        pairs = [split8(m, y[2 * rv]) for m, y in zip(mem, tok)]
        return _hk_left(*[[_cat([p[c]] + y[c * rv:(c + 1) * rv], 0) for p, y in zip(pairs, tok)] for c in range(2)])

    def rows_out(c):
        if len(c) == 1:
            return [(y[0:8], vregs(y, 1, 1 + rv)) for y in c[0]]
        got = []
        for y, w in zip(*c):
            ym, yt = join8(y[0:8], w[0:8])
            got.append((ym, vregs(y, 1, 1 + rv) + vregs(w, 1, 1 + rv) + [yt]))
        return got

    def probs(q, k):
        sc = _dot_nt(k, q.astype(BF16))
        sc = _cat([sc[0:M], jnp.where(mask, sc[M:L], -1e9 / scale)], 0)
        p = jnp.exp2((sc - jnp.max(sc, axis=0, keepdims=True)) * (scale * math.log2(math.e)))
        return p * _recip(jnp.sum(p, axis=0, keepdims=True))

    def out_copy(j):
        r0 = pl.multiple_of(j * QS, QS)
        return pltpu.make_async_copy(xbuf.at[pl.ds(r0, QS)], out_hbm.at[pl.ds(r0, QS)], sem_out.at[j])

    def quad(j, carry):
        xs = normed(pl.ds(pl.multiple_of(j * QS, QS), QS))
        qkv = {(t, h): [] for t in range(3) for h in range(H)}
        att = {h: [] for h in range(H)}
        outs = {n: [] for n in range(nd)}
        mem = membuf[...]
        for st in range(4):
            r, n_tok = (0, 2 * rv + 1) if st == 0 else ((st + 1) * rv + 1, rv)
            hl = left_operands([mem[:, cols(2 * k, 2)] for k in range(4)],
                               [vregs(xs[:, cols(2 * k, 2)], r, r + n_tok) for k in range(4)], st == 0)
            ol, cur, p, o = {}, {}, {}, {}

            def wq_part(t, g, lo, hi):
                return _hk_combine(hl, lambda f: _dot(
                    hl[f][1][:, lo:hi].astype(BF16),
                    weights(wa, o_qkv + ((t * ng + g) * nk + f) * wq + lo // 2, (hi - lo) // 2)))

            def wo_part(e, lo, hi):
                return _hk_combine(ol[lo], lambda f: _dot(
                    _cat([ol[g][f][1] for g in range(lo, hi)], 1).astype(BF16),
                    weights(wa, o_wo + ((e * nk + f) * ng + lo) * rq, (hi - lo) * rq)))

            def stash(q, c):
                for a, blocks in enumerate(c):
                    for b, y in enumerate(blocks):
                        pbuf[st, q, a, b] = y

            def resume(q, c):
                return [[pbuf[st, q, a, b] + y for b, y in enumerate(blocks)] for a, blocks in enumerate(c)]

            def proj(t, g):
                if g == 0 and st > 0 and t < 2:
                    c = resume(2 + t, wq_part(t, g, LANES, 2 * LANES))
                else:
                    c = wq_part(t, g, 0, 2 * LANES)
                got = []
                for h, (ym, yt) in zip(heads(g), rows_out(c)):
                    qkv[t, h] += yt
                    got.append(_cat([ym] + qkv[t, h][4 * st:4 * st + 4], 0))
                return got

            def attend(g, c):
                for e in (2 * c, 2 * c + 1):
                    if 0 <= g < ng:
                        p[g, e] = probs(cur[0, g][e], cur[1, g][e])
                if g > 0:
                    for e in (2 * c, 2 * c + 1):
                        o[e] = _dot(p[g - 1, e].T, cur[2, g - 1][e].astype(BF16))
                        att[heads(g - 1)[e]] += vregs(o[e], 1, 5)
                    if c:
                        ol[g - 1] = left_operands(
                            [o[e][0:8] for e in range(4)],
                            [att[h][st * rv:None if st == 3 else (st + 1) * rv] for h in heads(g - 1)], st == 3)

            if st > 0:
                for t in range(2):
                    stash(2 + t, wq_part(t, 0, 0, LANES))
            for g in range(ng):
                cur[0, g] = proj(0, g)
                cur[1, g] = proj(1, g)
                attend(g - 1, 1)
                cur[2, g] = proj(2, g)
                attend(g, 0)
            stash(0, wo_part(0, 0, 2))
            attend(ng - 1, 1)
            stash(1, wo_part(1, 0, 2))
            attend(ng, 0)
            stash(0, resume(0, wo_part(0, 2, 4)))
            attend(ng, 1)
            stash(1, resume(1, wo_part(1, 2, 4)))
            new = {}
            for e in range(2):
                for c, (ym, yt) in enumerate(rows_out(resume(e, wo_part(e, 4, ng)))):
                    new[2 * c + e] = ym
                    outs[2 * c + e] += yt
            mem = _cat([new[n] for n in range(nd)], 1)
            lo, hi = ((0, 2), (2, 6), (6, 8), (8, 16))[st]
            rr = pl.ds(pl.multiple_of(j * QS + 8 * lo, RC), 8 * (hi - lo))
            for n in range(nd):
                xbuf[rr, cols(n)] = (hs[n, rr, :] + _cat(outs[n][lo:hi], 0)).astype(BF16)
        membuf[...] = mem
        out_copy(j).start()
        return carry

    mem_copy.wait()
    membuf[...] = mem0[...].astype(F32)
    lax.fori_loop(0, S // QS, quad, 0)
    for j in range(S // QS):
        out_copy(j).wait()


@functools.partial(jax.jit, static_argnames=("A_seg_len",))
def pallas_parallel_sum__memory_aug_recurrent_mem_tr__mixer_s_mlp__prompt_kernel(
    A_x: jax.Array,
    A_mem0: jax.Array,
    A_Wq: jax.Array,
    A_Wk: jax.Array,
    A_Wv: jax.Array,
    A_Wo: jax.Array,
    A_seg_len: int,
    B_x: jax.Array,
    B_w1: jax.Array,
    B_w2: jax.Array,
    B_w3: jax.Array,
    B_w4: jax.Array,
):
    del B_x
    B, S, D = A_x.shape
    _, H, Dh = A_Wq.shape
    M = A_mem0.shape[1]
    seg = int(A_seg_len)
    F = B_w3.shape[1]
    assert (B, S, D, H, Dh, M, seg, F) == (1, 2048, 1024, 32, LANES, 8, 32, 3584)
    TM1, TM2 = 256, 128
    nd, nf, nk, nb2 = D // LANES, F // (4 * LANES), len(_HK), S // TM2

    hbm = pl.BlockSpec(memory_space=pl.ANY)
    dma = pltpu.SemaphoreType.DMA
    out = pl.pallas_call(
        functools.partial(_kernel, S=S, D=D, H=H, Dh=Dh, M=M, seg=seg, F=F, TM1=TM1, TM2=TM2),
        out_shape=jax.ShapeDtypeStruct((S, D), BF16),
        in_specs=[hbm] * 10,
        out_specs=hbm,
        scratch_shapes=[
            pltpu.VMEM((S, D), BF16),
            pltpu.VMEM((2, S, LANES), F32),
            pltpu.VMEM((nd, S + TM2, LANES), F32),
            pltpu.VMEM((2, 7, nd // 2, TM1 // 2, LANES), BF16),
            pltpu.VMEM((TM2, D), F32),
            pltpu.VMEM((49, nd // 4, TM2 // 4, LANES), BF16),
            pltpu.VMEM((49, nf, TM2 // 4, LANES), BF16),
            pltpu.VMEM((H * nk * D // 4, LANES), BF16),
            pltpu.VMEM((4 * 49 * (nf * D // 8 + 8), LANES), BF16),
            pltpu.SMEM((1,), jnp.int32),
            pltpu.VMEM((2, 12, (D // 4 // nb2) * H, LANES), BF16),
            pltpu.VMEM((12, (H // 2 + 2) * (D // 4 // nb2 + 4), LANES), U32),
            pltpu.VMEM((2, 4, nd, H * Dh // (4 * nb2), LANES), BF16),
            pltpu.VMEM((M, D), BF16),
            pltpu.VMEM((M, D), F32),
            pltpu.VMEM((4, 4, 2, 4, seg, LANES), F32),
            dma((S // TM1 + 1,)), dma((nd // 2 + 7,)), dma((2,)), dma((S // (4 * seg),)),
        ],
        compiler_params=pltpu.CompilerParams(
            vmem_limit_bytes=128 * 1024 * 1024, disable_bounds_checks=True, disable_semaphore_checks=True),
        name="rmt_s2mlp",
    )(A_x.reshape(S, D), A_mem0.reshape(M, D),
      A_Wq.reshape(D * H, Dh), A_Wk.reshape(D * H, Dh), A_Wv.reshape(D * H, Dh),
      A_Wo.reshape(H * Dh, D), B_w1, B_w2, B_w3, B_w4)
    return out.reshape(B, S, D)
```

```python
import functools
import math

import jax
import jax.numpy as jnp
from jax import lax
import jax.experimental.pallas as pl
import jax.experimental.pallas.tpu as pltpu

F32 = jnp.float32
BF16 = jnp.bfloat16
U32 = jnp.uint32
LANES = 128
EPS = 1e-5
PAD = 8


def _dot(a, b):
    return lax.dot_general(a, b, (((1,), (0,)), ((), ())), preferred_element_type=F32)


def _dot_nt(a, b):
    return lax.dot_general(a, b, (((1,), (1,)), ((), ())), preferred_element_type=F32)


def _cat(xs, axis):
    return xs[0] if len(xs) == 1 else jnp.concatenate(xs, axis=axis)


def _moments(x, z):
    s = _cat([pltpu.bitcast(z, F32)] * (x.shape[0] // 8), 0)
    for c in range(0, x.shape[1], LANES):
        s = s + x[:, c:c + LANES]
    m = jnp.sum(s, axis=-1, keepdims=True) * (1.0 / x.shape[1])
    d = x - m
    return m, d, jnp.mean(d * d, axis=-1, keepdims=True)


def _recip(x):
    r = pl.reciprocal(x, approx=True)
    return r * (2.0 - x * r)


def _gelu_of_twice(h):
    c = math.sqrt(2.0 / math.pi)
    return h + h * jnp.tanh(h * (2.0 * c + (8.0 * c * 0.044715) * (h * h)))


def _halves(w):
    return pltpu.bitcast(w, BF16)


def _unpack(w, z):
    return pltpu.bitcast(w << (z | 16), F32), pltpu.bitcast(w & (z | U32(0xFFFF0000)), F32)


def _widen(w, z):
    return _halves(w if z is None else w | z).astype(F32)


def _left(a11, a12, a21, a22):
    return (a11 + a22, a21 + a22, a11, a22, a11 + a12, a21 - a11, a12 - a22)


def _right(b11, b12, b21, b22):
    return (b11 + b22, b11, b12 - b22, b21 - b11, b22, b11 + b12, b21 + b22)


def _combine(m):
    m4 = m(3)
    m2 = m(1)
    c21 = m2 + m4
    m1 = m(0)
    c22 = m1 - m2
    c11 = m1 + m4
    c11 = c11 + m(6)
    m5 = m(4)
    c11 = c11 - m5
    m3 = m(2)
    c12 = m3 + m5
    c22 = c22 + m3
    c22 = c22 + m(5)
    return c11, c12, c21, c22


def _combine_late(m):
    m3 = m(2)
    m5 = m(4)
    c12 = m3 + m5
    c22 = m3 + m(5)
    m1 = m(0)
    c11 = m1 - m5
    c22 = c22 + m1
    m2 = m(1)
    c22 = c22 - m2
    m4 = m(3)
    c21 = m2 + m4
    c11 = c11 + m4
    c11 = c11 + m(6)
    return c11, c12, c21, c22


class _Blocks(tuple):
    def __add__(self, other):
        return _Blocks(a + b for a, b in zip(self, other))

    def __sub__(self, other):
        return _Blocks(a - b for a, b in zip(self, other))


def _left2(a):
    nested = [_Blocks(a[2 * i + u][2 * j + w] for u in range(2) for w in range(2))
              for i in range(2) for j in range(2)]
    return (_left(*g) for g in _left(*nested))


def _combine2(m, outer):
    c = outer(lambda a: _Blocks(_combine(lambda b: m(7 * a + b))))
    return [[c[2 * (i // 2) + j // 2][2 * (i % 2) + j % 2] for j in range(4)] for i in range(4)]


def _hopcroft_kerr(types):
    n = len(types)
    prods = []

    def add(left, out):
        prods.append((left, {}, out))
        return len(prods) - 1

    def use(block, terms):
        for f, s in terms:
            prods[f][1][block] = prods[f][1].get(block, 0) + s

    class Node:
        def __init__(self, t, xs, ys, plus, minus):
            self.t, self.xs, self.ys, self.plus, self.minus = t, xs, ys, plus, minus

    def mix(*parts):
        return {(i, t % 3): s * c for d, t, s in parts for i, c in d.items()}

    def pair(u, w):
        if (u.t - w.t) % 3 != 1:
            zwu, zuw, free = pair(w, u)
            return zuw, zwu, free
        t = u.t
        s = add(mix((u.xs, t + 2, 1), (w.xs, t, 1)), mix((u.ys, t + 2, 1), (w.ys, t, -1)))
        o1 = add(mix((u.xs, t, -1), (w.xs, t, 1)), mix((u.ys, t + 2, 1), (w.ys, t + 2, 1)))
        o2 = add(mix((u.xs, t + 2, -1), (w.xs, t + 2, 1)), mix((u.ys, t, 1), (w.ys, t, 1)))
        free = Node((t + 1) % 3, {**{i: -c for i, c in u.xs.items()}, **w.xs}, {**u.ys, **w.ys}, o1, o2)
        return ([(s, 1), (o1, -1), (u.minus, 1), (w.minus, -1)],
                [(s, 1), (o2, -1), (u.plus, 1), (w.plus, -1)], free)

    nodes = []
    for i, t in enumerate(types):
        e = {i: 1}
        nodes.append(Node(t, e, e, add(mix((e, t + 2, 1)), mix((e, t + 1, 1))),
                          add(mix((e, t + 1, 1)), mix((e, t + 2, 1)))))
        use((i, i), [(nodes[i].plus, 1), (nodes[i].minus, -1)])
    z, free = {}, {}
    for i in range(n):
        for j in range(i + 1, n):
            if types[i] != types[j]:
                z[i, j], z[j, i], free[i, j] = pair(nodes[i], nodes[j])
                free[j, i] = free[i, j]
    for i in range(n):
        for j in range(i + 1, n):
            if types[i] == types[j]:
                k = next(k for k in range(n) if types[k] != types[i])
                w = free[i, k]
                zwj, zjw, _ = pair(w, nodes[j])
                z[i, j] = [(f, w.xs[i] * c) for f, c in zwj] + z[k, j]
                z[j, i] = zjw + [(f, -c) for f, c in z[j, k]]
    for block, terms in z.items():
        use(block, terms)
    return [(left, {k: c for k, c in right.items() if c}, out) for left, right, out in prods]


def _signed_sum(terms):
    terms = sorted(terms, key=lambda t: -t[0])
    sign, y = terms[0]
    for s, x in terms[1:]:
        y = y + x if s == sign else y - x
    return sign, y


def _signed_value(terms):
    sign, y = _signed_sum(terms)
    return y if sign > 0 else -y


_HK = _hopcroft_kerr((0, 1, 2, 0))
_HK_ROW = [f for f, (left, _, out) in enumerate(_HK)
           if any(t != 2 for _, t in left) and any(t != 0 for _, t in out)]
_HK_RIGHT_SIGN = [_signed_sum([(c, 0) for c in right.values()])[0] for _, right, _ in _HK]


def _hk_left(upper, lower=None):
    if lower is None:
        base = [((1, u), (-1, u), None) for u in upper]
    else:
        base = [((1, u), (1, w), (-1, u + w)) for u, w in zip(upper, lower)]
    return {f: _signed_sum([(c * base[i][t][0], base[i][t][1]) for (i, t), c in _HK[f][0].items() if base[i][t]])
            for f in (_HK_ROW if lower is None else range(len(_HK)))}


def _hk_columns(f):
    js = [j for j, _ in _HK[f][2]]
    return min(js), max(js), f


def _hk_combine(left, m, midway=None):
    both = len(left) == len(_HK)
    acc = {}
    for n, f in enumerate(sorted(left, key=_hk_columns)):
        y = m(f)
        if midway and n + 1 == len(left) * 3 // 4:
            midway()
        for (j, t), c in _HK[f][2].items():
            c *= left[f][0] * _HK_RIGHT_SIGN[f]
            if both:
                acc[j, t] = _signed_sum([acc[j, t], (c, y)]) if (j, t) in acc else (c, y)
            elif t:
                c *= (0, -1, 1)[t]
                acc[j] = _signed_sum([acc[j], (c, y)]) if j in acc else (c, y)
    if not both:
        return [[_signed_value([acc[j]]) for j in range(4)]]
    return [[_signed_value([acc[j, p], (-acc[j, q][0], acc[j, q][1])]) for j in range(4)]
            for p, q in ((2, 1), (0, 2))]


class _Filler:
    def __init__(self, slots, jobs):
        self.slots, self.done, self.jobs, self.live = slots, 0, jobs, []

    def __call__(self, z):
        def step(g, v):
            try:
                g.send(v)
                return True
            except StopIteration:
                return False

        n = len(self.jobs)
        new = [job(z) for job in self.jobs[self.done * n // self.slots:(self.done + 1) * n // self.slots]]
        self.live = [g for g in new if step(g, None)] + [g for g in self.live if step(g, z)]
        self.done += 1

    def finish(self):
        while self.live or self.done < self.slots:
            self(jnp.zeros((8, LANES), U32))


def _run(jobs, group):
    _Filler(len(jobs) // group, jobs).finish()


def _kernel(x_hbm, mem0_hbm, wq_hbm, wk_hbm, wv_hbm, wo_hbm, w1_hbm, w2_hbm, w3_hbm, w4_hbm,
            out_hbm,
            xbuf, stat, hs, lf, lt, ly, lz, wa, wb, zero, stq, stt, sto, mem0, membuf, pbuf,
            sem_x, sem_w, sem_a, sem_out,
            *, S, D, H, Dh, M, seg, F, TM1, TM2):
    part = functools.partial
    L = M + seg
    nd = D // LANES
    nh = nd // 2
    Dk = D // 2
    rq = LANES // 2
    wk = Dk // 2
    wq = wk // 2
    nf = F // (4 * LANES)
    hp = H // 2
    ng = H // 4
    nk = len(_HK)
    nb1, nb2 = S // TM1, S // TM2
    h1, q2 = TM1 // 2, TM2 // 4
    RC = 16

    def cols(n, w=1):
        return slice(n * LANES, (n + w) * LANES)

    def heads(g):
        return [2 * g, 2 * g + 1, hp + 2 * g, hp + 2 * g + 1]

    fp = nf * wq + 8
    o_w3 = 0
    o_w4 = o_w3 + 49 * fp
    o_wo = 0
    o_qkv = o_wo + 2 * nk * ng * rq
    raw = {1: o_qkv, 2: o_qkv + nd * Dk, 3: o_qkv + 2 * nd * Dk, 4: o_qkv + 2 * nd * Dk + 4 * F}

    def words(ref, r0, rows):
        return ref.bitcast(U32)[pl.ds(r0, rows), :]

    def weights(ref, r0, rows):
        return _halves(words(ref, r0, rows))

    def view(ref, r0, rows):
        return ref.at[pl.ds(pl.multiple_of(2 * r0, RC), 2 * rows)]

    def put(ref, r, y):
        ref[2 * r:2 * r + RC, :] = y.astype(BF16)

    def w_copy(j, n):
        src, rows, sem = {1: (w1_hbm, Dk, n % nh), 2: (w2_hbm, Dk, nh),
                          3: (w3_hbm, Dk, nh + 1 + n % nf // 2), 4: (w4_hbm, F // 2, nh + 5 + n % 2)}[j]
        return pltpu.make_async_copy(src.at[:, cols(n)], wa.at[pl.ds(2 * (raw[j] + n * rows), 2 * rows)],
                                     sem_w.at[sem])

    def w_wait(sem, *spans):
        for r0, rows in spans:
            span = wa.at[pl.ds(2 * r0, 2 * rows)]
            pltpu.make_async_copy(span, span, sem_w.at[sem]).wait()

    def w3_copies(lo, hi):
        return [w_copy(3, p + j * nf) for p in range(lo, hi) for j in range(4)]

    def x_copy(i):
        r0 = pl.multiple_of(i * TM1, TM1)
        return pltpu.make_async_copy(x_hbm.at[pl.ds(r0, TM1)], xbuf.at[pl.ds(r0, TM1)], sem_x.at[i])

    fpi = D // 4 // nb2
    opi = ng * rq // nb2
    tp = fpi + 4

    def a_copies(i):
        cps = []
        for t, src in enumerate((wq_hbm, wk_hbm, wv_hbm)):
            for k in range(4):
                r0 = pl.multiple_of((k * (D // 4) + i * fpi) * H, fpi * H)
                cps.append(pltpu.make_async_copy(src.at[pl.ds(r0, fpi * H)],
                                                 stq.at[i % 2, 4 * t + k], sem_a.at[i % 2]))
        for k, h in enumerate(heads(i // (rq // opi))):
            r0 = pl.multiple_of(2 * (h * rq + i % (rq // opi) * opi), 2 * opi)
            for n in range(nd):
                cps.append(pltpu.make_async_copy(wo_hbm.at[pl.ds(r0, 2 * opi), cols(n)],
                                                 sto.at[i % 2, k, n], sem_a.at[i % 2]))
        return cps

    later = [
        lambda: [x_copy(4)] + [w_copy(2, n) for n in range(nh)],
        lambda: [x_copy(5)] + [w_copy(2, n) for n in range(nh, nd)],
        lambda: [x_copy(6)] + w3_copies(0, 1),
        lambda: [x_copy(7)] + w3_copies(1, 2),
        lambda: w3_copies(2, 3),
        lambda: w3_copies(3, 4),
        lambda: w3_copies(4, 6),
        lambda: w3_copies(6, 7),
        lambda: [w_copy(4, 0), w_copy(4, 2)],
        lambda: [w_copy(4, 4), w_copy(4, 6)],
        lambda: [w_copy(4, 1), w_copy(4, 3)],
        lambda: [w_copy(4, 5), w_copy(4, 7)],
        lambda: a_copies(0),
        lambda: a_copies(1),
    ]

    def start_later(i, lo, hi):
        for k in range(lo, min(hi, len(later))):
            @pl.when(i == k - lo)
            def _(k=k):
                for c in later[k]():
                    c.start()

    first = [pltpu.make_async_copy(x_hbm.at[pl.ds(r, TM1 // 8)], xbuf.at[pl.ds(r, TM1 // 8)], sem_x.at[0])
             for r in range(0, TM1, TM1 // 8)]
    for c in first:
        c.start()
    for n in range(nh // 2):
        w_copy(1, n).start()
        w_copy(1, n + nh).start()

    for n in range(nd):
        hs[n, 0:PAD, :] = jnp.zeros((PAD, LANES), F32)
        hs[n, PAD + S:PAD + S + PAD, :] = jnp.zeros((PAD, LANES), F32)
    for ref in (wa, wb):
        ref[0:RC, :] = jnp.zeros((RC, LANES), BF16)
    for c in range(stt.shape[0]):
        stt[c, 0:8, :] = jnp.zeros((8, LANES), U32)
    zero[0] = 0

    class Deadline:
        def __init__(self, probe=None, lag=0):
            self.probe, self.queue = probe, [None] * lag
            self.zero = jnp.full((8, LANES), zero[0], jnp.int32).astype(U32)

        def after(self, y):
            return pltpu.bitcast(y[0:8, 0:LANES], U32) & self.zero

        def __call__(self, w):
            self.queue.append(self.probe() & self.zero)
            z = self.queue.pop(0)
            if z is None:
                return w
            return _cat([_cat([w[0:8, 0:LANES] | z, w[8:, 0:LANES]], 0), w[:, LANES:]], 1)

    def norm_in(i, slot, r, z):
        a = []
        for half in range(2):
            rr = pl.ds(pl.multiple_of(i * TM1 + half * h1 + r, RC), RC)
            m, d, v = _moments(xbuf[rr, :].astype(F32), z)
            q = lax.rsqrt(v + EPS)
            stat[0, rr, :] = jnp.broadcast_to(m, (RC, LANES))
            stat[1, rr, :] = jnp.broadcast_to(q, (RC, LANES))
            a.append(d * (0.5 * q * lax.rsqrt(v * q * q + EPS)))
        for _ in range(3):
            yield
        for k, f in enumerate(_left(a[0][:, :Dk], a[0][:, Dk:], a[1][:, :Dk], a[1][:, Dk:])):
            for n in range(nh):
                lf[slot, k, n, pl.ds(r, RC), :] = f[:, cols(n)].astype(BF16)
            if k in (1, 4):
                yield

    def normed(rr):
        m, q = (_cat([stat[k, rr, :]] * nd, 1) for k in range(2))
        return (xbuf[rr, :].astype(F32) - m) * q

    def norm_first(q, carry):
        _run([part(norm_in, 0, 0, pl.multiple_of((4 * q + e) * RC, RC)) for e in range(4)], 4)
        return carry

    def prep1(n, carry):
        o = pl.multiple_of(raw[1] + n * Dk, Dk)
        src, dst = view(wa, o, (nh + 1) * Dk), view(wb, o_w4 + n * 7 * wk, 7 * wk)
        w_wait(n, (o, Dk), (o + nh * Dk, Dk))

        def job(r, _):
            w = [words(src, e + r, 8) for e in (0, nh * Dk, wk, nh * Dk + wk)]
            z = yield
            for k, f in enumerate(_right(*[_widen(x, z) for x in w])):
                put(dst, k * wk + r, f)

        _run([part(job, r) for r in range(0, wk, 8)], 2)
        return carry

    def b1(i, carry):
        @pl.when(i + 1 < nb1)
        def _():
            x_copy(i + 1).wait()

        r0 = pl.multiple_of(i * TM1, TM1)
        nxt = jnp.minimum(i + 1, nb1 - 1)
        fill = _Filler(7 * nh - 3, [part(norm_in, nxt, (i + 1) % 2, r) for r in range(0, h1, RC)])
        due = Deadline()

        def prod(n, k):
            w = lf.bitcast(U32)
            y = _dot(_halves(_cat([w[i % 2, k, c] for c in range(nh)], 1)), weights(wb, o_w4 + (n * 7 + k) * wk, wk))
            fill(due.after(y))
            return y

        for n in range(nh):
            for k, y in enumerate(_combine(part(prod, n))):
                hs[n + k % 2 * nh, pl.ds(r0 + PAD + k // 2 * h1, h1), :] = _gelu_of_twice(y)
        fill.finish()
        start_later(i, 0, nb1)
        return carry

    for c in first:
        c.wait()
    for n in range(nh // 2, nh):
        w_copy(1, n).start()
        w_copy(1, n + nh).start()
    lax.fori_loop(0, h1 // (4 * RC), norm_first, 0)
    x_copy(1).start()
    lax.fori_loop(0, nh, prep1, 0)
    x_copy(2).start()
    x_copy(3).start()
    mem_copy = pltpu.make_async_copy(mem0_hbm, mem0, sem_x.at[nb1])
    mem_copy.start()
    lax.fori_loop(0, nb1, b1, 0)

    shifts = (-1, 1, -2, 2)
    BK = 32
    HB = 64
    per = nf * (wq // BK) // (nb1 // 2)

    def prep34(second, u):
        src = jnp.where(second, raw[4] + u // (nf * rq // BK) * (F // 2) + u % (nf * rq // BK) * BK,
                        raw[3] + u // (wq // BK) * Dk + u % (wq // BK) * BK).astype(jnp.int32)
        src = [view(wa, src + k * jnp.where(second, nf * rq, wq), 3 * F + BK) for k in range(4)]
        dst = view(wb, jnp.where(second, o_w4, o_w3) + u.astype(jnp.int32) * BK, 48 * fp + BK)

        def job(r, z):
            def quarter(a, b):
                return _Blocks(_widen(words(src[2 * a + k], (2 * b + j) * F + r, 8), z if k == j else None)
                               for k in range(2) for j in range(2))

            for stage in ((1, 5, 3), (0, 4, 2, 6)):
                outer = _right(*[quarter(a, b) for a in range(2) for b in range(2)])
                for a in stage:
                    for b, f in enumerate(_right(*outer[a])):
                        put(dst, (7 * a + b) * fp + r, f)
                z = yield

        return [part(job, r) for r in range(0, BK, 8)]

    def b2(i, carry):
        for k in range(4):
            pl.when(i == k)(part(w_wait, nh + 1 + k, *[
                (raw[3] + j * F + 2 * k * Dk, min(2, nf - 2 * k) * Dk) for j in range(4)]))
        for e in range(2):
            pl.when(i == 4 + 2 * e)(part(w_wait, nh + 5 + e, *[
                (raw[4] + j * F + e * (F // 2), F // 2) for j in range(4)]))

        r0 = pl.multiple_of(i * TM1, TM1)
        jobs = [prep34(i >= nb1 // 2, (i.astype(U32) % (nb1 // 2)) * per + u) for u in range(per)]
        fill = _Filler(2 * nd * TM1 // HB - 6, sum(jobs, []))
        due = Deadline(lambda: words(wb, 0, 8), 4)

        def shifted(r):
            return [hs[n, pl.ds(r0 + PAD + r + shifts[n * 4 // nd], HB), :] for n in range(nd)]

        ahead = shifted(0)
        for r in range(0, TM1, HB):
            sh = ahead
            for c in range(nd):
                if c == nd - 2 and r + HB < TM1:
                    ahead = shifted(r + HB)
                y = None
                for k in range(0, nd, nh):
                    a = pltpu.bitcast(due(pltpu.bitcast(_cat(sh[k:k + nh], 1), U32)), F32)
                    p = _dot(a.astype(BF16), weights(wa, raw[2] + c * Dk + k * rq, nh * rq))
                    y = p if y is None else p + y
                    fill(due.after(y))
                hs[c, pl.ds(r0 + r, HB), :] = y
        fill.finish()
        start_later(i, nb1, 2 * nb1)
        return carry

    w_wait(nh, (raw[2], nd * Dk))
    lax.fori_loop(0, nb1, b2, 0)

    def norm_mid(i):
        def job(r, _):
            rr = pl.ds(pl.multiple_of(jnp.minimum(i, nb2 - 1) * TM2 + r, 8), 8)
            x1 = _cat([hs[n, rr, :] for n in range(nd)], 1) + normed(rr)
            y = x1 + xbuf[rr, :].astype(F32)
            z = yield
            for n in range(nd):
                hs[n, pl.ds(pl.multiple_of(i * TM2 + r, 8), 8), :] = y[:, cols(n)]
            _, d, v = _moments(x1, z)
            lt[r:r + 8, :] = d * (0.5 * lax.rsqrt(v + EPS))

        return [part(job, r) for r in range(0, TM2, 8)]

    def left_mid():
        def job(r, n, _):
            a = [[lt[u * q2 + r:u * q2 + r + RC, cols(2 * j + n)] for j in range(4)] for u in range(4)]
            for k, g in enumerate(_left2(a)):
                for b, f in enumerate(g):
                    ly[7 * k + b, n, r:r + RC, :] = f.astype(BF16)
                yield

        return [part(job, r, n) for r in range(0, q2, RC) for n in range(2)]

    def b3(i, carry):
        for buf in (stq, sto):
            pltpu.make_async_copy(buf.at[i % 2], buf.at[i % 2], sem_a.at[i % 2]).wait()

        dst_qkv = view(wa, o_qkv + i * (fpi // 2), (3 * ng * nk - 1) * wq + fpi // 2)
        dst_o = view(wa, o_wo + i * opi, (2 * nk - 1) * ng * rq + opi)
        stages = [range(8, 17), range(17, 26), range(0, 4), range(4, 8)]

        def turn(c, d, _):
            w = [stq.bitcast(U32)[i % 2, c, pl.ds(e * 8, 8), :] for e in range(2 * d, 2 * d + 4)]
            w[0] = w[0] | (yield)
            for e, x in enumerate(w):
                stt[c, pl.ds(e % 2 * 8 * tp + d + e // 2, 8, stride=tp), :] = x

        def prep_qkv(t, g, z):
            for stage in stages:
                def block(k, j):
                    r = heads(g)[j] // 2 * tp
                    return _cat([_unpack(stt[4 * t + k, r + e:r + e + 8, :], z)[j % 2] for e in (0, 8)], 0)

                for f in stage:
                    y = _signed_sum([(c, block(*key)) for key, c in _HK[f][1].items()])[1]
                    put(dst_qkv, ((t * ng + g) * nk + f) * wq, y)
                z = yield

        def prep_o(e, r, z):
            for stage in stages:
                for f in stage:
                    y = [(c, _widen(sto.bitcast(U32)[i % 2, k, 2 * j + e, r:r + 8, :], None if n else z))
                         for n, ((k, j), c) in enumerate(_HK[f][1].items())]
                    put(dst_o, (e * nk + f) * ng * rq + r, _signed_sum(y)[1])
                z = yield

        jobs = [part(prep_o, e, r) for e in range(2) for r in range(0, opi, 8)]
        jobs += [part(prep_qkv, t, g) for t in range(3) for g in range(ng)]
        r0 = pl.multiple_of(i * TM2, TM2)
        here = pl.ds(pl.multiple_of(zero[0], 8), 8)
        norm_slots = [k for k in range(49) if k // 7 in (3, 1)]
        prep_slots = norm_slots[3::3]
        fill = _Filler(nf * len(prep_slots) + 2 * 49 - 8, jobs)
        due = Deadline(lambda: words(wa, 0, 8), 5)
        fill_y = _Filler((nf - 1) * len(norm_slots), norm_mid(i + 1))
        due_y = Deadline(lambda: pltpu.bitcast(lt[here, 0:LANES], U32) | stt[zero[0], 0:8, :], 14)
        fill_t = _Filler((nf - 1) * len(norm_slots),
                         [part(turn, c, d) for c in range(12) for d in range(0, fpi, 2)])
        fill_z = _Filler(7 * 7, left_mid())
        due_z = Deadline(lambda: ly.bitcast(U32)[zero[0], 0, 0:8, :], 6)

        def up(p, k):
            w = ly.bitcast(U32)
            w = _cat([w[k, n] for n in range(2)], 1)
            if k in prep_slots:
                w = due(w)
            y = _dot(_halves(due_y(w) if k in norm_slots else w), weights(wb, o_w3 + k * fp + p * wq, wq))
            if k in norm_slots:
                z = due.after(y)
                fill_y(z)
                fill_t(z)
                if k in prep_slots:
                    fill(z)
            return y

        for p in range(nf):
            g = [[_gelu_of_twice(y) for y in row] for row in _combine2(part(up, p), _combine)]
            for a, group in enumerate(_left2(g)):
                for b, f in enumerate(group):
                    lz[7 * a + b, p] = f.astype(BF16)
        fill_y.finish()
        fill_t.finish()
        assert fill.done * len(jobs) // fill.slots <= 2 * opi // 8

        def down(e, k):
            w = lz.bitcast(U32)
            y = _dot(_halves(due_z(due(_cat([w[k, p] for p in range(nf)], 1)))),
                     weights(wb, o_w4 + k * fp + e * nf * rq, nf * rq))
            z = due.after(y)
            fill(z)
            fill_z(z)
            return y

        for e in range(2):
            for u, row in enumerate(_combine2(part(down, e), _combine_late)):
                for j, y in enumerate(row):
                    hs[2 * j + e, pl.ds(r0 + u * q2, q2), :] += y
        fill_z.finish()
        fill.finish()

        @pl.when(i + 2 < nb2)
        def _():
            for c in a_copies(i + 2):
                c.start()

        return carry

    _run(norm_mid(0), 2)
    _run(left_mid(), 1)
    lax.fori_loop(0, nb2, b3, 0)

    scale = Dh ** -0.5
    key = lax.broadcasted_iota(jnp.int32, (seg, L), 0) + M
    query = lax.broadcasted_iota(jnp.int32, (seg, L), 1)
    mask = (query < M) | (query >= key)
    QS = 4 * seg
    rv = (seg - M) // 8

    def upper(n):
        return lax.broadcasted_iota(jnp.int32, (8, n), 0) < 4

    def split8(mem, tok):
        u = upper(mem.shape[1])
        return jnp.where(u, mem, tok), pltpu.roll(jnp.where(u, tok, mem), 4, 0)

    def join8(t, b):
        u = upper(t.shape[1])
        b = pltpu.roll(b, 4, 0)
        return jnp.where(u, t, b), jnp.where(u, b, t)

    def vregs(y, lo, hi):
        return [y[8 * k:8 * k + 8] for k in range(lo, hi)]

    def left_operands(mem, tok, big):
        if not big:
            return _hk_left([_cat([m] + y, 0) for m, y in zip(mem, tok)])
        pairs = [split8(m, y[2 * rv]) for m, y in zip(mem, tok)]
        return _hk_left(*[[_cat([p[c]] + y[c * rv:(c + 1) * rv], 0) for p, y in zip(pairs, tok)] for c in range(2)])

    def rows_out(c):
        if len(c) == 1:
            return [(y[0:8], vregs(y, 1, 1 + rv)) for y in c[0]]
        got = []
        for y, w in zip(*c):
            ym, yt = join8(y[0:8], w[0:8])
            got.append((ym, vregs(y, 1, 1 + rv) + vregs(w, 1, 1 + rv) + [yt]))
        return got

    def probs(q, k):
        sc = _dot_nt(k, q.astype(BF16))
        sc = _cat([sc[0:M], jnp.where(mask, sc[M:L], -1e9 / scale)], 0)
        p = jnp.exp2((sc - jnp.max(sc, axis=0, keepdims=True)) * (scale * math.log2(math.e)))
        return p * _recip(jnp.sum(p, axis=0, keepdims=True))

    def out_copy(j):
        r0 = pl.multiple_of(j * QS, QS)
        return pltpu.make_async_copy(xbuf.at[pl.ds(r0, QS)], out_hbm.at[pl.ds(r0, QS)], sem_out.at[j])

    def quad(j, carry):
        xs = normed(pl.ds(pl.multiple_of(j * QS, QS), QS))
        qkv = {(t, h): [] for t in range(3) for h in range(H)}
        att = {h: [] for h in range(H)}
        outs = {n: [] for n in range(nd)}
        mem = membuf[...]
        for st in range(4):
            r, n_tok = (0, 2 * rv + 1) if st == 0 else ((st + 1) * rv + 1, rv)
            hl = left_operands([mem[:, cols(2 * k, 2)] for k in range(4)],
                               [vregs(xs[:, cols(2 * k, 2)], r, r + n_tok) for k in range(4)], st == 0)
            ol, cur, p, o = {}, {}, {}, {}

            def wq_part(t, g, lo, hi, midway=None):
                return _hk_combine(hl, lambda f: _dot(
                    hl[f][1][:, lo:hi].astype(BF16),
                    weights(wa, o_qkv + ((t * ng + g) * nk + f) * wq + lo // 2, (hi - lo) // 2)), midway)

            def wo_part(e, lo, hi):
                return _hk_combine(ol[lo], lambda f: _dot(
                    _cat([ol[g][f][1] for g in range(lo, hi)], 1).astype(BF16),
                    weights(wa, o_wo + ((e * nk + f) * ng + lo) * rq, (hi - lo) * rq)))

            def stash(q, c):
                for a, blocks in enumerate(c):
                    for b, y in enumerate(blocks):
                        pbuf[st, q, a, b] = y

            def resume(q, c):
                return [[pbuf[st, q, a, b] + y for b, y in enumerate(blocks)] for a, blocks in enumerate(c)]

            def proj(t, g, midway=None):
                if g == 0 and st > 0 and t < 2:
                    c = resume(2 + t, wq_part(t, g, LANES, 2 * LANES))
                else:
                    c = wq_part(t, g, 0, 2 * LANES, midway)
                got = []
                for h, (ym, yt) in zip(heads(g), rows_out(c)):
                    qkv[t, h] += yt
                    got.append(_cat([ym] + qkv[t, h][4 * st:4 * st + 4], 0))
                return got

            def attend(g, c):
                for e in (2 * c, 2 * c + 1):
                    if 0 <= g < ng:
                        p[g, e] = probs(cur[0, g][e], cur[1, g][e])
                if g > 0:
                    for e in (2 * c, 2 * c + 1):
                        o[e] = _dot(p[g - 1, e].T, cur[2, g - 1][e].astype(BF16))
                        att[heads(g - 1)[e]] += vregs(o[e], 1, 5)
                    if c:
                        ol[g - 1] = left_operands(
                            [o[e][0:8] for e in range(4)],
                            [att[h][st * rv:None if st == 3 else (st + 1) * rv] for h in heads(g - 1)], st == 3)

            if st > 0:
                for t in range(2):
                    stash(2 + t, wq_part(t, 0, 0, LANES))
            for g in range(ng):
                cur[0, g] = proj(0, g)
                cur[1, g] = proj(1, g, part(attend, g - 1, 1) if g else None)
                cur[2, g] = proj(2, g)
                attend(g, 0)
            stash(0, wo_part(0, 0, 2))
            attend(ng - 1, 1)
            stash(1, wo_part(1, 0, 2))
            attend(ng, 0)
            stash(0, resume(0, wo_part(0, 2, 4)))
            attend(ng, 1)
            stash(1, resume(1, wo_part(1, 2, 4)))
            new = {}
            for e in range(2):
                for c, (ym, yt) in enumerate(rows_out(resume(e, wo_part(e, 4, ng)))):
                    new[2 * c + e] = ym
                    outs[2 * c + e] += yt
            mem = _cat([new[n] for n in range(nd)], 1)
            lo, hi = ((0, 2), (2, 6), (6, 8), (8, 16))[st]
            rr = pl.ds(pl.multiple_of(j * QS + 8 * lo, RC), 8 * (hi - lo))
            for n in range(nd):
                xbuf[rr, cols(n)] = (hs[n, rr, :] + _cat(outs[n][lo:hi], 0)).astype(BF16)
        membuf[...] = mem
        out_copy(j).start()
        return carry

    mem_copy.wait()
    membuf[...] = mem0[...].astype(F32)
    lax.fori_loop(0, S // QS, quad, 0)
    for j in range(S // QS):
        out_copy(j).wait()


@functools.partial(jax.jit, static_argnames=("A_seg_len",))
def pallas_parallel_sum__memory_aug_recurrent_mem_tr__mixer_s_mlp__prompt_kernel(
    A_x: jax.Array,
    A_mem0: jax.Array,
    A_Wq: jax.Array,
    A_Wk: jax.Array,
    A_Wv: jax.Array,
    A_Wo: jax.Array,
    A_seg_len: int,
    B_x: jax.Array,
    B_w1: jax.Array,
    B_w2: jax.Array,
    B_w3: jax.Array,
    B_w4: jax.Array,
):
    del B_x
    B, S, D = A_x.shape
    _, H, Dh = A_Wq.shape
    M = A_mem0.shape[1]
    seg = int(A_seg_len)
    F = B_w3.shape[1]
    assert (B, S, D, H, Dh, M, seg, F) == (1, 2048, 1024, 32, LANES, 8, 32, 3584)
    TM1, TM2 = 256, 128
    nd, nf, nk, nb2 = D // LANES, F // (4 * LANES), len(_HK), S // TM2

    hbm = pl.BlockSpec(memory_space=pl.ANY)
    dma = pltpu.SemaphoreType.DMA
    out = pl.pallas_call(
        functools.partial(_kernel, S=S, D=D, H=H, Dh=Dh, M=M, seg=seg, F=F, TM1=TM1, TM2=TM2),
        out_shape=jax.ShapeDtypeStruct((S, D), BF16),
        in_specs=[hbm] * 10,
        out_specs=hbm,
        scratch_shapes=[
            pltpu.VMEM((S, D), BF16),
            pltpu.VMEM((2, S, LANES), F32),
            pltpu.VMEM((nd, S + TM2, LANES), F32),
            pltpu.VMEM((2, 7, nd // 2, TM1 // 2, LANES), BF16),
            pltpu.VMEM((TM2, D), F32),
            pltpu.VMEM((49, nd // 4, TM2 // 4, LANES), BF16),
            pltpu.VMEM((49, nf, TM2 // 4, LANES), BF16),
            pltpu.VMEM((H * nk * D // 4, LANES), BF16),
            pltpu.VMEM((4 * 49 * (nf * D // 8 + 8), LANES), BF16),
            pltpu.SMEM((1,), jnp.int32),
            pltpu.VMEM((2, 12, (D // 4 // nb2) * H, LANES), BF16),
            pltpu.VMEM((12, (H // 2 + 2) * (D // 4 // nb2 + 4), LANES), U32),
            pltpu.VMEM((2, 4, nd, H * Dh // (4 * nb2), LANES), BF16),
            pltpu.VMEM((M, D), BF16),
            pltpu.VMEM((M, D), F32),
            pltpu.VMEM((4, 4, 2, 4, seg, LANES), F32),
            dma((S // TM1 + 1,)), dma((nd // 2 + 7,)), dma((2,)), dma((S // (4 * seg),)),
        ],
        compiler_params=pltpu.CompilerParams(
            vmem_limit_bytes=128 * 1024 * 1024, disable_bounds_checks=True, disable_semaphore_checks=True),
        name="rmt_s2mlp",
    )(A_x.reshape(S, D), A_mem0.reshape(M, D),
      A_Wq.reshape(D * H, Dh), A_Wk.reshape(D * H, Dh), A_Wv.reshape(D * H, Dh),
      A_Wo.reshape(H * Dh, D), B_w1, B_w2, B_w3, B_w4)
    return out.reshape(B, S, D)
```

```python
import functools
import math

import jax
import jax.numpy as jnp
from jax import lax
import jax.experimental.pallas as pl
import jax.experimental.pallas.tpu as pltpu

F32 = jnp.float32
BF16 = jnp.bfloat16
U32 = jnp.uint32
LANES = 128
EPS = 1e-5
PAD = 8


def _dot(a, b):
    return lax.dot_general(a, b, (((1,), (0,)), ((), ())), preferred_element_type=F32)


def _dot_nt(a, b):
    return lax.dot_general(a, b, (((1,), (1,)), ((), ())), preferred_element_type=F32)


def _cat(xs, axis):
    return xs[0] if len(xs) == 1 else jnp.concatenate(xs, axis=axis)


def _moments(x, z):
    s = _cat([pltpu.bitcast(z, F32)] * (x.shape[0] // 8), 0)
    for c in range(0, x.shape[1], LANES):
        s = s + x[:, c:c + LANES]
    m = jnp.sum(s, axis=-1, keepdims=True) * (1.0 / x.shape[1])
    d = x - m
    return m, d, jnp.mean(d * d, axis=-1, keepdims=True)


def _recip(x):
    r = pl.reciprocal(x, approx=True)
    return r * (2.0 - x * r)


def _gelu_of_twice(h):
    c = math.sqrt(2.0 / math.pi)
    return h + h * jnp.tanh(h * (2.0 * c + (8.0 * c * 0.044715) * (h * h)))


def _halves(w):
    return pltpu.bitcast(w, BF16)


def _unpack(w, z):
    return pltpu.bitcast(w << (z | 16), F32), pltpu.bitcast(w & (z | U32(0xFFFF0000)), F32)


def _widen(w, z):
    return _halves(w if z is None else w | z).astype(F32)


def _left(a11, a12, a21, a22):
    return (a11 + a22, a21 + a22, a11, a22, a11 + a12, a21 - a11, a12 - a22)


def _right(b11, b12, b21, b22):
    return (b11 + b22, b11, b12 - b22, b21 - b11, b22, b11 + b12, b21 + b22)


_USE = (
    {0: 1, 3: 1}, {2: 1, 3: -1}, {1: 1, 3: 1}, {0: 1, 2: 1}, {0: -1, 1: 1}, {3: 1}, {0: 1})


def _combine(m, order):
    acc = {}
    for i in order:
        y = m(i)
        for c, s in _USE[i].items():
            acc[c] = _signed_sum([acc[c], (s, y)]) if c in acc else (s, y)
    return [acc[c][1] for c in range(4)]


class _Blocks(tuple):
    def __add__(self, other):
        return _Blocks(a + b for a, b in zip(self, other))

    def __sub__(self, other):
        return _Blocks(a - b for a, b in zip(self, other))


def _left2(a):
    nested = [_Blocks(a[2 * i + u][2 * j + w] for u in range(2) for w in range(2))
              for i in range(2) for j in range(2)]
    return (_left(*g) for g in _left(*nested))


def _combine2(m, outer, inner):
    c = _combine(lambda a: _Blocks(_combine(lambda b: m(7 * a + b), inner)), outer)
    return [[c[2 * (i // 2) + j // 2][2 * (i % 2) + j % 2] for j in range(4)] for i in range(4)]


def _hopcroft_kerr(types):
    n = len(types)
    prods = []

    def add(left, out):
        prods.append((left, {}, out))
        return len(prods) - 1

    def use(block, terms):
        for f, s in terms:
            prods[f][1][block] = prods[f][1].get(block, 0) + s

    class Node:
        def __init__(self, t, xs, ys, plus, minus):
            self.t, self.xs, self.ys, self.plus, self.minus = t, xs, ys, plus, minus

    def mix(*parts):
        return {(i, t % 3): s * c for d, t, s in parts for i, c in d.items()}

    def pair(u, w):
        if (u.t - w.t) % 3 != 1:
            zwu, zuw, free = pair(w, u)
            return zuw, zwu, free
        t = u.t
        s = add(mix((u.xs, t + 2, 1), (w.xs, t, 1)), mix((u.ys, t + 2, 1), (w.ys, t, -1)))
        o1 = add(mix((u.xs, t, -1), (w.xs, t, 1)), mix((u.ys, t + 2, 1), (w.ys, t + 2, 1)))
        o2 = add(mix((u.xs, t + 2, -1), (w.xs, t + 2, 1)), mix((u.ys, t, 1), (w.ys, t, 1)))
        free = Node((t + 1) % 3, {**{i: -c for i, c in u.xs.items()}, **w.xs}, {**u.ys, **w.ys}, o1, o2)
        return ([(s, 1), (o1, -1), (u.minus, 1), (w.minus, -1)],
                [(s, 1), (o2, -1), (u.plus, 1), (w.plus, -1)], free)

    nodes = []
    for i, t in enumerate(types):
        e = {i: 1}
        nodes.append(Node(t, e, e, add(mix((e, t + 2, 1)), mix((e, t + 1, 1))),
                          add(mix((e, t + 1, 1)), mix((e, t + 2, 1)))))
        use((i, i), [(nodes[i].plus, 1), (nodes[i].minus, -1)])
    z, free = {}, {}
    for i in range(n):
        for j in range(i + 1, n):
            if types[i] != types[j]:
                z[i, j], z[j, i], free[i, j] = pair(nodes[i], nodes[j])
                free[j, i] = free[i, j]
    for i in range(n):
        for j in range(i + 1, n):
            if types[i] == types[j]:
                k = next(k for k in range(n) if types[k] != types[i])
                w = free[i, k]
                zwj, zjw, _ = pair(w, nodes[j])
                z[i, j] = [(f, w.xs[i] * c) for f, c in zwj] + z[k, j]
                z[j, i] = zjw + [(f, -c) for f, c in z[j, k]]
    for block, terms in z.items():
        use(block, terms)
    return [(left, {k: c for k, c in right.items() if c}, out) for left, right, out in prods]


def _signed_sum(terms):
    terms = sorted(terms, key=lambda t: -t[0])
    sign, y = terms[0]
    for s, x in terms[1:]:
        y = y + x if s == sign else y - x
    return sign, y


def _signed_value(terms):
    sign, y = _signed_sum(terms)
    return y if sign > 0 else -y


_HK = _hopcroft_kerr((0, 1, 2, 0))
_HK_ROW = [f for f, (left, _, out) in enumerate(_HK)
           if any(t != 2 for _, t in left) and any(t != 0 for _, t in out)]
_HK_RIGHT_SIGN = [_signed_sum([(c, 0) for c in right.values()])[0] for _, right, _ in _HK]


def _hk_left(upper, lower=None):
    if lower is None:
        base = [((1, u), (-1, u), None) for u in upper]
    else:
        base = [((1, u), (1, w), (-1, u + w)) for u, w in zip(upper, lower)]
    return {f: _signed_sum([(c * base[i][t][0], base[i][t][1]) for (i, t), c in _HK[f][0].items() if base[i][t]])
            for f in (_HK_ROW if lower is None else range(len(_HK)))}


def _hk_columns(f):
    js = [j for j, _ in _HK[f][2]]
    return min(js), max(js), f


def _hk_combine(left, m, midway=None):
    both = len(left) == len(_HK)
    acc = {}
    for n, f in enumerate(sorted(left, key=_hk_columns)):
        y = m(f)
        if midway and n + 1 == len(left) * 3 // 4:
            midway()
        for (j, t), c in _HK[f][2].items():
            c *= left[f][0] * _HK_RIGHT_SIGN[f]
            if both:
                acc[j, t] = _signed_sum([acc[j, t], (c, y)]) if (j, t) in acc else (c, y)
            elif t:
                c *= (0, -1, 1)[t]
                acc[j] = _signed_sum([acc[j], (c, y)]) if j in acc else (c, y)
    if not both:
        return [[_signed_value([acc[j]]) for j in range(4)]]
    return [[_signed_value([acc[j, p], (-acc[j, q][0], acc[j, q][1])]) for j in range(4)]
            for p, q in ((2, 1), (0, 2))]


class _Filler:
    def __init__(self, slots, jobs):
        self.slots, self.done, self.jobs, self.live = slots, 0, jobs, []

    def __call__(self, z):
        def step(g, v):
            try:
                g.send(v)
                return True
            except StopIteration:
                return False

        n = len(self.jobs)
        new = [job(z) for job in self.jobs[self.done * n // self.slots:(self.done + 1) * n // self.slots]]
        self.live = [g for g in new if step(g, None)] + [g for g in self.live if step(g, z)]
        self.done += 1

    def finish(self):
        while self.live or self.done < self.slots:
            self(jnp.zeros((8, LANES), U32))


def _run(jobs, group):
    _Filler(len(jobs) // group, jobs).finish()


def _kernel(x_hbm, mem0_hbm, wq_hbm, wk_hbm, wv_hbm, wo_hbm, w1_hbm, w2_hbm, w3_hbm, w4_hbm,
            out_hbm,
            xbuf, stat, hs, lf, lt, ly, lz, wa, wb, zero, stq, stt, sto, mem0, membuf, pbuf,
            sem_x, sem_w, sem_a, sem_out,
            *, S, D, H, Dh, M, seg, F, TM1, TM2):
    part = functools.partial
    L = M + seg
    nd = D // LANES
    nh = nd // 2
    Dk = D // 2
    rq = LANES // 2
    wk = Dk // 2
    wq = wk // 2
    nf = F // (4 * LANES)
    hp = H // 2
    ng = H // 4
    nk = len(_HK)
    nb1, nb2 = S // TM1, S // TM2
    h1, q2 = TM1 // 2, TM2 // 4
    RC = 16

    def cols(n, w=1):
        return slice(n * LANES, (n + w) * LANES)

    def heads(g):
        return [2 * g, 2 * g + 1, hp + 2 * g, hp + 2 * g + 1]

    fp = nf * wq + 8
    o_w3 = 0
    o_w4 = o_w3 + 49 * fp
    o_wo = 0
    o_qkv = o_wo + 2 * nk * ng * rq
    raw = {1: o_qkv, 2: o_qkv + nd * Dk, 3: o_qkv + 2 * nd * Dk, 4: o_qkv + 2 * nd * Dk + 4 * F}

    def words(ref, r0, rows):
        return ref.bitcast(U32)[pl.ds(r0, rows), :]

    def weights(ref, r0, rows):
        return _halves(words(ref, r0, rows))

    def view(ref, r0, rows):
        return ref.at[pl.ds(pl.multiple_of(2 * r0, RC), 2 * rows)]

    def put(ref, r, y):
        ref[2 * r:2 * r + RC, :] = y.astype(BF16)

    def w_copy(j, n):
        src, rows, sem = {1: (w1_hbm, Dk, n % nh), 2: (w2_hbm, Dk, nh),
                          3: (w3_hbm, Dk, nh + 1 + n % nf // 2), 4: (w4_hbm, F // 2, nh + 5 + n % 2)}[j]
        return pltpu.make_async_copy(src.at[:, cols(n)], wa.at[pl.ds(2 * (raw[j] + n * rows), 2 * rows)],
                                     sem_w.at[sem])

    def w_wait(sem, *spans):
        for r0, rows in spans:
            span = wa.at[pl.ds(2 * r0, 2 * rows)]
            pltpu.make_async_copy(span, span, sem_w.at[sem]).wait()

    def w3_copies(lo, hi):
        return [w_copy(3, p + j * nf) for p in range(lo, hi) for j in range(4)]

    def x_copy(i):
        r0 = pl.multiple_of(i * TM1, TM1)
        return pltpu.make_async_copy(x_hbm.at[pl.ds(r0, TM1)], xbuf.at[pl.ds(r0, TM1)], sem_x.at[i])

    fpi = D // 4 // nb2
    opi = ng * rq // nb2
    tp = fpi + 4

    def a_copies(i):
        cps = []
        for t, src in enumerate((wq_hbm, wk_hbm, wv_hbm)):
            for k in range(4):
                r0 = pl.multiple_of((k * (D // 4) + i * fpi) * H, fpi * H)
                cps.append(pltpu.make_async_copy(src.at[pl.ds(r0, fpi * H)],
                                                 stq.at[i % 2, 4 * t + k], sem_a.at[i % 2]))
        for k, h in enumerate(heads(i // (rq // opi))):
            r0 = pl.multiple_of(2 * (h * rq + i % (rq // opi) * opi), 2 * opi)
            for n in range(nd):
                cps.append(pltpu.make_async_copy(wo_hbm.at[pl.ds(r0, 2 * opi), cols(n)],
                                                 sto.at[i % 2, k, n], sem_a.at[i % 2]))
        return cps

    later = [
        lambda: [x_copy(4)] + [w_copy(2, n) for n in range(nh)],
        lambda: [x_copy(5)] + [w_copy(2, n) for n in range(nh, nd)],
        lambda: [x_copy(6)] + w3_copies(0, 1),
        lambda: [x_copy(7)] + w3_copies(1, 2),
        lambda: w3_copies(2, 3),
        lambda: w3_copies(3, 4),
        lambda: w3_copies(4, 6),
        lambda: w3_copies(6, 7),
        lambda: [w_copy(4, 0), w_copy(4, 2)],
        lambda: [w_copy(4, 4), w_copy(4, 6)],
        lambda: [w_copy(4, 1), w_copy(4, 3)],
        lambda: [w_copy(4, 5), w_copy(4, 7)],
        lambda: a_copies(0),
        lambda: a_copies(1),
    ]

    def start_later(i, lo, hi):
        for k in range(lo, min(hi, len(later))):
            @pl.when(i == k - lo)
            def _(k=k):
                for c in later[k]():
                    c.start()

    first = [pltpu.make_async_copy(x_hbm.at[pl.ds(r, TM1 // 8)], xbuf.at[pl.ds(r, TM1 // 8)], sem_x.at[0])
             for r in range(0, TM1, TM1 // 8)]
    for c in first:
        c.start()
    for n in range(nh // 2):
        w_copy(1, n).start()
        w_copy(1, n + nh).start()

    for n in range(nd):
        hs[n, 0:PAD, :] = jnp.zeros((PAD, LANES), F32)
        hs[n, PAD + S:PAD + S + PAD, :] = jnp.zeros((PAD, LANES), F32)
    for ref in (wa, wb):
        ref[0:RC, :] = jnp.zeros((RC, LANES), BF16)
    for c in range(stt.shape[0]):
        stt[c, 0:8, :] = jnp.zeros((8, LANES), U32)
    zero[0] = 0

    class Deadline:
        def __init__(self, probe=None, lag=0):
            self.probe, self.queue = probe, [None] * lag
            self.zero = jnp.full((8, LANES), zero[0], jnp.int32).astype(U32)

        def after(self, y):
            return pltpu.bitcast(y[0:8, 0:LANES], U32) & self.zero

        def __call__(self, w):
            self.queue.append(self.probe() & self.zero)
            z = self.queue.pop(0)
            if z is None:
                return w
            return _cat([_cat([w[0:8, 0:LANES] | z, w[8:, 0:LANES]], 0), w[:, LANES:]], 1)

    def norm_in(i, slot, r, z):
        a = []
        for half in range(2):
            rr = pl.ds(pl.multiple_of(i * TM1 + half * h1 + r, RC), RC)
            m, d, v = _moments(xbuf[rr, :].astype(F32), z)
            q = lax.rsqrt(v + EPS)
            stat[0, rr, :] = jnp.broadcast_to(m, (RC, LANES))
            stat[1, rr, :] = jnp.broadcast_to(q, (RC, LANES))
            a.append(d * (0.5 * q * lax.rsqrt(v * q * q + EPS)))
        for _ in range(3):
            yield
        for k, f in enumerate(_left(a[0][:, :Dk], a[0][:, Dk:], a[1][:, :Dk], a[1][:, Dk:])):
            for n in range(nh):
                lf[slot, k, n, pl.ds(r, RC), :] = f[:, cols(n)].astype(BF16)
            if k in (1, 4):
                yield

    def normed(rr):
        m, q = (_cat([stat[k, rr, :]] * nd, 1) for k in range(2))
        return (xbuf[rr, :].astype(F32) - m) * q

    def norm_first(q, carry):
        _run([part(norm_in, 0, 0, pl.multiple_of((4 * q + e) * RC, RC)) for e in range(4)], 4)
        return carry

    def prep1(n, carry):
        o = pl.multiple_of(raw[1] + n * Dk, Dk)
        src, dst = view(wa, o, (nh + 1) * Dk), view(wb, o_w4 + n * 7 * wk, 7 * wk)
        w_wait(n, (o, Dk), (o + nh * Dk, Dk))

        def job(r, _):
            w = [words(src, e + r, 8) for e in (0, nh * Dk, wk, nh * Dk + wk)]
            z = yield
            for k, f in enumerate(_right(*[_widen(x, z) for x in w])):
                put(dst, k * wk + r, f)

        _run([part(job, r) for r in range(0, wk, 8)], 2)
        return carry

    def b1(i, carry):
        @pl.when(i + 1 < nb1)
        def _():
            x_copy(i + 1).wait()

        r0 = pl.multiple_of(i * TM1, TM1)
        nxt = jnp.minimum(i + 1, nb1 - 1)
        fill = _Filler(7 * nh - 3, [part(norm_in, nxt, (i + 1) % 2, r) for r in range(0, h1, RC)])
        due = Deadline()

        def prod(n, k):
            w = lf.bitcast(U32)
            y = _dot(_halves(_cat([w[i % 2, k, c] for c in range(nh)], 1)), weights(wb, o_w4 + (n * 7 + k) * wk, wk))
            fill(due.after(y))
            return y

        for n in range(nh):
            for k, y in enumerate(_combine(part(prod, n), (1, 0, 3, 6, 4, 2, 5))):
                hs[n + k % 2 * nh, pl.ds(r0 + PAD + k // 2 * h1, h1), :] = _gelu_of_twice(y)
        fill.finish()
        start_later(i, 0, nb1)
        return carry

    for c in first:
        c.wait()
    for n in range(nh // 2, nh):
        w_copy(1, n).start()
        w_copy(1, n + nh).start()
    lax.fori_loop(0, h1 // (4 * RC), norm_first, 0)
    x_copy(1).start()
    lax.fori_loop(0, nh, prep1, 0)
    x_copy(2).start()
    x_copy(3).start()
    mem_copy = pltpu.make_async_copy(mem0_hbm, mem0, sem_x.at[nb1])
    mem_copy.start()
    lax.fori_loop(0, nb1, b1, 0)

    shifts = (-1, 1, -2, 2)
    BK = 32
    HB = 64
    per = nf * (wq // BK) // (nb1 // 2)

    def prep34(second, u):
        src = jnp.where(second, raw[4] + u // (nf * rq // BK) * (F // 2) + u % (nf * rq // BK) * BK,
                        raw[3] + u // (wq // BK) * Dk + u % (wq // BK) * BK).astype(jnp.int32)
        src = [view(wa, src + k * jnp.where(second, nf * rq, wq), 3 * F + BK) for k in range(4)]
        dst = view(wb, jnp.where(second, o_w4, o_w3) + u.astype(jnp.int32) * BK, 48 * fp + BK)

        def job(r, z):
            def quarter(a, b):
                return _Blocks(_widen(words(src[2 * a + k], (2 * b + j) * F + r, 8), z if k == j else None)
                               for k in range(2) for j in range(2))

            for stage in ((1, 5, 3), (0, 4, 2, 6)):
                outer = _right(*[quarter(a, b) for a in range(2) for b in range(2)])
                for a in stage:
                    for b, f in enumerate(_right(*outer[a])):
                        put(dst, (7 * a + b) * fp + r, f)
                z = yield

        return [part(job, r) for r in range(0, BK, 8)]

    def b2(i, carry):
        for k in range(4):
            pl.when(i == k)(part(w_wait, nh + 1 + k, *[
                (raw[3] + j * F + 2 * k * Dk, min(2, nf - 2 * k) * Dk) for j in range(4)]))
        for e in range(2):
            pl.when(i == 4 + 2 * e)(part(w_wait, nh + 5 + e, *[
                (raw[4] + j * F + e * (F // 2), F // 2) for j in range(4)]))

        r0 = pl.multiple_of(i * TM1, TM1)
        jobs = [prep34(i >= nb1 // 2, (i.astype(U32) % (nb1 // 2)) * per + u) for u in range(per)]
        fill = _Filler(2 * nd * TM1 // HB - 6, sum(jobs, []))
        due = Deadline(lambda: words(wb, 0, 8), 4)

        def shifted(r):
            return [hs[n, pl.ds(r0 + PAD + r + shifts[n * 4 // nd], HB), :] for n in range(nd)]

        ahead = shifted(0)
        for r in range(0, TM1, HB):
            sh = ahead
            for c in range(nd):
                if c == nd - 2 and r + HB < TM1:
                    ahead = shifted(r + HB)
                y = None
                for k in range(0, nd, nh):
                    a = pltpu.bitcast(due(pltpu.bitcast(_cat(sh[k:k + nh], 1), U32)), F32)
                    p = _dot(a.astype(BF16), weights(wa, raw[2] + c * Dk + k * rq, nh * rq))
                    y = p if y is None else p + y
                    fill(due.after(y))
                hs[c, pl.ds(r0 + r, HB), :] = y
        fill.finish()
        start_later(i, nb1, 2 * nb1)
        return carry

    w_wait(nh, (raw[2], nd * Dk))
    lax.fori_loop(0, nb1, b2, 0)

    def norm_mid(i):
        def job(r, _):
            rr = pl.ds(pl.multiple_of(jnp.minimum(i, nb2 - 1) * TM2 + r, 8), 8)
            x1 = _cat([hs[n, rr, :] for n in range(nd)], 1) + normed(rr)
            y = x1 + xbuf[rr, :].astype(F32)
            z = yield
            for n in range(nd):
                hs[n, pl.ds(pl.multiple_of(i * TM2 + r, 8), 8), :] = y[:, cols(n)]
            _, d, v = _moments(x1, z)
            lt[r:r + 8, :] = d * (0.5 * lax.rsqrt(v + EPS))

        return [part(job, r) for r in range(0, TM2, 8)]

    def left_mid():
        def job(r, n, _):
            a = [[lt[u * q2 + r:u * q2 + r + RC, cols(2 * j + n)] for j in range(4)] for u in range(4)]
            for k, g in enumerate(_left2(a)):
                for b, f in enumerate(g):
                    ly[7 * k + b, n, r:r + RC, :] = f.astype(BF16)
                yield

        return [part(job, r, n) for r in range(0, q2, RC) for n in range(2)]

    def b3(i, carry):
        for buf in (stq, sto):
            pltpu.make_async_copy(buf.at[i % 2], buf.at[i % 2], sem_a.at[i % 2]).wait()

        dst_qkv = view(wa, o_qkv + i * (fpi // 2), (3 * ng * nk - 1) * wq + fpi // 2)
        dst_o = view(wa, o_wo + i * opi, (2 * nk - 1) * ng * rq + opi)
        stages = [range(8, 17), range(17, 26), range(0, 4), range(4, 8)]

        def turn(c, d, _):
            w = [stq.bitcast(U32)[i % 2, c, pl.ds(e * 8, 8), :] for e in range(2 * d, 2 * d + 4)]
            w[0] = w[0] | (yield)
            for e, x in enumerate(w):
                stt[c, pl.ds(e % 2 * 8 * tp + d + e // 2, 8, stride=tp), :] = x

        def prep_qkv(t, g, z):
            for stage in stages:
                def block(k, j):
                    r = heads(g)[j] // 2 * tp
                    return _cat([_unpack(stt[4 * t + k, r + e:r + e + 8, :], z)[j % 2] for e in (0, 8)], 0)

                for f in stage:
                    y = _signed_sum([(c, block(*key)) for key, c in _HK[f][1].items()])[1]
                    put(dst_qkv, ((t * ng + g) * nk + f) * wq, y)
                z = yield

        def prep_o(e, r, z):
            for stage in stages:
                for f in stage:
                    y = [(c, _widen(sto.bitcast(U32)[i % 2, k, 2 * j + e, r:r + 8, :], None if n else z))
                         for n, ((k, j), c) in enumerate(_HK[f][1].items())]
                    put(dst_o, (e * nk + f) * ng * rq + r, _signed_sum(y)[1])
                z = yield

        jobs = [part(prep_o, e, r) for e in range(2) for r in range(0, opi, 8)]
        jobs += [part(prep_qkv, t, g) for t in range(3) for g in range(ng)]
        r0 = pl.multiple_of(i * TM2, TM2)
        here = pl.ds(pl.multiple_of(zero[0], 8), 8)
        norm_slots = [k for k in range(49) if k // 7 in (3, 1)]
        prep_slots = norm_slots[3::3]
        fill = _Filler(nf * len(prep_slots) + 2 * 49 - 8, jobs)
        due = Deadline(lambda: words(wa, 0, 8), 5)
        fill_y = _Filler((nf - 1) * len(norm_slots), norm_mid(i + 1))
        due_y = Deadline(lambda: pltpu.bitcast(lt[here, 0:LANES], U32) | stt[zero[0], 0:8, :], 14)
        fill_t = _Filler((nf - 1) * len(norm_slots),
                         [part(turn, c, d) for c in range(12) for d in range(0, fpi, 2)])
        fill_z = _Filler(7 * 7, left_mid())
        due_z = Deadline(lambda: ly.bitcast(U32)[zero[0], 0, 0:8, :], 6)

        def up(p, k):
            w = ly.bitcast(U32)
            w = _cat([w[k, n] for n in range(2)], 1)
            if k in prep_slots:
                w = due(w)
            y = _dot(_halves(due_y(w) if k in norm_slots else w), weights(wb, o_w3 + k * fp + p * wq, wq))
            if k in norm_slots:
                z = due.after(y)
                fill_y(z)
                fill_t(z)
                if k in prep_slots:
                    fill(z)
            return y

        for p in range(nf):
            g = [[_gelu_of_twice(y) for y in row] for row in _combine2(part(up, p), (3, 1, 0, 6, 4, 2, 5), (3, 1, 0, 6, 4, 2, 5))]
            for a, group in enumerate(_left2(g)):
                for b, f in enumerate(group):
                    lz[7 * a + b, p] = f.astype(BF16)
        fill_y.finish()
        fill_t.finish()
        assert fill.done * len(jobs) // fill.slots <= 2 * opi // 8

        def down(e, k):
            w = lz.bitcast(U32)
            y = _dot(_halves(due_z(due(_cat([w[k, p] for p in range(nf)], 1)))),
                     weights(wb, o_w4 + k * fp + e * nf * rq, nf * rq))
            z = due.after(y)
            fill(z)
            fill_z(z)
            return y

        for e in range(2):
            for u, row in enumerate(_combine2(part(down, e), (4, 5, 1, 0, 6, 2, 3), (3, 1, 0, 2, 5, 6, 4))):
                for j, y in enumerate(row):
                    hs[2 * j + e, pl.ds(r0 + u * q2, q2), :] += y
        fill_z.finish()
        fill.finish()

        @pl.when(i + 2 < nb2)
        def _():
            for c in a_copies(i + 2):
                c.start()

        return carry

    _run(norm_mid(0), 2)
    _run(left_mid(), 1)
    lax.fori_loop(0, nb2, b3, 0)

    scale = Dh ** -0.5
    key = lax.broadcasted_iota(jnp.int32, (seg, L), 0) + M
    query = lax.broadcasted_iota(jnp.int32, (seg, L), 1)
    mask = (query < M) | (query >= key)
    QS = 4 * seg
    rv = (seg - M) // 8

    def upper(n):
        return lax.broadcasted_iota(jnp.int32, (8, n), 0) < 4

    def split8(mem, tok):
        u = upper(mem.shape[1])
        return jnp.where(u, mem, tok), pltpu.roll(jnp.where(u, tok, mem), 4, 0)

    def join8(t, b):
        u = upper(t.shape[1])
        b = pltpu.roll(b, 4, 0)
        return jnp.where(u, t, b), jnp.where(u, b, t)

    def vregs(y, lo, hi):
        return [y[8 * k:8 * k + 8] for k in range(lo, hi)]

    def left_operands(mem, tok, big):
        if not big:
            return _hk_left([_cat([m] + y, 0) for m, y in zip(mem, tok)])
        pairs = [split8(m, y[2 * rv]) for m, y in zip(mem, tok)]
        return _hk_left(*[[_cat([p[c]] + y[c * rv:(c + 1) * rv], 0) for p, y in zip(pairs, tok)] for c in range(2)])

    def rows_out(c):
        if len(c) == 1:
            return [(y[0:8], vregs(y, 1, 1 + rv)) for y in c[0]]
        got = []
        for y, w in zip(*c):
            ym, yt = join8(y[0:8], w[0:8])
            got.append((ym, vregs(y, 1, 1 + rv) + vregs(w, 1, 1 + rv) + [yt]))
        return got

    def probs(q, k):
        sc = _dot_nt(k, q.astype(BF16))
        sc = _cat([sc[0:M], jnp.where(mask, sc[M:L], -1e9 / scale)], 0)
        p = jnp.exp2((sc - jnp.max(sc, axis=0, keepdims=True)) * (scale * math.log2(math.e)))
        return p * _recip(jnp.sum(p, axis=0, keepdims=True))

    def out_copy(j):
        r0 = pl.multiple_of(j * QS, QS)
        return pltpu.make_async_copy(xbuf.at[pl.ds(r0, QS)], out_hbm.at[pl.ds(r0, QS)], sem_out.at[j])

    def quad(j, carry):
        xs = normed(pl.ds(pl.multiple_of(j * QS, QS), QS))
        qkv = {(t, h): [] for t in range(3) for h in range(H)}
        att = {h: [] for h in range(H)}
        outs = {n: [] for n in range(nd)}
        mem = membuf[...]
        for st in range(4):
            r, n_tok = (0, 2 * rv + 1) if st == 0 else ((st + 1) * rv + 1, rv)
            hl = left_operands([mem[:, cols(2 * k, 2)] for k in range(4)],
                               [vregs(xs[:, cols(2 * k, 2)], r, r + n_tok) for k in range(4)], st == 0)
            ol, cur, p, o = {}, {}, {}, {}

            def wq_part(t, g, lo, hi, midway=None):
                return _hk_combine(hl, lambda f: _dot(
                    hl[f][1][:, lo:hi].astype(BF16),
                    weights(wa, o_qkv + ((t * ng + g) * nk + f) * wq + lo // 2, (hi - lo) // 2)), midway)

            def wo_part(e, lo, hi):
                return _hk_combine(ol[lo], lambda f: _dot(
                    _cat([ol[g][f][1] for g in range(lo, hi)], 1).astype(BF16),
                    weights(wa, o_wo + ((e * nk + f) * ng + lo) * rq, (hi - lo) * rq)))

            def stash(q, c):
                for a, blocks in enumerate(c):
                    for b, y in enumerate(blocks):
                        pbuf[st, q, a, b] = y

            def resume(q, c):
                return [[pbuf[st, q, a, b] + y for b, y in enumerate(blocks)] for a, blocks in enumerate(c)]

            def proj(t, g, midway=None):
                if g == 0 and st > 0 and t < 2:
                    c = resume(2 + t, wq_part(t, g, LANES, 2 * LANES))
                else:
                    c = wq_part(t, g, 0, 2 * LANES, midway)
                got = []
                for h, (ym, yt) in zip(heads(g), rows_out(c)):
                    qkv[t, h] += yt
                    got.append(_cat([ym] + qkv[t, h][4 * st:4 * st + 4], 0))
                return got

            def attend(g, c):
                for e in (2 * c, 2 * c + 1):
                    if 0 <= g < ng:
                        p[g, e] = probs(cur[0, g][e], cur[1, g][e])
                if g > 0:
                    for e in (2 * c, 2 * c + 1):
                        o[e] = _dot(p[g - 1, e].T, cur[2, g - 1][e].astype(BF16))
                        att[heads(g - 1)[e]] += vregs(o[e], 1, 5)
                    if c:
                        ol[g - 1] = left_operands(
                            [o[e][0:8] for e in range(4)],
                            [att[h][st * rv:None if st == 3 else (st + 1) * rv] for h in heads(g - 1)], st == 3)

            if st > 0:
                for t in range(2):
                    stash(2 + t, wq_part(t, 0, 0, LANES))
            for g in range(ng):
                cur[0, g] = proj(0, g)
                cur[1, g] = proj(1, g, part(attend, g - 1, 1) if g else None)
                cur[2, g] = proj(2, g)
                attend(g, 0)
            stash(0, wo_part(0, 0, 2))
            attend(ng - 1, 1)
            stash(1, wo_part(1, 0, 2))
            attend(ng, 0)
            stash(0, resume(0, wo_part(0, 2, 4)))
            attend(ng, 1)
            stash(1, resume(1, wo_part(1, 2, 4)))
            new = {}
            for e in range(2):
                for c, (ym, yt) in enumerate(rows_out(resume(e, wo_part(e, 4, ng)))):
                    new[2 * c + e] = ym
                    outs[2 * c + e] += yt
            mem = _cat([new[n] for n in range(nd)], 1)
            lo, hi = ((0, 2), (2, 6), (6, 8), (8, 16))[st]
            rr = pl.ds(pl.multiple_of(j * QS + 8 * lo, RC), 8 * (hi - lo))
            for n in range(nd):
                xbuf[rr, cols(n)] = (hs[n, rr, :] + _cat(outs[n][lo:hi], 0)).astype(BF16)
        membuf[...] = mem
        out_copy(j).start()
        return carry

    mem_copy.wait()
    membuf[...] = mem0[...].astype(F32)
    lax.fori_loop(0, S // QS, quad, 0)
    for j in range(S // QS):
        out_copy(j).wait()


@functools.partial(jax.jit, static_argnames=("A_seg_len",))
def pallas_parallel_sum__memory_aug_recurrent_mem_tr__mixer_s_mlp__prompt_kernel(
    A_x: jax.Array,
    A_mem0: jax.Array,
    A_Wq: jax.Array,
    A_Wk: jax.Array,
    A_Wv: jax.Array,
    A_Wo: jax.Array,
    A_seg_len: int,
    B_x: jax.Array,
    B_w1: jax.Array,
    B_w2: jax.Array,
    B_w3: jax.Array,
    B_w4: jax.Array,
):
    del B_x
    B, S, D = A_x.shape
    _, H, Dh = A_Wq.shape
    M = A_mem0.shape[1]
    seg = int(A_seg_len)
    F = B_w3.shape[1]
    assert (B, S, D, H, Dh, M, seg, F) == (1, 2048, 1024, 32, LANES, 8, 32, 3584)
    TM1, TM2 = 256, 128
    nd, nf, nk, nb2 = D // LANES, F // (4 * LANES), len(_HK), S // TM2

    hbm = pl.BlockSpec(memory_space=pl.ANY)
    dma = pltpu.SemaphoreType.DMA
    out = pl.pallas_call(
        functools.partial(_kernel, S=S, D=D, H=H, Dh=Dh, M=M, seg=seg, F=F, TM1=TM1, TM2=TM2),
        out_shape=jax.ShapeDtypeStruct((S, D), BF16),
        in_specs=[hbm] * 10,
        out_specs=hbm,
        scratch_shapes=[
            pltpu.VMEM((S, D), BF16),
            pltpu.VMEM((2, S, LANES), F32),
            pltpu.VMEM((nd, S + TM2, LANES), F32),
            pltpu.VMEM((2, 7, nd // 2, TM1 // 2, LANES), BF16),
            pltpu.VMEM((TM2, D), F32),
            pltpu.VMEM((49, nd // 4, TM2 // 4, LANES), BF16),
            pltpu.VMEM((49, nf, TM2 // 4, LANES), BF16),
            pltpu.VMEM((H * nk * D // 4, LANES), BF16),
            pltpu.VMEM((4 * 49 * (nf * D // 8 + 8), LANES), BF16),
            pltpu.SMEM((1,), jnp.int32),
            pltpu.VMEM((2, 12, (D // 4 // nb2) * H, LANES), BF16),
            pltpu.VMEM((12, (H // 2 + 2) * (D // 4 // nb2 + 4), LANES), U32),
            pltpu.VMEM((2, 4, nd, H * Dh // (4 * nb2), LANES), BF16),
            pltpu.VMEM((M, D), BF16),
            pltpu.VMEM((M, D), F32),
            pltpu.VMEM((4, 4, 2, 4, seg, LANES), F32),
            dma((S // TM1 + 1,)), dma((nd // 2 + 7,)), dma((2,)), dma((S // (4 * seg),)),
        ],
        compiler_params=pltpu.CompilerParams(
            vmem_limit_bytes=128 * 1024 * 1024, disable_bounds_checks=True, disable_semaphore_checks=True),
        name="rmt_s2mlp",
    )(A_x.reshape(S, D), A_mem0.reshape(M, D),
      A_Wq.reshape(D * H, Dh), A_Wk.reshape(D * H, Dh), A_Wv.reshape(D * H, Dh),
      A_Wo.reshape(H * Dh, D), B_w1, B_w2, B_w3, B_w4)
    return out.reshape(B, S, D)
```
